```python
import jax
import jax.numpy as jnp

def _softmax(x, axis=-1):
    return jax.nn.softmax(x, axis=axis)
def _gelu(x):
    return jax.nn.gelu(x, approximate=True)
def _silu(x):
    return jax.nn.silu(x)
def _sigmoid(x):
    return jax.nn.sigmoid(x)
def _layernorm(x, axis=-1, eps=1e-5):
    m = jnp.mean(x, axis=axis, keepdims=True)
    v = jnp.var(x, axis=axis, keepdims=True)
    return (x - m) / jnp.sqrt(v + eps)
def _scatter_add(tgt, idx, src, axis=0):
    return tgt.at[idx].add(src)
def _segment_sum(src, seg, n):
    return jax.ops.segment_sum(src, seg, n)
class _Rng:
    def __init__(self, key):
        self._k = key
    def _next(self):
        self._k, sub = jax.random.split(self._k)
        return sub
    def normal(self, shape):
        return jax.random.normal(self._next(), shape, dtype=jnp.bfloat16)
    def randint(self, lo, hi, shape):
        return jax.random.randint(self._next(), shape, lo, hi, dtype=jnp.int32)
    def uniform(self, shape, lo=0.0, hi=1.0):
        return jax.random.uniform(self._next(), shape, jnp.bfloat16, lo, hi)
    def permutation(self, n):
        return jax.random.permutation(self._next(), n)


kernel_name = 'interleave_layers__sliding_block_cached__dense_activation_gelu__decode'

def setup_inputs():
    _rng = _Rng(jax.random.key(int.from_bytes(__import__("os").urandom(4), "little")))
    _w = (lambda a: (lambda t: t.astype(jnp.bfloat16) if jnp.issubdtype(t.dtype, jnp.floating) else t)(jnp.asarray(a)))
    def _A_setup():
        B, Sq, D = 1, 1, 640
        Hq, Hkv, Sk, Dh = 32, 32, 32768, 192
        assert Hq % Hkv == 0, (Hq, Hkv)
        return {
            "x": _w((lambda *s: _rng.normal(s) * 0.05)(B, Sq, D)),
            "k_cache": _w((lambda *s: _rng.normal(s) * 0.05)(B, Hkv, Sk, Dh)),
            "v_cache": _w((lambda *s: _rng.normal(s) * 0.05)(B, Hkv, Sk, Dh)),
            "wq": _w((lambda *s: _rng.normal(s) * 0.05)(D, Hq * Dh) * (D ** -0.5)),
            "wo": _w((lambda *s: _rng.normal(s) * 0.05)(Hq * Dh, D) * ((Hq * Dh) ** -0.5)),
        }
    _A_in = _A_setup()

    def _B_setup():
        B, S, D, F = 1, 1, 640, 1536
        return {
            "x": _w((lambda *s: _rng.normal(s) * 0.05)(B, S, D)),
            "w1": _w((lambda *s: _rng.normal(s) * 0.05)(D, F) * (D ** -0.5)),
            "b1": _w((lambda *s: _rng.normal(s) * 0.05)(F) * 0.01),
            "w2": _w((lambda *s: _rng.normal(s) * 0.05)(F, D) * (F ** -0.5)),
            "b2": _w((lambda *s: _rng.normal(s) * 0.05)(D) * 0.01),
        }
    _B_in = _B_setup()

    return {
        "A_x": _A_in["x"],
        "A_k_cache": _A_in["k_cache"],
        "A_v_cache": _A_in["v_cache"],
        "A_wq": _A_in["wq"],
        "A_wo": _A_in["wo"],
        "B_x": _B_in["x"],
        "B_w1": _B_in["w1"],
        "B_b1": _B_in["b1"],
        "B_w2": _B_in["w2"],
        "B_b2": _B_in["b2"],
    }

def reference(A_x, A_k_cache, A_v_cache, A_wq, A_wo, B_x, B_w1, B_b1, B_w2, B_b2):
    def _A_ref(x, k_cache, v_cache, wq, wo):
        B, Sq, D = x.shape
        Hq, Dh = 32, 192
        Hkv, Sk = k_cache.shape[1], k_cache.shape[2]
        W = min(4096, max(256, Sk // 4))
        rep = Hq // Hkv
        q = (lambda x, *d: x.transpose(*d))((x @ wq).reshape(B, Sq, Hq, Dh), 0, 2, 1, 3)
        k = jnp.repeat(k_cache[:, :, Sk - W:, :], rep, axis=1)
        v = jnp.repeat(v_cache[:, :, Sk - W:, :], rep, axis=1)
        scores = jnp.einsum("bhqd,bhkd->bhqk", q, k) * (Dh ** -0.5)
        p = _softmax(scores, axis=-1)
        o = jnp.einsum("bhqk,bhkd->bhqd", p, v)
        return (lambda x, *d: x.transpose(*d))(o, 0, 2, 1, 3).reshape(B, Sq, Hq * Dh) @ wo

    def _B_ref(x, w1, b1, w2, b2):
        h = jnp.einsum("bsd,df->bsf", x, w1) + b1
        h = _gelu(h)
        return jnp.einsum("bsf,fd->bsd", h, w2) + b2

    x = A_x
    x = x + _A_ref(_layernorm(x, axis=-1), A_k_cache, A_v_cache, A_wq, A_wo)
    x = x + _B_ref(_layernorm(x, axis=-1), B_w1, B_b1, B_w2, B_b2)
    x = x + _A_ref(_layernorm(x, axis=-1), A_k_cache, A_v_cache, A_wq, A_wo)
    x = x + _B_ref(_layernorm(x, axis=-1), B_w1, B_b1, B_w2, B_b2)
    return x
```

```python
import functools
import math

import jax
import jax.numpy as jnp
from jax import lax
import jax.experimental.pallas as pl
import jax.experimental.pallas.tpu as pltpu

F32 = jnp.float32
BF16 = jnp.bfloat16
U32 = jnp.uint32

D = 640
H = 32
DH = 192
F = 1536
EPS = 1e-5
R = 16


def _layernorm(x):
    m = jnp.mean(x, axis=-1, keepdims=True)
    xc = x - m
    v = jnp.mean(xc * xc, axis=-1, keepdims=True)
    return xc * lax.rsqrt(v + EPS)


def _gelu(x):
    c = math.sqrt(2.0 / math.pi)
    return 0.5 * x * (1.0 + jnp.tanh(c * (x + 0.044715 * (x * x * x))))


def _rows_to_lanes(b, n):
    return jnp.concatenate([b[i:i + 1, :] for i in range(n)], axis=1)


def _bf(ref_val):
    return pltpu.bitcast(ref_val, BF16)


def _kernel(x_hbm, kt_hbm, vt_hbm, wq_hbm, wo_hbm, w1_hbm, b1_hbm, w2_hbm, b2_hbm,
            o_ref,
            kbuf, vbuf, wq_buf, wo_buf, w1_buf, w2_buf, x_buf, b1_buf, b2_buf,
            q_buf, sem_k, sem_v, sem_w, *, sk, w):
    c_scale = (DH ** -0.5) * math.log2(math.e)

    def k_copy(h):
        return pltpu.make_async_copy(kt_hbm.at[0, h, :, pl.ds(sk - w, w)],
                                     kbuf.bitcast(BF16).at[h], sem_k.at[h])

    def v_copy(h):
        return pltpu.make_async_copy(vt_hbm.at[0, h, :, pl.ds(sk - w, w)],
                                     vbuf.bitcast(BF16).at[h], sem_v.at[h])

    wq_cp = pltpu.make_async_copy(wq_hbm, wq_buf.bitcast(BF16), sem_w.at[0])
    wo_cp = pltpu.make_async_copy(wo_hbm, wo_buf.bitcast(BF16), sem_w.at[1])
    w1_cp = pltpu.make_async_copy(w1_hbm, w1_buf.bitcast(BF16), sem_w.at[2])
    w2_cp = pltpu.make_async_copy(w2_hbm, w2_buf.bitcast(BF16), sem_w.at[3])
    x_cp = pltpu.make_async_copy(x_hbm, x_buf, sem_w.at[4])
    b1_cp = pltpu.make_async_copy(b1_hbm, b1_buf, sem_w.at[5])
    b2_cp = pltpu.make_async_copy(b2_hbm, b2_buf, sem_w.at[6])

    wq_cp.start()
    x_cp.start()
    b1_cp.start()
    b2_cp.start()
    wo_cp.start()
    k_copy(0).start()
    v_copy(0).start()
    x_cp.wait()
    b1_cp.wait()
    b2_cp.wait()

    x0 = jnp.broadcast_to(x_buf[...].astype(F32), (R, D))
    b1 = _rows_to_lanes(b1_buf[...].astype(F32), F // 128)
    b2 = _rows_to_lanes(b2_buf[...].astype(F32), D // 128)

    def compute_q(x):
        z = _layernorm(x).astype(BF16)
        q = jnp.dot(z, _bf(wq_buf[...]), preferred_element_type=F32) * c_scale
        for h in range(H):
            q_buf[h, :, 0:DH] = pltpu.bitcast(q[:, h * DH:(h + 1) * DH].astype(BF16), U32)

    def head(h, acc, first):
        if first:
            k_copy(h).wait()

            @pl.when(h + 1 < H)
            def _():
                k_copy(h + 1).start()

            @pl.when(h + 1 == H)
            def _():
                w1_cp.start()

        q = _bf(q_buf[h, :, 0:DH])
        s = jnp.dot(q, _bf(kbuf[h]), preferred_element_type=F32)
        m = jnp.max(s, axis=-1, keepdims=True)
        p = jnp.exp2(s - m)
        l = jnp.sum(p, axis=-1, keepdims=True)
        if first:
            v_copy(h).wait()

            @pl.when(h + 1 < H)
            def _():
                v_copy(h + 1).start()

            @pl.when(h + 1 == H)
            def _():
                w2_cp.start()

        o = lax.dot_general(p.astype(BF16), _bf(vbuf[h]), (((1,), (1,)), ((), ())),
                            preferred_element_type=F32)
        o = (o / l).astype(BF16)
        r0 = pl.multiple_of(h * (DH // 2), 8)
        return acc + jnp.dot(o, _bf(wo_buf[pl.ds(r0, DH // 2), :]), preferred_element_type=F32)

    def mlp(x):
        z = _layernorm(x).astype(BF16)
        hh = jnp.dot(z, _bf(w1_buf[...]), preferred_element_type=F32) + b1
        return _gelu(hh).astype(BF16)

    wq_cp.wait()
    compute_q(x0)
    wo_cp.wait()
    x1 = lax.fori_loop(0, H, functools.partial(head, first=True), x0)
    w1_cp.wait()
    g = mlp(x1)
    w2_cp.wait()
    x2 = x1 + jnp.dot(g, _bf(w2_buf[...]), preferred_element_type=F32) + b2

    compute_q(x2)
    x3 = lax.fori_loop(0, H, functools.partial(head, first=False), x2)
    g = mlp(x3)
    x4 = x3 + jnp.dot(g, _bf(w2_buf[...]), preferred_element_type=F32) + b2
    o_ref[...] = x4[0:1, :].astype(o_ref.dtype)


@jax.jit
def pallas_interleave_layers__sliding_block_cached__dense_activation_gelu__decode_kernel(
    A_x: jax.Array,
    A_k_cache: jax.Array,
    A_v_cache: jax.Array,
    A_wq: jax.Array,
    A_wo: jax.Array,
    B_x: jax.Array,
    B_w1: jax.Array,
    B_b1: jax.Array,
    B_w2: jax.Array,
    B_b2: jax.Array,
):
    sk = A_k_cache.shape[2]
    w = min(4096, max(256, sk // 4))
    kt = jnp.swapaxes(A_k_cache, 2, 3)
    vt = jnp.swapaxes(A_v_cache, 2, 3)
    any_spec = pl.BlockSpec(memory_space=pl.ANY)
    out = pl.pallas_call(
        functools.partial(_kernel, sk=sk, w=w),
        out_shape=jax.ShapeDtypeStruct((1, D), A_x.dtype),
        in_specs=[any_spec] * 9,
        out_specs=pl.BlockSpec(memory_space=pltpu.VMEM),
        scratch_shapes=[
            pltpu.VMEM((H, DH // 2, w), U32),
            pltpu.VMEM((H, DH // 2, w), U32),
            pltpu.VMEM((D // 2, H * DH), U32),
            pltpu.VMEM((H * DH // 2, D), U32),
            pltpu.VMEM((D // 2, F), U32),
            pltpu.VMEM((F // 2, D), U32),
            pltpu.VMEM((1, D), BF16),
            pltpu.VMEM((F // 128, 128), BF16),
            pltpu.VMEM((D // 128, 128), BF16),
            pltpu.VMEM((H, R // 2, 256), U32),
            pltpu.SemaphoreType.DMA((H,)),
            pltpu.SemaphoreType.DMA((H,)),
            pltpu.SemaphoreType.DMA((7,)),
        ],
        compiler_params=pltpu.CompilerParams(vmem_limit_bytes=126 * 1024 * 1024),
    )(A_x.reshape(1, D), kt, vt, A_wq, A_wo, B_w1, B_b1.reshape(F // 128, 128),
      B_w2, B_b2.reshape(D // 128, 128))
    return out.reshape(A_x.shape)
```

```python
import functools
import math

import jax
import jax.numpy as jnp
from jax import lax
import jax.experimental.pallas as pl
import jax.experimental.pallas.tpu as pltpu

F32 = jnp.float32
BF16 = jnp.bfloat16
U32 = jnp.uint32

D = 640
H = 32
DH = 192
F = 1536
EPS = 1e-5
R = 16
NP = H // 2
OPT = {'NS': 3}
U = int(OPT.get('U', 1))
CPS = float(OPT.get('CPS', 19.5))
LAT = float(OPT.get('LAT', 142))
GE = int(OPT.get('GE', 1))
NB = int(OPT.get('NB', 14))
BOFF = float(OPT.get('BOFF', 0))
LAT2 = float(OPT.get('LAT2', 142))
MOFF = float(OPT.get('MOFF', 50))
EOFF = float(OPT.get('EOFF', 48))
BE = int(OPT.get('BE', 2))
CHAIN = int(OPT.get('CHAIN', 1))
OPQ = int(OPT.get('OPQ', 0))
NS = int(OPT.get('NS', 2))
SKIP2 = int(OPT.get('SKIP2', 0))
SKIP1 = int(OPT.get('SKIP1', 0))


def _layernorm(x):
    m = jnp.mean(x, axis=-1, keepdims=True)
    xc = x - m
    v = jnp.mean(xc * xc, axis=-1, keepdims=True)
    return xc * lax.rsqrt(v + EPS)


def _gelu(x):
    c = math.sqrt(2.0 / math.pi)
    return 0.5 * x * (1.0 + jnp.tanh(c * (x + 0.044715 * (x * x * x))))


def _rows_to_lanes(b, n):
    return jnp.concatenate([b[i:i + 1, :] for i in range(n)], axis=1)


def _bf(ref_val):
    return pltpu.bitcast(ref_val, BF16)


def _pack(a, b):
    return pltpu.bitcast(pltpu.pack_elementwise([a, b], packed_dtype=BF16), U32)


def _unpack(x):
    return (pltpu.unpack_elementwise(x, index=0, packed_dtype=BF16, unpacked_dtype=F32),
            pltpu.unpack_elementwise(x, index=1, packed_dtype=BF16, unpacked_dtype=F32))


def _u32(val):
    return pltpu.bitcast(val, U32)


def _kernel(x_hbm, kt_hbm, vt_hbm, wq_hbm, wo_hbm, w1_hbm, b1_hbm, w2_hbm, b2_hbm,
            o_ref,
            kbuf, vbuf, wq_buf, wo_buf, w1_buf, w2_buf, x_buf, b1_buf, b2_buf,
            q_buf, s_buf0, s_buf1, accp_buf, z_buf, xacc_buf, p_buf,
            sem_k, sem_v, sem_w, *, sk, w):
    c_scale = (DH ** -0.5) * math.log2(math.e)
    nt = w // 128

    def k_copy(h):
        return pltpu.make_async_copy(kt_hbm.at[0, h, :, pl.ds(sk - w, w)],
                                     kbuf.bitcast(BF16).at[h], sem_k.at[h % 2])

    def v_copy(h):
        return pltpu.make_async_copy(vt_hbm.at[0, h, :, pl.ds(sk - w, w)],
                                     vbuf.bitcast(BF16).at[h], sem_v.at[h % 2])

    wq_cp = pltpu.make_async_copy(wq_hbm, wq_buf.bitcast(BF16), sem_w.at[0])
    wo_cp = pltpu.make_async_copy(wo_hbm, wo_buf.bitcast(BF16), sem_w.at[1])
    w1_cp = pltpu.make_async_copy(w1_hbm, w1_buf.bitcast(BF16), sem_w.at[2])
    w2_cp = pltpu.make_async_copy(w2_hbm, w2_buf.bitcast(BF16), sem_w.at[3])
    x_cp = pltpu.make_async_copy(x_hbm, x_buf, sem_w.at[4])
    b1_cp = pltpu.make_async_copy(b1_hbm, b1_buf, sem_w.at[5])
    b2_cp = pltpu.make_async_copy(b2_hbm, b2_buf, sem_w.at[6])

    if not SKIP1:
        wq_cp.start()
    x_cp.start()
    b1_cp.start()
    b2_cp.start()
    if not SKIP1:
        wo_cp.start()
        k_copy(0).start()
        v_copy(0).start()
    x_cp.wait()
    b1_cp.wait()
    b2_cp.wait()

    x0 = jnp.broadcast_to(x_buf[...].astype(F32), (R, D))
    b1 = _rows_to_lanes(b1_buf[...].astype(F32), F // 128)
    b2 = _rows_to_lanes(b2_buf[...].astype(F32), D // 128)

    def head1(h, acc):
        k_copy(h).wait()

        @pl.when(h + 1 < H)
        def _():
            k_copy(h + 1).start()

        @pl.when(h + 1 == H)
        def _():
            w1_cp.start()

        q = _bf(q_buf[h, :, 0:DH])
        s = jnp.dot(q, _bf(kbuf[h]), preferred_element_type=F32)
        m = jnp.max(s, axis=-1, keepdims=True)
        p = jnp.exp2(s - m)
        l = jnp.sum(p, axis=-1, keepdims=True)
        v_copy(h).wait()

        @pl.when(h + 1 < H)
        def _():
            v_copy(h + 1).start()

        @pl.when(h + 1 == H)
        def _():
            w2_cp.start()

        o = lax.dot_general(p.astype(BF16), _bf(vbuf[h]), (((1,), (1,)), ((), ())),
                            preferred_element_type=F32)
        o = (o / l).astype(BF16)
        r0 = pl.multiple_of(h * (DH // 2), 8)
        return acc + jnp.dot(o, _bf(wo_buf[pl.ds(r0, DH // 2), :]), preferred_element_type=F32)

    def mlp_hidden(x):
        z = _layernorm(x).astype(BF16)
        hh = jnp.dot(z, _bf(w1_buf[...]), preferred_element_type=F32) + b1
        return _gelu(hh).astype(BF16)

    accp_buf[...] = jnp.zeros(accp_buf.shape, U32)

    if not SKIP1:
        wq_cp.wait()
        z = _layernorm(x0).astype(BF16)
        q = jnp.dot(z, _bf(wq_buf[...]), preferred_element_type=F32) * c_scale
        for h in range(H):
            q_buf[h, :, 0:DH] = _u32(q[:, h * DH:(h + 1) * DH].astype(BF16))
        wo_cp.wait()
        x1 = lax.fori_loop(0, H, head1, x0)
        w1_cp.wait()
        g = mlp_hidden(x1)
        w2_cp.wait()
        x2 = x1 + jnp.dot(g, _bf(w2_buf[...]), preferred_element_type=F32) + b2
    else:
        x2 = x0

    if SKIP2:
        o_ref[...] = x2[0:1, :].astype(o_ref.dtype)
        return

    z_buf[...] = _u32(_layernorm(x2).astype(BF16))
    xacc_buf[...] = x2[0:8]
    lane = lax.broadcasted_iota(jnp.int32, (8, 128), 1)

    def dup_bf(v):
        return _bf(_pack(v, v))

    def q_pair(j):
        c0 = pl.multiple_of(j * (2 * DH), 128)
        q = jnp.dot(_bf(z_buf[...]), _bf(wq_buf[:, pl.ds(c0, 2 * DH)]),
                    preferred_element_type=F32)[0:8] * c_scale
        qp = _pack(q, q)
        q_buf[2 * j, :, 0:DH] = qp[:, 0:DH]
        q_buf[2 * j + 1, :, 0:DH] = qp[:, DH:2 * DH]
        return q

    def score_block(q32, h, t, s_out):
        s = jnp.dot(_bf(q32), _bf(kbuf[h, :, 128 * t:128 * (t + 1)]),
                    preferred_element_type=F32)[0:8]
        s_out[:, 128 * t:128 * (t + 1)] = s
        return s

    def row_max(ss):
        mx = ss[0]
        for s in ss[1:]:
            mx = jnp.maximum(mx, s)
        return jnp.broadcast_to(jnp.max(mx, axis=-1, keepdims=True), (8, 128))

    na = 12 // NS

    def pv_step(h, st, s_in, m, gvals, true_mask, state):
        sw, t = divmod(st, nt)
        if OPQ:
            ld = pl.ds(pl.multiple_of(state['zero'] + 128 * t, 128), 128)
        else:
            ld = pl.ds(128 * t, 128)
        if sw == 0:
            p = jnp.exp2(s_in[:, ld] - m)
            if NS > 1:
                p_buf[:, 128 * t:128 * (t + 1)] = p
        else:
            p = p_buf[:, ld]
        if CHAIN and t == 0 and state.get('last') is not None:
            gvals = list(gvals) + [state['last']]
        for gval in gvals:
            p = jnp.where(true_mask, p, gval)
        if sw == 0:
            state['l'] = p if t == 0 else state['l'] + p
        accs = state['accs']
        for a in range(sw * na, (sw + 1) * na):
            y0, y1 = _unpack(vbuf[h, 8 * a:8 * a + 8, 128 * t:128 * (t + 1)])
            for j, yy in ((2 * a, y0), (2 * a + 1, y1)):
                accs[j] = yy * p if t == 0 else accs[j] + yy * p
        state['last'] = accs[2 * (sw + 1) * na - 1]
        if t == nt - 1:
            for a in range(sw * na, (sw + 1) * na):
                r0 = state['half'] * (DH // 2) + 8 * a
                accp_buf[r0:r0 + 8, :] = _pack(accs[2 * a], accs[2 * a + 1])
            if sw == 0:
                state['inv'] = 1.0 / jnp.broadcast_to(
                    jnp.sum(state['l'], axis=-1, keepdims=True), (8, 128))

    def o_pair(accp, ie, io):
        ones = jnp.ones((R, 128), BF16)
        o = lax.dot_general(ones, _bf(accp), (((1,), (1,)), ((), ())),
                            preferred_element_type=F32)[0:8]
        inv = jnp.concatenate([ie, jnp.where(lane < 64, ie, io), io], axis=1)
        return o * inv

    def out_pair(o, j):
        r0 = pl.multiple_of(j * DH, 8)
        return jnp.dot(dup_bf(o), _bf(wo_buf[pl.ds(r0, DH), :]),
                       preferred_element_type=F32)[0:8]

    q_pair(0)
    q0 = q_buf[0, :, 0:DH]
    m0 = row_max([score_block(q0, 0, t, s_buf0) for t in range(nt)])
    q_pair(1)

    nst = NS * nt

    def step_of(cyc):
        return int(math.ceil(cyc * NS / CPS))

    def block(jj, carry):
        m_e, ie, io = carry
        prev_last = None
        for u in range(U):
            j = jj * U + u
            true_mask = (lane + j) >= 0
            h0 = 2 * j
            q1 = q_buf[h0 + 1, :, 0:DH]
            h2 = jnp.minimum(h0 + 2, H - 1)
            q2 = q_buf[h2, :, 0:DH]
            gates = {}

            def gate(cyc, v):
                gates.setdefault(min(step_of(cyc), 2 * nst - 1), []).append(v)

            accp_prev = accp_buf[...]
            zero = lax.shift_right_logical(j, 10) * 128
            se = dict(accs=[None] * 24, half=0, zero=zero, last=prev_last)
            done = 0
            ss1 = []
            for t in range(nt):
                qq = q1
                if u == 0 and 0 < t < NB:
                    need = int((12 * t + BOFF) * NS // CPS)
                    while done < need:
                        pv_step(h0, done, s_buf0, m_e, gates.get(done, ()), true_mask, se)
                        done += 1
                    if done > 0:
                        sw = (done - 1) // nt
                        cand = list(range(2 * sw * na, 2 * (sw + 1) * na))
                        parts = [q1[:, 0:128], q1[:, 128:DH]]
                        for e in range(BE):
                            c = cand[(BE * t + e) * 3 % len(cand)] if len(cand) % 3 else cand[(BE * t + e) * 5 % len(cand)]
                            w_ = parts[e % 2].shape[1]
                            parts[e % 2] = jnp.where(true_mask[:, 0:w_], parts[e % 2], pltpu.bitcast(se['accs'][c], U32)[:, 0:w_])
                        qq = jnp.concatenate(parts, axis=1)
                s = score_block(qq, h0 + 1, t, s_buf1)
                ss1.append(s)
                if t % GE == 0:
                    assert step_of(12 * t + LAT) >= done
                    gate(12 * t + LAT, s)
            m_o = row_max(ss1)
            gate(12 * nt + LAT + MOFF, m_o)
            o = o_pair(accp_prev, ie, io)
            gate(12 * nt + EOFF + LAT2, o[:, 256:384])
            base = 12 * nt + EOFF
            ss2 = []
            nxt = 0
            for st in range(done, nst):
                while nxt < nt and step_of(base + 12 * nxt + LAT2) <= st:
                    assert nxt < st
                    s = score_block(q2, h2, nxt, s_buf0)
                    ss2.append(s)
                    if nxt % GE == 0:
                        gate(base + 12 * nxt + LAT2, s)
                    nxt += 1
                pv_step(h0, st, s_buf0, m_e, gates.get(st, ()), true_mask, se)
            for t in range(nxt, nt):
                s = score_block(q2, h2, t, s_buf0)
                ss2.append(s)
                if t % GE == 0:
                    gate(base + 12 * t + LAT2, s)
            m_e = row_max(ss2)
            gate(base + 12 * nt + LAT2 + MOFF, m_e)
            xo = out_pair(o, jnp.maximum(j - 1, 0))
            xacc_buf[...] += xo
            base2 = base + 12 * nt
            for c in range(5):
                gate(base2 + 24 * c + LAT2, xo[:, 128 * c:128 * (c + 1)])
            qn = q_pair(jnp.minimum(j + 2, NP - 1))
            for c in range(3):
                gate(base2 + 120 + 40 * c + 20 + LAT2, qn[:, 128 * c:128 * (c + 1)])
            so = dict(accs=[None] * 24, half=1, zero=zero, last=se['last'])
            for st in range(nst):
                pv_step(h0 + 1, st, s_buf1, m_o, gates.get(nst + st, ()), true_mask, so)
            ie, io = se['inv'], so['inv']
            prev_last = so['last']
        return m_e, ie, io

    one = jnp.ones((8, 128), F32)
    _, ie, io = lax.fori_loop(0, NP // U, block, (m0, one, one))
    x3 = xacc_buf[...] + out_pair(o_pair(accp_buf[...], ie, io), NP - 1)
    x3 = jnp.concatenate([x3, x3], axis=0)
    g = mlp_hidden(x3)
    x4 = x3 + jnp.dot(g, _bf(w2_buf[...]), preferred_element_type=F32) + b2
    o_ref[...] = x4[0:1, :].astype(o_ref.dtype)


@jax.jit
def pallas_interleave_layers__sliding_block_cached__dense_activation_gelu__decode_kernel(
    A_x: jax.Array,
    A_k_cache: jax.Array,
    A_v_cache: jax.Array,
    A_wq: jax.Array,
    A_wo: jax.Array,
    B_x: jax.Array,
    B_w1: jax.Array,
    B_b1: jax.Array,
    B_w2: jax.Array,
    B_b2: jax.Array,
):
    sk = A_k_cache.shape[2]
    w = min(4096, max(256, sk // 4))
    kt = jnp.swapaxes(A_k_cache, 2, 3)
    vt = jnp.swapaxes(A_v_cache, 2, 3)
    any_spec = pl.BlockSpec(memory_space=pl.ANY)
    out = pl.pallas_call(
        functools.partial(_kernel, sk=sk, w=w),
        out_shape=jax.ShapeDtypeStruct((1, D), A_x.dtype),
        in_specs=[any_spec] * 9,
        out_specs=pl.BlockSpec(memory_space=pltpu.VMEM),
        scratch_shapes=[
            pltpu.VMEM((H, DH // 2, w), U32),
            pltpu.VMEM((H, DH // 2, w), U32),
            pltpu.VMEM((D // 2, H * DH), U32),
            pltpu.VMEM((H * DH // 2, D), U32),
            pltpu.VMEM((D // 2, F), U32),
            pltpu.VMEM((F // 2, D), U32),
            pltpu.VMEM((1, D), BF16),
            pltpu.VMEM((F // 128, 128), BF16),
            pltpu.VMEM((D // 128, 128), BF16),
            pltpu.VMEM((H, R // 2, 256), U32),
            pltpu.VMEM((8, w), F32),
            pltpu.VMEM((8, w), F32),
            pltpu.VMEM((DH, 128), U32),
            pltpu.VMEM((R // 2, D), U32),
            pltpu.VMEM((8, D), F32),
            pltpu.VMEM((8, w), F32),
            pltpu.SemaphoreType.DMA((2,)),
            pltpu.SemaphoreType.DMA((2,)),
            pltpu.SemaphoreType.DMA((7,)),
        ],
        compiler_params=pltpu.CompilerParams(vmem_limit_bytes=126 * 1024 * 1024),
    )(A_x.reshape(1, D), kt, vt, A_wq, A_wo, B_w1, B_b1.reshape(F // 128, 128),
      B_w2, B_b2.reshape(D // 128, 128))
    return out.reshape(A_x.shape)
```

```python
import functools
import math

import jax
import jax.numpy as jnp
from jax import lax
import jax.experimental.pallas as pl
import jax.experimental.pallas.tpu as pltpu

F32 = jnp.float32
BF16 = jnp.bfloat16
U32 = jnp.uint32

D = 640
H = 32
DH = 192
F = 1536
EPS = 1e-5
R = 16
NP = H // 2
OPT = {'MOFF': 130, 'SDT': 12}
U = int(OPT.get('U', 1))
SG = int(OPT.get('SG', 4))
SDT = float(OPT.get('SDT', 16))
SE = int(OPT.get('SE', 1))
CA = int(OPT.get('CA', 2))
CPS = float(OPT.get('CPS', 18.7))
LATP = float(OPT.get('LATP', 135))
T0 = float(OPT.get('T0', 12))
RHO1 = float(OPT.get('RHO1', 1.0))
RHO2 = float(OPT.get('RHO2', 1.0))
GE = int(OPT.get('GE', 1))
EE = int(OPT.get('EE', 1))
BE = int(OPT.get('BE', 1))
MOFF = float(OPT.get('MOFF', 110))
CHAIN = int(OPT.get('CHAIN', 1))
OPQ = int(OPT.get('OPQ', 0))
NS = int(OPT.get('NS', 3))
SKIP2 = int(OPT.get('SKIP2', 0))
SKIP1 = int(OPT.get('SKIP1', 0))


def _layernorm(x):
    m = jnp.mean(x, axis=-1, keepdims=True)
    xc = x - m
    v = jnp.mean(xc * xc, axis=-1, keepdims=True)
    return xc * lax.rsqrt(v + EPS)


def _gelu(x):
    c = math.sqrt(2.0 / math.pi)
    return 0.5 * x * (1.0 + jnp.tanh(c * (x + 0.044715 * (x * x * x))))


def _rows_to_lanes(b, n):
    return jnp.concatenate([b[i:i + 1, :] for i in range(n)], axis=1)


def _bf(ref_val):
    return pltpu.bitcast(ref_val, BF16)


def _pack(a, b):
    return pltpu.bitcast(pltpu.pack_elementwise([a, b], packed_dtype=BF16), U32)


def _unpack(x):
    return (pltpu.unpack_elementwise(x, index=0, packed_dtype=BF16, unpacked_dtype=F32),
            pltpu.unpack_elementwise(x, index=1, packed_dtype=BF16, unpacked_dtype=F32))


def _u32(val):
    return pltpu.bitcast(val, U32)


def _kernel(x_hbm, kx_hbm, vx_hbm, wq_hbm, wo_hbm, w1_hbm, b1_hbm, w2_hbm, b2_hbm,
            o_ref,
            kbuf, vbuf, wq_buf, wo_buf, w1_buf, w2_buf, x_buf, b1_buf, b2_buf,
            p_buf0, p_buf1, sp_buf, accp_buf, z_buf, xacc_buf, qv_buf,
            sem_k, sem_v, sem_w, *, sk, w):
    c_scale = (DH ** -0.5) * math.log2(math.e)
    nt = w // 128
    r0w = (sk - w) // 16
    nrw = w // 16

    def k_copy(h):
        return pltpu.make_async_copy(kx_hbm.at[h, :, :, pl.ds(r0w, nrw), :],
                                     kbuf.bitcast(BF16).at[h], sem_k.at[h % 2])

    def v_copy(h):
        return pltpu.make_async_copy(vx_hbm.at[h, :, :, pl.ds(r0w, nrw), :],
                                     vbuf.bitcast(BF16).at[h], sem_v.at[h % 2])

    wq_cp = pltpu.make_async_copy(wq_hbm, wq_buf.bitcast(BF16), sem_w.at[0])
    wo_cp = pltpu.make_async_copy(wo_hbm, wo_buf.bitcast(BF16), sem_w.at[1])
    w1_cp = pltpu.make_async_copy(w1_hbm, w1_buf, sem_w.at[2])
    w2_cp = pltpu.make_async_copy(w2_hbm, w2_buf, sem_w.at[3])
    x_cp = pltpu.make_async_copy(x_hbm, x_buf, sem_w.at[4])
    b1_cp = pltpu.make_async_copy(b1_hbm, b1_buf, sem_w.at[5])
    b2_cp = pltpu.make_async_copy(b2_hbm, b2_buf, sem_w.at[6])

    if not SKIP1:
        wq_cp.start()
    x_cp.start()
    b1_cp.start()
    b2_cp.start()
    if not SKIP1:
        wo_cp.start()
        k_copy(0).start()
        v_copy(0).start()
    x_cp.wait()
    b1_cp.wait()
    b2_cp.wait()

    x0 = jnp.broadcast_to(x_buf[...].astype(F32), (R, D))
    b1 = _rows_to_lanes(b1_buf[...].astype(F32), F // 128)
    b2 = _rows_to_lanes(b2_buf[...].astype(F32), D // 128)

    x0 = x0[0:8]
    lane = lax.broadcasted_iota(jnp.int32, (8, 128), 1)
    sub_lo = lax.broadcasted_iota(jnp.int32, (1, 8, 128), 1) < 4

    def dup_bf(v):
        return _bf(_pack(v, v))

    def mlp_hidden(x):
        hh = jnp.dot(dup_bf(_layernorm(x)), w1_buf[...], preferred_element_type=F32)[0:8] + b1
        return dup_bf(_gelu(hh))

    def swap_halves(ref2):
        n = ref2.shape[1]
        x0_ = ref2[0].reshape(n // 8, 8, 128)
        x1_ = ref2[1].reshape(n // 8, 8, 128)
        ref2[0] = jnp.where(sub_lo, x0_, pltpu.roll(x1_, 4, 1)).reshape(n, 128)
        ref2[1] = jnp.where(sub_lo, pltpu.roll(x0_, 4, 1), x1_).reshape(n, 128)

    def fix_wo(g8, carry):
        g0 = pl.multiple_of(g8 * 8, 8)
        v = [wo_buf[pl.ds(g0, 8), 8 * c:8 * c + 8, :] for c in range(5)]
        n = [jnp.where(sub_lo, v[0], v[2]),
             pltpu.roll(jnp.where(sub_lo, v[3], v[0]), 4, 1),
             jnp.where(sub_lo, v[1], v[3]),
             pltpu.roll(jnp.where(sub_lo, v[4], v[1]), 4, 1),
             jnp.where(sub_lo, v[2], v[4])]
        for c in range(5):
            wo_buf[pl.ds(g0, 8), 8 * c:8 * c + 8, :] = n[c]
        return carry

    def q_cols(z, j, c):
        ct = 3 * j + c
        r0 = pl.multiple_of((ct // 2) * 8, 8)
        rhs = wq_buf[:, ct % 2, pl.ds(r0, 8), :].reshape(D // 2, 128)
        return jnp.dot(_bf(z), _bf(rhs), preferred_element_type=F32)[0:8] * c_scale

    lo64 = lane < 64
    evn = (lane & 8) == 0
    zf = jnp.zeros((8, 128), F32)
    k_order = (
        list(range(0, 16, 2)) + list(range(1, 16, 2)) + [16, 18, 20, 22, 17, 19, 21, 23],
        list(range(8, 24, 2)) + list(range(9, 24, 2)) + [1, 3, 5, 7, 0, 2, 4, 6],
    )

    def store_q(qs, j):
        q0, q1, q2 = qs
        r1 = pltpu.roll(q1, 56, 1)

        def lhs(qf, a2):
            a0 = jnp.where(evn, qf, zf)
            b1_ = jnp.where(evn, zf, qf)
            a2 = jnp.where(evn, a2, zf)
            return [_pack(a0, pltpu.roll(a0, 8, 1)), _pack(pltpu.roll(b1_, 120, 1), b1_),
                    _pack(a2, pltpu.roll(a2, 8, 1))]

        we = lhs(q0, jnp.where(lo64, q1, r1))
        wo_ = lhs(q2, jnp.where(lo64, r1, q1))
        for hh, ww in ((2 * j, we), (2 * j + 1, wo_)):
            slot = hh % 4
            for c in range(4):
                for i in range(3):
                    qv_buf[slot, c, c:c + 1, 128 * i:128 * (i + 1)] = ww[i][c:c + 1, :]

    def q_pair(j):
        z = z_buf[...]
        store_q([q_cols(z, j, c) for c in range(3)], j)

    def score2(lhs, h, par, k):
        rhs = jnp.concatenate([kbuf[h, i // 2, i % 2, 8 * k:8 * k + 8, :] for i in k_order[par]], axis=0)
        return jnp.dot(_bf(lhs), _bf(rhs), preferred_element_type=F32)[0:8]

    ng = nt // 8

    def store_p(p, g, rs, p_out):
        for r in rs:
            p_out[pl.ds(64 * g + r, 8, stride=8), :] = p

    def softmax(sg, p_out):
        mx = sg[0]
        for s in sg[1:]:
            mx = jnp.maximum(mx, s)
        m = jnp.max(jnp.max(mx, axis=1, keepdims=True), axis=0, keepdims=True)
        l = None
        ps = []
        for g in range(ng):
            p = jnp.exp2(sg[g] - m)
            ps.append(p)
            if p_out is not None:
                store_p(p, g, range(8), p_out)
            l = p if l is None else l + p
        l = jnp.sum(jnp.sum(l, axis=1, keepdims=True), axis=0, keepdims=True)
        return ps, jnp.broadcast_to(1.0 / l, (8, 128))

    na = 12 // NS

    def pv_step(h, st, p_in, gvals, true_mask, state, chain=CHAIN):
        sw, t = divmod(st, nt)
        p = p_in[8 * t:8 * t + 8, :]
        if chain and t == 0 and state.get('last') is not None:
            gvals = list(gvals) + [state['last']]
        for gval in gvals:
            p = jnp.where(true_mask, p, gval)
        accs = state['accs']
        for a in range(sw * na, (sw + 1) * na):
            y0, y1 = _unpack(vbuf[h, a, t % 2, 8 * (t // 2):8 * (t // 2) + 8, :])
            for j, yy in ((2 * a, y0), (2 * a + 1, y1)):
                accs[j] = yy * p if t == 0 else accs[j] + yy * p
        state['last'] = accs[2 * (sw + 1) * na - 1]
        if t == nt - 1:
            for a in range(sw * na, (sw + 1) * na):
                r0 = state['half'] * (DH // 2) + 8 * a
                accp_buf[r0:r0 + 8, :] = _pack(accs[2 * a], accs[2 * a + 1])

    def o_pair(ones, accp, ie, io):
        o = lax.dot_general(_bf(ones), _bf(accp), (((1,), (1,)), ((), ())),
                            preferred_element_type=F32)[0:8]
        inv = jnp.concatenate([ie, jnp.where(lo64, ie, io), io], axis=1)
        return o * inv

    def out_cols(op, j, c):
        rhs = wo_buf[pl.ds(j * 24, 24), 8 * c:8 * c + 8, :].reshape(DH, 128)
        return jnp.dot(_bf(op), _bf(rhs), preferred_element_type=F32)[0:8]

    ones32 = jnp.full((8, 128), 0x3F803F80, U32)

    def scores_part(h, par, cs, sg):
        for c in cs:
            lhs = qv_buf[h % 4, c]
            for g in range(ng):
                s = score2(lhs, h, par, 4 * g + c)
                sg[g] = s if sg[g] is None else sg[g] + s
        return sg

    def pair1(j, carry):
        q_pair(j)
        invs = []
        for par in range(2):
            h = 2 * j + par
            k_copy(h).wait()

            @pl.when(h + 1 < H)
            def _():
                k_copy(h + 1).start()

            @pl.when(h + 1 == H)
            def _():
                w1_cp.start()

            _, inv = softmax(scores_part(h, par, range(4), [None] * ng), p_buf0)
            invs.append(inv)
            v_copy(h).wait()

            @pl.when(h + 1 < H)
            def _():
                v_copy(h + 1).start()

            @pl.when(h + 1 == H)
            def _():
                w2_cp.start()

            def fix_v(a, c):
                swap_halves(vbuf.at[h, a])
                return c
            lax.fori_loop(0, 12, fix_v, 0)
            state = dict(accs=[None] * 24, half=par, last=None)
            for st in range(NS * nt):
                pv_step(h, st, p_buf0, (), None, state, chain=False)
        o = o_pair(ones32, accp_buf[...], invs[0], invs[1])
        op = _pack(o, o)
        for c in range(5):
            xacc_buf[:, 128 * c:128 * (c + 1)] += out_cols(op, j, c)
        return carry

    qv_buf[...] = jnp.zeros(qv_buf.shape, U32)
    if not SKIP1:
        z = _layernorm(x0)
        z_buf[...] = _pack(z, z)
        xacc_buf[...] = x0
        wq_cp.wait()

        def fix_q(a, c):
            swap_halves(wq_buf.at[a])
            return c
        lax.fori_loop(0, D // 16, fix_q, 0)
        wo_cp.wait()
        lax.fori_loop(0, H * DH // 128, fix_wo, 0)
        lax.fori_loop(0, NP, pair1, 0)
        x1 = xacc_buf[...]
        accp_buf[...] = jnp.zeros(accp_buf.shape, U32)
        w1_cp.wait()
        g = mlp_hidden(x1)
        w2_cp.wait()
        x2 = x1 + jnp.dot(g, w2_buf[...], preferred_element_type=F32)[0:8] + b2
    else:
        accp_buf[...] = jnp.zeros(accp_buf.shape, U32)
        x2 = x0

    if SKIP2:
        o_ref[...] = x2[0:1, :].astype(o_ref.dtype)
        return

    z = _layernorm(x2)
    z_buf[...] = _pack(z, z)
    xacc_buf[...] = x2
    q_pair(0)
    _, inv0 = softmax(scores_part(0, 0, range(4), [None] * ng), p_buf0)
    if CA > 0:
        sg = scores_part(1, 1, range(CA), [None] * ng)
        for g in range(ng):
            sp_buf[g] = sg[g]
    q_pair(1)
    nst = NS * nt

    def block(jj, carry):
        ie_cur, ie, io = carry
        for u in range(U):
            j = jj * U + u
            true_mask = (lane + j) >= 0
            h0 = 2 * j
            h2 = jnp.minimum(h0 + 2, H - 2)
            h3 = jnp.minimum(h0 + 3, H - 1)
            accp_prev = accp_buf[...]
            env = dict(qs=[], nedge=0)
            env['s1'] = [sp_buf[g] for g in range(ng)] if CA > 0 else [None] * ng
            env['s2'] = [None] * ng
            env['s3'] = [None] * ng
            gates = {}
            cur = dict(state=None, st=-1)

            def gate(cyc, v):
                st = min(int(math.ceil(cyc * NS / CPS)), 2 * nst - 1)
                assert st > cur['st'], (st, cur['st'])
                gates.setdefault(st, []).append(v)

            def edge(x, n=BE):
                if cur['st'] < 0:
                    return x
                sw = (cur['st'] % nst) // nt
                cand = list(range(2 * sw * na, 2 * (sw + 1) * na))
                ntile = -(-x.shape[1] // 128)
                parts = [x[:, 128 * i:min(128 * (i + 1), x.shape[1])] for i in range(ntile)]
                for e in range(n):
                    c = cand[(env['nedge'] * 3) % len(cand)] if len(cand) % 3 else cand[(env['nedge'] * 5) % len(cand)]
                    env['nedge'] += 1
                    i = e % ntile
                    w_ = parts[i].shape[1]
                    parts[i] = jnp.where(true_mask[:, 0:w_], parts[i],
                                         pltpu.bitcast(cur['state']['accs'][c], U32)[:, 0:w_])
                return parts[0] if ntile == 1 else jnp.concatenate(parts, axis=1)

            jobs = []
            stores = {}

            def sched_stores(ps, p_out, t_ready):
                gate(t_ready, ps[-1])
                n = 8 // SG
                for i in range(ng * n):
                    g, k = divmod(i, n)
                    st = min(int(math.ceil((t_ready + SDT * i) * NS / CPS)) + 1, 2 * nst - 1)
                    stores.setdefault(st, []).append((ps[g], g, range(SG * k, SG * (k + 1)), p_out))

            def job_b(h, par, c, g, key, last):
                def fn(td):
                    lhs = edge(qv_buf[h % 4, c])
                    s = score2(lhs, h, par, 4 * g + c)
                    sg = env[key]
                    sg[g] = s if sg[g] is None else sg[g] + s
                    gate(td + LATP, sg[g])
                    if last == 'sm1':
                        ps, env['io'] = softmax(sg, None)
                        sched_stores(ps, p_buf1, td + LATP + MOFF)
                    elif last == 'sm2':
                        env['sm2'] = True
                    elif last == 'st':
                        for gg in range(ng):
                            sp_buf[gg] = sg[gg]
                return fn

            def job_e(td):
                o = o_pair(edge(ones32), accp_prev, ie, io)
                gate(td + LATP + 10, o[:, 256:384])
                env['op'] = _pack(o, o)

            def job_g(c):
                def fn(td):
                    xo = out_cols(edge(env['op']), jnp.maximum(j - 1, 0), c)
                    xacc_buf[:, 128 * c:128 * (c + 1)] += xo
                    gate(td + LATP, xo)
                return fn

            def job_a(c):
                def fn(td):
                    jn = jnp.minimum(j + 2, NP - 1)
                    qc = q_cols(edge(z_buf[...]), jn, c)
                    gate(td + LATP, qc)
                    env['qs'].append(qc)
                    if c == 2:
                        store_q(env['qs'], jn)
                return fn

            for c in range(CA, 4):
                for g in range(ng):
                    jobs.append((24, RHO1, job_b(h0 + 1, 1, c, g, 's1', 'sm1' if (c == 3 and g == ng - 1) else None)))
            jobs.append((48, RHO2, job_e))
            for c in range(4):
                for g in range(ng):
                    jobs.append((24, RHO2, job_b(h2, 0, c, g, 's2', 'sm2' if (c == 3 and g == ng - 1) else None)))
            for c in range(5):
                jobs.append((24, RHO2, job_g(c)))
            for c in range(CA):
                for g in range(ng):
                    jobs.append((24, RHO2, job_b(h3, 1, c, g, 's3', 'st' if (c == CA - 1 and g == ng - 1) else None)))
            for c in range(3):
                jobs.append((40, RHO2, job_a(c)))
            times = []
            tt = T0
            for cost, rho, _ in jobs:
                tt += cost * rho
                times.append(tt)

            se = dict(accs=[None] * 24, half=0, last=None)
            so = None
            nj = 0
            for st in range(2 * nst):
                while nj < len(jobs) and times[nj] <= st * CPS / NS:
                    jobs[nj][2](times[nj])
                    if env.get('sm2') is True:
                        env['sm2'] = times[nj]
                    nj += 1
                if st >= nst and isinstance(env.get('sm2'), float):
                    ps, env['ie'] = softmax(env['s2'], None)
                    sched_stores(ps, p_buf0, max(env['sm2'] + LATP + MOFF, (st + 8) * CPS / NS))
                    env['sm2'] = None
                for (pv_, g_, rs_, po_) in stores.get(st, ()):
                    assert not (po_ is p_buf1 and st > nst)
                    if SE:
                        pv_ = pltpu.bitcast(edge(pltpu.bitcast(pv_, U32), 1), F32)
                    store_p(pv_, g_, rs_, po_)
                if st < nst:
                    pv_step(h0, st, p_buf0, gates.get(st, ()), true_mask, se)
                    cur['state'] = se
                else:
                    if so is None:
                        so = dict(accs=[None] * 24, half=1, last=se['last'])
                    pv_step(h0 + 1, st - nst, p_buf1, gates.get(st, ()), true_mask, so)
                    cur['state'] = so
                cur['st'] = st
            assert nj == len(jobs)
            ie, io, ie_cur = ie_cur, env['io'], env['ie']
        return ie_cur, ie, io

    one = jnp.ones((8, 128), F32)
    _, ie, io = lax.fori_loop(0, NP // U, block, (inv0, one, one))
    o = o_pair(ones32, accp_buf[...], ie, io)
    op = _pack(o, o)
    x3 = xacc_buf[...] + jnp.concatenate([out_cols(op, NP - 1, c) for c in range(5)], axis=1)
    g = mlp_hidden(x3)
    x4 = x3 + jnp.dot(g, w2_buf[...], preferred_element_type=F32)[0:8] + b2
    o_ref[...] = x4[0:1, :].astype(o_ref.dtype)


@jax.jit
def pallas_interleave_layers__sliding_block_cached__dense_activation_gelu__decode_kernel(
    A_x: jax.Array,
    A_k_cache: jax.Array,
    A_v_cache: jax.Array,
    A_wq: jax.Array,
    A_wo: jax.Array,
    B_x: jax.Array,
    B_w1: jax.Array,
    B_b1: jax.Array,
    B_w2: jax.Array,
    B_b2: jax.Array,
):
    sk = A_k_cache.shape[2]
    w = min(4096, max(256, sk // 4))
    def tile_view(a):
        *lead, r, c = a.shape
        n = len(lead)
        a = a.reshape(*lead, r // 8, 8, c // 128, 128)
        a = a.transpose(*range(n), n, n + 2, n + 1, n + 3)
        return a.reshape(*lead, r // 16, 2, (c // 128) * 8, 128)

    kx = tile_view(jnp.swapaxes(A_k_cache, 2, 3)[0])
    vx = tile_view(jnp.swapaxes(A_v_cache, 2, 3)[0])
    wqx = tile_view(A_wq)
    wox = tile_view(A_wo).reshape(H * DH // 16, 80, 128)
    any_spec = pl.BlockSpec(memory_space=pl.ANY)
    out = pl.pallas_call(
        functools.partial(_kernel, sk=sk, w=w),
        out_shape=jax.ShapeDtypeStruct((1, D), A_x.dtype),
        in_specs=[any_spec] * 9,
        out_specs=pl.BlockSpec(memory_space=pltpu.VMEM),
        scratch_shapes=[
            pltpu.VMEM((H, DH // 16, 2, w // 32, 128), U32),
            pltpu.VMEM((H, DH // 16, 2, w // 32, 128), U32),
            pltpu.VMEM((D // 16, 2, H * DH // 32, 128), U32),
            pltpu.VMEM((H * DH // 16, 40, 128), U32),
            pltpu.VMEM((D, F), BF16),
            pltpu.VMEM((F, D), BF16),
            pltpu.VMEM((1, D), BF16),
            pltpu.VMEM((F // 128, 128), BF16),
            pltpu.VMEM((D // 128, 128), BF16),
            pltpu.VMEM((w // 16, 128), F32),
            pltpu.VMEM((w // 16, 128), F32),
            pltpu.VMEM((w // 1024, 8, 128), F32),
            pltpu.VMEM((DH, 128), U32),
            pltpu.VMEM((R // 2, D), U32),
            pltpu.VMEM((8, D), F32),
            pltpu.VMEM((4, 4, 8, 2 * DH), U32),
            pltpu.SemaphoreType.DMA((2,)),
            pltpu.SemaphoreType.DMA((2,)),
            pltpu.SemaphoreType.DMA((7,)),
        ],
        compiler_params=pltpu.CompilerParams(vmem_limit_bytes=126 * 1024 * 1024),
    )(A_x.reshape(1, D), kx, vx, wqx, wox, B_w1, B_b1.reshape(F // 128, 128),
      B_w2, B_b2.reshape(D // 128, 128))
    return out.reshape(A_x.shape)
```

```python
import functools
import math

import jax
import jax.numpy as jnp
from jax import lax
import jax.experimental.pallas as pl
import jax.experimental.pallas.tpu as pltpu

F32 = jnp.float32
BF16 = jnp.bfloat16
U32 = jnp.uint32

D = 640
H = 32
DH = 192
F = 1536
EPS = 1e-5
NP = H // 2
OPT = {}
NS = int(OPT.get('NS', 3))
CA = int(OPT.get('CA', 2))
CPS = float(OPT.get('CPS', 18.7))
LATP = float(OPT.get('LATP', 145))
T0 = float(OPT.get('T0', 12))
T0F = float(OPT.get('T0F', -200))
RHO = float(OPT.get('RHO', 1.0))
BE = int(OPT.get('BE', 1))
MOFF = float(OPT.get('MOFF', 130))
SG = int(OPT.get('SG', 4))
SDT = float(OPT.get('SDT', 12))
CHAIN = int(OPT.get('CHAIN', 1))
XE = int(OPT.get('XE', 6))
XO = int(OPT.get('XO', 7))
W2C = int(OPT.get('W2C', 4))
ORD = OPT.get('ORD', 'ebagn')
SKIP2 = int(OPT.get('SKIP2', 0))
SKIP1 = int(OPT.get('SKIP1', 0))


def _gelu(x):
    c = math.sqrt(2.0 / math.pi)
    return 0.5 * x * (1.0 + jnp.tanh(c * (x + 0.044715 * (x * x * x))))


def _rows_to_lanes(b, n):
    return jnp.concatenate([b[i:i + 1, :] for i in range(n)], axis=1)


def _bf(x):
    return pltpu.bitcast(x, BF16)


def _pack(a, b):
    return pltpu.bitcast(pltpu.pack_elementwise([a, b], packed_dtype=BF16), U32)


def _unpack(x):
    return (pltpu.unpack_elementwise(x, index=0, packed_dtype=BF16, unpacked_dtype=F32),
            pltpu.unpack_elementwise(x, index=1, packed_dtype=BF16, unpacked_dtype=F32))


def _dot(lhs32, rhs):
    return jnp.dot(_bf(lhs32), rhs, preferred_element_type=F32)[0:8]


def _dot_t(lhs32, rhs32):
    return lax.dot_general(_bf(lhs32), _bf(rhs32), (((1,), (1,)), ((), ())),
                           preferred_element_type=F32)[0:8]


def _ln_stats(xp):
    x = _unpack(xp)[0]
    m = jnp.mean(x, axis=-1, keepdims=True)
    xc = x - m
    v = jnp.mean(xc * xc, axis=-1, keepdims=True)
    return m, lax.rsqrt(v + EPS)


def _kernel(x_hbm, kx_hbm, vx_hbm, wq_hbm, wo_hbm, w1_hbm, b1_hbm, w2_hbm, b2_hbm,
            o_ref,
            kbuf, vbuf, wq_buf, wo_buf, w1_buf, w2_buf, x_buf, b1_buf, b2_buf,
            p_buf0, p_buf1, sp_buf, accp_buf, z_buf, xacc_buf, qv_buf, qraw_buf,
            csq_buf, cs1_buf, st_buf, tm_buf,
            sem_k, sem_v, sem_w, *, sk, w):
    c_scale = (DH ** -0.5) * math.log2(math.e)
    nt = w // 128
    ng = nt // 8
    na = 12 // NS
    nst = NS * nt
    r0w = (sk - w) // 16
    nrw = w // 16
    w2r = F // W2C

    def k_copy(h):
        return pltpu.make_async_copy(kx_hbm.at[h, :, :, pl.ds(r0w, nrw), :],
                                     kbuf.bitcast(BF16).at[h], sem_k.at[h & 1])

    def v_copy(h):
        return pltpu.make_async_copy(vx_hbm.at[h, :, :, pl.ds(r0w, nrw), :],
                                     vbuf.bitcast(BF16).at[h], sem_v.at[h & 1])

    wq_cp = pltpu.make_async_copy(wq_hbm, wq_buf.bitcast(BF16), sem_w.at[0])
    wo_cp = pltpu.make_async_copy(wo_hbm, wo_buf.bitcast(BF16), sem_w.at[1])
    w1_cp = pltpu.make_async_copy(w1_hbm, w1_buf, sem_w.at[2])
    x_cp = pltpu.make_async_copy(x_hbm, x_buf, sem_w.at[3])
    b1_cp = pltpu.make_async_copy(b1_hbm, b1_buf, sem_w.at[4])
    b2_cp = pltpu.make_async_copy(b2_hbm, b2_buf, sem_w.at[5])
    w2_cps = [pltpu.make_async_copy(w2_hbm.at[pl.ds(i * w2r, w2r), :],
                                    w2_buf.at[pl.ds(i * w2r, w2r), :], sem_w.at[6 + i])
              for i in range(W2C)]

    if not SKIP1:
        wq_cp.start()
    x_cp.start()
    b1_cp.start()
    b2_cp.start()
    if not SKIP1:
        wo_cp.start()
        k_copy(0).start()
        v_copy(0).start()
    x_cp.wait()
    b1_cp.wait()
    b2_cp.wait()

    x0 = jnp.broadcast_to(x_buf[...].astype(F32), (8, D))
    b1 = _rows_to_lanes(b1_buf[...].astype(F32), F // 128)
    b2 = _rows_to_lanes(b2_buf[...].astype(F32), D // 128)

    lane = lax.broadcasted_iota(jnp.int32, (8, 128), 1)
    sub_lo = lax.broadcasted_iota(jnp.int32, (1, 8, 128), 1) < 4
    lo64 = lane < 64
    evn = (lane & 8) == 0
    zf = jnp.zeros((8, 128), F32)
    ones32 = jnp.full((8, 128), 0x3F803F80, U32)
    k_order = (
        list(range(0, 16, 2)) + list(range(1, 16, 2)) + [16, 18, 20, 22, 17, 19, 21, 23],
        list(range(8, 24, 2)) + list(range(9, 24, 2)) + [1, 3, 5, 7, 0, 2, 4, 6],
    )

    def swap_halves(ref2):
        n = ref2.shape[1]
        a = ref2[0].reshape(n // 8, 8, 128)
        b = ref2[1].reshape(n // 8, 8, 128)
        ref2[0] = jnp.where(sub_lo, a, pltpu.roll(b, 4, 1)).reshape(n, 128)
        ref2[1] = jnp.where(sub_lo, pltpu.roll(a, 4, 1), b).reshape(n, 128)

    def fix_wq(a, carry):
        swap_halves(wq_buf.at[a])
        return carry

    def fix_wo(g8, carry):
        g0 = pl.multiple_of(g8 * 8, 8)
        v = [wo_buf[pl.ds(g0, 8), 8 * c:8 * c + 8, :] for c in range(5)]
        n = [jnp.where(sub_lo, v[0], v[2]),
             pltpu.roll(jnp.where(sub_lo, v[3], v[0]), 4, 1),
             jnp.where(sub_lo, v[1], v[3]),
             pltpu.roll(jnp.where(sub_lo, v[4], v[1]), 4, 1),
             jnp.where(sub_lo, v[2], v[4])]
        for c in range(5):
            wo_buf[pl.ds(g0, 8), 8 * c:8 * c + 8, :] = n[c]
        return carry

    def set_row(x):
        xp = _pack(x, x)
        z_buf[...] = xp
        m, r = _ln_stats(xp)
        rc = r * c_scale
        st_buf[0] = jnp.broadcast_to(rc, (8, 128))
        st_buf[1] = jnp.broadcast_to(m * rc, (8, 128))

    def wq_cols(ct):
        r0 = pl.multiple_of(lax.shift_right_logical(ct, 1) * 8, 8) if not isinstance(ct, int) else (ct // 2) * 8
        return _bf(wq_buf[:, ct & 1, pl.ds(r0, 8), :].reshape(D // 2, 128))

    def q_cols(z, j, c):
        ct = 3 * j + c
        return _dot(z, wq_cols(ct)) * st_buf[0] - csq_buf[ct] * st_buf[1]

    def store_q(qs, j):
        q0, q1, q2 = qs
        r1 = pltpu.roll(q1, 56, 1)

        def lhs(qf, a2):
            a0 = jnp.where(evn, qf, zf)
            b1_ = jnp.where(evn, zf, qf)
            a2 = jnp.where(evn, a2, zf)
            return [_pack(a0, pltpu.roll(a0, 8, 1)), _pack(pltpu.roll(b1_, 120, 1), b1_),
                    _pack(a2, pltpu.roll(a2, 8, 1))]

        for hh, ww in ((2 * j, lhs(q0, jnp.where(lo64, q1, r1))),
                       (2 * j + 1, lhs(q2, jnp.where(lo64, r1, q1)))):
            for c in range(4):
                for i in range(3):
                    qv_buf[hh & 3, c, c:c + 1, 128 * i:128 * (i + 1)] = ww[i][c:c + 1, :]

    def q_pair(j):
        z = z_buf[...]
        store_q([q_cols(z, j, c) for c in range(3)], j)

    def score2(lhs, h, par, k):
        rhs = jnp.concatenate([kbuf[h, i // 2, i % 2, 8 * k:8 * k + 8, :] for i in k_order[par]],
                              axis=0)
        return _dot(lhs, _bf(rhs))

    def scores_all(h, par):
        sg = [None] * ng
        for c in range(4):
            lhs = qv_buf[h & 3, c]
            for g in range(ng):
                s = score2(lhs, h, par, 4 * g + c)
                sg[g] = s if sg[g] is None else sg[g] + s
        return sg

    def store_p(p, g, rs, p_out):
        for r in rs:
            p_out[pl.ds(64 * g + r, 8, stride=8), :] = p

    def softmax(sg, p_out):
        mx = sg[0]
        for s in sg[1:]:
            mx = jnp.maximum(mx, s)
        m = jnp.max(jnp.max(mx, axis=1, keepdims=True), axis=0, keepdims=True)
        l = None
        ps = []
        for g in range(ng):
            p = jnp.exp2(sg[g] - m)
            ps.append(p)
            if p_out is not None:
                store_p(p, g, range(8), p_out)
            l = p if l is None else l + p
        l = jnp.sum(jnp.sum(l, axis=1, keepdims=True), axis=0, keepdims=True)
        return ps, jnp.broadcast_to(1.0 / l, (8, 128))

    def v_tile(h, a, t):
        return vbuf[h, a, t % 2, 8 * (t // 2):8 * (t // 2) + 8, :]

    def pv_step(h, sw, t, n_t, p_in, gvals, true_mask, state):
        p = p_in[8 * t:8 * t + 8, :]
        for gval in gvals:
            p = jnp.where(true_mask, p, gval)
        accs = state['accs']
        for a in range(sw * na, (sw + 1) * na):
            y0, y1 = _unpack(v_tile(h, a, t))
            for j, yy in ((2 * a, y0), (2 * a + 1, y1)):
                accs[j] = yy * p if t == 0 else accs[j] + yy * p
        state['sw'] = sw
        if t == n_t - 1:
            for a in range(sw * na, (sw + 1) * na):
                r0 = state['half'] * (DH // 2) + 8 * a
                accp_buf[r0:r0 + 8, :] = _pack(accs[2 * a], accs[2 * a + 1])

    def o_pair(ones, accp, ie, io):
        inv = jnp.concatenate([ie, jnp.where(lo64, ie, io), io], axis=1)
        return _dot_t(ones, accp) * inv

    def out_cols(op, g0, ngrp, c):
        rhs = wo_buf[pl.ds(g0, ngrp), 8 * c:8 * c + 8, :].reshape(ngrp * 8, 128)
        return _dot(op, _bf(rhs))

    def mlp_hidden(x):
        xp = _pack(x, x)
        m, r = _ln_stats(xp)
        hh = (_dot(xp, w1_buf[...]) - cs1_buf[...] * m) * r + b1
        g = _gelu(hh)
        return _pack(g, g)

    def pair1(j, carry):
        q_pair(j)
        invs = []
        for par in range(2):
            h = 2 * j + par
            k_copy(h).wait()

            @pl.when(h + 1 < H)
            def _():
                k_copy(h + 1).start()

            @pl.when(h + 1 == H)
            def _():
                w1_cp.start()

            _, inv = softmax(scores_all(h, par), p_buf0)
            invs.append(inv)
            v_copy(h).wait()

            @pl.when(h + 1 < H)
            def _():
                v_copy(h + 1).start()

            @pl.when(h + 1 == H)
            def _():
                for cp in w2_cps:
                    cp.start()

            def fix_v(a, c):
                swap_halves(vbuf.at[h, a])
                return c
            lax.fori_loop(0, DH // 16, fix_v, 0)
            state = dict(accs=[None] * 24, half=par)
            for sw in range(NS):
                for t in range(nt):
                    pv_step(h, sw, t, nt, p_buf0, (), None, state)
        o = o_pair(ones32, accp_buf[...], invs[0], invs[1])
        op = _pack(o, o)
        for c in range(5):
            xacc_buf[:, 128 * c:128 * (c + 1)] += out_cols(op, 24 * j, 24, c)
        return carry

    def colsum_q(ct, carry):
        ones = jnp.concatenate([ones32] * (D // 128), axis=1)
        csq_buf[ct] = _dot(ones, wq_cols(ct))
        return carry

    qv_buf[...] = jnp.zeros(qv_buf.shape, U32)
    tm_buf[...] = lane
    if not SKIP1:
        set_row(x0)
        xacc_buf[...] = x0
        wq_cp.wait()
        lax.fori_loop(0, D // 16, fix_wq, 0)
        lax.fori_loop(0, 3 * NP, colsum_q, 0)
        wo_cp.wait()
        lax.fori_loop(0, H * DH // 128, fix_wo, 0)
        lax.fori_loop(0, NP, pair1, 0)
        x1 = xacc_buf[...]
        w1_cp.wait()
        cs1_buf[...] = _dot(jnp.concatenate([ones32] * (D // 128), axis=1), w1_buf[...])
        gp = mlp_hidden(x1)
        x2 = x1 + b2
        for i in range(W2C):
            w2_cps[i].wait()
            x2 = x2 + _dot(gp[:, i * w2r:(i + 1) * w2r], w2_buf[i * w2r:(i + 1) * w2r, :])
    else:
        x2 = lax.fori_loop(0, 2, lambda i, x: x + 1.0, x0)

    if SKIP2:
        o_ref[...] = x2[0:1, :].astype(o_ref.dtype)
        return

    def block(j, carry, kind):
        ie_cur, ie, io = carry
        first, last = kind == 'first', kind == 'last'
        true_mask = tm_buf[...] >= 0
        h0 = 2 * j
        nts = (nt - XE, nt - XO) if last else (nt, nt)
        steps = [(par, sw, t) for par in range(2) for sw in range(NS) for t in range(nts[par])]
        n_even = NS * nts[0]
        env = dict(qs=[], nedge=0, s2=[None] * ng, s3=[None] * ng)
        env['s1'] = [None] * ng if first or CA == 0 else [sp_buf[g] for g in range(ng)]
        accp_prev = None if first else accp_buf[...]
        gates, stores = {}, {}
        cur = dict(state=None, st=-1)

        def step_at(cyc):
            return int(math.ceil(cyc * NS / CPS))

        def gate(cyc, v):
            st = step_at(cyc)
            if st < len(steps) and st > cur['st']:
                gates.setdefault(st, []).append(v)

        def edge(x, n=BE):
            if cur['st'] < 0:
                return x
            sw = cur['state']['sw']
            cand = list(range(2 * sw * na, 2 * (sw + 1) * na))
            ntile = -(-x.shape[1] // 128)
            parts = [x[:, 128 * i:min(128 * (i + 1), x.shape[1])] for i in range(ntile)]
            for e in range(n):
                mul = 3 if len(cand) % 3 else 5
                c = cand[(env['nedge'] * mul) % len(cand)]
                env['nedge'] += 1
                i = e % ntile
                w_ = parts[i].shape[1]
                parts[i] = jnp.where(true_mask[:, 0:w_], parts[i],
                                     pltpu.bitcast(cur['state']['accs'][c], U32)[:, 0:w_])
            return parts[0] if ntile == 1 else jnp.concatenate(parts, axis=1)

        def sched_stores(ps, p_out, t_ready, limit):
            gate(t_ready, ps[-1])
            n = 8 // SG
            for i in range(ng * n):
                g, k = divmod(i, n)
                st = min(max(step_at(t_ready + SDT * i) + 1, cur['st'] + 1), limit)
                stores.setdefault(st, []).append((ps[g], g, range(SG * k, SG * (k + 1)), p_out))

        def job_b(h, par, c, g, key, tail):
            def fn(td):
                s = score2(edge(qv_buf[h & 3, c]), h, par, 4 * g + c)
                sg = env[key]
                sg[g] = s if sg[g] is None else sg[g] + s
                gate(td + LATP, sg[g])
                if tail == 'sm1':
                    ps, env['io'] = softmax(sg, None)
                    sched_stores(ps, p_buf1, td + LATP + MOFF, n_even)
                    if not first and not last:
                        store_q([qraw_buf[i] for i in range(3)], j + 1)
                elif tail == 'sm2':
                    env['sm2'] = td
                elif tail == 'st':
                    for gg in range(ng):
                        sp_buf[gg] = sg[gg]
            return fn

        def job_e(td):
            o = o_pair(edge(ones32), accp_prev, ie, io)
            gate(td + LATP + 10, o[:, 256:384])
            env['op'] = _pack(o, o)

        def job_g(c):
            def fn(td):
                xo = out_cols(edge(env['op']), 24 * (j - 1), 24, c)
                xacc_buf[:, 128 * c:128 * (c + 1)] += xo
                gate(td + LATP, xo)
            return fn

        def job_a(c):
            def fn(td):
                jn = j + 2 if first else jnp.minimum(j + 2, NP - 1)
                qc = q_cols(edge(z_buf[...]), jn, c)
                gate(td + LATP, qc)
                qraw_buf[c] = qc
            return fn

        def job_x(par, t):
            def fn(td):
                p = (p_buf0, p_buf1)[par][8 * t:8 * t + 8, :]
                rhs = jnp.concatenate([v_tile(h0 + par, a, t) for a in range(DH // 16)], axis=0)
                o = _dot_t(edge(_pack(p, p)), rhs)
                key = 'x%d' % par
                env[key] = o if key not in env else env[key] + o
                gate(td + LATP, env[key][:, 0:128])
            return fn

        def finish_head(par, inv, lhs_edge):
            acc = accp_buf[par * (DH // 2):(par + 1) * (DH // 2), :]
            o = _dot_t(lhs_edge(ones32), acc)
            if 'x%d' % par in env:
                o = o + env['x%d' % par]
            o = o * jnp.concatenate([inv, inv[:, 0:DH - 128]], axis=1)
            return o

        def job_e30(td):
            o = finish_head(0, ie_cur, edge)
            gate(td + LATP + 10, o[:, 0:128])
            env['op30'] = _pack(o, o)

        def job_g30(c):
            def fn(td):
                xo = out_cols(edge(env['op30']), 12 * h0, 12, c)
                xacc_buf[:, 128 * c:128 * (c + 1)] += xo
                gate(td + LATP, xo)
            return fn

        jobs = []
        for c in range(0 if first else CA, 4):
            for g in range(ng):
                tail = 'sm1' if (c == 3 and g == ng - 1) else None
                jobs.append((24, None, job_b(h0 + 1, 1, c, g, 's1', tail)))
        groups = {
            'e': [] if first else [(48, None, job_e)],
            'b': [] if last else [(24, None, job_b(h0 + 2, 0, c, g, 's2',
                                                   'sm2' if (c == 3 and g == ng - 1) else None))
                                  for c in range(4) for g in range(ng)],
            'a': [] if last else [(40, None, job_a(c)) for c in range(3)],
            'g': [] if first else [(24, None, job_g(c)) for c in range(5)],
            'n': [] if last else [(24, None, job_b(h0 + 3, 1, c, g, 's3',
                                                   'st' if (c == CA - 1 and g == ng - 1) else None))
                                  for c in range(CA) for g in range(ng)],
        }
        if last:
            t_even_end = (n_even + 1) * CPS / NS
            jobs += groups['e'] + [(24, None, job_x(0, t)) for t in range(nts[0], nt)] + groups['g']
            jobs += [(24, t_even_end, job_x(1, t)) for t in range(nts[1], nt)]
            jobs += [(32, t_even_end, job_e30)]
            jobs += [(12, t_even_end + LATP + 60, job_g30(c)) for c in range(5)]
        else:
            for ch in ORD:
                jobs += groups[ch]
        times = []
        tt = T0F if first else T0
        for cost, earliest, _ in jobs:
            tt += cost * RHO
            if earliest is not None:
                tt = max(tt, earliest)
            times.append(tt)

        states = [dict(accs=[None] * 24, half=0), dict(accs=[None] * 24, half=1)]
        nj = 0
        prev_last = None
        for st, (par, sw, t) in enumerate(steps):
            while nj < len(jobs) and times[nj] <= st * CPS / NS:
                jobs[nj][2](times[nj])
                nj += 1
            if st >= n_even and env.get('sm2') is not None:
                ps, env['ie'] = softmax(env['s2'], None)
                sched_stores(ps, p_buf0, max(env['sm2'] + LATP + MOFF, (st + 8) * CPS / NS),
                             len(steps) - 1)
                env['sm2'] = None
            for (pv_, g_, rs_, po_) in stores.pop(st, ()):
                store_p(pltpu.bitcast(edge(pltpu.bitcast(pv_, U32), 1), F32), g_, rs_, po_)
            gv = list(gates.get(st, ()))
            if CHAIN and t == 0 and prev_last is not None:
                gv.append(prev_last)
            pv_step(h0 + par, sw, t, nts[par], (p_buf0, p_buf1)[par], gv, true_mask, states[par])
            prev_last = states[par]['accs'][2 * (sw + 1) * na - 1]
            cur['state'] = states[par]
            cur['st'] = st
        while nj < len(jobs):
            jobs[nj][2](times[nj])
            nj += 1
        assert not stores
        if last:
            o = finish_head(1, env['io'], lambda x: x)
            op = _pack(o, o)
            return xacc_buf[...] + jnp.concatenate(
                [out_cols(op, 12 * (h0 + 1), 12, c) for c in range(5)], axis=1)
        return env['ie'], ie_cur, env['io']

    set_row(x2)
    xacc_buf[...] = x2
    q_pair(0)
    q_pair(1)
    _, inv0 = softmax(scores_all(0, 0), p_buf0)
    carry = block(0, (inv0, None, None), 'first')
    carry = lax.fori_loop(1, NP - 1, functools.partial(block, kind='mid'), carry)
    x3 = block(NP - 1, carry, 'last')
    x4 = x3 + b2 + _dot(mlp_hidden(x3), w2_buf[...])
    o_ref[...] = x4[0:1, :].astype(o_ref.dtype)


@jax.jit
def pallas_interleave_layers__sliding_block_cached__dense_activation_gelu__decode_kernel(
    A_x: jax.Array,
    A_k_cache: jax.Array,
    A_v_cache: jax.Array,
    A_wq: jax.Array,
    A_wo: jax.Array,
    B_x: jax.Array,
    B_w1: jax.Array,
    B_b1: jax.Array,
    B_w2: jax.Array,
    B_b2: jax.Array,
):
    sk = A_k_cache.shape[2]
    w = min(4096, max(256, sk // 4))

    def tile_view(a):
        *lead, r, c = a.shape
        n = len(lead)
        a = a.reshape(*lead, r // 8, 8, c // 128, 128)
        a = a.transpose(*range(n), n, n + 2, n + 1, n + 3)
        return a.reshape(*lead, r // 16, 2, (c // 128) * 8, 128)

    kx = tile_view(jnp.swapaxes(A_k_cache, 2, 3)[0])
    vx = tile_view(jnp.swapaxes(A_v_cache, 2, 3)[0])
    wqx = tile_view(A_wq)
    wox = tile_view(A_wo).reshape(H * DH // 16, 80, 128)
    any_spec = pl.BlockSpec(memory_space=pl.ANY)
    out = pl.pallas_call(
        functools.partial(_kernel, sk=sk, w=w),
        out_shape=jax.ShapeDtypeStruct((1, D), A_x.dtype),
        in_specs=[any_spec] * 9,
        out_specs=pl.BlockSpec(memory_space=pltpu.VMEM),
        scratch_shapes=[
            pltpu.VMEM((H, DH // 16, 2, w // 32, 128), U32),
            pltpu.VMEM((H, DH // 16, 2, w // 32, 128), U32),
            pltpu.VMEM((D // 16, 2, H * DH // 32, 128), U32),
            pltpu.VMEM((H * DH // 16, 40, 128), U32),
            pltpu.VMEM((D, F), BF16),
            pltpu.VMEM((F, D), BF16),
            pltpu.VMEM((1, D), BF16),
            pltpu.VMEM((F // 128, 128), BF16),
            pltpu.VMEM((D // 128, 128), BF16),
            pltpu.VMEM((w // 16, 128), F32),
            pltpu.VMEM((w // 16, 128), F32),
            pltpu.VMEM((w // 1024, 8, 128), F32),
            pltpu.VMEM((DH, 128), U32),
            pltpu.VMEM((8, D), U32),
            pltpu.VMEM((8, D), F32),
            pltpu.VMEM((4, 4, 8, 2 * DH), U32),
            pltpu.VMEM((3, 8, 128), F32),
            pltpu.VMEM((3 * NP, 8, 128), F32),
            pltpu.VMEM((8, F), F32),
            pltpu.VMEM((2, 8, 128), F32),
            pltpu.VMEM((8, 128), jnp.int32),
            pltpu.SemaphoreType.DMA((2,)),
            pltpu.SemaphoreType.DMA((2,)),
            pltpu.SemaphoreType.DMA((6 + W2C,)),
        ],
        compiler_params=pltpu.CompilerParams(vmem_limit_bytes=126 * 1024 * 1024),
    )(A_x.reshape(1, D), kx, vx, wqx, wox, B_w1, B_b1.reshape(F // 128, 128),
      B_w2, B_b2.reshape(D // 128, 128))
    return out.reshape(A_x.shape)
```

```python
import functools
import math

import jax
import jax.numpy as jnp
from jax import lax
import jax.experimental.pallas as pl
import jax.experimental.pallas.tpu as pltpu

F32 = jnp.float32
BF16 = jnp.bfloat16
U32 = jnp.uint32

D = 640
H = 32
DH = 192
F = 1536
EPS = 1e-5
NP = H // 2
OPT = {'CHAIN': '0'}
NS = int(OPT.get('NS', 4))
CA = int(OPT.get('CA', 2))
CPS = float(OPT.get('CPS', 18.7))
LATP = float(OPT.get('LATP', 160))
T0 = float(OPT.get('T0', 12))
T0F = float(OPT.get('T0F', -200))
RHO = float(OPT.get('RHO', 1.0))
BE = int(OPT.get('BE', 6))
MOFF = float(OPT.get('MOFF', 160))
MOFF2 = float(OPT.get('MOFF2', 240))
EC = float(OPT.get('EC', 48))
SG = int(OPT.get('SG', 4))
SDT = float(OPT.get('SDT', 12))
CHAIN = int(OPT.get('CHAIN', 1))
XE = int(OPT.get('XE', 6))
XO = int(OPT.get('XO', 7))
W2C = int(OPT.get('W2C', 4))
ORD = OPT.get('ORD', 'ebagn')
OPQ = int(OPT.get('OPQ', 0))
LA = int(OPT.get('LA', 1))
NE = int(OPT.get('NE', 7))
EE = int(OPT.get('EE', 2))
SE = int(OPT.get('SE', 1))
EOFF = float(OPT.get('EOFF', 0))
SM = int(OPT.get('SM', 1))
OM = int(OPT.get('OM', 1))
SKIP2 = int(OPT.get('SKIP2', 0))
SKIP1 = int(OPT.get('SKIP1', 0))


def _gelu(x):
    c = math.sqrt(2.0 / math.pi)
    return 0.5 * x * (1.0 + jnp.tanh(c * (x + 0.044715 * (x * x * x))))


def _rows_to_lanes(b, n):
    return jnp.concatenate([b[i:i + 1, :] for i in range(n)], axis=1)


def _bf(x):
    return pltpu.bitcast(x, BF16)


def _pack(a, b):
    return pltpu.bitcast(pltpu.pack_elementwise([a, b], packed_dtype=BF16), U32)


def _unpack(x):
    return (pltpu.unpack_elementwise(x, index=0, packed_dtype=BF16, unpacked_dtype=F32),
            pltpu.unpack_elementwise(x, index=1, packed_dtype=BF16, unpacked_dtype=F32))


def _dot(lhs32, rhs):
    return jnp.dot(_bf(lhs32), rhs, preferred_element_type=F32)[0:8]


def _dot_t(lhs32, rhs32):
    return lax.dot_general(_bf(lhs32), _bf(rhs32), (((1,), (1,)), ((), ())),
                           preferred_element_type=F32)[0:8]


def _ln_stats(xp):
    x = _unpack(xp)[0]
    m = jnp.mean(x, axis=-1, keepdims=True)
    xc = x - m
    v = jnp.mean(xc * xc, axis=-1, keepdims=True)
    return m, lax.rsqrt(v + EPS)


def _kernel(x_hbm, kx_hbm, vx_hbm, wq_hbm, wo_hbm, w1_hbm, b1_hbm, w2_hbm, b2_hbm,
            o_ref,
            kbuf, vbuf, wq_buf, wo_buf, w1_buf, w2_buf, x_buf, b1_buf, b2_buf,
            p_buf0, p_buf1, sp_buf, accp_buf, z_buf, xacc_buf, qv_buf, qraw_buf,
            csq_buf, cs1_buf, st_buf, tm_buf, zs_ref, s2_buf, op_buf,
            sem_k, sem_v, sem_w, *, sk, w):
    c_scale = (DH ** -0.5) * math.log2(math.e)
    nt = w // 128
    ng = nt // 8
    na = 12 // NS
    nst = NS * nt
    r0w = (sk - w) // 16
    nrw = w // 16
    w2r = F // W2C

    def k_copy(h):
        return pltpu.make_async_copy(kx_hbm.at[h, :, :, pl.ds(r0w, nrw), :],
                                     kbuf.bitcast(BF16).at[h], sem_k.at[h & 1])

    def v_copy(h):
        return pltpu.make_async_copy(vx_hbm.at[h, :, :, pl.ds(r0w, nrw), :],
                                     vbuf.bitcast(BF16).at[h], sem_v.at[h & 1])

    wq_cp = pltpu.make_async_copy(wq_hbm, wq_buf.bitcast(BF16), sem_w.at[0])
    wo_cp = pltpu.make_async_copy(wo_hbm, wo_buf.bitcast(BF16), sem_w.at[1])
    w1_cp = pltpu.make_async_copy(w1_hbm, w1_buf, sem_w.at[2])
    x_cp = pltpu.make_async_copy(x_hbm, x_buf, sem_w.at[3])
    b1_cp = pltpu.make_async_copy(b1_hbm, b1_buf, sem_w.at[4])
    b2_cp = pltpu.make_async_copy(b2_hbm, b2_buf, sem_w.at[5])
    w2_cps = [pltpu.make_async_copy(w2_hbm.at[pl.ds(i * w2r, w2r), :],
                                    w2_buf.at[pl.ds(i * w2r, w2r), :], sem_w.at[6 + i])
              for i in range(W2C)]

    if not SKIP1:
        wq_cp.start()
    x_cp.start()
    b1_cp.start()
    b2_cp.start()
    if not SKIP1:
        wo_cp.start()
        k_copy(0).start()
        v_copy(0).start()
    x_cp.wait()
    b1_cp.wait()
    b2_cp.wait()

    x0 = jnp.broadcast_to(x_buf[...].astype(F32), (8, D))
    b1 = _rows_to_lanes(b1_buf[...].astype(F32), F // 128)
    b2 = _rows_to_lanes(b2_buf[...].astype(F32), D // 128)

    lane = lax.broadcasted_iota(jnp.int32, (8, 128), 1)
    sub_lo = lax.broadcasted_iota(jnp.int32, (1, 8, 128), 1) < 4
    lo64 = lane < 64
    evn = (lane & 8) == 0
    zf = jnp.zeros((8, 128), F32)
    ones32 = jnp.full((8, 128), 0x3F803F80, U32)
    k_order = (
        list(range(0, 16, 2)) + list(range(1, 16, 2)) + [16, 18, 20, 22, 17, 19, 21, 23],
        list(range(8, 24, 2)) + list(range(9, 24, 2)) + [1, 3, 5, 7, 0, 2, 4, 6],
    )

    def swap_halves(ref2):
        n = ref2.shape[1]
        a = ref2[0].reshape(n // 8, 8, 128)
        b = ref2[1].reshape(n // 8, 8, 128)
        ref2[0] = jnp.where(sub_lo, a, pltpu.roll(b, 4, 1)).reshape(n, 128)
        ref2[1] = jnp.where(sub_lo, pltpu.roll(a, 4, 1), b).reshape(n, 128)

    def fix_wq(a, carry):
        swap_halves(wq_buf.at[a])
        return carry

    def fix_wo(g8, carry):
        g0 = pl.multiple_of(g8 * 8, 8)
        v = [wo_buf[pl.ds(g0, 8), 8 * c:8 * c + 8, :] for c in range(5)]
        n = [jnp.where(sub_lo, v[0], v[2]),
             pltpu.roll(jnp.where(sub_lo, v[3], v[0]), 4, 1),
             jnp.where(sub_lo, v[1], v[3]),
             pltpu.roll(jnp.where(sub_lo, v[4], v[1]), 4, 1),
             jnp.where(sub_lo, v[2], v[4])]
        for c in range(5):
            wo_buf[pl.ds(g0, 8), 8 * c:8 * c + 8, :] = n[c]
        return carry

    def set_row(x):
        xp = _pack(x, x)
        z_buf[...] = xp
        m, r = _ln_stats(xp)
        rc = r * c_scale
        st_buf[0] = jnp.broadcast_to(rc, (8, 128))
        st_buf[1] = jnp.broadcast_to(m * rc, (8, 128))

    def wq_cols(ct):
        r0 = pl.multiple_of(lax.shift_right_logical(ct, 1) * 8, 8) if not isinstance(ct, int) else (ct // 2) * 8
        return _bf(wq_buf[:, ct & 1, pl.ds(r0, 8), :].reshape(D // 2, 128))

    def q_cols(z, j, c):
        ct = 3 * j + c
        return _dot(z, wq_cols(ct)) * st_buf[0] - csq_buf[ct] * st_buf[1]

    def store_q(qs, j):
        q0, q1, q2 = qs
        r1 = pltpu.roll(q1, 56, 1)

        def lhs(qf, a2):
            a0 = jnp.where(evn, qf, zf)
            b1_ = jnp.where(evn, zf, qf)
            a2 = jnp.where(evn, a2, zf)
            return [_pack(a0, pltpu.roll(a0, 8, 1)), _pack(pltpu.roll(b1_, 120, 1), b1_),
                    _pack(a2, pltpu.roll(a2, 8, 1))]

        for hh, ww in ((2 * j, lhs(q0, jnp.where(lo64, q1, r1))),
                       (2 * j + 1, lhs(q2, jnp.where(lo64, r1, q1)))):
            for c in range(4):
                for i in range(3):
                    qv_buf[hh & 3, c, c:c + 1, 128 * i:128 * (i + 1)] = ww[i][c:c + 1, :]

    def q_pair(j):
        z = z_buf[...]
        store_q([q_cols(z, j, c) for c in range(3)], j)

    def score2(lhs, h, par, k):
        rhs = jnp.concatenate([kbuf[h, i // 2, i % 2, 8 * k:8 * k + 8, :] for i in k_order[par]],
                              axis=0)
        return _dot(lhs, _bf(rhs))

    def scores_all(h, par):
        sg = [None] * ng
        for c in range(4):
            lhs = qv_buf[h & 3, c]
            for g in range(ng):
                s = score2(lhs, h, par, 4 * g + c)
                sg[g] = s if sg[g] is None else sg[g] + s
        return sg

    def store_p(p, g, rs, p_out):
        for r in rs:
            p_out[pl.ds(64 * g + r, 8, stride=8), :] = p

    def softmax(sg, p_out):
        mx = sg[0]
        for s in sg[1:]:
            mx = jnp.maximum(mx, s)
        m = jnp.max(jnp.max(mx, axis=1, keepdims=True), axis=0, keepdims=True)
        l = None
        ps = []
        for g in range(ng):
            p = jnp.exp2(sg[g] - m)
            ps.append(p)
            if p_out is not None:
                store_p(p, g, range(8), p_out)
            l = p if l is None else l + p
        l = jnp.sum(jnp.sum(l, axis=1, keepdims=True), axis=0, keepdims=True)
        return ps, jnp.broadcast_to(1.0 / l, (8, 128))

    def v_tile(h, a, t):
        return vbuf[h, a, t % 2, 8 * (t // 2):8 * (t // 2) + 8, :]

    def pv_step(h, sw, t, n_t, p_in, gvals, true_mask, state):
        if sw == 0 or true_mask is None or not OPQ:
            p = p_in[8 * t:8 * t + 8, :]
        else:
            p = p_in[pl.ds(pl.multiple_of(zs_ref[sw] + 8 * t, 8), 8), :]
        for i, gval in enumerate(gvals):
            assert i < 3
            p = jnp.where(true_mask[i], p, gval)
        accs = state['accs']
        for a in range(sw * na, (sw + 1) * na):
            y0, y1 = _unpack(v_tile(h, a, t))
            for j, yy in ((2 * a, y0), (2 * a + 1, y1)):
                accs[j] = yy * p if t == 0 else accs[j] + yy * p
        state['sw'] = sw
        if t == n_t - 1:
            for a in range(sw * na, (sw + 1) * na):
                r0 = state['half'] * (DH // 2) + 8 * a
                accp_buf[r0:r0 + 8, :] = _pack(accs[2 * a], accs[2 * a + 1])

    def o_pair(ones, accp, ie, io):
        inv = jnp.concatenate([ie, jnp.where(lo64, ie, io), io], axis=1)
        return _dot_t(ones, accp) * inv

    def out_cols(op, g0, ngrp, c):
        rhs = wo_buf[pl.ds(g0, ngrp), 8 * c:8 * c + 8, :].reshape(ngrp * 8, 128)
        return _dot(op, _bf(rhs))

    def mlp_hidden(x):
        xp = _pack(x, x)
        m, r = _ln_stats(xp)
        hh = (_dot(xp, w1_buf[...]) - cs1_buf[...] * m) * r + b1
        g = _gelu(hh)
        return _pack(g, g)

    def pair1(j, carry):
        q_pair(j)
        invs = []
        for par in range(2):
            h = 2 * j + par
            k_copy(h).wait()

            @pl.when(h + 1 < H)
            def _():
                k_copy(h + 1).start()

            @pl.when(h + 1 == H)
            def _():
                w1_cp.start()

            _, inv = softmax(scores_all(h, par), p_buf0)
            invs.append(inv)
            v_copy(h).wait()

            @pl.when(h + 1 < H)
            def _():
                v_copy(h + 1).start()

            @pl.when(h + 1 == H)
            def _():
                for cp in w2_cps:
                    cp.start()

            def fix_v(a, c):
                swap_halves(vbuf.at[h, a])
                return c
            lax.fori_loop(0, DH // 16, fix_v, 0)
            state = dict(accs=[None] * 24, half=par)
            for sw in range(NS):
                for t in range(nt):
                    pv_step(h, sw, t, nt, p_buf0, (), None, state)
        o = o_pair(ones32, accp_buf[...], invs[0], invs[1])
        op = _pack(o, o)
        for c in range(5):
            xacc_buf[:, 128 * c:128 * (c + 1)] += out_cols(op, 24 * j, 24, c)
        return carry

    def colsum_q(ct, carry):
        ones = jnp.concatenate([ones32] * (D // 128), axis=1)
        csq_buf[ct] = _dot(ones, wq_cols(ct))
        return carry

    qv_buf[...] = jnp.zeros(qv_buf.shape, U32)
    for i in range(3):
        tm_buf[i] = lane
    for sw in range(NS):
        zs_ref[sw] = 0
    if not SKIP1:
        set_row(x0)
        xacc_buf[...] = x0
        wq_cp.wait()
        lax.fori_loop(0, D // 16, fix_wq, 0)
        lax.fori_loop(0, 3 * NP, colsum_q, 0)
        wo_cp.wait()
        lax.fori_loop(0, H * DH // 128, fix_wo, 0)
        lax.fori_loop(0, NP, pair1, 0)
        x1 = xacc_buf[...]
        w1_cp.wait()
        cs1_buf[...] = _dot(jnp.concatenate([ones32] * (D // 128), axis=1), w1_buf[...])
        gp = mlp_hidden(x1)
        x2 = x1 + b2
        for i in range(W2C):
            w2_cps[i].wait()
            x2 = x2 + _dot(gp[:, i * w2r:(i + 1) * w2r], w2_buf[i * w2r:(i + 1) * w2r, :])
    else:
        x2 = lax.fori_loop(0, 2, lambda i, x: x + 1.0, x0)

    if SKIP2:
        o_ref[...] = x2[0:1, :].astype(o_ref.dtype)
        return

    def block(j, carry, kind):
        ie_cur, ie, io = carry
        first, last = kind == 'first', kind == 'last'
        true_mask = [tm_buf[i] >= 0 for i in range(3)]
        h0 = 2 * j
        nts = (nt - XE, nt - XO) if last else (nt, nt)
        steps = [(par, sw, t) for par in range(2) for sw in range(NS) for t in range(nts[par])]
        n_even = NS * nts[0]
        env = dict(qs=[], nedge=0, s2=[None] * ng, s3=[None] * ng)
        env['s1'] = [None] * ng
        accp_prev = None if first else accp_buf[...]
        gates, stores = {}, {}
        cur = dict(state=None, st=-1)

        def step_at(cyc):
            return int(math.ceil(cyc * NS / CPS))

        def gate(cyc, v):
            st = step_at(cyc)
            while len(gates.get(st, ())) >= 2:
                st += 1
            if st < len(steps) and st > cur['st']:
                gates.setdefault(st, []).append(v)

        def edge(x, n=BE, force=False):
            if cur['st'] < 0 or not (force or cur['edge']):
                return x
            sw = cur['state']['sw']
            cand = list(range(2 * sw * na, 2 * (sw + 1) * na))
            ntile = -(-x.shape[1] // 128)
            parts = [x[:, 128 * i:min(128 * (i + 1), x.shape[1])] for i in range(ntile)]
            for e in range(min(n, 3 * ntile)):
                k_ = env['nedge'] % len(cand)
                c = cand[(2 * k_) % len(cand) + (2 * k_) // len(cand)]
                env['nedge'] += 1
                i = e % ntile
                w_ = parts[i].shape[1]
                assert e // ntile < 3
                parts[i] = jnp.where(true_mask[e // ntile][:, 0:w_], parts[i],
                                     pltpu.bitcast(cur['state']['accs'][c], U32)[:, 0:w_])
            return parts[0] if ntile == 1 else jnp.concatenate(parts, axis=1)

        def sched_stores(ps, p_out, t_ready, limit):
            gate(t_ready, ps[-1])
            n = 8 // SG
            for i in range(ng * n):
                g, k = divmod(i, n)
                st = min(max(step_at(t_ready + SDT * i) + 1, cur['st'] + 1), limit)
                stores.setdefault(st, []).append((ps[g], g, range(SG * k, SG * (k + 1)), p_out))

        def job_b(h, par, c, g, key, tail):
            def fn(td):
                s = score2(edge(qv_buf[h & 3, c]), h, par, 4 * g + c)
                sg = env[key]
                sg[g] = s if c == 0 else sg[g] + s
                gate(td + LATP, sg[g])
                if c == 3 and (key == 's3' or SM):
                    (sp_buf if key != 's2' else s2_buf)[g] = sg[g]
                    sg[g] = None
                if tail == 'sm1':
                    sg = [sp_buf[gg] if sg[gg] is None else sg[gg] for gg in range(ng)]
                    ps, env['io'] = softmax(sg, None)
                    sched_stores(ps, p_buf1, td + LATP + MOFF, n_even)
                    if not first and not last:
                        store_q([qraw_buf[i] for i in range(3)], j + 1)
                elif tail == 'sm2':
                    env['sm2'] = td
            return fn

        def job_e(td):
            o = o_pair(edge(ones32), accp_prev, ie, io)
            gate(td + LATP + 10, o[:, 256:384])
            if OM:
                op_buf[...] = _pack(o, o)
            else:
                env['op'] = _pack(o, o)

        def job_g(c):
            def fn(td):
                xo = out_cols(edge(op_buf[...] if OM else env['op']), 24 * (j - 1), 24, c)
                xacc_buf[:, 128 * c:128 * (c + 1)] += xo
                gate(td + LATP, xo)
            return fn

        def job_a(c):
            def fn(td):
                jn = j + 2 if first else jnp.minimum(j + 2, NP - 1)
                qc = q_cols(edge(z_buf[...]), jn, c)
                gate(td + LATP, qc)
                qraw_buf[c] = qc
            return fn

        def job_x(par, t):
            def fn(td):
                p = (p_buf0, p_buf1)[par][8 * t:8 * t + 8, :]
                rhs = jnp.concatenate([v_tile(h0 + par, a, t) for a in range(DH // 16)], axis=0)
                o = _dot_t(edge(_pack(p, p)), rhs)
                key = 'x%d' % par
                env[key] = o if key not in env else env[key] + o
                gate(td + LATP, env[key][:, 0:128])
            return fn

        def finish_head(par, inv, lhs_edge):
            acc = accp_buf[par * (DH // 2):(par + 1) * (DH // 2), :]
            o = _dot_t(lhs_edge(ones32), acc)
            if 'x%d' % par in env:
                o = o + env['x%d' % par]
            o = o * jnp.concatenate([inv, inv[:, 0:DH - 128]], axis=1)
            return o

        def job_e30(td):
            o = finish_head(0, ie_cur, edge)
            gate(td + LATP + 10, o[:, 0:128])
            env['op30'] = _pack(o, o)

        def job_g30(c):
            def fn(td):
                xo = out_cols(edge(env['op30']), 12 * h0, 12, c)
                xacc_buf[:, 128 * c:128 * (c + 1)] += xo
                gate(td + LATP, xo)
            return fn

        jobs = []
        for g in range(0 if first else CA, ng):
            for c in range(4):
                tail = 'sm1' if (c == 3 and g == ng - 1) else None
                jobs.append((24, None, job_b(h0 + 1, 1, c, g, 's1', tail), 3))
        groups = {
            'e': [] if first else [(EC, None, job_e, 3)],
            'b': [] if last else [(24, None, job_b(h0 + 2, 0, c, g, 's2',
                                                   'sm2' if (c == 3 and g == ng - 1) else None), 3)
                                  for g in range(ng) for c in range(4)],
            'a': [] if last else [(40, None, job_a(c), 5) for c in range(3)],
            'g': [] if first else [(24, None, job_g(c), 3) for c in range(5)],
            'n': [] if last else [(24, None, job_b(h0 + 3, 1, c, g, 's3', None), 3)
                                  for g in range(CA) for c in range(4)],
        }
        if last:
            t_even_end = (n_even + 1) * CPS / NS
            jobs += groups['e'] + [(24, None, job_x(0, t), 2) for t in range(nts[0], nt)] + groups['g']
            jobs += [(24, t_even_end, job_x(1, t), 2) for t in range(nts[1], nt)]
            jobs += [(32, t_even_end, job_e30, 2)]
            jobs += [(12, t_even_end + LATP + 60, job_g30(c), 2) for c in range(5)]
        else:
            for ch in ORD:
                jobs += groups[ch]
        times = []
        tt = T0F if first else T0
        tile_t = []
        for cost, earliest, _, ntile in jobs:
            t_prev = tt
            tt += cost * RHO
            if earliest is not None:
                tt = max(tt, earliest)
            tile_t += [tt - cost * RHO * (ntile - 1 - i) / ntile for i in range(ntile)]
            times.append(tt)
        done_t = []
        k = 0
        for i, job in enumerate(jobs):
            k += job[3]
            t_g = times[i] + LATP
            if k - 1 + LA < len(tile_t):
                t_g = max(t_g, tile_t[k - 1 + LA])
            done_t.append(t_g - LATP)

        states = [dict(accs=[None] * 24, half=0), dict(accs=[None] * 24, half=1)]
        nj = 0
        prev_last = None
        for st, (par, sw, t) in enumerate(steps):
            while nj < len(jobs) and times[nj] + EOFF <= st * CPS / NS:
                cur['edge'] = (nj < NE and nj % EE == EE - 1) or LA == 0 or jobs[nj][1] is not None
                jobs[nj][2](done_t[nj])
                nj += 1
            if st >= n_even and env.get('sm2') is not None:
                sg2 = [s2_buf[gg] if env['s2'][gg] is None else env['s2'][gg] for gg in range(ng)]
                ps, env['ie'] = softmax(sg2, None)
                sched_stores(ps, p_buf0, max(env['sm2'] + LATP + MOFF2, (st + 8) * CPS / NS),
                             len(steps) - 1)
                env['sm2'] = None
            for (pv_, g_, rs_, po_) in stores.pop(st, ()):
                store_p(pltpu.bitcast(edge(pltpu.bitcast(pv_, U32), SE, True), F32), g_, rs_, po_)
            gv = list(gates.get(st, ()))
            if CHAIN and t == 0 and prev_last is not None:
                gv.append(prev_last)
            pv_step(h0 + par, sw, t, nts[par], (p_buf0, p_buf1)[par], gv, true_mask, states[par])
            prev_last = states[par]['accs'][2 * (sw + 1) * na - 1]
            cur['state'] = states[par]
            cur['st'] = st
        while nj < len(jobs):
            cur['edge'] = False
            jobs[nj][2](done_t[nj])
            nj += 1
        assert not stores
        if last:
            o = finish_head(1, env['io'], lambda x: x)
            op = _pack(o, o)
            return xacc_buf[...] + jnp.concatenate(
                [out_cols(op, 12 * (h0 + 1), 12, c) for c in range(5)], axis=1)
        return env['ie'], ie_cur, env['io']

    set_row(x2)
    xacc_buf[...] = x2
    q_pair(0)
    q_pair(1)
    _, inv0 = softmax(scores_all(0, 0), p_buf0)
    carry = block(0, (inv0, None, None), 'first')
    carry = lax.fori_loop(1, NP - 1, functools.partial(block, kind='mid'), carry)
    x3 = block(NP - 1, carry, 'last')
    x4 = x3 + b2 + _dot(mlp_hidden(x3), w2_buf[...])
    o_ref[...] = x4[0:1, :].astype(o_ref.dtype)


@jax.jit
def pallas_interleave_layers__sliding_block_cached__dense_activation_gelu__decode_kernel(
    A_x: jax.Array,
    A_k_cache: jax.Array,
    A_v_cache: jax.Array,
    A_wq: jax.Array,
    A_wo: jax.Array,
    B_x: jax.Array,
    B_w1: jax.Array,
    B_b1: jax.Array,
    B_w2: jax.Array,
    B_b2: jax.Array,
):
    sk = A_k_cache.shape[2]
    w = min(4096, max(256, sk // 4))

    def tile_view(a):
        *lead, r, c = a.shape
        n = len(lead)
        a = a.reshape(*lead, r // 8, 8, c // 128, 128)
        a = a.transpose(*range(n), n, n + 2, n + 1, n + 3)
        return a.reshape(*lead, r // 16, 2, (c // 128) * 8, 128)

    kx = tile_view(jnp.swapaxes(A_k_cache, 2, 3)[0])
    vx = tile_view(jnp.swapaxes(A_v_cache, 2, 3)[0])
    wqx = tile_view(A_wq)
    wox = tile_view(A_wo).reshape(H * DH // 16, 80, 128)
    any_spec = pl.BlockSpec(memory_space=pl.ANY)
    out = pl.pallas_call(
        functools.partial(_kernel, sk=sk, w=w),
        out_shape=jax.ShapeDtypeStruct((1, D), A_x.dtype),
        in_specs=[any_spec] * 9,
        out_specs=pl.BlockSpec(memory_space=pltpu.VMEM),
        scratch_shapes=[
            pltpu.VMEM((H, DH // 16, 2, w // 32, 128), U32),
            pltpu.VMEM((H, DH // 16, 2, w // 32, 128), U32),
            pltpu.VMEM((D // 16, 2, H * DH // 32, 128), U32),
            pltpu.VMEM((H * DH // 16, 40, 128), U32),
            pltpu.VMEM((D, F), BF16),
            pltpu.VMEM((F, D), BF16),
            pltpu.VMEM((1, D), BF16),
            pltpu.VMEM((F // 128, 128), BF16),
            pltpu.VMEM((D // 128, 128), BF16),
            pltpu.VMEM((w // 16, 128), F32),
            pltpu.VMEM((w // 16, 128), F32),
            pltpu.VMEM((w // 1024, 8, 128), F32),
            pltpu.VMEM((DH, 128), U32),
            pltpu.VMEM((8, D), U32),
            pltpu.VMEM((8, D), F32),
            pltpu.VMEM((4, 4, 8, 2 * DH), U32),
            pltpu.VMEM((3, 8, 128), F32),
            pltpu.VMEM((3 * NP, 8, 128), F32),
            pltpu.VMEM((8, F), F32),
            pltpu.VMEM((2, 8, 128), F32),
            pltpu.VMEM((3, 8, 128), jnp.int32),
            pltpu.SMEM((NS,), jnp.int32),
            pltpu.VMEM((w // 1024, 8, 128), F32),
            pltpu.VMEM((8, 2 * DH), U32),
            pltpu.SemaphoreType.DMA((2,)),
            pltpu.SemaphoreType.DMA((2,)),
            pltpu.SemaphoreType.DMA((6 + W2C,)),
        ],
        compiler_params=pltpu.CompilerParams(vmem_limit_bytes=126 * 1024 * 1024),
    )(A_x.reshape(1, D), kx, vx, wqx, wox, B_w1, B_b1.reshape(F // 128, 128),
      B_w2, B_b2.reshape(D // 128, 128))
    return out.reshape(A_x.shape)
```

```python
import functools
import math

import jax
import jax.numpy as jnp
from jax import lax
import jax.experimental.pallas as pl
import jax.experimental.pallas.tpu as pltpu

F32 = jnp.float32
BF16 = jnp.bfloat16
U32 = jnp.uint32

D = 640
H = 32
DH = 192
F = 1536
EPS = 1e-5
NP = H // 2
OPT = {}
NS = int(OPT.get('NS', 4))
CA = int(OPT.get('CA', 2))
CU = float(OPT.get('CU', 0.265))
XF = int(OPT.get('XF', 6))
CHUNKS = [int(c) for c in OPT.get('CHUNKS', '44322 1').replace(' ', '')]
LATP = float(OPT.get('LATP', 160))
T0 = float(OPT.get('T0', -10))
T0F = float(OPT.get('T0F', -200))
RHO = float(OPT.get('RHO', 1.0))
BE = int(OPT.get('BE', 6))
MOFF = float(OPT.get('MOFF', 160))
MOFF2 = float(OPT.get('MOFF2', 240))
EC = float(OPT.get('EC', 48))
SG = int(OPT.get('SG', 4))
SDT = float(OPT.get('SDT', 12))
CHAIN = int(OPT.get('CHAIN', 0))
XE = int(OPT.get('XE', 6))
XO = int(OPT.get('XO', 7))
W2R = [128 * int(c) for c in OPT.get('W2R', '5421')]
W2C = len(W2R)
W2S = [sum(W2R[:i]) for i in range(W2C)]
ORD = OPT.get('ORD', 'ebagn')
OPQ = int(OPT.get('OPQ', 0))
LA = int(OPT.get('LA', 1))
NE = int(OPT.get('NE', 7))
EE = int(OPT.get('EE', 2))
SE = int(OPT.get('SE', 1))
EOFF = float(OPT.get('EOFF', 0))
SM = int(OPT.get('SM', 1))
OM = int(OPT.get('OM', 1))
U = int(OPT.get('U', 2))
NF = int(OPT.get('NF', 0))
NL = int(OPT.get('NL', 0))
EDEL = float(OPT.get('EDEL', 70))
RHO0 = float(OPT.get('RHO0', 1.0))
RHOL = float(OPT.get('RHOL', 1.0))
BAR = int(OPT.get('BAR', 0))
IOFF = float(OPT.get('IOFF', 0))
DYN = int(OPT.get('DYN', 0))
MST = int(OPT.get('MST', 1))
DSC = int(OPT.get('DSC', 1))
DBC = int(OPT.get('DBC', 0))
SKIP2 = int(OPT.get('SKIP2', 0))
SKIP1 = int(OPT.get('SKIP1', 0))


def _gelu(x):
    c = math.sqrt(2.0 / math.pi)
    return 0.5 * x * (1.0 + jnp.tanh(c * (x + 0.044715 * (x * x * x))))


def _rows_to_lanes(b, n):
    return jnp.concatenate([b[i:i + 1, :] for i in range(n)], axis=1)


def _bf(x):
    return pltpu.bitcast(x, BF16)


def _pack(a, b):
    return pltpu.bitcast(pltpu.pack_elementwise([a, b], packed_dtype=BF16), U32)


def _unpack(x):
    return (pltpu.unpack_elementwise(x, index=0, packed_dtype=BF16, unpacked_dtype=F32),
            pltpu.unpack_elementwise(x, index=1, packed_dtype=BF16, unpacked_dtype=F32))


def _dot(lhs32, rhs):
    return jnp.dot(_bf(lhs32), rhs, preferred_element_type=F32)[0:8]


def _dot_t(lhs32, rhs32):
    return lax.dot_general(_bf(lhs32), _bf(rhs32), (((1,), (1,)), ((), ())),
                           preferred_element_type=F32)[0:8]


def _ln_stats(xp):
    x = _unpack(xp)[0]
    m = jnp.mean(x, axis=-1, keepdims=True)
    xc = x - m
    v = jnp.mean(xc * xc, axis=-1, keepdims=True)
    return m, lax.rsqrt(v + EPS)


def _kernel(x_hbm, kx_hbm, vx_hbm, wq_hbm, wo_hbm, w1_hbm, b1_hbm, w2_hbm, b2_hbm,
            o_ref,
            kbuf, vbuf, vf_buf, wq_buf, wo_buf, w1_buf, w2_buf, x_buf, b1_buf, b2_buf,
            p_buf0, p_buf1, sp_buf, accp_buf, z_buf, xacc_buf, qv_buf, qraw_buf,
            csq_buf, cs1_buf, st_buf, tm_buf, zs_ref, s2_buf, op_buf,
            sem_k, sem_v, sem_w, *, sk, w):
    c_scale = (DH ** -0.5) * math.log2(math.e)
    nt = w // 128
    ng = nt // 8
    na = 12 // NS
    nst = NS * nt
    r0w = (sk - w) // 16
    nrw = w // 16

    ntb = nt - XF
    starts = [sum(CHUNKS[:c]) for c in range(len(CHUNKS))]
    assert sum(CHUNKS) == NP

    def k_copy(c):
        rows = pl.ds(48 * starts[c], 48 * CHUNKS[c])
        return [pltpu.make_async_copy(kx_hbm.at[rows, pl.ds(r0w, nrw), :],
                                      kbuf.bitcast(BF16).at[rows], sem_k.at[c & 1])]

    def v_copy(c):
        rows = pl.ds(48 * starts[c], 48 * CHUNKS[c])
        cps = [pltpu.make_async_copy(vx_hbm.at[rows, pl.ds(r0w, 8 * ntb), :],
                                     vbuf.bitcast(BF16).at[rows], sem_v.at[c & 1])]
        if XF:
            cps.append(pltpu.make_async_copy(
                vx_hbm.at[rows, pl.ds(r0w + 8 * ntb, 8 * XF), :],
                vf_buf.bitcast(BF16).at[rows, pl.ds(8 * XF, 8 * XF), :], sem_v.at[2 + (c & 1)]))
        return cps

    wq_cp = pltpu.make_async_copy(wq_hbm, wq_buf.bitcast(BF16), sem_w.at[0])
    wo_cp = pltpu.make_async_copy(wo_hbm, wo_buf.bitcast(BF16), sem_w.at[1])
    w1_cp = pltpu.make_async_copy(w1_hbm, w1_buf, sem_w.at[2])
    x_cp = pltpu.make_async_copy(x_hbm, x_buf, sem_w.at[3])
    b1_cp = pltpu.make_async_copy(b1_hbm, b1_buf, sem_w.at[4])
    b2_cp = pltpu.make_async_copy(b2_hbm, b2_buf, sem_w.at[5])
    w2_cps = [pltpu.make_async_copy(w2_hbm.at[pl.ds(W2S[i], W2R[i]), :],
                                    w2_buf.at[pl.ds(W2S[i], W2R[i]), :], sem_w.at[6 + i])
              for i in range(W2C)]

    if not SKIP1:
        wq_cp.start()
    x_cp.start()
    b1_cp.start()
    b2_cp.start()
    if not SKIP1:
        wo_cp.start()
        for cp in k_copy(0) + v_copy(0):
            cp.start()
    x_cp.wait()
    b1_cp.wait()
    b2_cp.wait()

    x0 = jnp.broadcast_to(x_buf[...].astype(F32), (8, D))
    b1 = _rows_to_lanes(b1_buf[...].astype(F32), F // 128)
    b2 = _rows_to_lanes(b2_buf[...].astype(F32), D // 128)

    lane = lax.broadcasted_iota(jnp.int32, (8, 128), 1)
    sub_lo = lax.broadcasted_iota(jnp.int32, (1, 8, 128), 1) < 4
    lo64 = lane < 64
    sub = lax.broadcasted_iota(jnp.int32, (8, 128), 0)
    evn = (lane & 8) == 0
    zf = jnp.zeros((8, 128), F32)
    ones32 = jnp.full((8, 128), 0x3F803F80, U32)
    k_order = (
        list(range(0, 16, 2)) + list(range(1, 16, 2)) + [16, 18, 20, 22, 17, 19, 21, 23],
        list(range(8, 24, 2)) + list(range(9, 24, 2)) + [1, 3, 5, 7, 0, 2, 4, 6],
    )

    def swap_halves(ref2):
        n = ref2.shape[1]
        a = ref2[0].reshape(n // 8, 8, 128)
        b = ref2[1].reshape(n // 8, 8, 128)
        ref2[0] = jnp.where(sub_lo, a, pltpu.roll(b, 4, 1)).reshape(n, 128)
        ref2[1] = jnp.where(sub_lo, pltpu.roll(a, 4, 1), b).reshape(n, 128)

    def fix_wq(a, carry):
        swap_halves(wq_buf.at[a])
        return carry

    def fix_wo(g8, carry):
        g0 = pl.multiple_of(g8 * 8, 8)
        v = [wo_buf[pl.ds(g0, 8), 8 * c:8 * c + 8, :] for c in range(5)]
        n = [jnp.where(sub_lo, v[0], v[2]),
             pltpu.roll(jnp.where(sub_lo, v[3], v[0]), 4, 1),
             jnp.where(sub_lo, v[1], v[3]),
             pltpu.roll(jnp.where(sub_lo, v[4], v[1]), 4, 1),
             jnp.where(sub_lo, v[2], v[4])]
        for c in range(5):
            wo_buf[pl.ds(g0, 8), 8 * c:8 * c + 8, :] = n[c]
        return carry

    def set_row(x):
        xp = _pack(x, x)
        z_buf[...] = xp
        m, r = _ln_stats(xp)
        rc = r * c_scale
        st_buf[0] = jnp.broadcast_to(rc, (8, 128))
        st_buf[1] = jnp.broadcast_to(m * rc, (8, 128))

    def wq_cols(ct):
        r0 = pl.multiple_of(lax.shift_right_logical(ct, 1) * 8, 8) if not isinstance(ct, int) else (ct // 2) * 8
        return _bf(wq_buf[:, ct & 1, pl.ds(r0, 8), :].reshape(D // 2, 128))

    def q_cols(z, j, c):
        ct = 3 * j + c
        return _dot(z, wq_cols(ct)) * st_buf[0] - csq_buf[ct] * st_buf[1]

    def store_q(qs, j):
        q0, q1, q2 = qs
        r1 = pltpu.roll(q1, 56, 1)

        def lhs(qf, a2):
            a0 = jnp.where(evn, qf, zf)
            b1_ = jnp.where(evn, zf, qf)
            a2 = jnp.where(evn, a2, zf)
            return [_pack(a0, pltpu.roll(a0, 8, 1)), _pack(pltpu.roll(b1_, 120, 1), b1_),
                    _pack(a2, pltpu.roll(a2, 8, 1))]

        for hh, ww in ((2 * j, lhs(q0, jnp.where(lo64, q1, r1))),
                       (2 * j + 1, lhs(q2, jnp.where(lo64, r1, q1)))):
            for c in range(4):
                for i in range(3):
                    if MST:
                        pltpu.store(qv_buf.at[hh & 3, c, :, 128 * i:128 * (i + 1)], ww[i], mask=sub == c)
                    else:
                        qv_buf[hh & 3, c, c:c + 1, 128 * i:128 * (i + 1)] = ww[i][c:c + 1, :]

    def q_pair(j):
        z = z_buf[...]
        store_q([q_cols(z, j, c) for c in range(3)], j)

    def score2(lhs, h, par, k):
        rhs = jnp.concatenate([kbuf[24 * h + i, 8 * k:8 * k + 8, :] for i in k_order[par]],
                              axis=0)
        return _dot(lhs, _bf(rhs))

    def scores_all(h, par):
        sg = [None] * ng
        for c in range(4):
            lhs = qv_buf[h & 3, c]
            for g in range(ng):
                s = score2(lhs, h, par, 4 * g + c)
                sg[g] = s if sg[g] is None else sg[g] + s
        return sg

    def store_p(p, g, rs, p_out):
        for r in rs:
            p_out[pl.ds(64 * g + r, 8, stride=8), :] = p

    def softmax(sg, p_out):
        mx = sg[0]
        for s in sg[1:]:
            mx = jnp.maximum(mx, s)
        m = jnp.max(jnp.max(mx, axis=1, keepdims=True), axis=0, keepdims=True)
        l = None
        ps = []
        for g in range(ng):
            p = jnp.exp2(sg[g] - m)
            ps.append(p)
            if p_out is not None:
                store_p(p, g, range(8), p_out)
            l = p if l is None else l + p
        l = jnp.sum(jnp.sum(l, axis=1, keepdims=True), axis=0, keepdims=True)
        return ps, jnp.broadcast_to(1.0 / l, (8, 128))

    def v_tile(h, a, t):
        return vbuf[24 * h + 2 * a + t % 2, 8 * (t // 2):8 * (t // 2) + 8, :]

    def pv_step(h, sw, t, ts, p_in, gvals, true_mask, state):
        p = p_in[8 * t:8 * t + 8, :]
        for i, gval in enumerate(gvals):
            p = jnp.where(true_mask[i], p, gval)
        accs = state['accs']
        for a in range(sw * na, (sw + 1) * na):
            if t < ntb:
                ys = _unpack(v_tile(h, a, t))
            else:
                r = 8 * (t - ntb)
                ys = [pltpu.bitcast(vf_buf[24 * h + 2 * a + e, r:r + 8, :], F32) for e in range(2)]
            for e in range(2):
                j = 2 * a + e
                accs[j] = ys[e] * p if t == ts[0] else accs[j] + ys[e] * p
        state['sw'] = sw
        if t == ts[-1]:
            for a in range(sw * na, (sw + 1) * na):
                r0 = state['half'] * (DH // 2) + 8 * a
                accp_buf[state['slot'], r0:r0 + 8, :] = _pack(accs[2 * a], accs[2 * a + 1])

    def o_pair(ones, accp, ie, io):
        inv = jnp.concatenate([ie, jnp.where(lo64, ie, io), io], axis=1)
        return _dot_t(ones, accp) * inv

    def out_cols(op, g0, ngrp, c):
        rhs = wo_buf[pl.ds(g0, ngrp), 8 * c:8 * c + 8, :].reshape(ngrp * 8, 128)
        return _dot(op, _bf(rhs))

    def mlp_hidden(x):
        xp = _pack(x, x)
        m, r = _ln_stats(xp)
        hh = (_dot(xp, w1_buf[...]) - cs1_buf[...] * m) * r + b1
        g = _gelu(hh)
        return _pack(g, g)

    def fix_v(r2, carry):
        swap_halves(vbuf.at[pl.ds(2 * r2, 2)])
        if XF:
            n = 4 * XF
            a = vf_buf[2 * r2, n:2 * n, :].reshape(n // 8, 8, 128)
            b = vf_buf[2 * r2 + 1, n:2 * n, :].reshape(n // 8, 8, 128)
            t0 = _unpack(jnp.where(sub_lo, a, pltpu.roll(b, 4, 1)))
            t1 = _unpack(jnp.where(sub_lo, pltpu.roll(a, 4, 1), b))
            for e in range(2):
                for k in range(XF // 2):
                    vf_buf[2 * r2 + e, 16 * k:16 * k + 8, :] = pltpu.bitcast(t0[e][k], U32)
                    vf_buf[2 * r2 + e, 16 * k + 8:16 * k + 16, :] = pltpu.bitcast(t1[e][k], U32)
        return carry

    def next_copies(j, copy_fn, tail_cps):
        for c in range(len(CHUNKS)):
            @pl.when(j == starts[c])
            def _():
                for cp in copy_fn(c):
                    cp.wait()
                for cp in (copy_fn(c + 1) if c + 1 < len(CHUNKS) else tail_cps):
                    cp.start()

    def pair1(j, carry):
        q_pair(j)
        next_copies(j, k_copy, [w1_cp])
        invs = []
        for par in range(2):
            _, inv = softmax(scores_all(2 * j + par, par), (p_buf0, p_buf1)[par])
            invs.append(inv)
        next_copies(j, v_copy, w2_cps)
        lax.fori_loop(24 * j, 24 * (j + 1), fix_v, 0)
        for par in range(2):
            state = dict(accs=[None] * 24, half=par, slot=0)
            for sw in range(NS):
                for t in range(nt):
                    pv_step(2 * j + par, sw, t, range(nt), (p_buf0, p_buf1)[par], (), None, state)
        o = o_pair(ones32, accp_buf[0], invs[0], invs[1])
        op = _pack(o, o)
        for c in range(5):
            xacc_buf[:, 128 * c:128 * (c + 1)] += out_cols(op, 24 * j, 24, c)
        return carry

    def colsum_q(ct, carry):
        ones = jnp.concatenate([ones32] * (D // 128), axis=1)
        csq_buf[ct] = _dot(ones, wq_cols(ct))
        return carry

    qv_buf[...] = jnp.zeros(qv_buf.shape, U32)
    for i in range(3):
        tm_buf[i] = lane
    zs_ref[0] = 8 * nt
    if not SKIP1:
        set_row(x0)
        xacc_buf[...] = x0
        wq_cp.wait()
        lax.fori_loop(0, D // 16, fix_wq, 0)
        lax.fori_loop(0, 3 * NP, colsum_q, 0)
        wo_cp.wait()
        lax.fori_loop(0, H * DH // 128, fix_wo, 0)
        lax.fori_loop(0, NP, pair1, 0)
        x1 = xacc_buf[...]
        w1_cp.wait()
        cs1_buf[...] = _dot(jnp.concatenate([ones32] * (D // 128), axis=1), w1_buf[...])
        gp = mlp_hidden(x1)
        x2 = x1 + b2
        for i in range(W2C):
            w2_cps[i].wait()
            x2 = x2 + _dot(gp[:, W2S[i]:W2S[i] + W2R[i]], w2_buf[W2S[i]:W2S[i] + W2R[i], :])
    else:
        x2 = lax.fori_loop(0, 2, lambda i, x: x + 1.0, x0)

    if SKIP2:
        o_ref[...] = x2[0:1, :].astype(o_ref.dtype)
        return

    def block(j0, carry, kinds, jpar=None):
        true_mask = [tm_buf[i] >= 0 for i in range(3)]
        pad_row = pl.multiple_of(zs_ref[0], 8)
        steps = []
        info = []
        for u, kind in enumerate(kinds):
            xs = (XE, XO) if kind == 'last' else (0, 0)
            tss = [list(range(x, nt)) for x in xs]
            s0 = len(steps)
            steps += [(u, par, sw, t) for par in range(2) for sw in range(NS) for t in tss[par]]
            info.append(dict(tss=tss, s0=s0, s_odd=s0 + NS * len(tss[0]), s_end=len(steps)))
        t_step = [0.0]
        for (_, _, _, t) in steps:
            t_step.append(t_step[-1] + CU * na * (6 if t < ntb else 4))
        gates, stores = {}, {}
        cur = dict(state=None, st=-1, nedge=0)
        envs = [dict(s1=[None] * ng, s2=[None] * ng, s3=[None] * ng) for _ in kinds]
        envs[0]['ie_cur'], envs[0]['ie'], envs[0]['io_prev'] = carry

        def slot(u):
            return (j0 + u) & 1 if jpar is None else (jpar + u) & 1

        def step_at(cyc):
            return next((i for i, tt_ in enumerate(t_step) if tt_ >= cyc), len(t_step))

        def gate(cyc, v):
            st = step_at(cyc)
            while len(gates.get(st, ())) >= 2:
                st += 1
            if st < len(steps) and st > cur['st']:
                gates.setdefault(st, []).append(v)

        def edge(x, n=BE, force=False):
            if cur['st'] < 0 or not (force or cur['edge']):
                return x
            sw = cur['state']['sw']
            cand = list(range(2 * sw * na, 2 * (sw + 1) * na))
            ntile = -(-x.shape[1] // 128)
            parts = [x[:, 128 * i:min(128 * (i + 1), x.shape[1])] for i in range(ntile)]
            for e in range(min(n, 3 * ntile)):
                k_ = cur['nedge'] % len(cand)
                c = cand[(2 * k_) % len(cand) + (2 * k_) // len(cand)]
                cur['nedge'] += 1
                i = e % ntile
                w_ = parts[i].shape[1]
                parts[i] = jnp.where(true_mask[e // ntile][:, 0:w_], parts[i],
                                     pltpu.bitcast(cur['state']['accs'][c], U32)[:, 0:w_])
            return parts[0] if ntile == 1 else jnp.concatenate(parts, axis=1)

        def sched_stores(ps, inv, p_out, t_ready, lo, hi):
            gate(t_ready, ps[-1])
            if IOFF:
                gate(t_ready + IOFF, inv)
            n = 8 // SG
            t_first = max(t_ready, t_step[lo])
            for i in range(ng * n):
                g, k = divmod(i, n)
                st = min(max(step_at(t_first + SDT * i) + 1, cur['st'] + 1), hi)
                stores.setdefault(st, []).append((ps[g], g, range(SG * k, SG * (k + 1)), p_out))

        def pair_jobs(u):
            kind, env, inf = kinds[u], envs[u], info[u]
            first, last = kind == 'first', kind == 'last'
            j = j0 + u
            h0 = 2 * j

            def job_b(h, par, c, g, key, tail):
                def fn(td):
                    s = score2(edge(qv_buf[h & 3, c]), h, par, 4 * g + c)
                    sg = env[key]
                    sg[g] = s if c == 0 else sg[g] + s
                    gate(td + LATP, sg[g])
                    if c == 3:
                        (sp_buf if key != 's2' else s2_buf)[g] = sg[g]
                    if tail == 'sm1':
                        ps, env['io'] = softmax([sp_buf[gg] for gg in range(ng)], None)
                        sched_stores(ps, env['io'], p_buf1, td + LATP + MOFF, inf['s0'], inf['s_odd'])
                        if not first and not last:
                            store_q([qraw_buf[i] for i in range(3)], j + 1)
                    elif tail == 'sm2':
                        ps, env['ie_next'] = softmax([s2_buf[gg] for gg in range(ng)], None)
                        sched_stores(ps, env['ie_next'], p_buf0, td + LATP + MOFF2, inf['s_odd'], inf['s_end'] - 1)
                return fn

            def job_e(td):
                if u > 0:
                    env['ie'], env['io_prev'] = envs[u - 1]['ie_cur'], envs[u - 1]['io']
                    env['ie_cur'] = envs[u - 1]['ie_next']
                o = o_pair(edge(ones32), accp_buf[1 - slot(u)], env['ie'], env['io_prev'])
                gate(td + LATP + 10, o[:, 256:384])
                op_buf[...] = _pack(o, o)

            def job_g(c):
                def fn(td):
                    xo = out_cols(edge(op_buf[...]), 24 * (j - 1), 24, c)
                    xacc_buf[:, 128 * c:128 * (c + 1)] += xo
                    gate(td + LATP, xo)
                return fn

            def job_a(c):
                def fn(td):
                    jn = j + 2 if isinstance(j, int) else jnp.minimum(j + 2, NP - 1)
                    qc = q_cols(edge(z_buf[...]), jn, c)
                    gate(td + LATP, qc)
                    qraw_buf[c] = qc
                return fn

            def job_x(par, t):
                def fn(td):
                    p = (p_buf0, p_buf1)[par][8 * t:8 * t + 8, :]
                    rhs = jnp.concatenate([v_tile(h0 + par, a, t) for a in range(DH // 16)], axis=0)
                    o = _dot_t(edge(_pack(p, p)), rhs)
                    key = 'x%d' % par
                    env[key] = o if key not in env else env[key] + o
                    gate(td + LATP, env[key][:, 0:128])
                return fn

            def finish_head(par, inv, lhs_edge):
                acc = accp_buf[slot(u), par * (DH // 2):(par + 1) * (DH // 2), :]
                o = _dot_t(lhs_edge(ones32), acc)
                if 'x%d' % par in env:
                    o = o + env['x%d' % par]
                return o * jnp.concatenate([inv, inv[:, 0:DH - 128]], axis=1)

            env['finish_head'] = finish_head

            def job_e30(td):
                o = finish_head(0, env['ie_cur'], edge)
                gate(td + LATP + 10, o[:, 0:128])
                env['op30'] = _pack(o, o)

            def job_g30(c):
                def fn(td):
                    xo = out_cols(edge(env['op30']), 12 * h0, 12, c)
                    xacc_buf[:, 128 * c:128 * (c + 1)] += xo
                    gate(td + LATP, xo)
                return fn

            jobs = []
            for g in range(0 if first else CA, ng):
                for c in range(4):
                    tail = 'sm1' if (c == 3 and g == ng - 1) else None
                    jobs.append((24, None, job_b(h0 + 1, 1, c, g, 's1', tail), 3))
            t_pair = t_step[inf['s0']] + EDEL if u > 0 else None
            groups = {
                'e': [] if first else [(EC, t_pair, job_e, 3)],
                'b': [(24, None, job_b(h0 + 2, 0, c, g, 's2',
                                       'sm2' if (c == 3 and g == ng - 1) else None), 3)
                      for g in range(ng) for c in range(4)],
                'a': [] if isinstance(j, int) and j + 2 >= NP else
                     [(40, None, job_a(c), 5) for c in range(3)],
                'g': [] if first else [(24, None, job_g(c), 3) for c in range(5)],
                'n': [(24, None, job_b(h0 + 3, 1, c, g, 's3', None), 3)
                      for g in range(CA) for c in range(4)],
            }
            if last:
                t_odd = t_step[inf['s_odd'] + 1]
                jobs += groups['e'] + [(24, None, job_x(0, t), 2) for t in range(XE)] + groups['g']
                jobs += [(24, t_odd, job_x(1, t), 2) for t in range(XO)]
                jobs += [(32, t_odd, job_e30, 2)]
                jobs += [(12, t_odd + LATP + 60, job_g30(c), 2) for c in range(5)]
            else:
                for ch in ORD:
                    jobs += groups[ch]
            return jobs

        pjobs = [pair_jobs(u) for u in range(len(kinds))]
        jobs = [job for pj in pjobs for job in pj]
        rhos = [RHO if 0 < u < len(kinds) - 1 else (RHO0 if u == 0 else RHOL) for u, pj in enumerate(pjobs) for _ in pj]
        times = []
        tt = T0F if kinds[0] == 'first' else T0
        for (cost, earliest, _, _), rho in zip(jobs, rhos):
            tt += cost * rho
            if earliest is not None:
                tt = max(tt, earliest)
            times.append(tt)

        states = {}
        nj = 0
        for st, (u, par, sw, t) in enumerate(steps):
            while nj < len(jobs) and times[nj] + EOFF <= t_step[st]:
                if times[nj] > 0 and 'j0' not in cur:
                    cur['j0'] = nj
                rel = nj - cur.get('j0', nj + 1)
                cur['edge'] = (0 <= rel < NE and rel % EE == EE - 1) or jobs[nj][1] == times[nj]
                jobs[nj][2](times[nj])
                nj += 1
            for (pv_, g_, rs_, po_) in stores.pop(st, ()):
                store_p(pltpu.bitcast(edge(pltpu.bitcast(pv_, U32), SE, True), F32), g_, rs_, po_)
            state = states.setdefault((u, par), dict(accs=[None] * 24, half=par, slot=slot(u)))
            if BAR and sw > 0 and t == info[u]['tss'][par][0]:
                (p_buf0, p_buf1)[par][pl.ds(pad_row, 8), :] = zf
            pv_step(2 * (j0 + u) + par, sw, t, info[u]['tss'][par], (p_buf0, p_buf1)[par],
                    gates.get(st, ()), true_mask, state)
            cur['state'] = state
            cur['st'] = st
        cur['edge'] = False
        while nj < len(jobs):
            jobs[nj][2](times[nj])
            nj += 1
        assert not stores
        env = envs[-1]
        if kinds[-1] == 'last':
            o = env['finish_head'](1, env['io'], lambda x: x)
            op = _pack(o, o)
            return xacc_buf[...] + jnp.concatenate(
                [out_cols(op, 12 * (H - 1), 12, c) for c in range(5)], axis=1)
        return env['ie_next'], env['ie_cur'], env['io']

    set_row(x2)
    xacc_buf[...] = x2
    q_pair(0)
    q_pair(1)
    _, inv0 = softmax(scores_all(0, 0), p_buf0)
    carry = block(0, (inv0, None, None), ['first'] + ['mid'] * NF)
    n_mid = (NP - 2 - NF - NL) // U
    carry = lax.fori_loop(0, n_mid, lambda i, c: block(1 + NF + U * i, c, ['mid'] * U, (1 + NF) & 1 if U % 2 == 0 and not DYN else None), carry)
    x3 = block(NP - 1 - NL, carry, ['mid'] * NL + ['last'])
    x4 = x3 + b2 + _dot(mlp_hidden(x3), w2_buf[...])
    o_ref[...] = x4[0:1, :].astype(o_ref.dtype)


@jax.jit
def pallas_interleave_layers__sliding_block_cached__dense_activation_gelu__decode_kernel(
    A_x: jax.Array,
    A_k_cache: jax.Array,
    A_v_cache: jax.Array,
    A_wq: jax.Array,
    A_wo: jax.Array,
    B_x: jax.Array,
    B_w1: jax.Array,
    B_b1: jax.Array,
    B_w2: jax.Array,
    B_b2: jax.Array,
):
    sk = A_k_cache.shape[2]
    w = min(4096, max(256, sk // 4))

    def tile_view(a):
        *lead, r, c = a.shape
        n = len(lead)
        a = a.reshape(*lead, r // 8, 8, c // 128, 128)
        a = a.transpose(*range(n), n, n + 2, n + 1, n + 3)
        return a.reshape(*lead, r // 16, 2, (c // 128) * 8, 128)

    kx = tile_view(jnp.swapaxes(A_k_cache, 2, 3)[0]).reshape(H * DH // 8, sk // 16, 128)
    vx = tile_view(jnp.swapaxes(A_v_cache, 2, 3)[0]).reshape(H * DH // 8, sk // 16, 128)
    wqx = tile_view(A_wq)
    wox = tile_view(A_wo).reshape(H * DH // 16, 80, 128)
    any_spec = pl.BlockSpec(memory_space=pl.ANY)
    out = pl.pallas_call(
        functools.partial(_kernel, sk=sk, w=w),
        out_shape=jax.ShapeDtypeStruct((1, D), A_x.dtype),
        in_specs=[any_spec] * 9,
        out_specs=pl.BlockSpec(memory_space=pltpu.VMEM),
        scratch_shapes=[
            pltpu.VMEM((H * DH // 8, w // 32, 128), U32),
            pltpu.VMEM((H * DH // 8, w // 32 - 4 * XF, 128), U32),
            pltpu.VMEM((H * DH // 8, max(8 * XF, 8), 128), U32),
            pltpu.VMEM((D // 16, 2, H * DH // 32, 128), U32),
            pltpu.VMEM((H * DH // 16, 40, 128), U32),
            pltpu.VMEM((D, F), BF16),
            pltpu.VMEM((F, D), BF16),
            pltpu.VMEM((1, D), BF16),
            pltpu.VMEM((F // 128, 128), BF16),
            pltpu.VMEM((D // 128, 128), BF16),
            pltpu.VMEM((w // 16 + 8, 128), F32),
            pltpu.VMEM((w // 16 + 8, 128), F32),
            pltpu.VMEM((w // 1024, 8, 128), F32),
            pltpu.VMEM((2, DH, 128), U32),
            pltpu.VMEM((8, D), U32),
            pltpu.VMEM((8, D), F32),
            pltpu.VMEM((4, 4, 8, 2 * DH), U32),
            pltpu.VMEM((3, 8, 128), F32),
            pltpu.VMEM((3 * NP, 8, 128), F32),
            pltpu.VMEM((8, F), F32),
            pltpu.VMEM((2, 8, 128), F32),
            pltpu.VMEM((3, 8, 128), jnp.int32),
            pltpu.SMEM((NS,), jnp.int32),
            pltpu.VMEM((w // 1024, 8, 128), F32),
            pltpu.VMEM((8, 2 * DH), U32),
            pltpu.SemaphoreType.DMA((2,)),
            pltpu.SemaphoreType.DMA((4,)),
            pltpu.SemaphoreType.DMA((6 + W2C,)),
        ],
        compiler_params=pltpu.CompilerParams(vmem_limit_bytes=int(OPT.get('VM', 127)) * 1024 * 1024,
                                             disable_semaphore_checks=bool(DSC), disable_bounds_checks=bool(DBC)),
    )(A_x.reshape(1, D), kx, vx, wqx, wox, B_w1, B_b1.reshape(F // 128, 128),
      B_w2, B_b2.reshape(D // 128, 128))
    return out.reshape(A_x.shape)
```

```python
import functools
import math

import jax
import jax.numpy as jnp
from jax import lax
import jax.experimental.pallas as pl
import jax.experimental.pallas.tpu as pltpu

F32 = jnp.float32
BF16 = jnp.bfloat16
U32 = jnp.uint32

D = 640
H = 32
DH = 192
F = 1536
EPS = 1e-5
NP = H // 2
OPT = {'NF': '2', 'NL': '4', 'RHO': '1.1', 'RHOL': '1.04', 'XE': '7', 'XO': '7'}
NS = int(OPT.get('NS', 4))
CA = int(OPT.get('CA', 2))
CU = float(OPT.get('CU', 0.265))
XF = int(OPT.get('XF', 6))
CHUNKS = [int(c) for c in OPT.get('CHUNKS', '44322 1').replace(' ', '')]
LATP = float(OPT.get('LATP', 160))
T0 = float(OPT.get('T0', -10))
T0F = float(OPT.get('T0F', -200))
RHO = float(OPT.get('RHO', 1.0))
BE = int(OPT.get('BE', 6))
MOFF = float(OPT.get('MOFF', 160))
MOFF2 = float(OPT.get('MOFF2', 240))
EC = float(OPT.get('EC', 48))
SG = int(OPT.get('SG', 4))
SDT = float(OPT.get('SDT', 12))
CHAIN = int(OPT.get('CHAIN', 0))
XE = int(OPT.get('XE', 6))
XO = int(OPT.get('XO', 7))
W2R = [128 * int(c) for c in OPT.get('W2R', '5421')]
W2C = len(W2R)
W2S = [sum(W2R[:i]) for i in range(W2C)]
ORD = OPT.get('ORD', 'ebagn')
OPQ = int(OPT.get('OPQ', 0))
LA = int(OPT.get('LA', 1))
NE = int(OPT.get('NE', 7))
EE = int(OPT.get('EE', 2))
SE = int(OPT.get('SE', 1))
EOFF = float(OPT.get('EOFF', 0))
SM = int(OPT.get('SM', 1))
OM = int(OPT.get('OM', 1))
U = int(OPT.get('U', 2))
NF = int(OPT.get('NF', 0))
NL = int(OPT.get('NL', 0))
EDEL = float(OPT.get('EDEL', 70))
RHO0 = float(OPT.get('RHO0', 1.0))
RHOL = float(OPT.get('RHOL', 1.0))
BAR = int(OPT.get('BAR', 0))
IOFF = float(OPT.get('IOFF', 0))
DYN = int(OPT.get('DYN', 0))
MST = int(OPT.get('MST', 1))
DSC = int(OPT.get('DSC', 1))
DBC = int(OPT.get('DBC', 0))
REP = int(OPT.get('REP', 1))
PB = int(OPT.get('PB', 0))
SKIP2 = int(OPT.get('SKIP2', 0))
SKIP1 = int(OPT.get('SKIP1', 0))


def _gelu(x):
    c = math.sqrt(2.0 / math.pi)
    return 0.5 * x * (1.0 + jnp.tanh(c * (x + 0.044715 * (x * x * x))))


def _rows_to_lanes(b, n):
    return jnp.concatenate([b[i:i + 1, :] for i in range(n)], axis=1)


def _bf(x):
    return pltpu.bitcast(x, BF16)


def _pack(a, b):
    return pltpu.bitcast(pltpu.pack_elementwise([a, b], packed_dtype=BF16), U32)


def _unpack(x):
    return (pltpu.unpack_elementwise(x, index=0, packed_dtype=BF16, unpacked_dtype=F32),
            pltpu.unpack_elementwise(x, index=1, packed_dtype=BF16, unpacked_dtype=F32))


def _dot(lhs32, rhs):
    return jnp.dot(_bf(lhs32), rhs, preferred_element_type=F32)[0:8]


def _dot_t(lhs32, rhs32):
    return lax.dot_general(_bf(lhs32), _bf(rhs32), (((1,), (1,)), ((), ())),
                           preferred_element_type=F32)[0:8]


def _ln_stats(xp):
    x = _unpack(xp)[0]
    m = jnp.mean(x, axis=-1, keepdims=True)
    xc = x - m
    v = jnp.mean(xc * xc, axis=-1, keepdims=True)
    return m, lax.rsqrt(v + EPS)


def _kernel(x_hbm, kx_hbm, vx_hbm, wq_hbm, wo_hbm, w1_hbm, b1_hbm, w2_hbm, b2_hbm,
            o_ref,
            kbuf, vbuf, vf_buf, wq_buf, wo_buf, w1_buf, w2_buf, x_buf, b1_buf, b2_buf,
            p_buf0, p_buf1, sp_buf, accp_buf, z_buf, xacc_buf, qv_buf, qraw_buf,
            csq_buf, cs1_buf, st_buf, tm_buf, zs_ref, s2_buf, op_buf,
            sem_k, sem_v, sem_w, *, sk, w):
    c_scale = (DH ** -0.5) * math.log2(math.e)
    nt = w // 128
    ng = nt // 8
    na = 12 // NS
    nst = NS * nt
    r0w = (sk - w) // 16
    nrw = w // 16

    ntb = nt - XF
    starts = [sum(CHUNKS[:c]) for c in range(len(CHUNKS))]
    assert sum(CHUNKS) == NP

    def k_copy(c):
        rows = pl.ds(48 * starts[c], 48 * CHUNKS[c])
        return [pltpu.make_async_copy(kx_hbm.at[rows, pl.ds(r0w, nrw), :],
                                      kbuf.bitcast(BF16).at[rows], sem_k.at[c & 1])]

    def v_copy(c):
        rows = pl.ds(48 * starts[c], 48 * CHUNKS[c])
        cps = [pltpu.make_async_copy(vx_hbm.at[rows, pl.ds(r0w, 8 * ntb), :],
                                     vbuf.bitcast(BF16).at[rows], sem_v.at[c & 1])]
        if XF:
            cps.append(pltpu.make_async_copy(
                vx_hbm.at[rows, pl.ds(r0w + 8 * ntb, 8 * XF), :],
                vf_buf.bitcast(BF16).at[rows, pl.ds(8 * XF, 8 * XF), :], sem_v.at[2 + (c & 1)]))
        return cps

    wq_cp = pltpu.make_async_copy(wq_hbm, wq_buf.bitcast(BF16), sem_w.at[0])
    wo_cp = pltpu.make_async_copy(wo_hbm, wo_buf.bitcast(BF16), sem_w.at[1])
    w1_cp = pltpu.make_async_copy(w1_hbm, w1_buf, sem_w.at[2])
    x_cp = pltpu.make_async_copy(x_hbm, x_buf, sem_w.at[3])
    b1_cp = pltpu.make_async_copy(b1_hbm, b1_buf, sem_w.at[4])
    b2_cp = pltpu.make_async_copy(b2_hbm, b2_buf, sem_w.at[5])
    w2_cps = [pltpu.make_async_copy(w2_hbm.at[pl.ds(W2S[i], W2R[i]), :],
                                    w2_buf.at[pl.ds(W2S[i], W2R[i]), :], sem_w.at[6 + i])
              for i in range(W2C)]

    if not SKIP1:
        wq_cp.start()
    x_cp.start()
    b1_cp.start()
    b2_cp.start()
    if not SKIP1:
        wo_cp.start()
        for cp in k_copy(0) + v_copy(0):
            cp.start()
    x_cp.wait()
    b1_cp.wait()
    b2_cp.wait()

    x0 = jnp.broadcast_to(x_buf[...].astype(F32), (8, D))
    b1 = _rows_to_lanes(b1_buf[...].astype(F32), F // 128)
    b2 = _rows_to_lanes(b2_buf[...].astype(F32), D // 128)

    lane = lax.broadcasted_iota(jnp.int32, (8, 128), 1)
    sub_lo = lax.broadcasted_iota(jnp.int32, (1, 8, 128), 1) < 4
    lo64 = lane < 64
    sub = lax.broadcasted_iota(jnp.int32, (8, 128), 0)
    evn = (lane & 8) == 0
    zf = jnp.zeros((8, 128), F32)
    ones32 = jnp.full((8, 128), 0x3F803F80, U32)
    k_order = (
        list(range(0, 16, 2)) + list(range(1, 16, 2)) + [16, 18, 20, 22, 17, 19, 21, 23],
        list(range(8, 24, 2)) + list(range(9, 24, 2)) + [1, 3, 5, 7, 0, 2, 4, 6],
    )

    def swap_halves(ref2):
        n = ref2.shape[1]
        a = ref2[0].reshape(n // 8, 8, 128)
        b = ref2[1].reshape(n // 8, 8, 128)
        ref2[0] = jnp.where(sub_lo, a, pltpu.roll(b, 4, 1)).reshape(n, 128)
        ref2[1] = jnp.where(sub_lo, pltpu.roll(a, 4, 1), b).reshape(n, 128)

    def fix_wq(a, carry):
        swap_halves(wq_buf.at[a])
        return carry

    def fix_wo(g8, carry):
        g0 = pl.multiple_of(g8 * 8, 8)
        v = [wo_buf[pl.ds(g0, 8), 8 * c:8 * c + 8, :] for c in range(5)]
        n = [jnp.where(sub_lo, v[0], v[2]),
             pltpu.roll(jnp.where(sub_lo, v[3], v[0]), 4, 1),
             jnp.where(sub_lo, v[1], v[3]),
             pltpu.roll(jnp.where(sub_lo, v[4], v[1]), 4, 1),
             jnp.where(sub_lo, v[2], v[4])]
        for c in range(5):
            wo_buf[pl.ds(g0, 8), 8 * c:8 * c + 8, :] = n[c]
        return carry

    def set_row(x):
        xp = _pack(x, x)
        z_buf[...] = xp
        m, r = _ln_stats(xp)
        rc = r * c_scale
        st_buf[0] = jnp.broadcast_to(rc, (8, 128))
        st_buf[1] = jnp.broadcast_to(m * rc, (8, 128))

    def wq_cols(ct):
        r0 = pl.multiple_of(lax.shift_right_logical(ct, 1) * 8, 8) if not isinstance(ct, int) else (ct // 2) * 8
        return _bf(wq_buf[:, ct & 1, pl.ds(r0, 8), :].reshape(D // 2, 128))

    def q_cols(z, j, c):
        ct = 3 * j + c
        return _dot(z, wq_cols(ct)) * st_buf[0] - csq_buf[ct] * st_buf[1]

    def store_q(qs, j):
        q0, q1, q2 = qs
        r1 = pltpu.roll(q1, 56, 1)

        def lhs(qf, a2):
            a0 = jnp.where(evn, qf, zf)
            b1_ = jnp.where(evn, zf, qf)
            a2 = jnp.where(evn, a2, zf)
            return [_pack(a0, pltpu.roll(a0, 8, 1)), _pack(pltpu.roll(b1_, 120, 1), b1_),
                    _pack(a2, pltpu.roll(a2, 8, 1))]

        for hh, ww in ((2 * j, lhs(q0, jnp.where(lo64, q1, r1))),
                       (2 * j + 1, lhs(q2, jnp.where(lo64, r1, q1)))):
            for c in range(4):
                for i in range(3):
                    if MST:
                        pltpu.store(qv_buf.at[hh & 3, c, :, 128 * i:128 * (i + 1)], ww[i], mask=sub == c)
                    else:
                        qv_buf[hh & 3, c, c:c + 1, 128 * i:128 * (i + 1)] = ww[i][c:c + 1, :]

    def q_pair(j):
        z = z_buf[...]
        store_q([q_cols(z, j, c) for c in range(3)], j)

    def score2(lhs, h, par, k):
        rhs = jnp.concatenate([kbuf[24 * h + i, 8 * k:8 * k + 8, :] for i in k_order[par]],
                              axis=0)
        return _dot(lhs, _bf(rhs))

    def scores_all(h, par):
        sg = [None] * ng
        for c in range(4):
            lhs = qv_buf[h & 3, c]
            for g in range(ng):
                s = score2(lhs, h, par, 4 * g + c)
                sg[g] = s if sg[g] is None else sg[g] + s
        return sg

    def store_p(p, g, rs, p_out):
        for r in rs:
            if PB:
                p_out[0, 64 * g + 8 * r:64 * g + 8 * r + 8, :] = jnp.broadcast_to(p[r:r + 1, :], (8, 128))
            else:
                p_out[0, pl.ds(64 * g + r, 8, stride=8), :] = p

    def softmax(sg, p_out):
        mx = sg[0]
        for s in sg[1:]:
            mx = jnp.maximum(mx, s)
        m = jnp.max(jnp.max(mx, axis=1, keepdims=True), axis=0, keepdims=True)
        l = None
        ps = []
        for g in range(ng):
            p = jnp.exp2(sg[g] - m)
            ps.append(p)
            if p_out is not None:
                store_p(p, g, range(8), p_out)
            l = p if l is None else l + p
        l = jnp.sum(jnp.sum(l, axis=1, keepdims=True), axis=0, keepdims=True)
        return ps, jnp.broadcast_to(1.0 / l, (8, 128))

    def v_tile(h, a, t):
        return vbuf[24 * h + 2 * a + t % 2, 8 * (t // 2):8 * (t // 2) + 8, :]

    def pv_step(h, sw, t, ts, p_in, gvals, true_mask, state):
        p = p_in[state['z'][sw], 8 * t:8 * t + 8, :]
        for i, gval in enumerate(gvals):
            p = jnp.where(true_mask[i], p, gval)
        accs = state['accs']
        for a in range(sw * na, (sw + 1) * na):
            if t < ntb:
                ys = _unpack(v_tile(h, a, t))
            else:
                r = 8 * (t - ntb)
                ys = [pltpu.bitcast(vf_buf[24 * h + 2 * a + e, r:r + 8, :], F32) for e in range(2)]
            for e in range(2):
                j = 2 * a + e
                accs[j] = ys[e] * p if t == ts[0] else accs[j] + ys[e] * p
        state['sw'] = sw
        if t == ts[-1]:
            for a in range(sw * na, (sw + 1) * na):
                r0 = state['half'] * (DH // 2) + 8 * a
                accp_buf[state['slot'], r0:r0 + 8, :] = _pack(accs[2 * a], accs[2 * a + 1])

    def o_pair(ones, accp, ie, io):
        inv = jnp.concatenate([ie, jnp.where(lo64, ie, io), io], axis=1)
        return _dot_t(ones, accp) * inv

    def out_cols(op, g0, ngrp, c):
        rhs = wo_buf[pl.ds(g0, ngrp), 8 * c:8 * c + 8, :].reshape(ngrp * 8, 128)
        return _dot(op, _bf(rhs))

    def mlp_hidden(x):
        xp = _pack(x, x)
        m, r = _ln_stats(xp)
        hh = (_dot(xp, w1_buf[...]) - cs1_buf[...] * m) * r + b1
        g = _gelu(hh)
        return _pack(g, g)

    def fix_v(r2, carry):
        swap_halves(vbuf.at[pl.ds(2 * r2, 2)])
        if XF:
            n = 4 * XF
            a = vf_buf[2 * r2, n:2 * n, :].reshape(n // 8, 8, 128)
            b = vf_buf[2 * r2 + 1, n:2 * n, :].reshape(n // 8, 8, 128)
            t0 = _unpack(jnp.where(sub_lo, a, pltpu.roll(b, 4, 1)))
            t1 = _unpack(jnp.where(sub_lo, pltpu.roll(a, 4, 1), b))
            for e in range(2):
                for k in range(XF // 2):
                    vf_buf[2 * r2 + e, 16 * k:16 * k + 8, :] = pltpu.bitcast(t0[e][k], U32)
                    vf_buf[2 * r2 + e, 16 * k + 8:16 * k + 16, :] = pltpu.bitcast(t1[e][k], U32)
        return carry

    def next_copies(j, copy_fn, tail_cps):
        for c in range(len(CHUNKS)):
            @pl.when(j == starts[c])
            def _():
                for cp in copy_fn(c):
                    cp.wait()
                for cp in (copy_fn(c + 1) if c + 1 < len(CHUNKS) else tail_cps):
                    cp.start()

    def pair1(j, carry):
        q_pair(j)
        next_copies(j, k_copy, [w1_cp])
        invs = []
        for par in range(2):
            _, inv = softmax(scores_all(2 * j + par, par), (p_buf0, p_buf1)[par])
            invs.append(inv)
        next_copies(j, v_copy, w2_cps)
        lax.fori_loop(24 * j, 24 * (j + 1), fix_v, 0)
        for par in range(2):
            state = dict(accs=[None] * 24, half=par, slot=0, z=[0] * NS)
            for sw in range(NS):
                for t in range(nt):
                    pv_step(2 * j + par, sw, t, range(nt), (p_buf0, p_buf1)[par], (), None, state)
        o = o_pair(ones32, accp_buf[0], invs[0], invs[1])
        op = _pack(o, o)
        for c in range(5):
            xacc_buf[:, 128 * c:128 * (c + 1)] += out_cols(op, 24 * j, 24, c)
        return carry

    def colsum_q(ct, carry):
        ones = jnp.concatenate([ones32] * (D // 128), axis=1)
        csq_buf[ct] = _dot(ones, wq_cols(ct))
        return carry

    qv_buf[...] = jnp.zeros(qv_buf.shape, U32)
    for i in range(3):
        tm_buf[i] = lane
    for sw in range(NS):
        zs_ref[sw] = 0
    if not SKIP1:
        set_row(x0)
        xacc_buf[...] = x0
        wq_cp.wait()
        lax.fori_loop(0, D // 16, fix_wq, 0)
        lax.fori_loop(0, 3 * NP, colsum_q, 0)
        wo_cp.wait()
        lax.fori_loop(0, H * DH // 128, fix_wo, 0)
        lax.fori_loop(0, NP, pair1, 0)
        x1 = xacc_buf[...]
        w1_cp.wait()
        cs1_buf[...] = _dot(jnp.concatenate([ones32] * (D // 128), axis=1), w1_buf[...])
        gp = mlp_hidden(x1)
        x2 = x1 + b2
        for i in range(W2C):
            w2_cps[i].wait()
            x2 = x2 + _dot(gp[:, W2S[i]:W2S[i] + W2R[i]], w2_buf[W2S[i]:W2S[i] + W2R[i], :])
    else:
        x2 = lax.fori_loop(0, 2, lambda i, x: x + 1.0, x0)

    if SKIP2:
        o_ref[...] = x2[0:1, :].astype(o_ref.dtype)
        return

    def block(j0, carry, kinds, jpar=None):
        true_mask = [tm_buf[i] >= 0 for i in range(3)]
        zs = [0] + [zs_ref[sw] if OPQ else 0 for sw in range(1, NS)]
        steps = []
        info = []
        for u, kind in enumerate(kinds):
            xs = (XE, XO) if kind == 'last' else (0, 0)
            tss = [list(range(x, nt)) for x in xs]
            s0 = len(steps)
            steps += [(u, par, sw, t) for par in range(2) for sw in range(NS) for t in tss[par]]
            info.append(dict(tss=tss, s0=s0, s_odd=s0 + NS * len(tss[0]), s_end=len(steps)))
        t_step = [0.0]
        for (_, _, _, t) in steps:
            t_step.append(t_step[-1] + CU * na * (6 if t < ntb else 4))
        gates, stores = {}, {}
        cur = dict(state=None, st=-1, nedge=0)
        envs = [dict(s1=[None] * ng, s2=[None] * ng, s3=[None] * ng) for _ in kinds]
        envs[0]['ie_cur'], envs[0]['ie'], envs[0]['io_prev'] = carry

        def slot(u):
            return (j0 + u) & 1 if jpar is None else (jpar + u) & 1

        def step_at(cyc):
            return next((i for i, tt_ in enumerate(t_step) if tt_ >= cyc), len(t_step))

        def gate(cyc, v):
            st = step_at(cyc)
            while len(gates.get(st, ())) >= 2:
                st += 1
            if st < len(steps) and st > cur['st']:
                gates.setdefault(st, []).append(v)

        def edge(x, n=BE, force=False):
            if cur['st'] < 0 or not (force or cur['edge']):
                return x
            sw = cur['state']['sw']
            cand = list(range(2 * sw * na, 2 * (sw + 1) * na))
            ntile = -(-x.shape[1] // 128)
            parts = [x[:, 128 * i:min(128 * (i + 1), x.shape[1])] for i in range(ntile)]
            for e in range(min(n, 3 * ntile)):
                k_ = cur['nedge'] % len(cand)
                c = cand[(2 * k_) % len(cand) + (2 * k_) // len(cand)]
                cur['nedge'] += 1
                i = e % ntile
                w_ = parts[i].shape[1]
                parts[i] = jnp.where(true_mask[e // ntile][:, 0:w_], parts[i],
                                     pltpu.bitcast(cur['state']['accs'][c], U32)[:, 0:w_])
            return parts[0] if ntile == 1 else jnp.concatenate(parts, axis=1)

        def sched_stores(ps, inv, p_out, t_ready, lo, hi):
            gate(t_ready, ps[-1])
            if IOFF:
                gate(t_ready + IOFF, inv)
            n = 8 // SG
            t_first = max(t_ready, t_step[lo])
            for i in range(ng * n):
                g, k = divmod(i, n)
                st = min(max(step_at(t_first + SDT * i) + 1, cur['st'] + 1), hi)
                stores.setdefault(st, []).append((ps[g], g, range(SG * k, SG * (k + 1)), p_out))

        def pair_jobs(u):
            kind, env, inf = kinds[u], envs[u], info[u]
            first, last = kind == 'first', kind == 'last'
            j = j0 + u
            h0 = 2 * j

            def job_b(h, par, c, g, key, tail):
                def fn(td):
                    s = score2(edge(qv_buf[h & 3, c]), h, par, 4 * g + c)
                    sg = env[key]
                    sg[g] = s if c == 0 else sg[g] + s
                    gate(td + LATP, sg[g])
                    if c == 3:
                        (sp_buf if key != 's2' else s2_buf)[g] = sg[g]
                    if tail == 'sm1':
                        ps, env['io'] = softmax([sp_buf[gg] for gg in range(ng)], None)
                        sched_stores(ps, env['io'], p_buf1, td + LATP + MOFF, inf['s0'], inf['s_odd'])
                        if not first and not last:
                            store_q([qraw_buf[i] for i in range(3)], j + 1)
                    elif tail == 'sm2':
                        ps, env['ie_next'] = softmax([s2_buf[gg] for gg in range(ng)], None)
                        sched_stores(ps, env['ie_next'], p_buf0, td + LATP + MOFF2, inf['s_odd'], inf['s_end'] - 1)
                return fn

            def job_e(td):
                if u > 0:
                    env['ie'], env['io_prev'] = envs[u - 1]['ie_cur'], envs[u - 1]['io']
                    env['ie_cur'] = envs[u - 1]['ie_next']
                o = o_pair(edge(ones32), accp_buf[1 - slot(u)], env['ie'], env['io_prev'])
                gate(td + LATP + 10, o[:, 256:384])
                op_buf[...] = _pack(o, o)

            def job_g(c):
                def fn(td):
                    xo = out_cols(edge(op_buf[...]), 24 * (j - 1), 24, c)
                    xacc_buf[:, 128 * c:128 * (c + 1)] += xo
                    gate(td + LATP, xo)
                return fn

            def job_a(c):
                def fn(td):
                    jn = j + 2 if isinstance(j, int) else jnp.minimum(j + 2, NP - 1)
                    qc = q_cols(edge(z_buf[...]), jn, c)
                    gate(td + LATP, qc)
                    qraw_buf[c] = qc
                return fn

            def job_x(par, t):
                def fn(td):
                    p = (p_buf0, p_buf1)[par][0, 8 * t:8 * t + 8, :]
                    rhs = jnp.concatenate([v_tile(h0 + par, a, t) for a in range(DH // 16)], axis=0)
                    o = _dot_t(edge(_pack(p, p)), rhs)
                    key = 'x%d' % par
                    env[key] = o if key not in env else env[key] + o
                    gate(td + LATP, env[key][:, 0:128])
                return fn

            def finish_head(par, inv, lhs_edge):
                acc = accp_buf[slot(u), par * (DH // 2):(par + 1) * (DH // 2), :]
                o = _dot_t(lhs_edge(ones32), acc)
                if 'x%d' % par in env:
                    o = o + env['x%d' % par]
                return o * jnp.concatenate([inv, inv[:, 0:DH - 128]], axis=1)

            env['finish_head'] = finish_head

            def job_e30(td):
                o = finish_head(0, env['ie_cur'], edge)
                gate(td + LATP + 10, o[:, 0:128])
                env['op30'] = _pack(o, o)

            def job_g30(c):
                def fn(td):
                    xo = out_cols(edge(env['op30']), 12 * h0, 12, c)
                    xacc_buf[:, 128 * c:128 * (c + 1)] += xo
                    gate(td + LATP, xo)
                return fn

            jobs = []
            for g in range(0 if first else CA, ng):
                for c in range(4):
                    tail = 'sm1' if (c == 3 and g == ng - 1) else None
                    jobs.append((24, None, job_b(h0 + 1, 1, c, g, 's1', tail), 3))
            t_pair = t_step[inf['s0']] + EDEL if u > 0 else None
            groups = {
                'e': [] if first else [(EC, t_pair, job_e, 3)],
                'b': [(24, None, job_b(h0 + 2, 0, c, g, 's2',
                                       'sm2' if (c == 3 and g == ng - 1) else None), 3)
                      for g in range(ng) for c in range(4)],
                'a': [] if isinstance(j, int) and j + 2 >= NP else
                     [(40, None, job_a(c), 5) for c in range(3)],
                'g': [] if first else [(24, None, job_g(c), 3) for c in range(5)],
                'n': [(24, None, job_b(h0 + 3, 1, c, g, 's3', None), 3)
                      for g in range(CA) for c in range(4)],
            }
            if last:
                t_odd = t_step[inf['s_odd'] + 1]
                jobs += groups['e'] + [(24, None, job_x(0, t), 2) for t in range(XE)] + groups['g']
                jobs += [(24, t_odd, job_x(1, t), 2) for t in range(XO)]
                jobs += [(32, t_odd, job_e30, 2)]
                jobs += [(12, t_odd + LATP + 60, job_g30(c), 2) for c in range(5)]
            else:
                for ch in ORD:
                    jobs += groups[ch]
            return jobs

        pjobs = [pair_jobs(u) for u in range(len(kinds))]
        jobs = [job for pj in pjobs for job in pj]
        rhos = [RHO if 0 < u < len(kinds) - 1 else (RHO0 if u == 0 else RHOL) for u, pj in enumerate(pjobs) for _ in pj]
        times = []
        tt = T0F if kinds[0] == 'first' else T0
        for (cost, earliest, _, _), rho in zip(jobs, rhos):
            tt += cost * rho
            if earliest is not None:
                tt = max(tt, earliest)
            times.append(tt)

        states = {}
        nj = 0
        for st, (u, par, sw, t) in enumerate(steps):
            while nj < len(jobs) and times[nj] + EOFF <= t_step[st]:
                if times[nj] > 0 and 'j0' not in cur:
                    cur['j0'] = nj
                rel = nj - cur.get('j0', nj + 1)
                cur['edge'] = (0 <= rel < NE and rel % EE == EE - 1) or jobs[nj][1] == times[nj]
                jobs[nj][2](times[nj])
                nj += 1
            for (pv_, g_, rs_, po_) in stores.pop(st, ()):
                store_p(pltpu.bitcast(edge(pltpu.bitcast(pv_, U32), SE, True), F32), g_, rs_, po_)
            state = states.setdefault((u, par), dict(accs=[None] * 24, half=par, slot=slot(u), z=zs))
            pv_step(2 * (j0 + u) + par, sw, t, info[u]['tss'][par], (p_buf0, p_buf1)[par],
                    gates.get(st, ()), true_mask, state)
            cur['state'] = state
            cur['st'] = st
        cur['edge'] = False
        while nj < len(jobs):
            jobs[nj][2](times[nj])
            nj += 1
        assert not stores
        env = envs[-1]
        if kinds[-1] == 'last':
            o = env['finish_head'](1, env['io'], lambda x: x)
            op = _pack(o, o)
            return xacc_buf[...] + jnp.concatenate(
                [out_cols(op, 12 * (H - 1), 12, c) for c in range(5)], axis=1)
        return env['ie_next'], env['ie_cur'], env['io']

    set_row(x2)
    xacc_buf[...] = x2
    q_pair(0)
    q_pair(1)
    _, inv0 = softmax(scores_all(0, 0), p_buf0)
    carry = block(0, (inv0, None, None), ['first'] + ['mid'] * NF)
    n_mid = (NP - 2 - NF - NL) // U
    carry = lax.fori_loop(0, n_mid * REP, lambda i, c: block(1 + NF + U * (i if REP == 1 else lax.rem(i, n_mid)), c, ['mid'] * U, (1 + NF) & 1 if U % 2 == 0 and not DYN else None), carry)
    x3 = block(NP - 1 - NL, carry, ['mid'] * NL + ['last'])
    x4 = x3 + b2 + _dot(mlp_hidden(x3), w2_buf[...])
    o_ref[...] = x4[0:1, :].astype(o_ref.dtype)


@jax.jit
def pallas_interleave_layers__sliding_block_cached__dense_activation_gelu__decode_kernel(
    A_x: jax.Array,
    A_k_cache: jax.Array,
    A_v_cache: jax.Array,
    A_wq: jax.Array,
    A_wo: jax.Array,
    B_x: jax.Array,
    B_w1: jax.Array,
    B_b1: jax.Array,
    B_w2: jax.Array,
    B_b2: jax.Array,
):
    sk = A_k_cache.shape[2]
    w = min(4096, max(256, sk // 4))

    def tile_view(a):
        *lead, r, c = a.shape
        n = len(lead)
        a = a.reshape(*lead, r // 8, 8, c // 128, 128)
        a = a.transpose(*range(n), n, n + 2, n + 1, n + 3)
        return a.reshape(*lead, r // 16, 2, (c // 128) * 8, 128)

    kx = tile_view(jnp.swapaxes(A_k_cache, 2, 3)[0]).reshape(H * DH // 8, sk // 16, 128)
    vx = tile_view(jnp.swapaxes(A_v_cache, 2, 3)[0]).reshape(H * DH // 8, sk // 16, 128)
    wqx = tile_view(A_wq)
    wox = tile_view(A_wo).reshape(H * DH // 16, 80, 128)
    any_spec = pl.BlockSpec(memory_space=pl.ANY)
    out = pl.pallas_call(
        functools.partial(_kernel, sk=sk, w=w),
        out_shape=jax.ShapeDtypeStruct((1, D), A_x.dtype),
        in_specs=[any_spec] * 9,
        out_specs=pl.BlockSpec(memory_space=pltpu.VMEM),
        scratch_shapes=[
            pltpu.VMEM((H * DH // 8, w // 32, 128), U32),
            pltpu.VMEM((H * DH // 8, w // 32 - 4 * XF, 128), U32),
            pltpu.VMEM((H * DH // 8, max(8 * XF, 8), 128), U32),
            pltpu.VMEM((D // 16, 2, H * DH // 32, 128), U32),
            pltpu.VMEM((H * DH // 16, 40, 128), U32),
            pltpu.VMEM((D, F), BF16),
            pltpu.VMEM((F, D), BF16),
            pltpu.VMEM((1, D), BF16),
            pltpu.VMEM((F // 128, 128), BF16),
            pltpu.VMEM((D // 128, 128), BF16),
            pltpu.VMEM((1, w // 16, 128), F32),
            pltpu.VMEM((1, w // 16, 128), F32),
            pltpu.VMEM((w // 1024, 8, 128), F32),
            pltpu.VMEM((2, DH, 128), U32),
            pltpu.VMEM((8, D), U32),
            pltpu.VMEM((8, D), F32),
            pltpu.VMEM((4, 4, 8, 2 * DH), U32),
            pltpu.VMEM((3, 8, 128), F32),
            pltpu.VMEM((3 * NP, 8, 128), F32),
            pltpu.VMEM((8, F), F32),
            pltpu.VMEM((2, 8, 128), F32),
            pltpu.VMEM((3, 8, 128), jnp.int32),
            pltpu.SMEM((NS,), jnp.int32),
            pltpu.VMEM((w // 1024, 8, 128), F32),
            pltpu.VMEM((8, 2 * DH), U32),
            pltpu.SemaphoreType.DMA((2,)),
            pltpu.SemaphoreType.DMA((4,)),
            pltpu.SemaphoreType.DMA((6 + W2C,)),
        ],
        compiler_params=pltpu.CompilerParams(vmem_limit_bytes=int(OPT.get('VM', 127)) * 1024 * 1024,
                                             disable_semaphore_checks=bool(DSC), disable_bounds_checks=bool(DBC)),
    )(A_x.reshape(1, D), kx, vx, wqx, wox, B_w1, B_b1.reshape(F // 128, 128),
      B_w2, B_b2.reshape(D // 128, 128))
    return out.reshape(A_x.shape)
```

```python
import functools
import math

import jax
import jax.numpy as jnp
from jax import lax
import jax.experimental.pallas as pl
import jax.experimental.pallas.tpu as pltpu

F32 = jnp.float32
BF16 = jnp.bfloat16
U32 = jnp.uint32

D = 640
H = 32
DH = 192
F = 1536
EPS = 1e-5
NP = H // 2
OPT = {'OPQ2': '1'}
NS = int(OPT.get('NS', 4))
CA = int(OPT.get('CA', 2))
CU = float(OPT.get('CU', 0.26))
XF = int(OPT.get('XF', 6))
CHUNKS = [int(c) for c in OPT.get('CHUNKS', '44322 1').replace(' ', '')]
LATP = float(OPT.get('LATP', 160))
T0 = float(OPT.get('T0', -10))
T0F = float(OPT.get('T0F', -200))
RHO = float(OPT.get('RHO', 1.07))
BE = int(OPT.get('BE', 6))
MOFF = float(OPT.get('MOFF', 160))
MOFF2 = float(OPT.get('MOFF2', 240))
EC = float(OPT.get('EC', 48))
SG = int(OPT.get('SG', 4))
SDT = float(OPT.get('SDT', 12))
CHAIN = int(OPT.get('CHAIN', 0))
XE = int(OPT.get('XE', 7))
XO = int(OPT.get('XO', 7))
W2R = [128 * int(c) for c in OPT.get('W2R', '5421')]
W2C = len(W2R)
W2S = [sum(W2R[:i]) for i in range(W2C)]
ORD = OPT.get('ORD', 'ebagn')
OPQ = int(OPT.get('OPQ', 0))
LA = int(OPT.get('LA', 1))
NE = int(OPT.get('NE', 7))
EE = int(OPT.get('EE', 2))
SE = int(OPT.get('SE', 1))
EOFF = float(OPT.get('EOFF', 0))
SM = int(OPT.get('SM', 1))
OM = int(OPT.get('OM', 1))
U = int(OPT.get('U', 2))
NF = int(OPT.get('NF', 0))
NL = int(OPT.get('NL', 0))
EDEL = float(OPT.get('EDEL', 70))
RHO0 = float(OPT.get('RHO0', 1.0))
RHOL = float(OPT.get('RHOL', 1.0))
BAR = int(OPT.get('BAR', 0))
IOFF = float(OPT.get('IOFF', 0))
DYN = int(OPT.get('DYN', 0))
MST = int(OPT.get('MST', 1))
DSC = int(OPT.get('DSC', 1))
DBC = int(OPT.get('DBC', 0))
REP = int(OPT.get('REP', 1))
PB = int(OPT.get('PB', 0))
ALL = int(OPT.get('ALL', 1))
LEAD = float(OPT.get('LEAD', 100))
OPQ2 = int(OPT.get('OPQ2', 0))
SKIP2 = int(OPT.get('SKIP2', 0))
SKIP1 = int(OPT.get('SKIP1', 0))


def _gelu(x):
    c = math.sqrt(2.0 / math.pi)
    return 0.5 * x * (1.0 + jnp.tanh(c * (x + 0.044715 * (x * x * x))))


def _rows_to_lanes(b, n):
    return jnp.concatenate([b[i:i + 1, :] for i in range(n)], axis=1)


def _bf(x):
    return pltpu.bitcast(x, BF16)


def _pack(a, b):
    return pltpu.bitcast(pltpu.pack_elementwise([a, b], packed_dtype=BF16), U32)


def _unpack(x):
    return (pltpu.unpack_elementwise(x, index=0, packed_dtype=BF16, unpacked_dtype=F32),
            pltpu.unpack_elementwise(x, index=1, packed_dtype=BF16, unpacked_dtype=F32))


def _dot(lhs32, rhs):
    return jnp.dot(_bf(lhs32), rhs, preferred_element_type=F32)[0:8]


def _dot_t(lhs32, rhs32):
    return lax.dot_general(_bf(lhs32), _bf(rhs32), (((1,), (1,)), ((), ())),
                           preferred_element_type=F32)[0:8]


def _ln_stats(xp):
    x = _unpack(xp)[0]
    m = jnp.mean(x, axis=-1, keepdims=True)
    xc = x - m
    v = jnp.mean(xc * xc, axis=-1, keepdims=True)
    return m, lax.rsqrt(v + EPS)


def _kernel(x_hbm, kx_hbm, vx_hbm, wq_hbm, wo_hbm, w1_hbm, b1_hbm, w2_hbm, b2_hbm,
            o_ref,
            kbuf, vbuf, vf_buf, wq_buf, wo_buf, w1_buf, w2_buf, x_buf, b1_buf, b2_buf,
            p_buf0, p_buf1, sp_buf, accp_buf, z_buf, xacc_buf, qv_buf, qraw_buf,
            csq_buf, cs1_buf, st_buf, tm_buf, zs_ref, s2_buf, op_buf, l_buf,
            sem_k, sem_v, sem_w, *, sk, w):
    c_scale = (DH ** -0.5) * math.log2(math.e)
    nt = w // 128
    ng = nt // 8
    na = 12 // NS
    nst = NS * nt
    r0w = (sk - w) // 16
    nrw = w // 16

    ntb = nt - XF
    starts = [sum(CHUNKS[:c]) for c in range(len(CHUNKS))]
    assert sum(CHUNKS) == NP

    def k_copy(c):
        rows = pl.ds(48 * starts[c], 48 * CHUNKS[c])
        return [pltpu.make_async_copy(kx_hbm.at[rows, pl.ds(r0w, nrw), :],
                                      kbuf.bitcast(BF16).at[rows], sem_k.at[c & 1])]

    def v_copy(c):
        rows = pl.ds(48 * starts[c], 48 * CHUNKS[c])
        cps = [pltpu.make_async_copy(vx_hbm.at[rows, pl.ds(r0w, 8 * ntb), :],
                                     vbuf.bitcast(BF16).at[rows], sem_v.at[c & 1])]
        if XF:
            cps.append(pltpu.make_async_copy(
                vx_hbm.at[rows, pl.ds(r0w + 8 * ntb, 8 * XF), :],
                vf_buf.bitcast(BF16).at[rows, pl.ds(8 * XF, 8 * XF), :], sem_v.at[2 + (c & 1)]))
        return cps

    wq_cp = pltpu.make_async_copy(wq_hbm, wq_buf.bitcast(BF16), sem_w.at[0])
    wo_cp = pltpu.make_async_copy(wo_hbm, wo_buf.bitcast(BF16), sem_w.at[1])
    w1_cp = pltpu.make_async_copy(w1_hbm, w1_buf, sem_w.at[2])
    x_cp = pltpu.make_async_copy(x_hbm, x_buf, sem_w.at[3])
    b1_cp = pltpu.make_async_copy(b1_hbm, b1_buf, sem_w.at[4])
    b2_cp = pltpu.make_async_copy(b2_hbm, b2_buf, sem_w.at[5])
    w2_cps = [pltpu.make_async_copy(w2_hbm.at[pl.ds(W2S[i], W2R[i]), :],
                                    w2_buf.at[pl.ds(W2S[i], W2R[i]), :], sem_w.at[6 + i])
              for i in range(W2C)]

    if not SKIP1:
        wq_cp.start()
    x_cp.start()
    b1_cp.start()
    b2_cp.start()
    if not SKIP1:
        wo_cp.start()
        for cp in k_copy(0) + v_copy(0):
            cp.start()
    x_cp.wait()
    b1_cp.wait()
    b2_cp.wait()

    x0 = jnp.broadcast_to(x_buf[...].astype(F32), (8, D))
    b1 = _rows_to_lanes(b1_buf[...].astype(F32), F // 128)
    b2 = _rows_to_lanes(b2_buf[...].astype(F32), D // 128)

    lane = lax.broadcasted_iota(jnp.int32, (8, 128), 1)
    sub_lo = lax.broadcasted_iota(jnp.int32, (1, 8, 128), 1) < 4
    lo64 = lane < 64
    sub = lax.broadcasted_iota(jnp.int32, (8, 128), 0)
    evn = (lane & 8) == 0
    zf = jnp.zeros((8, 128), F32)
    ones32 = jnp.full((8, 128), 0x3F803F80, U32)
    k_order = (
        list(range(0, 16, 2)) + list(range(1, 16, 2)) + [16, 18, 20, 22, 17, 19, 21, 23],
        list(range(8, 24, 2)) + list(range(9, 24, 2)) + [1, 3, 5, 7, 0, 2, 4, 6],
    )

    def swap_halves(ref2):
        n = ref2.shape[1]
        a = ref2[0].reshape(n // 8, 8, 128)
        b = ref2[1].reshape(n // 8, 8, 128)
        ref2[0] = jnp.where(sub_lo, a, pltpu.roll(b, 4, 1)).reshape(n, 128)
        ref2[1] = jnp.where(sub_lo, pltpu.roll(a, 4, 1), b).reshape(n, 128)

    def fix_wq(a, carry):
        swap_halves(wq_buf.at[a])
        return carry

    def fix_wo(g8, carry):
        g0 = pl.multiple_of(g8 * 8, 8)
        v = [wo_buf[pl.ds(g0, 8), 8 * c:8 * c + 8, :] for c in range(5)]
        n = [jnp.where(sub_lo, v[0], v[2]),
             pltpu.roll(jnp.where(sub_lo, v[3], v[0]), 4, 1),
             jnp.where(sub_lo, v[1], v[3]),
             pltpu.roll(jnp.where(sub_lo, v[4], v[1]), 4, 1),
             jnp.where(sub_lo, v[2], v[4])]
        for c in range(5):
            wo_buf[pl.ds(g0, 8), 8 * c:8 * c + 8, :] = n[c]
        return carry

    def set_row(x):
        xp = _pack(x, x)
        z_buf[...] = xp
        m, r = _ln_stats(xp)
        rc = r * c_scale
        st_buf[0] = jnp.broadcast_to(rc, (8, 128))
        st_buf[1] = jnp.broadcast_to(m * rc, (8, 128))

    def wq_cols(ct):
        r0 = pl.multiple_of(lax.shift_right_logical(ct, 1) * 8, 8) if not isinstance(ct, int) else (ct // 2) * 8
        return _bf(wq_buf[:, ct & 1, pl.ds(r0, 8), :].reshape(D // 2, 128))

    def q_cols(z, j, c):
        ct = 3 * j + c
        return _dot(z, wq_cols(ct)) * st_buf[0] - csq_buf[ct] * st_buf[1]

    def store_q(qs, j):
        q0, q1, q2 = qs
        r1 = pltpu.roll(q1, 56, 1)

        def lhs(qf, a2):
            a0 = jnp.where(evn, qf, zf)
            b1_ = jnp.where(evn, zf, qf)
            a2 = jnp.where(evn, a2, zf)
            return [_pack(a0, pltpu.roll(a0, 8, 1)), _pack(pltpu.roll(b1_, 120, 1), b1_),
                    _pack(a2, pltpu.roll(a2, 8, 1))]

        for hh, ww in ((2 * j, lhs(q0, jnp.where(lo64, q1, r1))),
                       (2 * j + 1, lhs(q2, jnp.where(lo64, r1, q1)))):
            for c in range(4):
                for i in range(3):
                    if MST:
                        pltpu.store(qv_buf.at[hh & 3, c, :, 128 * i:128 * (i + 1)], ww[i], mask=sub == c)
                    else:
                        qv_buf[hh & 3, c, c:c + 1, 128 * i:128 * (i + 1)] = ww[i][c:c + 1, :]

    def q_pair(j):
        z = z_buf[...]
        store_q([q_cols(z, j, c) for c in range(3)], j)

    def score2(lhs, h, par, k):
        rhs = jnp.concatenate([kbuf[24 * h + i, 8 * k:8 * k + 8, :] for i in k_order[par]],
                              axis=0)
        return _dot(lhs, _bf(rhs))

    def scores_all(h, par):
        sg = [None] * ng
        for c in range(4):
            lhs = qv_buf[h & 3, c]
            for g in range(ng):
                s = score2(lhs, h, par, 4 * g + c)
                sg[g] = s if sg[g] is None else sg[g] + s
        return sg

    def store_p(p, g, rs, p_out):
        for r in rs:
            if PB:
                p_out[0, 64 * g + 8 * r:64 * g + 8 * r + 8, :] = jnp.broadcast_to(p[r:r + 1, :], (8, 128))
            else:
                p_out[0, pl.ds(64 * g + r, 8, stride=8), :] = p

    def inv_sum(l):
        l = jnp.sum(jnp.sum(l, axis=1, keepdims=True), axis=0, keepdims=True)
        return jnp.broadcast_to(1.0 / l, (8, 128))

    def softmax(sg, p_out):
        mx = sg[0]
        for s in sg[1:]:
            mx = jnp.maximum(mx, s)
        m = jnp.max(jnp.max(mx, axis=1, keepdims=True), axis=0, keepdims=True)
        l = None
        ps = []
        for g in range(ng):
            p = jnp.exp2(sg[g] - m)
            ps.append(p)
            if p_out is not None:
                store_p(p, g, range(8), p_out)
            l = p if l is None else l + p
        if p_out is None:
            return ps, l
        return ps, inv_sum(l)

    def v_tile(h, a, t):
        return vbuf[24 * h + 2 * a + t % 2, 8 * (t // 2):8 * (t // 2) + 8, :]

    def pv_step(h, sw, t, ts, p_in, gvals, true_mask, state):
        p = p_in[state['z'][sw], 8 * t:8 * t + 8, :]
        for i, gval in enumerate(gvals):
            p = jnp.where(true_mask[i], p, gval)
        accs = state['accs']
        for a in range(sw * na, (sw + 1) * na):
            if t < ntb:
                ys = _unpack(v_tile(h, a, t))
            else:
                r = 8 * (t - ntb)
                ys = [pltpu.bitcast(vf_buf[24 * h + 2 * a + e, r:r + 8, :], F32) for e in range(2)]
            for e in range(2):
                j = 2 * a + e
                accs[j] = ys[e] * p if t == ts[0] else accs[j] + ys[e] * p
        state['sw'] = sw
        if t == ts[-1]:
            for a in range(sw * na, (sw + 1) * na):
                r0 = state['half'] * (DH // 2) + 8 * a
                accp_buf[state['slot'], r0:r0 + 8, :] = _pack(accs[2 * a], accs[2 * a + 1])

    def o_pair(ones, accp, ie, io):
        inv = jnp.concatenate([ie, jnp.where(lo64, ie, io), io], axis=1)
        return _dot_t(ones, accp) * inv

    def out_cols(op, g0, ngrp, c):
        rhs = wo_buf[pl.ds(g0, ngrp), 8 * c:8 * c + 8, :].reshape(ngrp * 8, 128)
        return _dot(op, _bf(rhs))

    def mlp_hidden(x):
        xp = _pack(x, x)
        m, r = _ln_stats(xp)
        hh = (_dot(xp, w1_buf[...]) - cs1_buf[...] * m) * r + b1
        g = _gelu(hh)
        return _pack(g, g)

    def fix_v(r2, carry):
        swap_halves(vbuf.at[pl.ds(2 * r2, 2)])
        if XF:
            n = 4 * XF
            a = vf_buf[2 * r2, n:2 * n, :].reshape(n // 8, 8, 128)
            b = vf_buf[2 * r2 + 1, n:2 * n, :].reshape(n // 8, 8, 128)
            t0 = _unpack(jnp.where(sub_lo, a, pltpu.roll(b, 4, 1)))
            t1 = _unpack(jnp.where(sub_lo, pltpu.roll(a, 4, 1), b))
            for e in range(2):
                for k in range(XF // 2):
                    vf_buf[2 * r2 + e, 16 * k:16 * k + 8, :] = pltpu.bitcast(t0[e][k], U32)
                    vf_buf[2 * r2 + e, 16 * k + 8:16 * k + 16, :] = pltpu.bitcast(t1[e][k], U32)
        return carry

    def next_copies(j, copy_fn, tail_cps):
        for c in range(len(CHUNKS)):
            @pl.when(j == starts[c])
            def _():
                for cp in copy_fn(c):
                    cp.wait()
                for cp in (copy_fn(c + 1) if c + 1 < len(CHUNKS) else tail_cps):
                    cp.start()

    def pair1(j, carry):
        q_pair(j)
        next_copies(j, k_copy, [w1_cp])
        invs = []
        for par in range(2):
            _, inv = softmax(scores_all(2 * j + par, par), (p_buf0, p_buf1)[par])
            invs.append(inv)
        next_copies(j, v_copy, w2_cps)
        lax.fori_loop(24 * j, 24 * (j + 1), fix_v, 0)
        for par in range(2):
            state = dict(accs=[None] * 24, half=par, slot=0, z=[0] * NS)
            for sw in range(NS):
                for t in range(nt):
                    pv_step(2 * j + par, sw, t, range(nt), (p_buf0, p_buf1)[par], (), None, state)
        o = o_pair(ones32, accp_buf[0], invs[0], invs[1])
        op = _pack(o, o)
        for c in range(5):
            xacc_buf[:, 128 * c:128 * (c + 1)] += out_cols(op, 24 * j, 24, c)
        return carry

    def colsum_q(ct, carry):
        ones = jnp.concatenate([ones32] * (D // 128), axis=1)
        csq_buf[ct] = _dot(ones, wq_cols(ct))
        return carry

    qv_buf[...] = jnp.zeros(qv_buf.shape, U32)
    for i in range(3):
        tm_buf[i] = lane
    for sw in range(NS):
        zs_ref[sw] = 0
    if not SKIP1:
        set_row(x0)
        xacc_buf[...] = x0
        wq_cp.wait()
        lax.fori_loop(0, D // 16, fix_wq, 0)
        lax.fori_loop(0, 3 * NP, colsum_q, 0)
        wo_cp.wait()
        lax.fori_loop(0, H * DH // 128, fix_wo, 0)
        lax.fori_loop(0, NP, pair1, 0)
        x1 = xacc_buf[...]
        w1_cp.wait()
        cs1_buf[...] = _dot(jnp.concatenate([ones32] * (D // 128), axis=1), w1_buf[...])
        gp = mlp_hidden(x1)
        x2 = x1 + b2
        for i in range(W2C):
            w2_cps[i].wait()
            x2 = x2 + _dot(gp[:, W2S[i]:W2S[i] + W2R[i]], w2_buf[W2S[i]:W2S[i] + W2R[i], :])
    else:
        x2 = lax.fori_loop(0, 2, lambda i, x: x + 1.0, x0)

    if SKIP2:
        o_ref[...] = x2[0:1, :].astype(o_ref.dtype)
        return

    def block(j0, carry, kinds, jpar=None):
        true_mask = [tm_buf[i] >= 0 for i in range(3)]
        zs = [0] + [zs_ref[sw] if OPQ else 0 for sw in range(1, NS)]
        steps = []
        info = []
        for u, kind in enumerate(kinds):
            xs = (XE, XO) if kind == 'last' else (0, 0)
            tss = [list(range(x, nt)) for x in xs]
            s0 = len(steps)
            steps += [(u, par, sw, t) for par in range(2) for sw in range(NS) for t in tss[par]]
            info.append(dict(tss=tss, s0=s0, s_odd=s0 + NS * len(tss[0]), s_end=len(steps)))
        t_step = [0.0]
        for (_, _, _, t) in steps:
            t_step.append(t_step[-1] + CU * na * (6 if t < ntb else 4))
        gates, stores = {}, {}
        cur = dict(state=None, st=-1, nedge=0)
        envs = [dict(s1=[None] * ng, s2=[None] * ng, s3=[None] * ng) for _ in kinds]

        zq = zs_ref[0] if OPQ2 else 0

        def get_inv(h):
            return inv_sum(l_buf[zq + (h & 3)])

        def slot(u):
            return (j0 + u) & 1 if jpar is None else (jpar + u) & 1

        def step_at(cyc):
            return next((i for i, tt_ in enumerate(t_step) if tt_ >= cyc), len(t_step))

        def gate(cyc, v):
            st = step_at(cyc)
            while len(gates.get(st, ())) >= 2:
                st += 1
            if st < len(steps) and st > cur['st']:
                gates.setdefault(st, []).append(v)

        def edge(x, n=BE, force=False):
            if cur['st'] < 0 or not (force or cur['edge']):
                return x
            sw = cur['state']['sw']
            cand = list(range(2 * sw * na, 2 * (sw + 1) * na))
            ntile = -(-x.shape[1] // 128)
            parts = [x[:, 128 * i:min(128 * (i + 1), x.shape[1])] for i in range(ntile)]
            for e in range(min(n, 3 * ntile)):
                k_ = cur['nedge'] % len(cand)
                c = cand[(2 * k_) % len(cand) + (2 * k_) // len(cand)]
                cur['nedge'] += 1
                i = e % ntile
                w_ = parts[i].shape[1]
                parts[i] = jnp.where(true_mask[e // ntile][:, 0:w_], parts[i],
                                     pltpu.bitcast(cur['state']['accs'][c], U32)[:, 0:w_])
            return parts[0] if ntile == 1 else jnp.concatenate(parts, axis=1)

        def sched_stores(ps, lsum, h, p_out, t_ready, lo, hi):
            gate(t_ready, ps[-1])
            st_l = min(max(step_at(t_ready + 10), cur['st'] + 1), len(steps) - 1)
            stores.setdefault(st_l, []).append((lsum, h, None, None))
            n = 8 // SG
            t_first = max(t_ready, t_step[lo])
            for i in range(ng * n):
                g, k = divmod(i, n)
                st = min(max(step_at(t_first + SDT * i) + 1, cur['st'] + 1), hi)
                stores.setdefault(st, []).append((ps[g], g, range(SG * k, SG * (k + 1)), p_out))

        def pair_jobs(u):
            kind, env, inf = kinds[u], envs[u], info[u]
            first, last = kind == 'first', kind == 'last'
            j = j0 + u
            h0 = 2 * j

            def job_b(h, par, c, g, key, tail):
                def fn(td):
                    s = score2(edge(qv_buf[h & 3, c]), h, par, 4 * g + c)
                    sg = env[key]
                    sg[g] = s if c == 0 else sg[g] + s
                    gate(td + LATP, sg[g])
                    if c == 3:
                        (sp_buf if key != 's2' else s2_buf)[g] = sg[g]
                    if tail == 'sm1':
                        ps, lsum = softmax([sp_buf[zq + gg] for gg in range(ng)], None)
                        sched_stores(ps, lsum, h, p_buf1, td + LATP + MOFF, inf['s0'], inf['s_odd'])
                        if not first and not last:
                            store_q([qraw_buf[zq + i] for i in range(3)], j + 1)
                    elif tail == 'sm2':
                        ps, lsum = softmax([s2_buf[zq + gg] for gg in range(ng)], None)
                        sched_stores(ps, lsum, h, p_buf0, td + LATP + MOFF2, inf['s_odd'], inf['s_end'] - 1)
                return fn

            def job_e(td):
                o = o_pair(edge(ones32), accp_buf[1 - slot(u)], get_inv(h0 - 2), get_inv(h0 - 1))
                gate(td + LATP + 10, o[:, 256:384])
                op_buf[...] = _pack(o, o)

            def job_g(c):
                def fn(td):
                    xo = out_cols(edge(op_buf[...]), 24 * (j - 1), 24, c)
                    xacc_buf[:, 128 * c:128 * (c + 1)] += xo
                    gate(td + LATP, xo)
                return fn

            def job_a(c):
                def fn(td):
                    jn = j + 2 if isinstance(j, int) else jnp.minimum(j + 2, NP - 1)
                    qc = q_cols(edge(z_buf[...]), jn, c)
                    gate(td + LATP, qc)
                    qraw_buf[c] = qc
                return fn

            def job_x(par, t):
                def fn(td):
                    p = (p_buf0, p_buf1)[par][0, 8 * t:8 * t + 8, :]
                    rhs = jnp.concatenate([v_tile(h0 + par, a, t) for a in range(DH // 16)], axis=0)
                    o = _dot_t(edge(_pack(p, p)), rhs)
                    key = 'x%d' % par
                    env[key] = o if key not in env else env[key] + o
                    gate(td + LATP, env[key][:, 0:128])
                return fn

            def finish_head(par, inv, lhs_edge):
                acc = accp_buf[slot(u), par * (DH // 2):(par + 1) * (DH // 2), :]
                o = _dot_t(lhs_edge(ones32), acc)
                if 'x%d' % par in env:
                    o = o + env['x%d' % par]
                return o * jnp.concatenate([inv, inv[:, 0:DH - 128]], axis=1)

            env['finish_head'] = finish_head

            def job_e30(td):
                o = finish_head(0, get_inv(h0), edge)
                gate(td + LATP + 10, o[:, 0:128])
                env['op30'] = _pack(o, o)

            def job_g30(c):
                def fn(td):
                    xo = out_cols(edge(env['op30']), 12 * h0, 12, c)
                    xacc_buf[:, 128 * c:128 * (c + 1)] += xo
                    gate(td + LATP, xo)
                return fn

            jobs = []
            for g in range(0 if first else CA, ng):
                for c in range(4):
                    tail = 'sm1' if (c == 3 and g == ng - 1) else None
                    jobs.append((24, None, job_b(h0 + 1, 1, c, g, 's1', tail), 3))
            t_pair = t_step[inf['s0']] + EDEL if u > 0 else None
            groups = {
                'e': [] if first else [(EC, t_pair, job_e, 3)],
                'b': [(24, None, job_b(h0 + 2, 0, c, g, 's2',
                                       'sm2' if (c == 3 and g == ng - 1) else None), 3)
                      for g in range(ng) for c in range(4)],
                'a': [] if isinstance(j, int) and j + 2 >= NP else
                     [(40, None, job_a(c), 5) for c in range(3)],
                'g': [] if first else [(24, None, job_g(c), 3) for c in range(5)],
                'n': [(24, None, job_b(h0 + 3, 1, c, g, 's3', None), 3)
                      for g in range(CA) for c in range(4)],
            }
            if last:
                t_odd = t_step[inf['s_odd'] + 1]
                jobs += groups['e'] + [(24, None, job_x(0, t), 2) for t in range(XE)] + groups['g']
                jobs += [(24, t_odd, job_x(1, t), 2) for t in range(XO)]
                jobs += [(32, t_odd, job_e30, 2)]
                jobs += [(12, t_odd + LATP + 60, job_g30(c), 2) for c in range(5)]
            else:
                for ch in ORD:
                    jobs += groups[ch]
            return jobs

        pjobs = [pair_jobs(u) for u in range(len(kinds))]
        jobs = [job for pj in pjobs for job in pj]
        times = []
        tt = T0F if kinds[0] == 'first' else T0
        for u, pj in enumerate(pjobs):
            rho = RHO if 0 < u < len(kinds) - 1 else (RHO0 if u == 0 else RHOL)
            if u > 0 and LEAD is not None:
                tt = max(tt, t_step[info[u]['s0']] - LEAD)
            for (cost, earliest, _, _) in pj:
                tt += cost * rho
                if earliest is not None:
                    tt = max(tt, earliest)
                times.append(tt)

        states = {}
        nj = 0
        for st, (u, par, sw, t) in enumerate(steps):
            while nj < len(jobs) and times[nj] + EOFF <= t_step[st]:
                if times[nj] > 0 and 'j0' not in cur:
                    cur['j0'] = nj
                rel = nj - cur.get('j0', nj + 1)
                cur['edge'] = (0 <= rel < NE and rel % EE == EE - 1) or jobs[nj][1] == times[nj]
                jobs[nj][2](times[nj])
                nj += 1
            for (pv_, g_, rs_, po_) in stores.pop(st, ()):
                pv_ = pltpu.bitcast(edge(pltpu.bitcast(pv_, U32), SE, True), F32)
                if po_ is None:
                    l_buf[g_ & 3] = pv_
                else:
                    store_p(pv_, g_, rs_, po_)
            state = states.setdefault((u, par), dict(accs=[None] * 24, half=par, slot=slot(u), z=zs))
            pv_step(2 * (j0 + u) + par, sw, t, info[u]['tss'][par], (p_buf0, p_buf1)[par],
                    gates.get(st, ()), true_mask, state)
            cur['state'] = state
            cur['st'] = st
        cur['edge'] = False
        while nj < len(jobs):
            jobs[nj][2](times[nj])
            nj += 1
        assert not stores
        env = envs[-1]
        if kinds[-1] == 'last':
            o = env['finish_head'](1, get_inv(H - 1), lambda x: x)
            op = _pack(o, o)
            return xacc_buf[...] + jnp.concatenate(
                [out_cols(op, 12 * (H - 1), 12, c) for c in range(5)], axis=1)
        return carry

    set_row(x2)
    xacc_buf[...] = x2
    q_pair(0)
    q_pair(1)
    ps0, l0 = softmax(scores_all(0, 0), None)
    for g in range(ng):
        store_p(ps0[g], g, range(8), p_buf0)
    l_buf[0] = l0
    if ALL:
        x3 = block(0, 0, ['first'] + ['mid'] * (NP - 2) + ['last'])
    else:
        carry = block(0, 0, ['first'] + ['mid'] * NF)
        n_mid = (NP - 2 - NF - NL) // U
        if n_mid:
            carry = lax.fori_loop(0, n_mid * REP, lambda i, c: block(1 + NF + U * (i if REP == 1 else lax.rem(i, n_mid)), c, ['mid'] * U, (1 + NF) & 1 if U % 2 == 0 and not DYN else None), carry)
        x3 = block(NP - 1 - NL, carry, ['mid'] * NL + ['last'])
    x4 = x3 + b2 + _dot(mlp_hidden(x3), w2_buf[...])
    o_ref[...] = x4[0:1, :].astype(o_ref.dtype)


@jax.jit
def pallas_interleave_layers__sliding_block_cached__dense_activation_gelu__decode_kernel(
    A_x: jax.Array,
    A_k_cache: jax.Array,
    A_v_cache: jax.Array,
    A_wq: jax.Array,
    A_wo: jax.Array,
    B_x: jax.Array,
    B_w1: jax.Array,
    B_b1: jax.Array,
    B_w2: jax.Array,
    B_b2: jax.Array,
):
    sk = A_k_cache.shape[2]
    w = min(4096, max(256, sk // 4))

    def tile_view(a):
        *lead, r, c = a.shape
        n = len(lead)
        a = a.reshape(*lead, r // 8, 8, c // 128, 128)
        a = a.transpose(*range(n), n, n + 2, n + 1, n + 3)
        return a.reshape(*lead, r // 16, 2, (c // 128) * 8, 128)

    kx = tile_view(jnp.swapaxes(A_k_cache, 2, 3)[0]).reshape(H * DH // 8, sk // 16, 128)
    vx = tile_view(jnp.swapaxes(A_v_cache, 2, 3)[0]).reshape(H * DH // 8, sk // 16, 128)
    wqx = tile_view(A_wq)
    wox = tile_view(A_wo).reshape(H * DH // 16, 80, 128)
    any_spec = pl.BlockSpec(memory_space=pl.ANY)
    out = pl.pallas_call(
        functools.partial(_kernel, sk=sk, w=w),
        out_shape=jax.ShapeDtypeStruct((1, D), A_x.dtype),
        in_specs=[any_spec] * 9,
        out_specs=pl.BlockSpec(memory_space=pltpu.VMEM),
        scratch_shapes=[
            pltpu.VMEM((H * DH // 8, w // 32, 128), U32),
            pltpu.VMEM((H * DH // 8, w // 32 - 4 * XF, 128), U32),
            pltpu.VMEM((H * DH // 8, max(8 * XF, 8), 128), U32),
            pltpu.VMEM((D // 16, 2, H * DH // 32, 128), U32),
            pltpu.VMEM((H * DH // 16, 40, 128), U32),
            pltpu.VMEM((D, F), BF16),
            pltpu.VMEM((F, D), BF16),
            pltpu.VMEM((1, D), BF16),
            pltpu.VMEM((F // 128, 128), BF16),
            pltpu.VMEM((D // 128, 128), BF16),
            pltpu.VMEM((1, w // 16, 128), F32),
            pltpu.VMEM((1, w // 16, 128), F32),
            pltpu.VMEM((w // 1024, 8, 128), F32),
            pltpu.VMEM((2, DH, 128), U32),
            pltpu.VMEM((8, D), U32),
            pltpu.VMEM((8, D), F32),
            pltpu.VMEM((4, 4, 8, 2 * DH), U32),
            pltpu.VMEM((3, 8, 128), F32),
            pltpu.VMEM((3 * NP, 8, 128), F32),
            pltpu.VMEM((8, F), F32),
            pltpu.VMEM((2, 8, 128), F32),
            pltpu.VMEM((3, 8, 128), jnp.int32),
            pltpu.SMEM((NS,), jnp.int32),
            pltpu.VMEM((w // 1024, 8, 128), F32),
            pltpu.VMEM((8, 2 * DH), U32),
            pltpu.VMEM((4, 8, 128), F32),
            pltpu.SemaphoreType.DMA((2,)),
            pltpu.SemaphoreType.DMA((4,)),
            pltpu.SemaphoreType.DMA((6 + W2C,)),
        ],
        compiler_params=pltpu.CompilerParams(vmem_limit_bytes=int(OPT.get('VM', 127)) * 1024 * 1024,
                                             disable_semaphore_checks=bool(DSC), disable_bounds_checks=bool(DBC)),
    )(A_x.reshape(1, D), kx, vx, wqx, wox, B_w1, B_b1.reshape(F // 128, 128),
      B_w2, B_b2.reshape(D // 128, 128))
    return out.reshape(A_x.shape)
```

```python
import functools
import math

import jax
import jax.numpy as jnp
from jax import lax
import jax.experimental.pallas as pl
import jax.experimental.pallas.tpu as pltpu

F32 = jnp.float32
BF16 = jnp.bfloat16
U32 = jnp.uint32

D = 640
H = 32
DH = 192
F = 1536
EPS = 1e-5
NP = H // 2
OPT = {'T0F': '-100'}
NS = int(OPT.get('NS', 4))
CA = int(OPT.get('CA', 2))
CU = float(OPT.get('CU', 0.26))
XF = int(OPT.get('XF', 6))
CHUNKS = [int(c) for c in OPT.get('CHUNKS', '44322 1').replace(' ', '')]
LATP = float(OPT.get('LATP', 160))
T0 = float(OPT.get('T0', -10))
T0F = float(OPT.get('T0F', -200))
RHO = float(OPT.get('RHO', 1.07))
BE = int(OPT.get('BE', 6))
MOFF = float(OPT.get('MOFF', 160))
MOFF2 = float(OPT.get('MOFF2', 240))
EC = float(OPT.get('EC', 48))
SG = int(OPT.get('SG', 4))
SDT = float(OPT.get('SDT', 12))
CHAIN = int(OPT.get('CHAIN', 0))
XE = int(OPT.get('XE', 7))
XO = int(OPT.get('XO', 7))
W2R = [128 * int(c) for c in OPT.get('W2R', '5421')]
W2C = len(W2R)
W2S = [sum(W2R[:i]) for i in range(W2C)]
ORD = OPT.get('ORD', 'ebagn')
OPQ = int(OPT.get('OPQ', 0))
LA = int(OPT.get('LA', 1))
NE = int(OPT.get('NE', 7))
EE = int(OPT.get('EE', 2))
SE = int(OPT.get('SE', 1))
EOFF = float(OPT.get('EOFF', 0))
SM = int(OPT.get('SM', 1))
OM = int(OPT.get('OM', 1))
U = int(OPT.get('U', 2))
NF = int(OPT.get('NF', 0))
NL = int(OPT.get('NL', 0))
EDEL = float(OPT.get('EDEL', 70))
RHO0 = float(OPT.get('RHO0', 1.0))
RHOL = float(OPT.get('RHOL', 1.0))
BAR = int(OPT.get('BAR', 0))
IOFF = float(OPT.get('IOFF', 0))
DYN = int(OPT.get('DYN', 0))
MST = int(OPT.get('MST', 1))
DSC = int(OPT.get('DSC', 1))
DBC = int(OPT.get('DBC', 0))
REP = int(OPT.get('REP', 1))
PB = int(OPT.get('PB', 0))
ALL = int(OPT.get('ALL', 1))
LEAD = float(OPT.get('LEAD', 100))
OPQ2 = int(OPT.get('OPQ2', 1))
SKIP2 = int(OPT.get('SKIP2', 0))
SKIP1 = int(OPT.get('SKIP1', 0))


def _gelu(x):
    c = math.sqrt(2.0 / math.pi)
    return 0.5 * x * (1.0 + jnp.tanh(c * (x + 0.044715 * (x * x * x))))


def _rows_to_lanes(b, n):
    return jnp.concatenate([b[i:i + 1, :] for i in range(n)], axis=1)


def _bf(x):
    return pltpu.bitcast(x, BF16)


def _pack(a, b):
    return pltpu.bitcast(pltpu.pack_elementwise([a, b], packed_dtype=BF16), U32)


def _unpack(x):
    return (pltpu.unpack_elementwise(x, index=0, packed_dtype=BF16, unpacked_dtype=F32),
            pltpu.unpack_elementwise(x, index=1, packed_dtype=BF16, unpacked_dtype=F32))


def _dot(lhs32, rhs):
    return jnp.dot(_bf(lhs32), rhs, preferred_element_type=F32)[0:8]


def _dot_t(lhs32, rhs32):
    return lax.dot_general(_bf(lhs32), _bf(rhs32), (((1,), (1,)), ((), ())),
                           preferred_element_type=F32)[0:8]


def _ln_stats(xp, shift):
    x = _unpack(xp)[0] - shift
    m = jnp.mean(x, axis=-1, keepdims=True)
    v = jnp.maximum(jnp.mean(x * x, axis=-1, keepdims=True) - m * m, 0.0)
    return m + shift, lax.rsqrt(v + EPS)


def _mean(x):
    return jnp.mean(x, axis=-1, keepdims=True)


def _kernel(x_hbm, kx_hbm, vx_hbm, wq_hbm, wo_hbm, w1_hbm, b1_hbm, w2_hbm, b2_hbm,
            o_ref,
            kbuf, vbuf, vf_buf, wq_buf, wo_buf, w1_buf, w2_buf, x_buf, b1_buf, b2_buf,
            p_buf0, p_buf1, sp_buf, accp_buf, z_buf, xacc_buf, qv_buf, qraw_buf,
            csq_buf, cs1_buf, st_buf, tm_buf, zs_ref, s2_buf, op_buf, l_buf, wx_buf, lhs0_buf,
            sem_k, sem_v, sem_w, *, sk, w):
    c_scale = (DH ** -0.5) * math.log2(math.e)
    nt = w // 128
    ng = nt // 8
    na = 12 // NS
    nst = NS * nt
    r0w = (sk - w) // 16
    nrw = w // 16

    ntb = nt - XF
    starts = [sum(CHUNKS[:c]) for c in range(len(CHUNKS))]
    assert sum(CHUNKS) == NP

    def k_copy(c):
        rows = pl.ds(48 * starts[c], 48 * CHUNKS[c])
        return [pltpu.make_async_copy(kx_hbm.at[rows, pl.ds(r0w, nrw), :],
                                      kbuf.bitcast(BF16).at[rows], sem_k.at[c & 1])]

    def v_copy(c):
        rows = pl.ds(48 * starts[c], 48 * CHUNKS[c])
        cps = [pltpu.make_async_copy(vx_hbm.at[rows, pl.ds(r0w, 8 * ntb), :],
                                     vbuf.bitcast(BF16).at[rows], sem_v.at[c & 1])]
        if XF:
            cps.append(pltpu.make_async_copy(
                vx_hbm.at[rows, pl.ds(r0w + 8 * ntb, 8 * XF), :],
                vf_buf.bitcast(BF16).at[rows, pl.ds(8 * XF, 8 * XF), :], sem_v.at[2 + (c & 1)]))
        return cps

    wq_cp = pltpu.make_async_copy(wq_hbm, wq_buf.bitcast(BF16), sem_w.at[0])
    wo_cp = pltpu.make_async_copy(wo_hbm, wo_buf.bitcast(BF16), sem_w.at[1])
    w1_cp = pltpu.make_async_copy(w1_hbm, w1_buf, sem_w.at[2])
    x_cp = pltpu.make_async_copy(x_hbm, x_buf, sem_w.at[3])
    b1_cp = pltpu.make_async_copy(b1_hbm, b1_buf, sem_w.at[4])
    b2_cp = pltpu.make_async_copy(b2_hbm, b2_buf, sem_w.at[5])
    w2_cps = [pltpu.make_async_copy(w2_hbm.at[pl.ds(W2S[i], W2R[i]), :],
                                    w2_buf.at[pl.ds(W2S[i], W2R[i]), :], sem_w.at[6 + i])
              for i in range(W2C)]

    if not SKIP1:
        wq_cp.start()
    x_cp.start()
    b1_cp.start()
    b2_cp.start()
    if not SKIP1:
        wo_cp.start()
        for cp in k_copy(0) + v_copy(0):
            cp.start()
    x_cp.wait()
    b1_cp.wait()
    b2_cp.wait()

    x0 = jnp.broadcast_to(x_buf[...].astype(F32), (8, D))
    b1 = _rows_to_lanes(b1_buf[...].astype(F32), F // 128)
    b2 = _rows_to_lanes(b2_buf[...].astype(F32), D // 128)

    lane = lax.broadcasted_iota(jnp.int32, (8, 128), 1)
    sub_lo = lax.broadcasted_iota(jnp.int32, (1, 8, 128), 1) < 4
    lo64 = lane < 64
    sub = lax.broadcasted_iota(jnp.int32, (8, 128), 0)
    evn = (lane & 8) == 0
    zf = jnp.zeros((8, 128), F32)
    ones32 = jnp.full((8, 128), 0x3F803F80, U32)
    k_order = (
        list(range(0, 16, 2)) + list(range(1, 16, 2)) + [16, 18, 20, 22, 17, 19, 21, 23],
        list(range(8, 24, 2)) + list(range(9, 24, 2)) + [1, 3, 5, 7, 0, 2, 4, 6],
    )

    def swap_halves(ref2):
        n = ref2.shape[1]
        a = ref2[0].reshape(n // 8, 8, 128)
        b = ref2[1].reshape(n // 8, 8, 128)
        ref2[0] = jnp.where(sub_lo, a, pltpu.roll(b, 4, 1)).reshape(n, 128)
        ref2[1] = jnp.where(sub_lo, pltpu.roll(a, 4, 1), b).reshape(n, 128)

    def fix_wq(a, carry):
        swap_halves(wq_buf.at[a])
        return carry

    def fix_wo(g8, carry):
        g0 = pl.multiple_of(g8 * 8, 8)
        v = [wo_buf[pl.ds(g0, 8), 8 * c:8 * c + 8, :] for c in range(5)]
        n = [jnp.where(sub_lo, v[0], v[2]),
             pltpu.roll(jnp.where(sub_lo, v[3], v[0]), 4, 1),
             jnp.where(sub_lo, v[1], v[3]),
             pltpu.roll(jnp.where(sub_lo, v[4], v[1]), 4, 1),
             jnp.where(sub_lo, v[2], v[4])]
        for c in range(5):
            wo_buf[pl.ds(g0, 8), 8 * c:8 * c + 8, :] = n[c]
        return carry

    def set_row(x, shift):
        xp = _pack(x, x)
        z_buf[...] = xp
        m, r = _ln_stats(xp, shift)
        rc = r * c_scale
        st_buf[0] = jnp.broadcast_to(rc, (8, 128))
        st_buf[1] = jnp.broadcast_to(m * rc, (8, 128))

    def wq_cols(ct):
        r0 = pl.multiple_of(lax.shift_right_logical(ct, 1) * 8, 8) if not isinstance(ct, int) else (ct // 2) * 8
        return _bf(wq_buf[:, ct & 1, pl.ds(r0, 8), :].reshape(D // 2, 128))

    def q_cols(z, j, c):
        ct = 3 * j + c
        return _dot(z, wq_cols(ct)) * st_buf[0] - csq_buf[ct] * st_buf[1]

    def store_lhs(hh, ww):
        for c in range(4):
            for i in range(3):
                pltpu.store(qv_buf.at[hh & 3, c, :, 128 * i:128 * (i + 1)], ww[i], mask=sub == c)

    def store_q(qs, j, pars=(0, 1)):
        q0, q1, q2 = qs
        r56, r64, r8 = (pltpu.roll(q1, s, 1) for s in (56, 64, 8))

        def lhs(qf, a2, b2):
            a0 = jnp.where(evn, qf, zf)
            b1_ = jnp.where(evn, zf, qf)
            return [_pack(a0, pltpu.roll(a0, 8, 1)), _pack(pltpu.roll(b1_, 120, 1), b1_),
                    _pack(jnp.where(evn, a2, zf), jnp.where(evn, zf, b2))]

        if 0 in pars:
            store_lhs(2 * j, lhs(q0, jnp.where(lo64, q1, r56), jnp.where(lo64, r8, r64)))
        if 1 in pars:
            store_lhs(2 * j + 1, lhs(q2, jnp.where(lo64, r56, q1), jnp.where(lo64, r64, r8)))

    def q_pair(j):
        z = z_buf[...]
        store_q([q_cols(z, j, c) for c in range(3)], j)

    def score2(lhs, h, par, k):
        rhs = jnp.concatenate([kbuf[24 * h + i, 8 * k:8 * k + 8, :] for i in k_order[par]],
                              axis=0)
        return _dot(lhs, _bf(rhs))

    def scores_all(h, par):
        sg = [None] * ng
        for c in range(4):
            lhs = qv_buf[h & 3, c]
            for g in range(ng):
                s = score2(lhs, h, par, 4 * g + c)
                sg[g] = s if sg[g] is None else sg[g] + s
        return sg

    def store_p(p, g, rs, p_out):
        for r in rs:
            if PB:
                p_out[0, 64 * g + 8 * r:64 * g + 8 * r + 8, :] = jnp.broadcast_to(p[r:r + 1, :], (8, 128))
            else:
                p_out[0, pl.ds(64 * g + r, 8, stride=8), :] = p

    def inv_sum(l):
        l = jnp.sum(jnp.sum(l, axis=1, keepdims=True), axis=0, keepdims=True)
        return jnp.broadcast_to(1.0 / l, (8, 128))

    def softmax(sg, p_out):
        mx = sg[0]
        for s in sg[1:]:
            mx = jnp.maximum(mx, s)
        m = jnp.max(jnp.max(mx, axis=1, keepdims=True), axis=0, keepdims=True)
        l = None
        ps = []
        for g in range(ng):
            p = jnp.exp2(sg[g] - m)
            ps.append(p)
            if p_out is not None:
                store_p(p, g, range(8), p_out)
            l = p if l is None else l + p
        if p_out is None:
            return ps, l
        return ps, inv_sum(l)

    def v_tile(h, a, t):
        return vbuf[24 * h + 2 * a + t % 2, 8 * (t // 2):8 * (t // 2) + 8, :]

    def pv_step(h, sw, t, ts, p_in, gvals, true_mask, state):
        p = p_in[state['z'][sw], 8 * t:8 * t + 8, :]
        for i, gval in enumerate(gvals):
            p = jnp.where(true_mask[i], p, gval)
        accs = state['accs']
        for a in range(sw * na, (sw + 1) * na):
            if t < ntb:
                ys = _unpack(v_tile(h, a, t))
            else:
                r = 8 * (t - ntb)
                ys = [pltpu.bitcast(vf_buf[24 * h + 2 * a + e, r:r + 8, :], F32) for e in range(2)]
            for e in range(2):
                j = 2 * a + e
                accs[j] = ys[e] * p if t == ts[0] else accs[j] + ys[e] * p
        state['sw'] = sw
        if t == ts[-1]:
            for a in range(sw * na, (sw + 1) * na):
                r0 = state['half'] * (DH // 2) + 8 * a
                accp_buf[state['slot'], r0:r0 + 8, :] = _pack(accs[2 * a], accs[2 * a + 1])

    def o_pair(ones, accp, ie, io):
        inv = jnp.concatenate([ie, jnp.where(lo64, ie, io), io], axis=1)
        return _dot_t(ones, accp) * inv

    def out_cols(op, g0, ngrp, c):
        rhs = wo_buf[pl.ds(g0, ngrp), 8 * c:8 * c + 8, :].reshape(ngrp * 8, 128)
        return _dot(op, _bf(rhs))

    def mlp_hidden(x, shift):
        xp = _pack(x, x)
        m, r = _ln_stats(xp, shift)
        hh = (_dot(xp, w1_buf[...]) - cs1_buf[...] * m) * r + b1
        g = _gelu(hh)
        return _pack(g, g)

    def fix_v(r2, carry):
        swap_halves(vbuf.at[pl.ds(2 * r2, 2)])
        if XF:
            n = 4 * XF
            a = vf_buf[2 * r2, n:2 * n, :].reshape(n // 8, 8, 128)
            b = vf_buf[2 * r2 + 1, n:2 * n, :].reshape(n // 8, 8, 128)
            t0 = _unpack(jnp.where(sub_lo, a, pltpu.roll(b, 4, 1)))
            t1 = _unpack(jnp.where(sub_lo, pltpu.roll(a, 4, 1), b))
            for e in range(2):
                for k in range(XF // 2):
                    vf_buf[2 * r2 + e, 16 * k:16 * k + 8, :] = pltpu.bitcast(t0[e][k], U32)
                    vf_buf[2 * r2 + e, 16 * k + 8:16 * k + 16, :] = pltpu.bitcast(t1[e][k], U32)
        return carry

    def next_copies(j, copy_fn, tail_cps):
        for c in range(len(CHUNKS)):
            @pl.when(j == starts[c])
            def _():
                for cp in copy_fn(c):
                    cp.wait()
                for cp in (copy_fn(c + 1) if c + 1 < len(CHUNKS) else tail_cps):
                    cp.start()

    def pair1(j, carry):
        q_pair(j)
        next_copies(j, k_copy, [w1_cp])
        invs = []
        for par in range(2):
            _, inv = softmax(scores_all(2 * j + par, par), (p_buf0, p_buf1)[par])
            invs.append(inv)
        next_copies(j, v_copy, w2_cps)
        lax.fori_loop(24 * j, 24 * (j + 1), fix_v, 0)
        for par in range(2):
            state = dict(accs=[None] * 24, half=par, slot=0, z=[0] * NS)
            for sw in range(NS):
                for t in range(nt):
                    pv_step(2 * j + par, sw, t, range(nt), (p_buf0, p_buf1)[par], (), None, state)
        o = o_pair(ones32, accp_buf[0], invs[0], invs[1])
        op = _pack(o, o)
        for c in range(5):
            xacc_buf[:, 128 * c:128 * (c + 1)] += out_cols(op, 24 * j, 24, c)
        return carry

    def expand(t0, t1):
        return [jnp.where(evn, t0, pltpu.roll(t0, 8, 1)),
                jnp.where(evn, pltpu.roll(t0, 120, 1), t0),
                jnp.where(evn, jnp.where(lo64, t1, pltpu.roll(t1, 56, 1)),
                          jnp.where(lo64, pltpu.roll(t1, 8, 1), pltpu.roll(t1, 64, 1)))]

    def expand_wq(a, carry):
        e = expand(wq_buf[a, 0, 0:8, :], wq_buf[a, 1, 0:8, :])
        for i in range(3):
            wx_buf[i, a] = e[i]
        return carry

    def colsum_q(ct, carry):
        ones = jnp.concatenate([ones32] * (D // 128), axis=1)
        csq_buf[ct] = _dot(ones, wq_cols(ct))
        return carry

    qv_buf[...] = jnp.zeros(qv_buf.shape, U32)
    for i in range(3):
        tm_buf[i] = lane
    for sw in range(NS):
        zs_ref[sw] = 0
    if not SKIP1:
        set_row(x0, _mean(x0))
        xacc_buf[...] = x0
        wq_cp.wait()
        lax.fori_loop(0, D // 16, fix_wq, 0)
        lax.fori_loop(0, 3 * NP, colsum_q, 0)
        lax.fori_loop(0, D // 16, expand_wq, 0)
        e = expand(csq_buf[0], csq_buf[1])
        for i in range(3):
            csq_buf[3 * NP + i] = e[i]
        wo_cp.wait()
        lax.fori_loop(0, H * DH // 128, fix_wo, 0)
        lax.fori_loop(0, NP, pair1, 0)
        x1 = xacc_buf[...]
        w1_cp.wait()
        cs1_buf[...] = _dot(jnp.concatenate([ones32] * (D // 128), axis=1), w1_buf[...])
        gp = mlp_hidden(x1, _mean(x1))
        x2 = x1 + b2
        for i in range(W2C):
            if i == W2C - 1:
                shift2 = _mean(x2)
            w2_cps[i].wait()
            x2 = x2 + _dot(gp[:, W2S[i]:W2S[i] + W2R[i]], w2_buf[W2S[i]:W2S[i] + W2R[i], :])
    else:
        x2 = lax.fori_loop(0, 2, lambda i, x: x + 1.0, x0)
        shift2 = _mean(x0)

    if SKIP2:
        o_ref[...] = x2[0:1, :].astype(o_ref.dtype)
        return

    def block(j0, carry, kinds, jpar=None):
        true_mask = [tm_buf[i] >= 0 for i in range(3)]
        zs = [0] + [zs_ref[sw] if OPQ else 0 for sw in range(1, NS)]
        steps = []
        info = []
        for u, kind in enumerate(kinds):
            xs = (XE, XO) if kind == 'last' else (0, 0)
            tss = [list(range(x, nt)) for x in xs]
            s0 = len(steps)
            steps += [(u, par, sw, t) for par in range(2) for sw in range(NS) for t in tss[par]]
            info.append(dict(tss=tss, s0=s0, s_odd=s0 + NS * len(tss[0]), s_end=len(steps)))
        t_step = [0.0]
        for (_, _, _, t) in steps:
            t_step.append(t_step[-1] + CU * na * (6 if t < ntb else 4))
        gates, stores = {}, {}
        cur = dict(state=None, st=-1, nedge=0)
        envs = [dict(s1=[None] * ng, s2=[None] * ng, s3=[None] * ng) for _ in kinds]

        zq = zs_ref[0] if OPQ2 else 0

        def get_inv(h):
            return inv_sum(l_buf[zq + (h & 3)])

        def slot(u):
            return (j0 + u) & 1 if jpar is None else (jpar + u) & 1

        def step_at(cyc):
            return next((i for i, tt_ in enumerate(t_step) if tt_ >= cyc), len(t_step))

        def gate(cyc, v):
            st = step_at(cyc)
            while len(gates.get(st, ())) >= 2:
                st += 1
            if st < len(steps) and st > cur['st']:
                gates.setdefault(st, []).append(v)

        def edge(x, n=BE, force=False):
            if cur['st'] < 0 or not (force or cur['edge']):
                return x
            sw = cur['state']['sw']
            cand = list(range(2 * sw * na, 2 * (sw + 1) * na))
            ntile = -(-x.shape[1] // 128)
            parts = [x[:, 128 * i:min(128 * (i + 1), x.shape[1])] for i in range(ntile)]
            for e in range(min(n, 3 * ntile)):
                k_ = cur['nedge'] % len(cand)
                c = cand[(2 * k_) % len(cand) + (2 * k_) // len(cand)]
                cur['nedge'] += 1
                i = e % ntile
                w_ = parts[i].shape[1]
                parts[i] = jnp.where(true_mask[e // ntile][:, 0:w_], parts[i],
                                     pltpu.bitcast(cur['state']['accs'][c], U32)[:, 0:w_])
            return parts[0] if ntile == 1 else jnp.concatenate(parts, axis=1)

        def sched_stores(ps, lsum, h, p_out, t_ready, lo, hi):
            gate(t_ready, ps[-1])
            st_l = min(max(step_at(t_ready + 10), cur['st'] + 1), len(steps) - 1)
            stores.setdefault(st_l, []).append((lsum, h, None, None))
            n = 8 // SG
            t_first = max(t_ready, t_step[lo])
            for i in range(ng * n):
                g, k = divmod(i, n)
                st = min(max(step_at(t_first + SDT * i) + 1, cur['st'] + 1), hi)
                stores.setdefault(st, []).append((ps[g], g, range(SG * k, SG * (k + 1)), p_out))

        def pair_jobs(u):
            kind, env, inf = kinds[u], envs[u], info[u]
            first, last = kind == 'first', kind == 'last'
            j = j0 + u
            h0 = 2 * j

            def job_b(h, par, c, g, key, tail):
                def fn(td):
                    s = score2(edge(qv_buf[h & 3, c]), h, par, 4 * g + c)
                    sg = env[key]
                    sg[g] = s if c == 0 else sg[g] + s
                    gate(td + LATP, sg[g])
                    if c == 3:
                        (sp_buf if key != 's2' else s2_buf)[g] = sg[g]
                    if tail == 'sm1':
                        ps, lsum = softmax([sp_buf[zq + gg] for gg in range(ng)], None)
                        sched_stores(ps, lsum, h, p_buf1, td + LATP + MOFF, inf['s0'], inf['s_odd'])
                        if not first and not last:
                            store_q([qraw_buf[zq + i] for i in range(3)], j + 1)
                    elif tail == 'sm2':
                        ps, lsum = softmax([s2_buf[zq + gg] for gg in range(ng)], None)
                        sched_stores(ps, lsum, h, p_buf0, td + LATP + MOFF2, inf['s_odd'], inf['s_end'] - 1)
                return fn

            def job_e(td):
                if isinstance(j, int) and j == 1:
                    x = _dot_t(edge(lhs0_buf[...]), accp_buf[1 - slot(u)])
                    row = lambda i, r: jnp.broadcast_to(x[r:r + 1, 128 * i:128 * (i + 1)], (8, 128))
                    ie, io = get_inv(0), get_inv(1)
                    o = jnp.concatenate([row(0, 0) * ie, jnp.where(lo64, row(1, 0) * ie, row(1, 1) * io),
                                         row(2, 1) * io], axis=1)
                else:
                    o = o_pair(edge(ones32), accp_buf[1 - slot(u)], get_inv(h0 - 2), get_inv(h0 - 1))
                gate(td + LATP + 10, o[:, 256:384])
                op_buf[...] = _pack(o, o)

            def job_g(c):
                def fn(td):
                    xo = out_cols(edge(op_buf[...]), 24 * (j - 1), 24, c)
                    xacc_buf[:, 128 * c:128 * (c + 1)] += xo
                    gate(td + LATP, xo)
                return fn

            def job_a(c):
                def fn(td):
                    jn = j + 2 if isinstance(j, int) else jnp.minimum(j + 2, NP - 1)
                    qc = q_cols(edge(z_buf[...]), jn, c)
                    gate(td + LATP, qc)
                    qraw_buf[c] = qc
                return fn

            def job_x(par, t):
                def fn(td):
                    p = (p_buf0, p_buf1)[par][0, 8 * t:8 * t + 8, :]
                    rhs = jnp.concatenate([v_tile(h0 + par, a, t) for a in range(DH // 16)], axis=0)
                    o = _dot_t(edge(_pack(p, p)), rhs)
                    key = 'x%d' % par
                    env[key] = o if key not in env else env[key] + o
                    gate(td + LATP, env[key][:, 0:128])
                return fn

            def finish_head(par, inv, lhs_edge):
                acc = accp_buf[slot(u), par * (DH // 2):(par + 1) * (DH // 2), :]
                o = _dot_t(lhs_edge(ones32), acc)
                if 'x%d' % par in env:
                    o = o + env['x%d' % par]
                return o * jnp.concatenate([inv, inv[:, 0:DH - 128]], axis=1)

            env['finish_head'] = finish_head

            def job_e30(td):
                o = finish_head(0, get_inv(h0), edge)
                gate(td + LATP + 10, o[:, 0:128])
                env['op30'] = _pack(o, o)

            def job_g30(c):
                def fn(td):
                    xo = out_cols(edge(env['op30']), 12 * h0, 12, c)
                    xacc_buf[:, 128 * c:128 * (c + 1)] += xo
                    gate(td + LATP, xo)
                return fn

            jobs = []
            for g in range(0 if first else CA, ng):
                for c in range(4):
                    tail = 'sm1' if (c == 3 and g == ng - 1) else None
                    jobs.append((24, None, job_b(h0 + 1, 1, c, g, 's1', tail), 3))
            t_pair = t_step[inf['s0']] + EDEL if u > 0 else None
            groups = {
                'e': [] if first else [(EC, t_pair, job_e, 3)],
                'b': [(24, None, job_b(h0 + 2, 0, c, g, 's2',
                                       'sm2' if (c == 3 and g == ng - 1) else None), 3)
                      for g in range(ng) for c in range(4)],
                'a': [] if isinstance(j, int) and j + 2 >= NP else
                     [(40, None, job_a(c), 5) for c in range(3)],
                'g': [] if first else [(24, None, job_g(c), 3) for c in range(5)],
                'n': [(24, None, job_b(h0 + 3, 1, c, g, 's3', None), 3)
                      for g in range(CA) for c in range(4)],
            }
            if last:
                t_odd = t_step[inf['s_odd'] + 1]
                jobs += groups['e'] + [(24, None, job_x(0, t), 2) for t in range(XE)] + groups['g']
                jobs += [(24, t_odd, job_x(1, t), 2) for t in range(XO)]
                jobs += [(32, t_odd, job_e30, 2)]
                jobs += [(12, t_odd + LATP + 60, job_g30(c), 2) for c in range(5)]
            else:
                for ch in ORD:
                    jobs += groups[ch]
            return jobs

        pjobs = [pair_jobs(u) for u in range(len(kinds))]
        jobs = [job for pj in pjobs for job in pj]
        times = []
        tt = T0F if kinds[0] == 'first' else T0
        for u, pj in enumerate(pjobs):
            rho = RHO if 0 < u < len(kinds) - 1 else (RHO0 if u == 0 else RHOL)
            if u > 0 and LEAD is not None:
                tt = max(tt, t_step[info[u]['s0']] - LEAD)
            for (cost, earliest, _, _) in pj:
                tt += cost * rho
                if earliest is not None:
                    tt = max(tt, earliest)
                times.append(tt)

        states = {}
        nj = 0
        for st, (u, par, sw, t) in enumerate(steps):
            while nj < len(jobs) and times[nj] + EOFF <= t_step[st]:
                if times[nj] > 0 and 'j0' not in cur:
                    cur['j0'] = nj
                rel = nj - cur.get('j0', nj + 1)
                cur['edge'] = (0 <= rel < NE and rel % EE == EE - 1) or jobs[nj][1] == times[nj]
                jobs[nj][2](times[nj])
                nj += 1
            for (pv_, g_, rs_, po_) in stores.pop(st, ()):
                pv_ = pltpu.bitcast(edge(pltpu.bitcast(pv_, U32), SE, True), F32)
                if po_ is None:
                    l_buf[g_ & 3] = pv_
                else:
                    store_p(pv_, g_, rs_, po_)
            state = states.setdefault((u, par), dict(accs=[None] * 24, half=par, slot=slot(u), z=zs))
            pv_step(2 * (j0 + u) + par, sw, t, info[u]['tss'][par], (p_buf0, p_buf1)[par],
                    gates.get(st, ()), true_mask, state)
            cur['state'] = state
            cur['st'] = st
        cur['edge'] = False
        while nj < len(jobs):
            jobs[nj][2](times[nj])
            nj += 1
        assert not stores
        env = envs[-1]
        if kinds[-1] == 'last':
            o = env['finish_head'](1, get_inv(H - 1), lambda x: x)
            op = _pack(o, o)
            xp_ = xacc_buf[...]
            return xp_ + jnp.concatenate(
                [out_cols(op, 12 * (H - 1), 12, c) for c in range(5)], axis=1), _mean(xp_)
        return carry

    set_row(x2, shift2)
    xacc_buf[...] = x2
    z = z_buf[...]
    qx = [_dot(z, _bf(wx_buf[i].reshape(D // 2, 128))) * st_buf[0] - csq_buf[3 * NP + i] * st_buf[1]
          for i in range(3)]
    w0 = [_pack(jnp.where(evn, q_, zf), jnp.where(evn, zf, q_)) for q_ in qx]
    store_q([None, q_cols(z, 0, 1), q_cols(z, 0, 2)], 0, pars=(1,))
    sg = [None] * ng
    for g in range(ng):
        for c in range(4):
            lhs = jnp.concatenate([jnp.where(sub == c, w_, jnp.zeros_like(w_)) for w_ in w0], axis=1)
            s = score2(lhs, 0, 0, 4 * g + c)
            sg[g] = s if c == 0 else sg[g] + s
    q_pair(1)
    mx = jnp.maximum(jnp.maximum(sg[0], sg[1]), jnp.maximum(sg[2], sg[3]))
    m0 = jnp.broadcast_to(jnp.max(mx, axis=0, keepdims=True), (8, 128))
    l0 = None
    for g in range(ng):
        p = jnp.exp2(sg[g] - m0)
        store_p(p, g, range(8), p_buf0)
        l0 = p if l0 is None else l0 + p
    c0 = jnp.exp2(m0 - jnp.max(m0, axis=1, keepdims=True))
    lhs0_buf[...] = _pack(c0, jnp.ones((8, 128), F32))
    l_buf[0] = l0 * _unpack(_pack(c0, c0))[0]
    if ALL:
        x3, shift3 = block(0, 0, ['first'] + ['mid'] * (NP - 2) + ['last'])
    else:
        carry = block(0, 0, ['first'] + ['mid'] * NF)
        n_mid = (NP - 2 - NF - NL) // U
        if n_mid:
            carry = lax.fori_loop(0, n_mid * REP, lambda i, c: block(1 + NF + U * (i if REP == 1 else lax.rem(i, n_mid)), c, ['mid'] * U, (1 + NF) & 1 if U % 2 == 0 and not DYN else None), carry)
        x3, shift3 = block(NP - 1 - NL, carry, ['mid'] * NL + ['last'])
    x4 = x3 + b2 + _dot(mlp_hidden(x3, shift3), w2_buf[...])
    o_ref[...] = x4[0:1, :].astype(o_ref.dtype)


@jax.jit
def pallas_interleave_layers__sliding_block_cached__dense_activation_gelu__decode_kernel(
    A_x: jax.Array,
    A_k_cache: jax.Array,
    A_v_cache: jax.Array,
    A_wq: jax.Array,
    A_wo: jax.Array,
    B_x: jax.Array,
    B_w1: jax.Array,
    B_b1: jax.Array,
    B_w2: jax.Array,
    B_b2: jax.Array,
):
    sk = A_k_cache.shape[2]
    w = min(4096, max(256, sk // 4))

    def tile_view(a):
        *lead, r, c = a.shape
        n = len(lead)
        a = a.reshape(*lead, r // 8, 8, c // 128, 128)
        a = a.transpose(*range(n), n, n + 2, n + 1, n + 3)
        return a.reshape(*lead, r // 16, 2, (c // 128) * 8, 128)

    kx = tile_view(jnp.swapaxes(A_k_cache, 2, 3)[0]).reshape(H * DH // 8, sk // 16, 128)
    vx = tile_view(jnp.swapaxes(A_v_cache, 2, 3)[0]).reshape(H * DH // 8, sk // 16, 128)
    wqx = tile_view(A_wq)
    wox = tile_view(A_wo).reshape(H * DH // 16, 80, 128)
    any_spec = pl.BlockSpec(memory_space=pl.ANY)
    out = pl.pallas_call(
        functools.partial(_kernel, sk=sk, w=w),
        out_shape=jax.ShapeDtypeStruct((1, D), A_x.dtype),
        in_specs=[any_spec] * 9,
        out_specs=pl.BlockSpec(memory_space=pltpu.VMEM),
        scratch_shapes=[
            pltpu.VMEM((H * DH // 8, w // 32, 128), U32),
            pltpu.VMEM((H * DH // 8, w // 32 - 4 * XF, 128), U32),
            pltpu.VMEM((H * DH // 8, max(8 * XF, 8), 128), U32),
            pltpu.VMEM((D // 16, 2, H * DH // 32, 128), U32),
            pltpu.VMEM((H * DH // 16, 40, 128), U32),
            pltpu.VMEM((D, F), BF16),
            pltpu.VMEM((F, D), BF16),
            pltpu.VMEM((1, D), BF16),
            pltpu.VMEM((F // 128, 128), BF16),
            pltpu.VMEM((D // 128, 128), BF16),
            pltpu.VMEM((1, w // 16, 128), F32),
            pltpu.VMEM((1, w // 16, 128), F32),
            pltpu.VMEM((w // 1024, 8, 128), F32),
            pltpu.VMEM((2, DH, 128), U32),
            pltpu.VMEM((8, D), U32),
            pltpu.VMEM((8, D), F32),
            pltpu.VMEM((4, 4, 8, 2 * DH), U32),
            pltpu.VMEM((3, 8, 128), F32),
            pltpu.VMEM((3 * NP + 3, 8, 128), F32),
            pltpu.VMEM((8, F), F32),
            pltpu.VMEM((2, 8, 128), F32),
            pltpu.VMEM((3, 8, 128), jnp.int32),
            pltpu.SMEM((NS,), jnp.int32),
            pltpu.VMEM((w // 1024, 8, 128), F32),
            pltpu.VMEM((8, 2 * DH), U32),
            pltpu.VMEM((4, 8, 128), F32),
            pltpu.VMEM((3, D // 16, 8, 128), U32),
            pltpu.VMEM((8, 128), U32),
            pltpu.SemaphoreType.DMA((2,)),
            pltpu.SemaphoreType.DMA((4,)),
            pltpu.SemaphoreType.DMA((6 + W2C,)),
        ],
        compiler_params=pltpu.CompilerParams(vmem_limit_bytes=int(OPT.get('VM', 127)) * 1024 * 1024,
                                             disable_semaphore_checks=bool(DSC), disable_bounds_checks=bool(DBC)),
    )(A_x.reshape(1, D), kx, vx, wqx, wox, B_w1, B_b1.reshape(F // 128, 128),
      B_w2, B_b2.reshape(D // 128, 128))
    return out.reshape(A_x.shape)
```

```python
import functools
import math

import jax
import jax.numpy as jnp
from jax import lax
import jax.experimental.pallas as pl
import jax.experimental.pallas.tpu as pltpu

F32 = jnp.float32
BF16 = jnp.bfloat16
U32 = jnp.uint32

D = 640
H = 32
DH = 192
F = 1536
EPS = 1e-5
NP = H // 2
OPT = {'XB': '16'}
NS = int(OPT.get('NS', 4))
CA = int(OPT.get('CA', 2))
CU = float(OPT.get('CU', 0.26))
XF = int(OPT.get('XF', 6))
CHUNKS = [int(c) for c in OPT.get('CHUNKS', '44322 1').replace(' ', '')]
LATP = float(OPT.get('LATP', 160))
T0 = float(OPT.get('T0', -10))
T0F = float(OPT.get('T0F', -100))
RHO = float(OPT.get('RHO', 1.07))
BE = int(OPT.get('BE', 6))
MOFF = float(OPT.get('MOFF', 160))
MOFF2 = float(OPT.get('MOFF2', 240))
EC = float(OPT.get('EC', 48))
SG = int(OPT.get('SG', 4))
SDT = float(OPT.get('SDT', 12))
CHAIN = int(OPT.get('CHAIN', 0))
XE = int(OPT.get('XE', 7))
XO = int(OPT.get('XO', 7))
W2R = [128 * int(c) for c in OPT.get('W2R', '5421')]
W2C = len(W2R)
W2S = [sum(W2R[:i]) for i in range(W2C)]
ORD = OPT.get('ORD', 'ebagn')
OPQ = int(OPT.get('OPQ', 0))
LA = int(OPT.get('LA', 1))
NE = int(OPT.get('NE', 7))
EE = int(OPT.get('EE', 2))
SE = int(OPT.get('SE', 1))
EOFF = float(OPT.get('EOFF', 0))
SM = int(OPT.get('SM', 1))
OM = int(OPT.get('OM', 1))
U = int(OPT.get('U', 2))
NF = int(OPT.get('NF', 0))
NL = int(OPT.get('NL', 0))
EDEL = float(OPT.get('EDEL', 70))
RHO0 = float(OPT.get('RHO0', 1.0))
RHOL = float(OPT.get('RHOL', 1.0))
BAR = int(OPT.get('BAR', 0))
IOFF = float(OPT.get('IOFF', 0))
DYN = int(OPT.get('DYN', 0))
MST = int(OPT.get('MST', 1))
DSC = int(OPT.get('DSC', 1))
DBC = int(OPT.get('DBC', 0))
REP = int(OPT.get('REP', 1))
PB = int(OPT.get('PB', 0))
ALL = int(OPT.get('ALL', 1))
LEAD = float(OPT.get('LEAD', 100))
OPQ2 = int(OPT.get('OPQ2', 1))
XB = int(OPT.get('XB', 16))
XB1 = int(OPT.get('XB1', 6))
NGT = int(OPT.get('NGT', 12))
MOFL = float(OPT.get('MOFL', 60))
SKIP2 = int(OPT.get('SKIP2', 0))
SKIP1 = int(OPT.get('SKIP1', 0))


def _gelu(x):
    c = math.sqrt(2.0 / math.pi)
    return 0.5 * x * (1.0 + jnp.tanh(c * (x + 0.044715 * (x * x * x))))


def _rows_to_lanes(b, n):
    return jnp.concatenate([b[i:i + 1, :] for i in range(n)], axis=1)


def _bf(x):
    return pltpu.bitcast(x, BF16)


def _pack(a, b):
    return pltpu.bitcast(pltpu.pack_elementwise([a, b], packed_dtype=BF16), U32)


def _unpack(x):
    return (pltpu.unpack_elementwise(x, index=0, packed_dtype=BF16, unpacked_dtype=F32),
            pltpu.unpack_elementwise(x, index=1, packed_dtype=BF16, unpacked_dtype=F32))


def _dot(lhs32, rhs):
    return jnp.dot(_bf(lhs32), rhs, preferred_element_type=F32)[0:8]


def _dot_t(lhs32, rhs32):
    return lax.dot_general(_bf(lhs32), _bf(rhs32), (((1,), (1,)), ((), ())),
                           preferred_element_type=F32)[0:8]


def _ln_stats(xp, shift):
    x = _unpack(xp)[0] - shift
    m = jnp.mean(x, axis=-1, keepdims=True)
    v = jnp.maximum(jnp.mean(x * x, axis=-1, keepdims=True) - m * m, 0.0)
    return m + shift, lax.rsqrt(v + EPS)


def _mean(x):
    return jnp.mean(x, axis=-1, keepdims=True)


def _kernel(x_hbm, kx_hbm, vx_hbm, wq_hbm, wo_hbm, w1_hbm, b1_hbm, w2_hbm, b2_hbm,
            o_ref,
            kbuf, vbuf, vf_buf, wq_buf, wo_buf, w1_buf, w2_buf, x_buf, b1_buf, b2_buf,
            p_buf0, p_buf1, sp_buf, accp_buf, z_buf, xacc_buf, qv_buf, qraw_buf,
            csq_buf, cs1_buf, st_buf, tm_buf, zs_ref, s2_buf, op_buf, l_buf, wx_buf, lhs0_buf,
            sem_k, sem_v, sem_w, *, sk, w):
    c_scale = (DH ** -0.5) * math.log2(math.e)
    nt = w // 128
    ng = nt // 8
    na = 12 // NS
    nst = NS * nt
    r0w = (sk - w) // 16
    nrw = w // 16

    ntb = nt - XF
    starts = [sum(CHUNKS[:c]) for c in range(len(CHUNKS))]
    assert sum(CHUNKS) == NP

    def k_copy(c):
        rows = pl.ds(48 * starts[c], 48 * CHUNKS[c])
        return [pltpu.make_async_copy(kx_hbm.at[rows, pl.ds(r0w, nrw), :],
                                      kbuf.bitcast(BF16).at[rows], sem_k.at[c & 1])]

    def v_copy(c):
        rows = pl.ds(48 * starts[c], 48 * CHUNKS[c])
        cps = [pltpu.make_async_copy(vx_hbm.at[rows, pl.ds(r0w, 8 * ntb), :],
                                     vbuf.bitcast(BF16).at[rows], sem_v.at[c & 1])]
        if XF:
            cps.append(pltpu.make_async_copy(
                vx_hbm.at[rows, pl.ds(r0w + 8 * ntb, 8 * XF), :],
                vf_buf.bitcast(BF16).at[rows, pl.ds(8 * XF, 8 * XF), :], sem_v.at[2 + (c & 1)]))
        return cps

    wq_cp = pltpu.make_async_copy(wq_hbm, wq_buf.bitcast(BF16), sem_w.at[0])
    wo_cp = pltpu.make_async_copy(wo_hbm, wo_buf.bitcast(BF16), sem_w.at[1])
    w1_cp = pltpu.make_async_copy(w1_hbm, w1_buf, sem_w.at[2])
    x_cp = pltpu.make_async_copy(x_hbm, x_buf, sem_w.at[3])
    b1_cp = pltpu.make_async_copy(b1_hbm, b1_buf, sem_w.at[4])
    b2_cp = pltpu.make_async_copy(b2_hbm, b2_buf, sem_w.at[5])
    w2_cps = [pltpu.make_async_copy(w2_hbm.at[pl.ds(W2S[i], W2R[i]), :],
                                    w2_buf.at[pl.ds(W2S[i], W2R[i]), :], sem_w.at[6 + i])
              for i in range(W2C)]

    if not SKIP1:
        wq_cp.start()
    x_cp.start()
    b1_cp.start()
    b2_cp.start()
    if not SKIP1:
        wo_cp.start()
        for cp in k_copy(0) + v_copy(0):
            cp.start()
    x_cp.wait()
    b1_cp.wait()
    b2_cp.wait()

    x0 = jnp.broadcast_to(x_buf[...].astype(F32), (8, D))
    b1 = _rows_to_lanes(b1_buf[...].astype(F32), F // 128)
    b2 = _rows_to_lanes(b2_buf[...].astype(F32), D // 128)

    lane = lax.broadcasted_iota(jnp.int32, (8, 128), 1)
    sub_lo = lax.broadcasted_iota(jnp.int32, (1, 8, 128), 1) < 4
    lo64 = lane < 64
    sub = lax.broadcasted_iota(jnp.int32, (8, 128), 0)
    evn = (lane & 8) == 0
    zf = jnp.zeros((8, 128), F32)
    ones32 = jnp.full((8, 128), 0x3F803F80, U32)
    k_order = (
        list(range(0, 16, 2)) + list(range(1, 16, 2)) + [16, 18, 20, 22, 17, 19, 21, 23],
        list(range(8, 24, 2)) + list(range(9, 24, 2)) + [1, 3, 5, 7, 0, 2, 4, 6],
    )

    def swap_halves(ref2):
        n = ref2.shape[1]
        a = ref2[0].reshape(n // 8, 8, 128)
        b = ref2[1].reshape(n // 8, 8, 128)
        ref2[0] = jnp.where(sub_lo, a, pltpu.roll(b, 4, 1)).reshape(n, 128)
        ref2[1] = jnp.where(sub_lo, pltpu.roll(a, 4, 1), b).reshape(n, 128)

    def fix_wq(a, carry):
        swap_halves(wq_buf.at[a])
        return carry

    def fix_wo(g8, carry):
        g0 = pl.multiple_of(g8 * 8, 8)
        v = [wo_buf[pl.ds(g0, 8), 8 * c:8 * c + 8, :] for c in range(5)]
        n = [jnp.where(sub_lo, v[0], v[2]),
             pltpu.roll(jnp.where(sub_lo, v[3], v[0]), 4, 1),
             jnp.where(sub_lo, v[1], v[3]),
             pltpu.roll(jnp.where(sub_lo, v[4], v[1]), 4, 1),
             jnp.where(sub_lo, v[2], v[4])]
        for c in range(5):
            wo_buf[pl.ds(g0, 8), 8 * c:8 * c + 8, :] = n[c]
        return carry

    def set_row(x, shift):
        xp = _pack(x, x)
        z_buf[...] = xp
        m, r = _ln_stats(xp, shift)
        rc = r * c_scale
        st_buf[0] = jnp.broadcast_to(rc, (8, 128))
        st_buf[1] = jnp.broadcast_to(m * rc, (8, 128))

    def wq_cols(ct):
        r0 = pl.multiple_of(lax.shift_right_logical(ct, 1) * 8, 8) if not isinstance(ct, int) else (ct // 2) * 8
        return _bf(wq_buf[:, ct & 1, pl.ds(r0, 8), :].reshape(D // 2, 128))

    def q_cols(z, j, c):
        ct = 3 * j + c
        return _dot(z, wq_cols(ct)) * st_buf[0] - csq_buf[ct] * st_buf[1]

    def store_lhs(hh, ww):
        for c in range(4):
            for i in range(3):
                pltpu.store(qv_buf.at[hh & 3, c, :, 128 * i:128 * (i + 1)], ww[i], mask=sub == c)

    def store_q(qs, j, pars=(0, 1)):
        q0, q1, q2 = qs
        r56, r64, r8 = (pltpu.roll(q1, s, 1) for s in (56, 64, 8))

        def lhs(qf, a2, b2):
            a0 = jnp.where(evn, qf, zf)
            b1_ = jnp.where(evn, zf, qf)
            return [_pack(a0, pltpu.roll(a0, 8, 1)), _pack(pltpu.roll(b1_, 120, 1), b1_),
                    _pack(jnp.where(evn, a2, zf), jnp.where(evn, zf, b2))]

        if 0 in pars:
            store_lhs(2 * j, lhs(q0, jnp.where(lo64, q1, r56), jnp.where(lo64, r8, r64)))
        if 1 in pars:
            store_lhs(2 * j + 1, lhs(q2, jnp.where(lo64, r56, q1), jnp.where(lo64, r64, r8)))

    def q_pair(j):
        z = z_buf[...]
        store_q([q_cols(z, j, c) for c in range(3)], j)

    def score2(lhs, h, par, k):
        rhs = jnp.concatenate([kbuf[24 * h + i, 8 * k:8 * k + 8, :] for i in k_order[par]],
                              axis=0)
        return _dot(lhs, _bf(rhs))

    def scores_all(h, par):
        sg = [None] * ng
        for c in range(4):
            lhs = qv_buf[h & 3, c]
            for g in range(ng):
                s = score2(lhs, h, par, 4 * g + c)
                sg[g] = s if sg[g] is None else sg[g] + s
        return sg

    def store_p(p, g, rs, p_out):
        for r in rs:
            if PB:
                p_out[0, 64 * g + 8 * r:64 * g + 8 * r + 8, :] = jnp.broadcast_to(p[r:r + 1, :], (8, 128))
            else:
                p_out[0, pl.ds(64 * g + r, 8, stride=8), :] = p

    def inv_sum(l):
        l = jnp.sum(jnp.sum(l, axis=1, keepdims=True), axis=0, keepdims=True)
        return jnp.broadcast_to(1.0 / l, (8, 128))

    def softmax(sg, p_out):
        mx = sg[0]
        for s in sg[1:]:
            mx = jnp.maximum(mx, s)
        m = jnp.max(jnp.max(mx, axis=1, keepdims=True), axis=0, keepdims=True)
        l = None
        ps = []
        for g in range(ng):
            p = jnp.exp2(sg[g] - m)
            ps.append(p)
            if p_out is not None:
                store_p(p, g, range(8), p_out)
            l = p if l is None else l + p
        if p_out is None:
            return ps, l
        return ps, inv_sum(l)

    def softmax_lane(sg):
        mx = jnp.maximum(jnp.maximum(sg[0], sg[1]), jnp.maximum(sg[2], sg[3]))
        m = jnp.broadcast_to(jnp.max(mx, axis=0, keepdims=True), (8, 128))
        ps = [jnp.exp2(s - m) for s in sg]
        c = jnp.exp2(m - jnp.max(m, axis=1, keepdims=True))
        c = _unpack(_pack(c, c))[0]
        return ps, ((ps[0] + ps[1]) + (ps[2] + ps[3])) * c, c

    def v_tile(h, a, t):
        return vbuf[24 * h + 2 * a + t % 2, 8 * (t // 2):8 * (t // 2) + 8, :]

    def pv_step(h, tiles, t, ts, p_in, gvals, true_mask, state):
        p = p_in[0, 8 * t:8 * t + 8, :]
        for i, gval in enumerate(gvals):
            p = jnp.where(true_mask[i], p, gval)
        accs = state['accs']
        for a in tiles:
            if t < ntb:
                ys = _unpack(v_tile(h, a, t))
            else:
                r = 8 * (t - ntb)
                ys = [pltpu.bitcast(vf_buf[24 * h + 2 * a + e, r:r + 8, :], F32) for e in range(2)]
            for e in range(2):
                j = 2 * a + e
                accs[j] = ys[e] * p if t == ts[0] else accs[j] + ys[e] * p
        state['tiles'] = tiles
        if t == ts[-1]:
            for a in tiles:
                r0 = state['half'] * (DH // 2) + 8 * a
                accp_buf[state['slot'], r0:r0 + 8, :] = _pack(accs[2 * a], accs[2 * a + 1])

    def o_pair(ones, accp, ie, io):
        inv = jnp.concatenate([ie, jnp.where(lo64, ie, io), io], axis=1)
        return _dot_t(ones, accp) * inv

    def out_cols(op, g0, ngrp, c):
        rhs = wo_buf[pl.ds(g0, ngrp), 8 * c:8 * c + 8, :].reshape(ngrp * 8, 128)
        return _dot(op, _bf(rhs))

    def mlp_hidden(x, shift):
        xp = _pack(x, x)
        m, r = _ln_stats(xp, shift)
        hh = (_dot(xp, w1_buf[...]) - cs1_buf[...] * m) * r + b1
        g = _gelu(hh)
        return _pack(g, g)

    def fix_v(r2, carry):
        swap_halves(vbuf.at[pl.ds(2 * r2, 2)])
        if XF:
            n = 4 * XF
            a = vf_buf[2 * r2, n:2 * n, :].reshape(n // 8, 8, 128)
            b = vf_buf[2 * r2 + 1, n:2 * n, :].reshape(n // 8, 8, 128)
            t0 = _unpack(jnp.where(sub_lo, a, pltpu.roll(b, 4, 1)))
            t1 = _unpack(jnp.where(sub_lo, pltpu.roll(a, 4, 1), b))
            for e in range(2):
                for k in range(XF // 2):
                    vf_buf[2 * r2 + e, 16 * k:16 * k + 8, :] = pltpu.bitcast(t0[e][k], U32)
                    vf_buf[2 * r2 + e, 16 * k + 8:16 * k + 16, :] = pltpu.bitcast(t1[e][k], U32)
        return carry

    def next_copies(j, copy_fn, tail_cps):
        for c in range(len(CHUNKS)):
            @pl.when(j == starts[c])
            def _():
                for cp in copy_fn(c):
                    cp.wait()
                for cp in (copy_fn(c + 1) if c + 1 < len(CHUNKS) else tail_cps):
                    cp.start()

    def pair1(j, carry):
        q_pair(j)
        next_copies(j, k_copy, [w1_cp])
        invs = []
        for par in range(2):
            _, inv = softmax(scores_all(2 * j + par, par), (p_buf0, p_buf1)[par])
            invs.append(inv)
        next_copies(j, v_copy, w2_cps)
        lax.fori_loop(24 * j, 24 * (j + 1), fix_v, 0)
        for par in range(2):
            state = dict(accs=[None] * 24, half=par, slot=0, z=[0] * NS)
            for sw in range(NS):
                for t in range(nt):
                    pv_step(2 * j + par, range(sw * na, (sw + 1) * na), t, range(nt),
                            (p_buf0, p_buf1)[par], (), None, state)
        o = o_pair(ones32, accp_buf[0], invs[0], invs[1])
        op = _pack(o, o)
        for c in range(5):
            xacc_buf[:, 128 * c:128 * (c + 1)] += out_cols(op, 24 * j, 24, c)
        return carry

    def expand(t0, t1):
        return [jnp.where(evn, t0, pltpu.roll(t0, 8, 1)),
                jnp.where(evn, pltpu.roll(t0, 120, 1), t0),
                jnp.where(evn, jnp.where(lo64, t1, pltpu.roll(t1, 56, 1)),
                          jnp.where(lo64, pltpu.roll(t1, 8, 1), pltpu.roll(t1, 64, 1)))]

    def expand_wq(a, carry):
        e = expand(wq_buf[a, 0, 0:8, :], wq_buf[a, 1, 0:8, :])
        for i in range(3):
            wx_buf[i, a] = e[i]
        return carry

    def colsum_q(ct, carry):
        ones = jnp.concatenate([ones32] * (D // 128), axis=1)
        csq_buf[ct] = _dot(ones, wq_cols(ct))
        return carry

    qv_buf[...] = jnp.zeros(qv_buf.shape, U32)
    for i in range(3):
        tm_buf[i] = lane
    for sw in range(NS):
        zs_ref[sw] = 0
    if not SKIP1:
        set_row(x0, _mean(x0))
        xacc_buf[...] = x0
        wq_cp.wait()
        lax.fori_loop(0, D // 16, fix_wq, 0)
        lax.fori_loop(0, 3 * NP, colsum_q, 0)
        lax.fori_loop(0, D // 16, expand_wq, 0)
        e = expand(csq_buf[0], csq_buf[1])
        for i in range(3):
            csq_buf[3 * NP + i] = e[i]
        wo_cp.wait()
        lax.fori_loop(0, H * DH // 128, fix_wo, 0)
        lax.fori_loop(0, NP, pair1, 0)
        x1 = xacc_buf[...]
        w1_cp.wait()
        cs1_buf[...] = _dot(jnp.concatenate([ones32] * (D // 128), axis=1), w1_buf[...])
        gp = mlp_hidden(x1, _mean(x1))
        x2 = x1 + b2
        for i in range(W2C):
            if i == W2C - 1:
                shift2 = _mean(x2)
            w2_cps[i].wait()
            x2 = x2 + _dot(gp[:, W2S[i]:W2S[i] + W2R[i]], w2_buf[W2S[i]:W2S[i] + W2R[i], :])
    else:
        x2 = lax.fori_loop(0, 2, lambda i, x: x + 1.0, x0)
        shift2 = _mean(x0)

    if SKIP2:
        o_ref[...] = x2[0:1, :].astype(o_ref.dtype)
        return

    def block(j0, carry, kinds, jpar=None):
        true_mask = [tm_buf[i] >= 0 for i in range(3)]
        zs = [0] + [zs_ref[sw] if OPQ else 0 for sw in range(1, NS)]
        steps = []
        info = []
        std = [list(range(sw * na, (sw + 1) * na)) for sw in range(NS)]
        for u, kind in enumerate(kinds):
            if kind == 'last':
                sweeps = [[(tl, list(range(XE, nt))) for tl in std],
                          [([5, 6, 7], list(range(XO, nt))), ([2, 3, 4], list(range(XO, nt))),
                           ([0, 1], list(range(XO, nt))), ([8, 9, 10, 11], list(range(XB, nt)))]]
            else:
                sweeps = [[(tl, list(range(nt))) for tl in std]] * 2
            s0 = len(steps)
            steps += [(u, 0, tl, t, ts) for tl, ts in sweeps[0] for t in ts]
            s_odd = len(steps)
            steps += [(u, 1, tl, t, ts) for tl, ts in sweeps[1] for t in ts]
            info.append(dict(s0=s0, s_odd=s_odd, s_end=len(steps),
                             s_tail=len(steps) - len(sweeps[1][-1][1])))
        t_step = [0.0]
        for (_, _, tl, t, _) in steps:
            t_step.append(t_step[-1] + CU * len(tl) * (6 if t < ntb else 4))
        gates, stores = {}, {}
        cur = dict(state=None, st=-1, nedge=0)
        envs = [dict(s1=[None] * ng, s2=[None] * ng, s3=[None] * ng) for _ in kinds]

        zq = zs_ref[0] if OPQ2 else 0

        def get_inv(h):
            return inv_sum(l_buf[zq + (h & 3)])

        def slot(u):
            return (j0 + u) & 1 if jpar is None else (jpar + u) & 1

        def step_at(cyc):
            return next((i for i, tt_ in enumerate(t_step) if tt_ >= cyc), len(t_step))

        def gate(cyc, v):
            st = step_at(cyc)
            while len(gates.get(st, ())) >= 2:
                st += 1
            if st < len(steps) - NGT and st > cur['st']:
                gates.setdefault(st, []).append(v)

        def edge(x, n=BE, force=False):
            if cur['st'] < 0 or not (force or cur['edge']):
                return x
            cand = [2 * a + e for a in cur['state']['tiles'] for e in range(2)]
            ntile = -(-x.shape[1] // 128)
            parts = [x[:, 128 * i:min(128 * (i + 1), x.shape[1])] for i in range(ntile)]
            for e in range(min(n, 3 * ntile)):
                k_ = cur['nedge'] % len(cand)
                c = cand[(2 * k_) % len(cand) + (2 * k_) // len(cand)]
                cur['nedge'] += 1
                i = e % ntile
                w_ = parts[i].shape[1]
                parts[i] = jnp.where(true_mask[e // ntile][:, 0:w_], parts[i],
                                     pltpu.bitcast(cur['state']['accs'][c], U32)[:, 0:w_])
            return parts[0] if ntile == 1 else jnp.concatenate(parts, axis=1)

        def sched_stores(ps, lsum, h, p_out, t_ready, lo, hi, l_off=10):
            gate(t_ready, ps[-1])
            st_l = min(max(step_at(t_ready + l_off), cur['st'] + 1), len(steps) - 1)
            stores.setdefault(st_l, []).append((lsum, h, None, None))
            n = 8 // SG
            t_first = max(t_ready, t_step[lo])
            for i in range(ng * n):
                g, k = divmod(i, n)
                st = min(max(step_at(t_first + SDT * i) + 1, cur['st'] + 1), hi)
                stores.setdefault(st, []).append((ps[g], g, range(SG * k, SG * (k + 1)), p_out))

        def pair_jobs(u):
            kind, env, inf = kinds[u], envs[u], info[u]
            first, last = kind == 'first', kind == 'last'
            j = j0 + u
            h0 = 2 * j

            def job_b(h, par, c, g, key, tail):
                def fn(td):
                    s = score2(edge(qv_buf[h & 3, c]), h, par, 4 * g + c)
                    sg = env[key]
                    sg[g] = s if c == 0 else sg[g] + s
                    gate(td + LATP, sg[g])
                    if c == 3:
                        (sp_buf if key != 's2' else s2_buf)[g] = sg[g]
                    if tail == 'sm1' and first:
                        ps, lsum, c1 = softmax_lane([sp_buf[zq + gg] for gg in range(ng)])
                        lhs0_buf[...] = _pack(c0, c1)
                        sched_stores(ps, lsum, h, p_buf1, td + LATP + MOFL, inf['s0'], inf['s_odd'], 130)
                    elif tail == 'sm1':
                        ps, lsum = softmax([sp_buf[zq + gg] for gg in range(ng)], None)
                        sched_stores(ps, lsum, h, p_buf1, td + LATP + MOFF, inf['s0'], inf['s_odd'])
                        if not first and not last:
                            store_q([qraw_buf[zq + i] for i in range(3)], j + 1)
                    elif tail == 'sm2':
                        ps, lsum = softmax([s2_buf[zq + gg] for gg in range(ng)], None)
                        sched_stores(ps, lsum, h, p_buf0, td + LATP + MOFF2, inf['s_odd'], inf['s_end'] - 1)
                return fn

            def job_e(td):
                if isinstance(j, int) and j == 1:
                    x = _dot_t(edge(lhs0_buf[...]), accp_buf[1 - slot(u)])
                    row = lambda i, r: jnp.broadcast_to(x[r:r + 1, 128 * i:128 * (i + 1)], (8, 128))
                    ie, io = get_inv(0), get_inv(1)
                    o = jnp.concatenate([row(0, 0) * ie, jnp.where(lo64, row(1, 0) * ie, row(1, 1) * io),
                                         row(2, 1) * io], axis=1)
                else:
                    o = o_pair(edge(ones32), accp_buf[1 - slot(u)], get_inv(h0 - 2), get_inv(h0 - 1))
                gate(td + LATP + 10, o[:, 256:384])
                op_buf[...] = _pack(o, o)

            def job_g(c):
                def fn(td):
                    xo = out_cols(edge(op_buf[...]), 24 * (j - 1), 24, c)
                    xacc_buf[:, 128 * c:128 * (c + 1)] += xo
                    gate(td + LATP, xo)
                return fn

            def job_a(c):
                def fn(td):
                    jn = j + 2 if isinstance(j, int) else jnp.minimum(j + 2, NP - 1)
                    qc = q_cols(edge(z_buf[...]), jn, c)
                    gate(td + LATP, qc)
                    qraw_buf[c] = qc
                return fn

            def job_x(par, t, tiles, key):
                def fn(td):
                    p = (p_buf0, p_buf1)[par][0, 8 * t:8 * t + 8, :]
                    rhs = jnp.concatenate([v_tile(h0 + par, a, t) for a in tiles], axis=0)
                    o = _dot_t(edge(_pack(p, p)), rhs)
                    env[key] = o if key not in env else env[key] + o
                    gate(td + LATP, env[key][:, 0:128] if len(tiles) >= 8 else
                         jnp.concatenate([env[key], env[key]], axis=1))
                return fn

            def finish(par, a0, a1, key, lhs_edge):
                r0 = par * (DH // 2)
                o = _dot_t(lhs_edge(ones32), accp_buf[slot(u), r0 + 8 * a0:r0 + 8 * a1, :])
                if key in env:
                    o = o + env[key]
                inv = get_inv(h0 + par)
                n = 16 * (a1 - a0)
                return o * (inv[:, 0:n] if n <= 128 else jnp.concatenate([inv, inv[:, 0:n - 128]], axis=1))

            env['finish'] = finish

            def job_fin(par, a0, a1, key):
                def fn(td):
                    o = finish(par, a0, a1, key, edge)
                    gate(td + LATP + 10, o[:, 0:128])
                    env['op' + key] = _pack(o, o)
                return fn

            def job_gfin(par, a0, a1, key, c):
                def fn(td):
                    xo = out_cols(edge(env['op' + key]), 12 * (h0 + par) + a0, a1 - a0, c)
                    xacc_buf[:, 128 * c:128 * (c + 1)] += xo
                    gate(td + LATP, xo)
                return fn

            jobs = []
            for g in range(0 if first else CA, ng):
                for c in range(4):
                    tail = 'sm1' if (c == 3 and g == ng - 1) else None
                    jobs.append((24, None, job_b(h0 + 1, 1, c, g, 's1', tail), 3))
            t_pair = t_step[inf['s0']] + EDEL if u > 0 else None
            groups = {
                'e': [] if first else [(EC, t_pair, job_e, 3)],
                'b': [(24, None, job_b(h0 + 2, 0, c, g, 's2',
                                       'sm2' if (c == 3 and g == ng - 1) else None), 3)
                      for g in range(ng) for c in range(4)],
                'a': [] if isinstance(j, int) and j + 2 >= NP else
                     [(40, None, job_a(c), 5) for c in range(3)],
                'g': [] if first else [(24, None, job_g(c), 3) for c in range(5)],
                'n': [(24, None, job_b(h0 + 3, 1, c, g, 's3', None), 3)
                      for g in range(CA) for c in range(4)],
            }
            if last:
                t_odd = t_step[inf['s_odd'] + 1]
                t_tail = t_step[inf['s_tail'] + 1]
                al, ah = list(range(8)), list(range(8, 12))
                jobs += groups['e'] + [(24, None, job_x(0, t, al + ah, 'x0'), 2) for t in range(XE)]
                jobs += groups['g']
                jobs += [(32, t_odd, job_fin(0, 0, 12, 'x0'), 2)]
                jobs += [(16, None, job_x(1, t, al, 'x1a'), 1) for t in range(XO)]
                jobs += [(12, t_odd + LATP + 60, job_gfin(0, 0, 12, 'x0', c), 2) for c in range(5)]
                jobs += [(8, None, job_x(1, t, ah, 'x1b'), 1) for t in range(XB1)]
                jobs += [(16, t_tail, job_fin(1, 0, 8, 'x1a'), 1)]
                jobs += [(8, None, job_x(1, t, ah, 'x1b'), 1) for t in range(XB1, XB)]
            else:
                for ch in ORD:
                    jobs += groups[ch]
            return jobs

        pjobs = [pair_jobs(u) for u in range(len(kinds))]
        jobs = [job for pj in pjobs for job in pj]
        times = []
        tt = T0F if kinds[0] == 'first' else T0
        for u, pj in enumerate(pjobs):
            rho = RHO if 0 < u < len(kinds) - 1 else (RHO0 if u == 0 else RHOL)
            if u > 0 and LEAD is not None:
                tt = max(tt, t_step[info[u]['s0']] - LEAD)
            for (cost, earliest, _, _) in pj:
                tt += cost * rho
                if earliest is not None:
                    tt = max(tt, earliest)
                times.append(tt)

        states = {}
        nj = 0
        for st, (u, par, tl, t, ts) in enumerate(steps):
            while nj < len(jobs) and times[nj] + EOFF <= t_step[st]:
                if times[nj] > 0 and 'j0' not in cur:
                    cur['j0'] = nj
                rel = nj - cur.get('j0', nj + 1)
                cur['edge'] = (0 <= rel < NE and rel % EE == EE - 1) or jobs[nj][1] == times[nj]
                jobs[nj][2](times[nj])
                nj += 1
            for (pv_, g_, rs_, po_) in stores.pop(st, ()):
                pv_ = pltpu.bitcast(edge(pltpu.bitcast(pv_, U32), SE, True), F32)
                if po_ is None:
                    l_buf[g_ & 3] = pv_
                else:
                    store_p(pv_, g_, rs_, po_)
            state = states.setdefault((u, par), dict(accs=[None] * 24, half=par, slot=slot(u)))
            pv_step(2 * (j0 + u) + par, tl, t, ts, (p_buf0, p_buf1)[par],
                    gates.get(st, ()), true_mask, state)
            cur['state'] = state
            cur['st'] = st
        cur['edge'] = False
        while nj < len(jobs):
            jobs[nj][2](times[nj])
            nj += 1
        assert not stores
        env = envs[-1]
        if kinds[-1] == 'last':
            o = env['finish'](1, 8, 12, 'x1b', lambda x: x)
            op = _pack(o, o)
            xa = [out_cols(env['opx1a'], 12 * (H - 1), 8, c) for c in range(5)]
            xb = [out_cols(op, 12 * (H - 1) + 8, 4, c) for c in range(5)]
            return (xacc_buf[...] + jnp.concatenate(xa, axis=1)) + jnp.concatenate(xb, axis=1), shift2
        return carry

    set_row(x2, shift2)
    xacc_buf[...] = x2
    z = z_buf[...]
    qx = [_dot(z, _bf(wx_buf[i].reshape(D // 2, 128))) * st_buf[0] - csq_buf[3 * NP + i] * st_buf[1]
          for i in range(3)]
    w0 = [_pack(jnp.where(evn, q_, zf), jnp.where(evn, zf, q_)) for q_ in qx]
    store_q([None, q_cols(z, 0, 1), q_cols(z, 0, 2)], 0, pars=(1,))
    sg = [None] * ng
    for g in range(ng):
        for c in range(4):
            lhs = jnp.concatenate([jnp.where(sub == c, w_, jnp.zeros_like(w_)) for w_ in w0], axis=1)
            s = score2(lhs, 0, 0, 4 * g + c)
            sg[g] = s if c == 0 else sg[g] + s
    q_pair(1)
    ps0, l0, c0 = softmax_lane(sg)
    for g in range(ng):
        store_p(ps0[g], g, range(8), p_buf0)
    l_buf[0] = l0
    if ALL:
        x3, shift3 = block(0, 0, ['first'] + ['mid'] * (NP - 2) + ['last'])
    else:
        carry = block(0, 0, ['first'] + ['mid'] * NF)
        n_mid = (NP - 2 - NF - NL) // U
        if n_mid:
            carry = lax.fori_loop(0, n_mid * REP, lambda i, c: block(1 + NF + U * (i if REP == 1 else lax.rem(i, n_mid)), c, ['mid'] * U, (1 + NF) & 1 if U % 2 == 0 and not DYN else None), carry)
        x3, shift3 = block(NP - 1 - NL, carry, ['mid'] * NL + ['last'])
    x4 = x3 + b2 + _dot(mlp_hidden(x3, shift3), w2_buf[...])
    o_ref[...] = x4[0:1, :].astype(o_ref.dtype)


@jax.jit
def pallas_interleave_layers__sliding_block_cached__dense_activation_gelu__decode_kernel(
    A_x: jax.Array,
    A_k_cache: jax.Array,
    A_v_cache: jax.Array,
    A_wq: jax.Array,
    A_wo: jax.Array,
    B_x: jax.Array,
    B_w1: jax.Array,
    B_b1: jax.Array,
    B_w2: jax.Array,
    B_b2: jax.Array,
):
    sk = A_k_cache.shape[2]
    w = min(4096, max(256, sk // 4))

    def tile_view(a):
        *lead, r, c = a.shape
        n = len(lead)
        a = a.reshape(*lead, r // 8, 8, c // 128, 128)
        a = a.transpose(*range(n), n, n + 2, n + 1, n + 3)
        return a.reshape(*lead, r // 16, 2, (c // 128) * 8, 128)

    kx = tile_view(jnp.swapaxes(A_k_cache, 2, 3)[0]).reshape(H * DH // 8, sk // 16, 128)
    vx = tile_view(jnp.swapaxes(A_v_cache, 2, 3)[0]).reshape(H * DH // 8, sk // 16, 128)
    wqx = tile_view(A_wq)
    wox = tile_view(A_wo).reshape(H * DH // 16, 80, 128)
    any_spec = pl.BlockSpec(memory_space=pl.ANY)
    out = pl.pallas_call(
        functools.partial(_kernel, sk=sk, w=w),
        out_shape=jax.ShapeDtypeStruct((1, D), A_x.dtype),
        in_specs=[any_spec] * 9,
        out_specs=pl.BlockSpec(memory_space=pltpu.VMEM),
        scratch_shapes=[
            pltpu.VMEM((H * DH // 8, w // 32, 128), U32),
            pltpu.VMEM((H * DH // 8, w // 32 - 4 * XF, 128), U32),
            pltpu.VMEM((H * DH // 8, max(8 * XF, 8), 128), U32),
            pltpu.VMEM((D // 16, 2, H * DH // 32, 128), U32),
            pltpu.VMEM((H * DH // 16, 40, 128), U32),
            pltpu.VMEM((D, F), BF16),
            pltpu.VMEM((F, D), BF16),
            pltpu.VMEM((1, D), BF16),
            pltpu.VMEM((F // 128, 128), BF16),
            pltpu.VMEM((D // 128, 128), BF16),
            pltpu.VMEM((1, w // 16, 128), F32),
            pltpu.VMEM((1, w // 16, 128), F32),
            pltpu.VMEM((w // 1024, 8, 128), F32),
            pltpu.VMEM((2, DH, 128), U32),
            pltpu.VMEM((8, D), U32),
            pltpu.VMEM((8, D), F32),
            pltpu.VMEM((4, 4, 8, 2 * DH), U32),
            pltpu.VMEM((3, 8, 128), F32),
            pltpu.VMEM((3 * NP + 3, 8, 128), F32),
            pltpu.VMEM((8, F), F32),
            pltpu.VMEM((2, 8, 128), F32),
            pltpu.VMEM((3, 8, 128), jnp.int32),
            pltpu.SMEM((NS,), jnp.int32),
            pltpu.VMEM((w // 1024, 8, 128), F32),
            pltpu.VMEM((8, 2 * DH), U32),
            pltpu.VMEM((4, 8, 128), F32),
            pltpu.VMEM((3, D // 16, 8, 128), U32),
            pltpu.VMEM((8, 128), U32),
            pltpu.SemaphoreType.DMA((2,)),
            pltpu.SemaphoreType.DMA((4,)),
            pltpu.SemaphoreType.DMA((6 + W2C,)),
        ],
        compiler_params=pltpu.CompilerParams(vmem_limit_bytes=int(OPT.get('VM', 127)) * 1024 * 1024,
                                             disable_semaphore_checks=bool(DSC), disable_bounds_checks=bool(DBC)),
    )(A_x.reshape(1, D), kx, vx, wqx, wox, B_w1, B_b1.reshape(F // 128, 128),
      B_w2, B_b2.reshape(D // 128, 128))
    return out.reshape(A_x.shape)
```

```python
import functools
import math

import jax
import jax.numpy as jnp
from jax import lax
import jax.experimental.pallas as pl
import jax.experimental.pallas.tpu as pltpu

F32 = jnp.float32
BF16 = jnp.bfloat16
U32 = jnp.uint32

D = 640
H = 32
DH = 192
F = 1536
EPS = 1e-5
NP = H // 2
OPT = {'XM': '1', 'XMP': '2', 'RHO': '1.02'}
NS = int(OPT.get('NS', 4))
CA = int(OPT.get('CA', 2))
CU = float(OPT.get('CU', 0.26))
XF = int(OPT.get('XF', 6))
CHUNKS = [int(c) for c in OPT.get('CHUNKS', '44322 1').replace(' ', '')]
LATP = float(OPT.get('LATP', 160))
T0 = float(OPT.get('T0', -10))
T0F = float(OPT.get('T0F', -100))
RHO = float(OPT.get('RHO', 1.07))
BE = int(OPT.get('BE', 6))
MOFF = float(OPT.get('MOFF', 160))
MOFF2 = float(OPT.get('MOFF2', 240))
EC = float(OPT.get('EC', 48))
SG = int(OPT.get('SG', 4))
SDT = float(OPT.get('SDT', 12))
CHAIN = int(OPT.get('CHAIN', 0))
XE = int(OPT.get('XE', 7))
XO = int(OPT.get('XO', 7))
W2R = [128 * int(c) for c in OPT.get('W2R', '5421')]
W2C = len(W2R)
W2S = [sum(W2R[:i]) for i in range(W2C)]
ORD = OPT.get('ORD', 'ebxagn')
OPQ = int(OPT.get('OPQ', 0))
LA = int(OPT.get('LA', 1))
NE = int(OPT.get('NE', 7))
EE = int(OPT.get('EE', 2))
SE = int(OPT.get('SE', 1))
EOFF = float(OPT.get('EOFF', 0))
SM = int(OPT.get('SM', 1))
OM = int(OPT.get('OM', 1))
U = int(OPT.get('U', 2))
NF = int(OPT.get('NF', 0))
NL = int(OPT.get('NL', 0))
EDEL = float(OPT.get('EDEL', 70))
RHO0 = float(OPT.get('RHO0', 1.0))
RHOL = float(OPT.get('RHOL', 1.0))
BAR = int(OPT.get('BAR', 0))
IOFF = float(OPT.get('IOFF', 0))
DYN = int(OPT.get('DYN', 0))
MST = int(OPT.get('MST', 1))
DSC = int(OPT.get('DSC', 1))
DBC = int(OPT.get('DBC', 0))
REP = int(OPT.get('REP', 1))
PB = int(OPT.get('PB', 0))
ALL = int(OPT.get('ALL', 1))
LEAD = float(OPT.get('LEAD', 100))
OPQ2 = int(OPT.get('OPQ2', 1))
XB = int(OPT.get('XB', 16))
XB1 = int(OPT.get('XB1', 6))
NGT = int(OPT.get('NGT', 12))
MOFL = float(OPT.get('MOFL', 60))
XM = int(OPT.get('XM', 1))
XMP = int(OPT.get('XMP', 2))
RF = float(OPT.get('RF', 0))
SKIP2 = int(OPT.get('SKIP2', 0))
SKIP1 = int(OPT.get('SKIP1', 0))


def _gelu(x):
    c = math.sqrt(2.0 / math.pi)
    return 0.5 * x * (1.0 + jnp.tanh(c * (x + 0.044715 * (x * x * x))))


def _rows_to_lanes(b, n):
    return jnp.concatenate([b[i:i + 1, :] for i in range(n)], axis=1)


def _bf(x):
    return pltpu.bitcast(x, BF16)


def _pack(a, b):
    return pltpu.bitcast(pltpu.pack_elementwise([a, b], packed_dtype=BF16), U32)


def _unpack(x):
    return (pltpu.unpack_elementwise(x, index=0, packed_dtype=BF16, unpacked_dtype=F32),
            pltpu.unpack_elementwise(x, index=1, packed_dtype=BF16, unpacked_dtype=F32))


def _dot(lhs32, rhs):
    return jnp.dot(_bf(lhs32), rhs, preferred_element_type=F32)[0:8]


def _dot_t(lhs32, rhs32):
    return lax.dot_general(_bf(lhs32), _bf(rhs32), (((1,), (1,)), ((), ())),
                           preferred_element_type=F32)[0:8]


def _ln_stats(xp, shift):
    x = _unpack(xp)[0] - shift
    m = jnp.mean(x, axis=-1, keepdims=True)
    v = jnp.maximum(jnp.mean(x * x, axis=-1, keepdims=True) - m * m, 0.0)
    return m + shift, lax.rsqrt(v + EPS)


def _mean(x):
    return jnp.mean(x, axis=-1, keepdims=True)


def _kernel(x_hbm, kx_hbm, vx_hbm, wq_hbm, wo_hbm, w1_hbm, b1_hbm, w2_hbm, b2_hbm,
            o_ref,
            kbuf, vbuf, vf_buf, wq_buf, wo_buf, w1_buf, w2_buf, x_buf, b1_buf, b2_buf,
            p_buf0, p_buf1, sp_buf, accp_buf, z_buf, xacc_buf, qv_buf, qraw_buf,
            csq_buf, cs1_buf, st_buf, tm_buf, zs_ref, s2_buf, op_buf, l_buf, wx_buf, lhs0_buf, xo_buf,
            sem_k, sem_v, sem_w, *, sk, w):
    c_scale = (DH ** -0.5) * math.log2(math.e)
    nt = w // 128
    ng = nt // 8
    na = 12 // NS
    nst = NS * nt
    r0w = (sk - w) // 16
    nrw = w // 16

    ntb = nt - XF
    starts = [sum(CHUNKS[:c]) for c in range(len(CHUNKS))]
    assert sum(CHUNKS) == NP

    def k_copy(c):
        rows = pl.ds(48 * starts[c], 48 * CHUNKS[c])
        return [pltpu.make_async_copy(kx_hbm.at[rows, pl.ds(r0w, nrw), :],
                                      kbuf.bitcast(BF16).at[rows], sem_k.at[c & 1])]

    def v_copy(c):
        rows = pl.ds(48 * starts[c], 48 * CHUNKS[c])
        cps = [pltpu.make_async_copy(vx_hbm.at[rows, pl.ds(r0w, 8 * ntb), :],
                                     vbuf.bitcast(BF16).at[rows], sem_v.at[c & 1])]
        if XF:
            cps.append(pltpu.make_async_copy(
                vx_hbm.at[rows, pl.ds(r0w + 8 * ntb, 8 * XF), :],
                vf_buf.bitcast(BF16).at[rows, pl.ds(8 * XF, 8 * XF), :], sem_v.at[2 + (c & 1)]))
        return cps

    wq_cp = pltpu.make_async_copy(wq_hbm, wq_buf.bitcast(BF16), sem_w.at[0])
    wo_cp = pltpu.make_async_copy(wo_hbm, wo_buf.bitcast(BF16), sem_w.at[1])
    w1_cp = pltpu.make_async_copy(w1_hbm, w1_buf, sem_w.at[2])
    x_cp = pltpu.make_async_copy(x_hbm, x_buf, sem_w.at[3])
    b1_cp = pltpu.make_async_copy(b1_hbm, b1_buf, sem_w.at[4])
    b2_cp = pltpu.make_async_copy(b2_hbm, b2_buf, sem_w.at[5])
    w2_cps = [pltpu.make_async_copy(w2_hbm.at[pl.ds(W2S[i], W2R[i]), :],
                                    w2_buf.at[pl.ds(W2S[i], W2R[i]), :], sem_w.at[6 + i])
              for i in range(W2C)]

    if not SKIP1:
        wq_cp.start()
    x_cp.start()
    b1_cp.start()
    b2_cp.start()
    if not SKIP1:
        wo_cp.start()
        for cp in k_copy(0) + v_copy(0):
            cp.start()
    x_cp.wait()
    b1_cp.wait()
    b2_cp.wait()

    x0 = jnp.broadcast_to(x_buf[...].astype(F32), (8, D))
    b1 = _rows_to_lanes(b1_buf[...].astype(F32), F // 128)
    b2 = _rows_to_lanes(b2_buf[...].astype(F32), D // 128)

    lane = lax.broadcasted_iota(jnp.int32, (8, 128), 1)
    sub_lo = lax.broadcasted_iota(jnp.int32, (1, 8, 128), 1) < 4
    lo64 = lane < 64
    sub = lax.broadcasted_iota(jnp.int32, (8, 128), 0)
    evn = (lane & 8) == 0
    zf = jnp.zeros((8, 128), F32)
    ones32 = jnp.full((8, 128), 0x3F803F80, U32)
    k_order = (
        list(range(0, 16, 2)) + list(range(1, 16, 2)) + [16, 18, 20, 22, 17, 19, 21, 23],
        list(range(8, 24, 2)) + list(range(9, 24, 2)) + [1, 3, 5, 7, 0, 2, 4, 6],
    )

    def swap_halves(ref2):
        n = ref2.shape[1]
        a = ref2[0].reshape(n // 8, 8, 128)
        b = ref2[1].reshape(n // 8, 8, 128)
        ref2[0] = jnp.where(sub_lo, a, pltpu.roll(b, 4, 1)).reshape(n, 128)
        ref2[1] = jnp.where(sub_lo, pltpu.roll(a, 4, 1), b).reshape(n, 128)

    def fix_wq(a, carry):
        swap_halves(wq_buf.at[a])
        return carry

    def fix_wo(g8, carry):
        g0 = pl.multiple_of(g8 * 8, 8)
        v = [wo_buf[pl.ds(g0, 8), 8 * c:8 * c + 8, :] for c in range(5)]
        n = [jnp.where(sub_lo, v[0], v[2]),
             pltpu.roll(jnp.where(sub_lo, v[3], v[0]), 4, 1),
             jnp.where(sub_lo, v[1], v[3]),
             pltpu.roll(jnp.where(sub_lo, v[4], v[1]), 4, 1),
             jnp.where(sub_lo, v[2], v[4])]
        for c in range(5):
            wo_buf[pl.ds(g0, 8), 8 * c:8 * c + 8, :] = n[c]
        return carry

    def set_row(x, shift):
        xp = _pack(x, x)
        z_buf[...] = xp
        m, r = _ln_stats(xp, shift)
        rc = r * c_scale
        st_buf[0] = jnp.broadcast_to(rc, (8, 128))
        st_buf[1] = jnp.broadcast_to(m * rc, (8, 128))

    def wq_cols(ct):
        r0 = pl.multiple_of(lax.shift_right_logical(ct, 1) * 8, 8) if not isinstance(ct, int) else (ct // 2) * 8
        return _bf(wq_buf[:, ct & 1, pl.ds(r0, 8), :].reshape(D // 2, 128))

    def q_cols(z, j, c):
        ct = 3 * j + c
        return _dot(z, wq_cols(ct)) * st_buf[0] - csq_buf[ct] * st_buf[1]

    def store_lhs(hh, ww):
        for c in range(4):
            for i in range(3):
                pltpu.store(qv_buf.at[hh & 3, c, :, 128 * i:128 * (i + 1)], ww[i], mask=sub == c)

    def store_q(qs, j, pars=(0, 1)):
        q0, q1, q2 = qs
        r56, r64, r8 = (pltpu.roll(q1, s, 1) for s in (56, 64, 8))

        def lhs(qf, a2, b2):
            a0 = jnp.where(evn, qf, zf)
            b1_ = jnp.where(evn, zf, qf)
            return [_pack(a0, pltpu.roll(a0, 8, 1)), _pack(pltpu.roll(b1_, 120, 1), b1_),
                    _pack(jnp.where(evn, a2, zf), jnp.where(evn, zf, b2))]

        if 0 in pars:
            store_lhs(2 * j, lhs(q0, jnp.where(lo64, q1, r56), jnp.where(lo64, r8, r64)))
        if 1 in pars:
            store_lhs(2 * j + 1, lhs(q2, jnp.where(lo64, r56, q1), jnp.where(lo64, r64, r8)))

    def q_pair(j):
        z = z_buf[...]
        store_q([q_cols(z, j, c) for c in range(3)], j)

    def score2(lhs, h, par, k):
        rhs = jnp.concatenate([kbuf[24 * h + i, 8 * k:8 * k + 8, :] for i in k_order[par]],
                              axis=0)
        return _dot(lhs, _bf(rhs))

    def scores_all(h, par):
        sg = [None] * ng
        for c in range(4):
            lhs = qv_buf[h & 3, c]
            for g in range(ng):
                s = score2(lhs, h, par, 4 * g + c)
                sg[g] = s if sg[g] is None else sg[g] + s
        return sg

    def store_p(p, g, rs, p_out):
        for r in rs:
            if PB:
                p_out[0, 64 * g + 8 * r:64 * g + 8 * r + 8, :] = jnp.broadcast_to(p[r:r + 1, :], (8, 128))
            else:
                p_out[0, pl.ds(64 * g + r, 8, stride=8), :] = p

    def inv_sum(l):
        l = jnp.sum(jnp.sum(l, axis=1, keepdims=True), axis=0, keepdims=True)
        return jnp.broadcast_to(1.0 / l, (8, 128))

    def softmax(sg, p_out):
        mx = sg[0]
        for s in sg[1:]:
            mx = jnp.maximum(mx, s)
        m = jnp.max(jnp.max(mx, axis=1, keepdims=True), axis=0, keepdims=True)
        l = None
        ps = []
        for g in range(ng):
            p = jnp.exp2(sg[g] - m)
            ps.append(p)
            if p_out is not None:
                store_p(p, g, range(8), p_out)
            l = p if l is None else l + p
        if p_out is None:
            return ps, l
        return ps, inv_sum(l)

    def softmax_lane(sg):
        mx = jnp.maximum(jnp.maximum(sg[0], sg[1]), jnp.maximum(sg[2], sg[3]))
        m = jnp.broadcast_to(jnp.max(mx, axis=0, keepdims=True), (8, 128))
        ps = [jnp.exp2(s - m) for s in sg]
        c = jnp.exp2(m - jnp.max(m, axis=1, keepdims=True))
        c = _unpack(_pack(c, c))[0]
        return ps, ((ps[0] + ps[1]) + (ps[2] + ps[3])) * c, c

    def v_tile(h, a, t):
        return vbuf[24 * h + 2 * a + t % 2, 8 * (t // 2):8 * (t // 2) + 8, :]

    def pv_step(h, tiles, t, ts, p_in, gvals, true_mask, state):
        p = p_in[0, 8 * t:8 * t + 8, :]
        for i, gval in enumerate(gvals):
            p = jnp.where(true_mask[i], p, gval)
        accs = state['accs']
        for a in tiles:
            if t < ntb:
                ys = _unpack(v_tile(h, a, t))
            else:
                r = 8 * (t - ntb)
                ys = [pltpu.bitcast(vf_buf[24 * h + 2 * a + e, r:r + 8, :], F32) for e in range(2)]
            for e in range(2):
                j = 2 * a + e
                accs[j] = ys[e] * p if t == ts[0] else accs[j] + ys[e] * p
        state['tiles'] = tiles
        if t == ts[-1]:
            for a in tiles:
                r0 = state['half'] * (DH // 2) + 8 * a
                accp_buf[state['slot'], r0:r0 + 8, :] = _pack(accs[2 * a], accs[2 * a + 1])

    def o_pair(ones, accp, ie, io):
        inv = jnp.concatenate([ie, jnp.where(lo64, ie, io), io], axis=1)
        return _dot_t(ones, accp) * inv

    def out_cols(op, g0, ngrp, c):
        rhs = wo_buf[pl.ds(g0, ngrp), 8 * c:8 * c + 8, :].reshape(ngrp * 8, 128)
        return _dot(op, _bf(rhs))

    def mlp_hidden(x, shift):
        xp = _pack(x, x)
        m, r = _ln_stats(xp, shift)
        hh = (_dot(xp, w1_buf[...]) - cs1_buf[...] * m) * r + b1
        g = _gelu(hh)
        return _pack(g, g)

    def fix_v(r2, carry):
        swap_halves(vbuf.at[pl.ds(2 * r2, 2)])
        if XF:
            n = 4 * XF
            a = vf_buf[2 * r2, n:2 * n, :].reshape(n // 8, 8, 128)
            b = vf_buf[2 * r2 + 1, n:2 * n, :].reshape(n // 8, 8, 128)
            t0 = _unpack(jnp.where(sub_lo, a, pltpu.roll(b, 4, 1)))
            t1 = _unpack(jnp.where(sub_lo, pltpu.roll(a, 4, 1), b))
            for e in range(2):
                for k in range(XF // 2):
                    vf_buf[2 * r2 + e, 16 * k:16 * k + 8, :] = pltpu.bitcast(t0[e][k], U32)
                    vf_buf[2 * r2 + e, 16 * k + 8:16 * k + 16, :] = pltpu.bitcast(t1[e][k], U32)
        return carry

    def next_copies(j, copy_fn, tail_cps):
        for c in range(len(CHUNKS)):
            @pl.when(j == starts[c])
            def _():
                for cp in copy_fn(c):
                    cp.wait()
                for cp in (copy_fn(c + 1) if c + 1 < len(CHUNKS) else tail_cps):
                    cp.start()

    def pair1(j, carry):
        q_pair(j)
        next_copies(j, k_copy, [w1_cp])
        invs = []
        for par in range(2):
            _, inv = softmax(scores_all(2 * j + par, par), (p_buf0, p_buf1)[par])
            invs.append(inv)
        next_copies(j, v_copy, w2_cps)
        lax.fori_loop(24 * j, 24 * (j + 1), fix_v, 0)
        for par in range(2):
            state = dict(accs=[None] * 24, half=par, slot=0, z=[0] * NS)
            for sw in range(NS):
                for t in range(nt):
                    pv_step(2 * j + par, range(sw * na, (sw + 1) * na), t, range(nt),
                            (p_buf0, p_buf1)[par], (), None, state)
        o = o_pair(ones32, accp_buf[0], invs[0], invs[1])
        op = _pack(o, o)
        for c in range(5):
            xacc_buf[:, 128 * c:128 * (c + 1)] += out_cols(op, 24 * j, 24, c)
        return carry

    def expand(t0, t1):
        return [jnp.where(evn, t0, pltpu.roll(t0, 8, 1)),
                jnp.where(evn, pltpu.roll(t0, 120, 1), t0),
                jnp.where(evn, jnp.where(lo64, t1, pltpu.roll(t1, 56, 1)),
                          jnp.where(lo64, pltpu.roll(t1, 8, 1), pltpu.roll(t1, 64, 1)))]

    def expand_wq(a, carry):
        e = expand(wq_buf[a, 0, 0:8, :], wq_buf[a, 1, 0:8, :])
        for i in range(3):
            wx_buf[i, a] = e[i]
        return carry

    def colsum_q(ct, carry):
        ones = jnp.concatenate([ones32] * (D // 128), axis=1)
        csq_buf[ct] = _dot(ones, wq_cols(ct))
        return carry

    qv_buf[...] = jnp.zeros(qv_buf.shape, U32)
    for i in range(3):
        tm_buf[i] = lane
    for sw in range(NS):
        zs_ref[sw] = 0
    if not SKIP1:
        set_row(x0, _mean(x0))
        xacc_buf[...] = x0
        wq_cp.wait()
        lax.fori_loop(0, D // 16, fix_wq, 0)
        lax.fori_loop(0, 3 * NP, colsum_q, 0)
        lax.fori_loop(0, D // 16, expand_wq, 0)
        e = expand(csq_buf[0], csq_buf[1])
        for i in range(3):
            csq_buf[3 * NP + i] = e[i]
        wo_cp.wait()
        lax.fori_loop(0, H * DH // 128, fix_wo, 0)
        lax.fori_loop(0, NP, pair1, 0)
        x1 = xacc_buf[...]
        w1_cp.wait()
        cs1_buf[...] = _dot(jnp.concatenate([ones32] * (D // 128), axis=1), w1_buf[...])
        gp = mlp_hidden(x1, _mean(x1))
        x2 = x1 + b2
        for i in range(W2C):
            if i == W2C - 1:
                shift2 = _mean(x2)
            w2_cps[i].wait()
            x2 = x2 + _dot(gp[:, W2S[i]:W2S[i] + W2R[i]], w2_buf[W2S[i]:W2S[i] + W2R[i], :])
    else:
        x2 = lax.fori_loop(0, 2, lambda i, x: x + 1.0, x0)
        shift2 = _mean(x0)

    if SKIP2:
        o_ref[...] = x2[0:1, :].astype(o_ref.dtype)
        return

    def block(j0, carry, kinds, jpar=None):
        true_mask = [tm_buf[i] >= 0 for i in range(3)]
        zs = [0] + [zs_ref[sw] if OPQ else 0 for sw in range(1, NS)]
        steps = []
        info = []
        def xm(j):
            return XM if (j % XMP == XMP - 1 and 0 < j < NP - 1) else 0

        std = [list(range(sw * na, (sw + 1) * na)) for sw in range(NS)]
        for u, kind in enumerate(kinds):
            if kind == 'last':
                sweeps = [[(tl, list(range(XE, nt))) for tl in std],
                          [([5, 6, 7], list(range(XO, nt))), ([2, 3, 4], list(range(XO, nt))),
                           ([0, 1], list(range(XO, nt))), ([8, 9, 10, 11], list(range(XB, nt)))]]
            else:
                sweeps = [[(tl, list(range(xm(j0 + u), nt))) for tl in std]] * 2
            s0 = len(steps)
            steps += [(u, 0, tl, t, ts) for tl, ts in sweeps[0] for t in ts]
            s_odd = len(steps)
            steps += [(u, 1, tl, t, ts) for tl, ts in sweeps[1] for t in ts]
            info.append(dict(s0=s0, s_odd=s_odd, s_end=len(steps),
                             s_tail=len(steps) - len(sweeps[1][-1][1])))
        t_step = [0.0]
        for (_, _, tl, t, _) in steps:
            t_step.append(t_step[-1] + CU * len(tl) * (6 if t < ntb else 4))
        gates, stores = {}, {}
        cur = dict(state=None, st=-1, nedge=0)
        envs = [dict(s1=[None] * ng, s2=[None] * ng, s3=[None] * ng) for _ in kinds]

        zq = zs_ref[0] if OPQ2 else 0

        def get_inv(h):
            return inv_sum(l_buf[zq + (h & 3)])

        def slot(u):
            return (j0 + u) & 1 if jpar is None else (jpar + u) & 1

        def step_at(cyc):
            return next((i for i, tt_ in enumerate(t_step) if tt_ >= cyc), len(t_step))

        def gate(cyc, v):
            st = step_at(cyc)
            while len(gates.get(st, ())) >= 2:
                st += 1
            if st < len(steps) - NGT and st > cur['st']:
                gates.setdefault(st, []).append(v)

        def edge(x, n=BE, force=False):
            if cur['st'] < 0 or not (force or cur['edge']):
                return x
            cand = [2 * a + e for a in cur['state']['tiles'] for e in range(2)]
            ntile = -(-x.shape[1] // 128)
            parts = [x[:, 128 * i:min(128 * (i + 1), x.shape[1])] for i in range(ntile)]
            for e in range(min(n, 3 * ntile)):
                k_ = cur['nedge'] % len(cand)
                c = cand[(2 * k_) % len(cand) + (2 * k_) // len(cand)]
                cur['nedge'] += 1
                i = e % ntile
                w_ = parts[i].shape[1]
                parts[i] = jnp.where(true_mask[e // ntile][:, 0:w_], parts[i],
                                     pltpu.bitcast(cur['state']['accs'][c], U32)[:, 0:w_])
            return parts[0] if ntile == 1 else jnp.concatenate(parts, axis=1)

        def sched_stores(ps, lsum, h, p_out, t_ready, lo, hi, l_off=10):
            gate(t_ready, ps[-1])
            st_l = min(max(step_at(t_ready + l_off), cur['st'] + 1), len(steps) - 1)
            stores.setdefault(st_l, []).append((lsum, h, None, None))
            n = 8 // SG
            t_first = max(t_ready, t_step[lo])
            for i in range(ng * n):
                g, k = divmod(i, n)
                st = min(max(step_at(t_first + SDT * i) + 1, cur['st'] + 1), hi)
                stores.setdefault(st, []).append((ps[g], g, range(SG * k, SG * (k + 1)), p_out))

        def pair_jobs(u):
            kind, env, inf = kinds[u], envs[u], info[u]
            first, last = kind == 'first', kind == 'last'
            j = j0 + u
            h0 = 2 * j

            def job_b(h, par, c, g, key, tail):
                def fn(td):
                    s = score2(edge(qv_buf[h & 3, c]), h, par, 4 * g + c)
                    sg = env[key]
                    sg[g] = s if c == 0 else sg[g] + s
                    gate(td + LATP, sg[g])
                    if c == 3:
                        (sp_buf if key != 's2' else s2_buf)[g] = sg[g]
                    if tail == 'sm1' and first:
                        ps, lsum, c1 = softmax_lane([sp_buf[zq + gg] for gg in range(ng)])
                        lhs0_buf[...] = _pack(c0, c1)
                        sched_stores(ps, lsum, h, p_buf1, td + LATP + MOFL, inf['s0'], inf['s_odd'], 130)
                    elif tail == 'sm1':
                        ps, lsum = softmax([sp_buf[zq + gg] for gg in range(ng)], None)
                        sched_stores(ps, lsum, h, p_buf1, td + LATP + MOFF, inf['s0'], inf['s_odd'])
                        if not first and not last:
                            store_q([qraw_buf[zq + i] for i in range(3)], j + 1)
                    elif tail == 'sm2':
                        ps, lsum = softmax([s2_buf[zq + gg] for gg in range(ng)], None)
                        sched_stores(ps, lsum, h, p_buf0, td + LATP + MOFF2, inf['s_odd'], inf['s_end'] - 1)
                return fn

            def job_e(td):
                if j == 1 or xm(j - 1):
                    x = _dot_t(edge(lhs0_buf[...] if j == 1 else ones32), accp_buf[1 - slot(u)])
                    if xm(j - 1):
                        x = x + xo_buf[zq]
                    row = lambda i, r: jnp.broadcast_to(x[r:r + 1, 128 * i:128 * (i + 1)], (8, 128))
                    ie, io = get_inv(h0 - 2), get_inv(h0 - 1)
                    o = jnp.concatenate([row(0, 0) * ie, jnp.where(lo64, row(1, 0) * ie, row(1, 1) * io),
                                         row(2, 1) * io], axis=1)
                else:
                    o = o_pair(edge(ones32), accp_buf[1 - slot(u)], get_inv(h0 - 2), get_inv(h0 - 1))
                gate(td + LATP + 10, o[:, 256:384])
                op_buf[...] = _pack(o, o)

            def job_g(c):
                def fn(td):
                    xo = out_cols(edge(op_buf[...]), 24 * (j - 1), 24, c)
                    xacc_buf[:, 128 * c:128 * (c + 1)] += xo
                    gate(td + LATP, xo)
                return fn

            def job_a(c):
                def fn(td):
                    jn = j + 2 if isinstance(j, int) else jnp.minimum(j + 2, NP - 1)
                    qc = q_cols(edge(z_buf[...]), jn, c)
                    gate(td + LATP, qc)
                    qraw_buf[c] = qc
                return fn

            def job_x(par, t, tiles, key):
                def fn(td):
                    p = (p_buf0, p_buf1)[par][0, 8 * t:8 * t + 8, :]
                    rhs = jnp.concatenate([v_tile(h0 + par, a, t) for a in tiles], axis=0)
                    o = _dot_t(edge(_pack(p, p)), rhs)
                    env[key] = o if key not in env else env[key] + o
                    gate(td + LATP, env[key][:, 0:128] if len(tiles) >= 8 else
                         jnp.concatenate([env[key], env[key]], axis=1))
                return fn

            def job_xp(t):
                def fn(td):
                    assert j > 0
                    lhs = _pack(p_buf0[0, 8 * t:8 * t + 8, :], p_buf1[0, 8 * t:8 * t + 8, :])
                    rhs = jnp.concatenate([v_tile(h0 + par, a, t) for par in range(2)
                                           for a in range(DH // 16)], axis=0)
                    o = _dot_t(edge(lhs), rhs)
                    env['xp'] = o if 'xp' not in env else env['xp'] + o
                    gate(td + LATP + 20, env['xp'][:, 256:384])
                    if t == xm(j) - 1:
                        xo_buf[0] = env['xp']
                return fn

            def finish(par, a0, a1, key, lhs_edge):
                r0 = par * (DH // 2)
                o = _dot_t(lhs_edge(ones32), accp_buf[slot(u), r0 + 8 * a0:r0 + 8 * a1, :])
                if key in env:
                    o = o + env[key]
                inv = get_inv(h0 + par)
                n = 16 * (a1 - a0)
                return o * (inv[:, 0:n] if n <= 128 else jnp.concatenate([inv, inv[:, 0:n - 128]], axis=1))

            env['finish'] = finish

            def job_fin(par, a0, a1, key):
                def fn(td):
                    o = finish(par, a0, a1, key, edge)
                    gate(td + LATP + 10, o[:, 0:128])
                    env['op' + key] = _pack(o, o)
                return fn

            def job_gfin(par, a0, a1, key, c):
                def fn(td):
                    xo = out_cols(edge(env['op' + key]), 12 * (h0 + par) + a0, a1 - a0, c)
                    xacc_buf[:, 128 * c:128 * (c + 1)] += xo
                    gate(td + LATP, xo)
                return fn

            jobs = []
            for g in range(0 if first else CA, ng):
                for c in range(4):
                    tail = 'sm1' if (c == 3 and g == ng - 1) else None
                    jobs.append((24, None, job_b(h0 + 1, 1, c, g, 's1', tail), 3))
            t_pair = t_step[inf['s0']] + EDEL if u > 0 else None
            groups = {
                'e': [] if first else [(EC, t_pair, job_e, 3)],
                'b': [(24, None, job_b(h0 + 2, 0, c, g, 's2',
                                       'sm2' if (c == 3 and g == ng - 1) else None), 3)
                      for g in range(ng) for c in range(4)],
                'a': [] if isinstance(j, int) and j + 2 >= NP else
                     [(40, None, job_a(c), 5) for c in range(3)],
                'x': [(EC, t_step[inf['s_odd'] + 1], job_xp(t), 3) for t in range(xm(j))],
                'g': [] if first else [(24, None, job_g(c), 3) for c in range(5)],
                'n': [(24, None, job_b(h0 + 3, 1, c, g, 's3', None), 3)
                      for g in range(CA) for c in range(4)],
            }
            if last:
                t_odd = t_step[inf['s_odd'] + 1]
                t_tail = t_step[inf['s_tail'] + 1]
                al, ah = list(range(8)), list(range(8, 12))
                jobs += groups['e'] + [(24, None, job_x(0, t, al + ah, 'x0'), 2) for t in range(XE)]
                jobs += groups['g']
                jobs += [(32, t_odd, job_fin(0, 0, 12, 'x0'), 2)]
                jobs += [(16, None, job_x(1, t, al, 'x1a'), 1) for t in range(XO)]
                jobs += [(12, t_odd + LATP + 60, job_gfin(0, 0, 12, 'x0', c), 2) for c in range(5)]
                jobs += [(8, None, job_x(1, t, ah, 'x1b'), 1) for t in range(XB1)]
                jobs += [(16, t_tail, job_fin(1, 0, 8, 'x1a'), 1)]
                jobs += [(8, None, job_x(1, t, ah, 'x1b'), 1) for t in range(XB1, XB)]
            else:
                for ch in ORD:
                    jobs += groups[ch]
            return jobs

        pjobs = [pair_jobs(u) for u in range(len(kinds))]
        jobs = [job for pj in pjobs for job in pj]
        times = []
        tt = T0F if kinds[0] == 'first' else T0
        for u, pj in enumerate(pjobs):
            rho = RHO if 0 < u < len(kinds) - 1 else (RHO0 if u == 0 else RHOL)
            if RF and 0 < u < len(kinds) - 1:
                dur = t_step[info[u]['s_end']] - t_step[info[u]['s0']]
                rho = max(1.0, RF * dur / sum(job[0] for job in pj))
            if u > 0 and LEAD is not None:
                tt = max(tt, t_step[info[u]['s0']] - LEAD)
            for (cost, earliest, _, _) in pj:
                tt += cost * rho
                if earliest is not None:
                    tt = max(tt, earliest)
                times.append(tt)

        states = {}
        nj = 0
        for st, (u, par, tl, t, ts) in enumerate(steps):
            while nj < len(jobs) and times[nj] + EOFF <= t_step[st]:
                if times[nj] > 0 and 'j0' not in cur:
                    cur['j0'] = nj
                rel = nj - cur.get('j0', nj + 1)
                cur['edge'] = (0 <= rel < NE and rel % EE == EE - 1) or jobs[nj][1] == times[nj]
                jobs[nj][2](times[nj])
                nj += 1
            for (pv_, g_, rs_, po_) in stores.pop(st, ()):
                pv_ = pltpu.bitcast(edge(pltpu.bitcast(pv_, U32), SE, True), F32)
                if po_ is None:
                    l_buf[g_ & 3] = pv_
                else:
                    store_p(pv_, g_, rs_, po_)
            state = states.setdefault((u, par), dict(accs=[None] * 24, half=par, slot=slot(u)))
            pv_step(2 * (j0 + u) + par, tl, t, ts, (p_buf0, p_buf1)[par],
                    gates.get(st, ()), true_mask, state)
            cur['state'] = state
            cur['st'] = st
        cur['edge'] = False
        while nj < len(jobs):
            jobs[nj][2](times[nj])
            nj += 1
        assert not stores
        env = envs[-1]
        if kinds[-1] == 'last':
            o = env['finish'](1, 8, 12, 'x1b', lambda x: x)
            op = _pack(o, o)
            xa = [out_cols(env['opx1a'], 12 * (H - 1), 8, c) for c in range(5)]
            xb = [out_cols(op, 12 * (H - 1) + 8, 4, c) for c in range(5)]
            return (xacc_buf[...] + jnp.concatenate(xa, axis=1)) + jnp.concatenate(xb, axis=1), shift2
        return carry

    set_row(x2, shift2)
    xacc_buf[...] = x2
    z = z_buf[...]
    qx = [_dot(z, _bf(wx_buf[i].reshape(D // 2, 128))) * st_buf[0] - csq_buf[3 * NP + i] * st_buf[1]
          for i in range(3)]
    w0 = [_pack(jnp.where(evn, q_, zf), jnp.where(evn, zf, q_)) for q_ in qx]
    store_q([None, q_cols(z, 0, 1), q_cols(z, 0, 2)], 0, pars=(1,))
    sg = [None] * ng
    for g in range(ng):
        for c in range(4):
            lhs = jnp.concatenate([jnp.where(sub == c, w_, jnp.zeros_like(w_)) for w_ in w0], axis=1)
            s = score2(lhs, 0, 0, 4 * g + c)
            sg[g] = s if c == 0 else sg[g] + s
    q_pair(1)
    ps0, l0, c0 = softmax_lane(sg)
    for g in range(ng):
        store_p(ps0[g], g, range(8), p_buf0)
    l_buf[0] = l0
    if ALL:
        x3, shift3 = block(0, 0, ['first'] + ['mid'] * (NP - 2) + ['last'])
    else:
        carry = block(0, 0, ['first'] + ['mid'] * NF)
        n_mid = (NP - 2 - NF - NL) // U
        if n_mid:
            carry = lax.fori_loop(0, n_mid * REP, lambda i, c: block(1 + NF + U * (i if REP == 1 else lax.rem(i, n_mid)), c, ['mid'] * U, (1 + NF) & 1 if U % 2 == 0 and not DYN else None), carry)
        x3, shift3 = block(NP - 1 - NL, carry, ['mid'] * NL + ['last'])
    x4 = x3 + b2 + _dot(mlp_hidden(x3, shift3), w2_buf[...])
    o_ref[...] = x4[0:1, :].astype(o_ref.dtype)


@jax.jit
def pallas_interleave_layers__sliding_block_cached__dense_activation_gelu__decode_kernel(
    A_x: jax.Array,
    A_k_cache: jax.Array,
    A_v_cache: jax.Array,
    A_wq: jax.Array,
    A_wo: jax.Array,
    B_x: jax.Array,
    B_w1: jax.Array,
    B_b1: jax.Array,
    B_w2: jax.Array,
    B_b2: jax.Array,
):
    sk = A_k_cache.shape[2]
    w = min(4096, max(256, sk // 4))

    def tile_view(a):
        *lead, r, c = a.shape
        n = len(lead)
        a = a.reshape(*lead, r // 8, 8, c // 128, 128)
        a = a.transpose(*range(n), n, n + 2, n + 1, n + 3)
        return a.reshape(*lead, r // 16, 2, (c // 128) * 8, 128)

    kx = tile_view(jnp.swapaxes(A_k_cache, 2, 3)[0]).reshape(H * DH // 8, sk // 16, 128)
    vx = tile_view(jnp.swapaxes(A_v_cache, 2, 3)[0]).reshape(H * DH // 8, sk // 16, 128)
    wqx = tile_view(A_wq)
    wox = tile_view(A_wo).reshape(H * DH // 16, 80, 128)
    any_spec = pl.BlockSpec(memory_space=pl.ANY)
    out = pl.pallas_call(
        functools.partial(_kernel, sk=sk, w=w),
        out_shape=jax.ShapeDtypeStruct((1, D), A_x.dtype),
        in_specs=[any_spec] * 9,
        out_specs=pl.BlockSpec(memory_space=pltpu.VMEM),
        scratch_shapes=[
            pltpu.VMEM((H * DH // 8, w // 32, 128), U32),
            pltpu.VMEM((H * DH // 8, w // 32 - 4 * XF, 128), U32),
            pltpu.VMEM((H * DH // 8, max(8 * XF, 8), 128), U32),
            pltpu.VMEM((D // 16, 2, H * DH // 32, 128), U32),
            pltpu.VMEM((H * DH // 16, 40, 128), U32),
            pltpu.VMEM((D, F), BF16),
            pltpu.VMEM((F, D), BF16),
            pltpu.VMEM((1, D), BF16),
            pltpu.VMEM((F // 128, 128), BF16),
            pltpu.VMEM((D // 128, 128), BF16),
            pltpu.VMEM((1, w // 16, 128), F32),
            pltpu.VMEM((1, w // 16, 128), F32),
            pltpu.VMEM((w // 1024, 8, 128), F32),
            pltpu.VMEM((2, DH, 128), U32),
            pltpu.VMEM((8, D), U32),
            pltpu.VMEM((8, D), F32),
            pltpu.VMEM((4, 4, 8, 2 * DH), U32),
            pltpu.VMEM((3, 8, 128), F32),
            pltpu.VMEM((3 * NP + 3, 8, 128), F32),
            pltpu.VMEM((8, F), F32),
            pltpu.VMEM((2, 8, 128), F32),
            pltpu.VMEM((3, 8, 128), jnp.int32),
            pltpu.SMEM((NS,), jnp.int32),
            pltpu.VMEM((w // 1024, 8, 128), F32),
            pltpu.VMEM((8, 2 * DH), U32),
            pltpu.VMEM((4, 8, 128), F32),
            pltpu.VMEM((3, D // 16, 8, 128), U32),
            pltpu.VMEM((8, 128), U32),
            pltpu.VMEM((1, 8, 2 * DH), F32),
            pltpu.SemaphoreType.DMA((2,)),
            pltpu.SemaphoreType.DMA((4,)),
            pltpu.SemaphoreType.DMA((6 + W2C,)),
        ],
        compiler_params=pltpu.CompilerParams(vmem_limit_bytes=int(OPT.get('VM', 127)) * 1024 * 1024,
                                             disable_semaphore_checks=bool(DSC), disable_bounds_checks=bool(DBC)),
    )(A_x.reshape(1, D), kx, vx, wqx, wox, B_w1, B_b1.reshape(F // 128, 128),
      B_w2, B_b2.reshape(D // 128, 128))
    return out.reshape(A_x.shape)
```

```python
import functools
import math

import jax
import jax.numpy as jnp
from jax import lax
import jax.experimental.pallas as pl
import jax.experimental.pallas.tpu as pltpu

F32 = jnp.float32
BF16 = jnp.bfloat16
U32 = jnp.uint32

D = 640
H = 32
DH = 192
F = 1536
EPS = 1e-5
NP = H // 2
OPT = {}
NS = int(OPT.get('NS', 4))
CA = int(OPT.get('CA', 2))
CU = float(OPT.get('CU', 0.26))
XF = int(OPT.get('XF', 6))
CHUNKS = [int(c) for c in OPT.get('CHUNKS', '44322 1').replace(' ', '')]
LATP = float(OPT.get('LATP', 160))
T0 = float(OPT.get('T0', -10))
T0F = float(OPT.get('T0F', -100))
RHO = float(OPT.get('RHO', 1.02))
BE = int(OPT.get('BE', 6))
MOFF = float(OPT.get('MOFF', 160))
MOFF2 = float(OPT.get('MOFF2', 240))
EC = float(OPT.get('EC', 48))
SG = int(OPT.get('SG', 4))
SDT = float(OPT.get('SDT', 12))
CHAIN = int(OPT.get('CHAIN', 0))
XE = int(OPT.get('XE', 7))
XO = int(OPT.get('XO', 7))
W2R = [128 * int(c) for c in OPT.get('W2R', '5421')]
W2C = len(W2R)
W2S = [sum(W2R[:i]) for i in range(W2C)]
ORD = OPT.get('ORD', 'ebxagn')
OPQ = int(OPT.get('OPQ', 0))
LA = int(OPT.get('LA', 1))
NE = int(OPT.get('NE', 7))
EE = int(OPT.get('EE', 2))
SE = int(OPT.get('SE', 1))
EOFF = float(OPT.get('EOFF', 0))
SM = int(OPT.get('SM', 1))
OM = int(OPT.get('OM', 1))
U = int(OPT.get('U', 2))
NF = int(OPT.get('NF', 0))
NL = int(OPT.get('NL', 0))
EDEL = float(OPT.get('EDEL', 70))
RHO0 = float(OPT.get('RHO0', 1.0))
RHOL = float(OPT.get('RHOL', 1.0))
BAR = int(OPT.get('BAR', 0))
IOFF = float(OPT.get('IOFF', 0))
DYN = int(OPT.get('DYN', 0))
MST = int(OPT.get('MST', 1))
DSC = int(OPT.get('DSC', 1))
DBC = int(OPT.get('DBC', 0))
REP = int(OPT.get('REP', 1))
PB = int(OPT.get('PB', 0))
ALL = int(OPT.get('ALL', 1))
LEAD = float(OPT.get('LEAD', 100))
OPQ2 = int(OPT.get('OPQ2', 1))
XB = int(OPT.get('XB', 16))
XB1 = int(OPT.get('XB1', 6))
NGT = int(OPT.get('NGT', 12))
MOFL = float(OPT.get('MOFL', 60))
XM = int(OPT.get('XM', 1))
XMP = int(OPT.get('XMP', 2))
RF = float(OPT.get('RF', 0))
SKIP2 = int(OPT.get('SKIP2', 0))
SKIP1 = int(OPT.get('SKIP1', 0))


def _gelu(x):
    c = math.sqrt(2.0 / math.pi)
    return 0.5 * x * (1.0 + jnp.tanh(c * (x + 0.044715 * (x * x * x))))


def _rows_to_lanes(b, n):
    return jnp.concatenate([b[i:i + 1, :] for i in range(n)], axis=1)


def _bf(x):
    return pltpu.bitcast(x, BF16)


def _pack(a, b):
    return pltpu.bitcast(pltpu.pack_elementwise([a, b], packed_dtype=BF16), U32)


def _unpack(x):
    return (pltpu.unpack_elementwise(x, index=0, packed_dtype=BF16, unpacked_dtype=F32),
            pltpu.unpack_elementwise(x, index=1, packed_dtype=BF16, unpacked_dtype=F32))


def _dot(lhs32, rhs):
    return jnp.dot(_bf(lhs32), rhs, preferred_element_type=F32)[0:8]


def _dot_t(lhs32, rhs32):
    return lax.dot_general(_bf(lhs32), _bf(rhs32), (((1,), (1,)), ((), ())),
                           preferred_element_type=F32)[0:8]


def _ln_stats(xp, shift):
    x = _unpack(xp)[0] - shift
    m = jnp.mean(x, axis=-1, keepdims=True)
    v = jnp.maximum(jnp.mean(x * x, axis=-1, keepdims=True) - m * m, 0.0)
    return m + shift, lax.rsqrt(v + EPS)


def _mean(x):
    return jnp.mean(x, axis=-1, keepdims=True)


def _kernel(x_hbm, kx_hbm, vx_hbm, wq_hbm, wo_hbm, w1_hbm, b1_hbm, w2_hbm, b2_hbm,
            o_ref,
            kbuf, vbuf, vf_buf, wq_buf, wo_buf, w1_buf, w2_buf, x_buf, b1_buf, b2_buf,
            p_buf0, p_buf1, sp_buf, accp_buf, z_buf, xacc_buf, qv_buf, qraw_buf,
            csq_buf, cs1_buf, st_buf, tm_buf, zs_ref, s2_buf, op_buf, l_buf, wx_buf, lhs0_buf, xo_buf,
            sem_k, sem_v, sem_w, *, sk, w):
    c_scale = (DH ** -0.5) * math.log2(math.e)
    nt = w // 128
    ng = nt // 8
    na = 12 // NS
    nst = NS * nt
    r0w = (sk - w) // 16
    nrw = w // 16

    ntb = nt - XF
    starts = [sum(CHUNKS[:c]) for c in range(len(CHUNKS))]
    assert sum(CHUNKS) == NP

    def k_copy(c):
        rows = pl.ds(24 * starts[c], 24 * CHUNKS[c])
        return [pltpu.make_async_copy(kx_hbm.at[rows, :, pl.ds(r0w, nrw), :],
                                      kbuf.bitcast(BF16).at[rows], sem_k.at[c & 1])]

    def v_copy(c):
        rows = pl.ds(24 * starts[c], 24 * CHUNKS[c])
        cps = [pltpu.make_async_copy(vx_hbm.at[rows, :, pl.ds(r0w, 8 * ntb), :],
                                     vbuf.bitcast(BF16).at[rows], sem_v.at[c & 1])]
        if XF:
            cps.append(pltpu.make_async_copy(
                vx_hbm.at[rows, :, pl.ds(r0w + 8 * ntb, 8 * XF), :],
                vf_buf.bitcast(BF16).at[rows, :, pl.ds(8 * XF, 8 * XF), :], sem_v.at[2 + (c & 1)]))
        return cps

    wq_cp = pltpu.make_async_copy(wq_hbm, wq_buf.bitcast(BF16), sem_w.at[0])
    wo_cp = pltpu.make_async_copy(wo_hbm, wo_buf.bitcast(BF16), sem_w.at[1])
    w1_cp = pltpu.make_async_copy(w1_hbm, w1_buf, sem_w.at[2])
    x_cp = pltpu.make_async_copy(x_hbm, x_buf, sem_w.at[3])
    b1_cp = pltpu.make_async_copy(b1_hbm, b1_buf, sem_w.at[4])
    b2_cp = pltpu.make_async_copy(b2_hbm, b2_buf, sem_w.at[5])
    w2_cps = [pltpu.make_async_copy(w2_hbm.at[pl.ds(W2S[i], W2R[i]), :],
                                    w2_buf.at[pl.ds(W2S[i], W2R[i]), :], sem_w.at[6 + i])
              for i in range(W2C)]

    if not SKIP1:
        wq_cp.start()
    x_cp.start()
    b1_cp.start()
    b2_cp.start()
    if not SKIP1:
        wo_cp.start()
        for cp in k_copy(0) + v_copy(0):
            cp.start()
    x_cp.wait()
    b1_cp.wait()
    b2_cp.wait()

    x0 = jnp.broadcast_to(x_buf[...].astype(F32), (8, D))
    b1 = _rows_to_lanes(b1_buf[...].astype(F32), F // 128)
    b2 = _rows_to_lanes(b2_buf[...].astype(F32), D // 128)

    lane = lax.broadcasted_iota(jnp.int32, (8, 128), 1)
    sub_lo = lax.broadcasted_iota(jnp.int32, (1, 8, 128), 1) < 4
    lo64 = lane < 64
    sub = lax.broadcasted_iota(jnp.int32, (8, 128), 0)
    evn = (lane & 8) == 0
    zf = jnp.zeros((8, 128), F32)
    ones32 = jnp.full((8, 128), 0x3F803F80, U32)
    k_order = (((0, 8, 0), (0, 8, 1), (8, 4, 0), (8, 4, 1)),
               ((4, 8, 0), (4, 8, 1), (0, 4, 1), (0, 4, 0)))

    def swap_halves(ref2):
        n = ref2.shape[1]
        a = ref2[0].reshape(n // 8, 8, 128)
        b = ref2[1].reshape(n // 8, 8, 128)
        ref2[0] = jnp.where(sub_lo, a, pltpu.roll(b, 4, 1)).reshape(n, 128)
        ref2[1] = jnp.where(sub_lo, pltpu.roll(a, 4, 1), b).reshape(n, 128)

    def fix_wq(a, carry):
        swap_halves(wq_buf.at[a])
        return carry

    def fix_wo(g8, carry):
        g0 = pl.multiple_of(g8 * 8, 8)
        v = [wo_buf[pl.ds(g0, 8), 8 * c:8 * c + 8, :] for c in range(5)]
        n = [jnp.where(sub_lo, v[0], v[2]),
             pltpu.roll(jnp.where(sub_lo, v[3], v[0]), 4, 1),
             jnp.where(sub_lo, v[1], v[3]),
             pltpu.roll(jnp.where(sub_lo, v[4], v[1]), 4, 1),
             jnp.where(sub_lo, v[2], v[4])]
        for c in range(5):
            wo_buf[pl.ds(g0, 8), 8 * c:8 * c + 8, :] = n[c]
        return carry

    def set_row(x, shift):
        xp = _pack(x, x)
        z_buf[...] = xp
        m, r = _ln_stats(xp, shift)
        rc = r * c_scale
        st_buf[0] = jnp.broadcast_to(rc, (8, 128))
        st_buf[1] = jnp.broadcast_to(m * rc, (8, 128))

    def wq_cols(ct):
        r0 = pl.multiple_of(lax.shift_right_logical(ct, 1) * 8, 8) if not isinstance(ct, int) else (ct // 2) * 8
        return _bf(wq_buf[:, ct & 1, pl.ds(r0, 8), :].reshape(D // 2, 128))

    def q_cols(z, j, c):
        ct = 3 * j + c
        return _dot(z, wq_cols(ct)) * st_buf[0] - csq_buf[ct] * st_buf[1]

    def store_lhs(hh, ww):
        for c in range(4):
            for i in range(3):
                pltpu.store(qv_buf.at[hh & 3, c, :, 128 * i:128 * (i + 1)], ww[i], mask=sub == c)

    def store_q(qs, j, pars=(0, 1)):
        q0, q1, q2 = qs
        r56, r64, r8 = (pltpu.roll(q1, s, 1) for s in (56, 64, 8))

        def lhs(qf, a2, b2):
            a0 = jnp.where(evn, qf, zf)
            b1_ = jnp.where(evn, zf, qf)
            return [_pack(a0, pltpu.roll(a0, 8, 1)), _pack(pltpu.roll(b1_, 120, 1), b1_),
                    _pack(jnp.where(evn, a2, zf), jnp.where(evn, zf, b2))]

        if 0 in pars:
            store_lhs(2 * j, lhs(q0, jnp.where(lo64, q1, r56), jnp.where(lo64, r8, r64)))
        if 1 in pars:
            store_lhs(2 * j + 1, lhs(q2, jnp.where(lo64, r56, q1), jnp.where(lo64, r64, r8)))

    def q_pair(j):
        z = z_buf[...]
        store_q([q_cols(z, j, c) for c in range(3)], j)

    def score2(lhs, h, par, k):
        rhs = jnp.concatenate([kbuf[pl.ds(12 * h + a, n), e, 8 * k:8 * k + 8, :]
                               for a, n, e in k_order[par]], axis=0)
        return _dot(lhs, _bf(rhs.reshape(DH, 128)))

    def scores_all(h, par):
        sg = [None] * ng
        for c in range(4):
            lhs = qv_buf[h & 3, c]
            for g in range(ng):
                s = score2(lhs, h, par, 4 * g + c)
                sg[g] = s if sg[g] is None else sg[g] + s
        return sg

    def store_p(p, g, rs, p_out):
        for r in rs:
            if PB:
                p_out[0, 64 * g + 8 * r:64 * g + 8 * r + 8, :] = jnp.broadcast_to(p[r:r + 1, :], (8, 128))
            else:
                p_out[0, pl.ds(64 * g + r, 8, stride=8), :] = p

    def inv_sum(l):
        l = jnp.sum(jnp.sum(l, axis=1, keepdims=True), axis=0, keepdims=True)
        return jnp.broadcast_to(1.0 / l, (8, 128))

    def softmax(sg, p_out):
        mx = sg[0]
        for s in sg[1:]:
            mx = jnp.maximum(mx, s)
        m = jnp.max(jnp.max(mx, axis=1, keepdims=True), axis=0, keepdims=True)
        l = None
        ps = []
        for g in range(ng):
            p = jnp.exp2(sg[g] - m)
            ps.append(p)
            if p_out is not None:
                store_p(p, g, range(8), p_out)
            l = p if l is None else l + p
        if p_out is None:
            return ps, l
        return ps, inv_sum(l)

    def softmax_lane(sg):
        mx = jnp.maximum(jnp.maximum(sg[0], sg[1]), jnp.maximum(sg[2], sg[3]))
        m = jnp.broadcast_to(jnp.max(mx, axis=0, keepdims=True), (8, 128))
        ps = [jnp.exp2(s - m) for s in sg]
        c = jnp.exp2(m - jnp.max(m, axis=1, keepdims=True))
        c = _unpack(_pack(c, c))[0]
        return ps, ((ps[0] + ps[1]) + (ps[2] + ps[3])) * c, c

    def v_tiles(h, a0, n, t):
        return vbuf[pl.ds(12 * h + a0, n), t % 2, 8 * (t // 2):8 * (t // 2) + 8, :]

    def pv_step(h, tiles, t, ts, p_in, gvals, true_mask, state):
        a0, n = tiles
        p = p_in[0, 8 * t:8 * t + 8, :]
        for i, gval in enumerate(gvals):
            p = jnp.where(true_mask[i], p, gval)
        if t < ntb:
            ys = _unpack(v_tiles(h, a0, n, t))
        else:
            r = 8 * (t - ntb)
            ys = [pltpu.bitcast(vf_buf[pl.ds(12 * h + a0, n), e, r:r + 8, :], F32) for e in range(2)]
        if t == ts[0]:
            state['accs'] = [y * p for y in ys]
        else:
            state['accs'] = [acc + y * p for acc, y in zip(state['accs'], ys)]
        if t == ts[-1]:
            r0 = state['half'] * (DH // 2) + 8 * a0
            accp_buf[state['slot'], r0:r0 + 8 * n, :] = _pack(*state['accs']).reshape(8 * n, 128)

    def o_pair(ones, accp, ie, io):
        inv = jnp.concatenate([ie, jnp.where(lo64, ie, io), io], axis=1)
        return _dot_t(ones, accp) * inv

    def out_cols(op, g0, ngrp, c):
        rhs = wo_buf[pl.ds(g0, ngrp), 8 * c:8 * c + 8, :].reshape(ngrp * 8, 128)
        return _dot(op, _bf(rhs))

    def mlp_hidden(x, shift):
        xp = _pack(x, x)
        m, r = _ln_stats(xp, shift)
        hh = (_dot(xp, w1_buf[...]) - cs1_buf[...] * m) * r + b1
        g = _gelu(hh)
        return _pack(g, g)

    def fix_v(r2, carry):
        swap_halves(vbuf.at[r2])
        if XF:
            n = 4 * XF
            a = vf_buf[r2, 0, n:2 * n, :].reshape(n // 8, 8, 128)
            b = vf_buf[r2, 1, n:2 * n, :].reshape(n // 8, 8, 128)
            t0 = _unpack(jnp.where(sub_lo, a, pltpu.roll(b, 4, 1)))
            t1 = _unpack(jnp.where(sub_lo, pltpu.roll(a, 4, 1), b))
            for e in range(2):
                for k in range(XF // 2):
                    vf_buf[r2, e, 16 * k:16 * k + 8, :] = pltpu.bitcast(t0[e][k], U32)
                    vf_buf[r2, e, 16 * k + 8:16 * k + 16, :] = pltpu.bitcast(t1[e][k], U32)
        return carry

    def next_copies(j, copy_fn, tail_cps):
        for c in range(len(CHUNKS)):
            @pl.when(j == starts[c])
            def _():
                for cp in copy_fn(c):
                    cp.wait()
                for cp in (copy_fn(c + 1) if c + 1 < len(CHUNKS) else tail_cps):
                    cp.start()

    def pair1(j, carry):
        q_pair(j)
        next_copies(j, k_copy, [w1_cp])
        invs = []
        for par in range(2):
            _, inv = softmax(scores_all(2 * j + par, par), (p_buf0, p_buf1)[par])
            invs.append(inv)
        next_copies(j, v_copy, w2_cps)
        lax.fori_loop(24 * j, 24 * (j + 1), fix_v, 0)
        for par in range(2):
            state = dict(half=par, slot=0)
            for sw in range(NS):
                for t in range(nt):
                    pv_step(2 * j + par, (sw * na, na), t, range(nt),
                            (p_buf0, p_buf1)[par], (), None, state)
        o = o_pair(ones32, accp_buf[0], invs[0], invs[1])
        op = _pack(o, o)
        for c in range(5):
            xacc_buf[:, 128 * c:128 * (c + 1)] += out_cols(op, 24 * j, 24, c)
        return carry

    def expand(t0, t1):
        return [jnp.where(evn, t0, pltpu.roll(t0, 8, 1)),
                jnp.where(evn, pltpu.roll(t0, 120, 1), t0),
                jnp.where(evn, jnp.where(lo64, t1, pltpu.roll(t1, 56, 1)),
                          jnp.where(lo64, pltpu.roll(t1, 8, 1), pltpu.roll(t1, 64, 1)))]

    def expand_wq(a, carry):
        e = expand(wq_buf[a, 0, 0:8, :], wq_buf[a, 1, 0:8, :])
        for i in range(3):
            wx_buf[i, a] = e[i]
        return carry

    def colsum_q(ct, carry):
        ones = jnp.concatenate([ones32] * (D // 128), axis=1)
        csq_buf[ct] = _dot(ones, wq_cols(ct))
        return carry

    qv_buf[...] = jnp.zeros(qv_buf.shape, U32)
    for i in range(3):
        tm_buf[i] = lane
    for sw in range(NS):
        zs_ref[sw] = 0
    if not SKIP1:
        set_row(x0, _mean(x0))
        xacc_buf[...] = x0
        wq_cp.wait()
        lax.fori_loop(0, D // 16, fix_wq, 0)
        lax.fori_loop(0, 3 * NP, colsum_q, 0)
        lax.fori_loop(0, D // 16, expand_wq, 0)
        e = expand(csq_buf[0], csq_buf[1])
        for i in range(3):
            csq_buf[3 * NP + i] = e[i]
        wo_cp.wait()
        lax.fori_loop(0, H * DH // 128, fix_wo, 0)
        lax.fori_loop(0, NP, pair1, 0)
        x1 = xacc_buf[...]
        w1_cp.wait()
        cs1_buf[...] = _dot(jnp.concatenate([ones32] * (D // 128), axis=1), w1_buf[...])
        gp = mlp_hidden(x1, _mean(x1))
        x2 = x1 + b2
        for i in range(W2C):
            if i == W2C - 1:
                shift2 = _mean(x2)
            w2_cps[i].wait()
            x2 = x2 + _dot(gp[:, W2S[i]:W2S[i] + W2R[i]], w2_buf[W2S[i]:W2S[i] + W2R[i], :])
    else:
        x2 = lax.fori_loop(0, 2, lambda i, x: x + 1.0, x0)
        shift2 = _mean(x0)

    if SKIP2:
        o_ref[...] = x2[0:1, :].astype(o_ref.dtype)
        return

    def block(j0, carry, kinds, jpar=None):
        true_mask = [tm_buf[i] >= 0 for i in range(3)]
        zs = [0] + [zs_ref[sw] if OPQ else 0 for sw in range(1, NS)]
        steps = []
        info = []
        def xm(j):
            return XM if (j % XMP == XMP - 1 and 0 < j < NP - 1) else 0

        std = [(sw * na, na) for sw in range(NS)]
        for u, kind in enumerate(kinds):
            if kind == 'last':
                sweeps = [[(tl, list(range(XE, nt))) for tl in std],
                          [((5, 3), list(range(XO, nt))), ((2, 3), list(range(XO, nt))),
                           ((0, 2), list(range(XO, nt))), ((8, 4), list(range(XB, nt)))]]
            else:
                sweeps = [[(tl, list(range(xm(j0 + u), nt))) for tl in std]] * 2
            s0 = len(steps)
            steps += [(u, 0, tl, t, ts) for tl, ts in sweeps[0] for t in ts]
            s_odd = len(steps)
            steps += [(u, 1, tl, t, ts) for tl, ts in sweeps[1] for t in ts]
            info.append(dict(s0=s0, s_odd=s_odd, s_end=len(steps),
                             s_tail=len(steps) - len(sweeps[1][-1][1])))
        t_step = [0.0]
        for (_, _, tl, t, _) in steps:
            t_step.append(t_step[-1] + CU * tl[1] * (6 if t < ntb else 4))
        gates, stores = {}, {}
        cur = dict(state=None, st=-1, nedge=0)
        envs = [dict(s1=[None] * ng, s2=[None] * ng, s3=[None] * ng) for _ in kinds]

        zq = zs_ref[0] if OPQ2 else 0

        def get_inv(h):
            return inv_sum(l_buf[zq + (h & 3)])

        def slot(u):
            return (j0 + u) & 1 if jpar is None else (jpar + u) & 1

        def step_at(cyc):
            return next((i for i, tt_ in enumerate(t_step) if tt_ >= cyc), len(t_step))

        def gate(cyc, v):
            st = step_at(cyc)
            while len(gates.get(st, ())) >= 2:
                st += 1
            if st < len(steps) - NGT and st > cur['st']:
                gates.setdefault(st, []).append(v)

        def edge(x, n=BE, force=False):
            if cur['st'] < 0 or not (force or cur['edge']):
                return x
            accs = cur['state']['accs']
            cand = [(e, a) for e in range(2) for a in range(accs[0].shape[0])]
            ntile = -(-x.shape[1] // 128)
            parts = [x[:, 128 * i:min(128 * (i + 1), x.shape[1])] for i in range(ntile)]
            for e in range(min(n, 3 * ntile)):
                ce, ca = cand[cur['nedge'] % len(cand)]
                cur['nedge'] += 1
                i = e % ntile
                w_ = parts[i].shape[1]
                parts[i] = jnp.where(true_mask[e // ntile][:, 0:w_], parts[i],
                                     pltpu.bitcast(accs[ce][ca], U32)[:, 0:w_])
            return parts[0] if ntile == 1 else jnp.concatenate(parts, axis=1)

        def sched_stores(ps, lsum, h, p_out, t_ready, lo, hi, l_off=10):
            gate(t_ready, ps[-1])
            st_l = min(max(step_at(t_ready + l_off), cur['st'] + 1), len(steps) - 1)
            stores.setdefault(st_l, []).append((lsum, h, None, None))
            n = 8 // SG
            t_first = max(t_ready, t_step[lo])
            for i in range(ng * n):
                g, k = divmod(i, n)
                st = min(max(step_at(t_first + SDT * i) + 1, cur['st'] + 1), hi)
                stores.setdefault(st, []).append((ps[g], g, range(SG * k, SG * (k + 1)), p_out))

        def pair_jobs(u):
            kind, env, inf = kinds[u], envs[u], info[u]
            first, last = kind == 'first', kind == 'last'
            j = j0 + u
            h0 = 2 * j

            def job_b(h, par, c, g, key, tail):
                def fn(td):
                    s = score2(edge(qv_buf[h & 3, c]), h, par, 4 * g + c)
                    sg = env[key]
                    sg[g] = s if c == 0 else sg[g] + s
                    gate(td + LATP, sg[g])
                    if c == 3:
                        (sp_buf if key != 's2' else s2_buf)[g] = sg[g]
                    if tail == 'sm1' and first:
                        ps, lsum, c1 = softmax_lane([sp_buf[zq + gg] for gg in range(ng)])
                        lhs0_buf[...] = _pack(c0, c1)
                        sched_stores(ps, lsum, h, p_buf1, td + LATP + MOFL, inf['s0'], inf['s_odd'], 130)
                    elif tail == 'sm1':
                        ps, lsum = softmax([sp_buf[zq + gg] for gg in range(ng)], None)
                        sched_stores(ps, lsum, h, p_buf1, td + LATP + MOFF, inf['s0'], inf['s_odd'])
                        if not first and not last:
                            store_q([qraw_buf[zq + i] for i in range(3)], j + 1)
                    elif tail == 'sm2':
                        ps, lsum = softmax([s2_buf[zq + gg] for gg in range(ng)], None)
                        sched_stores(ps, lsum, h, p_buf0, td + LATP + MOFF2, inf['s_odd'], inf['s_end'] - 1)
                return fn

            def job_e(td):
                if j == 1 or xm(j - 1):
                    x = _dot_t(edge(lhs0_buf[...] if j == 1 else ones32), accp_buf[1 - slot(u)])
                    if xm(j - 1):
                        x = x + xo_buf[zq]
                    row = lambda i, r: jnp.broadcast_to(x[r:r + 1, 128 * i:128 * (i + 1)], (8, 128))
                    ie, io = get_inv(h0 - 2), get_inv(h0 - 1)
                    o = jnp.concatenate([row(0, 0) * ie, jnp.where(lo64, row(1, 0) * ie, row(1, 1) * io),
                                         row(2, 1) * io], axis=1)
                else:
                    o = o_pair(edge(ones32), accp_buf[1 - slot(u)], get_inv(h0 - 2), get_inv(h0 - 1))
                gate(td + LATP + 10, o[:, 256:384])
                op_buf[...] = _pack(o, o)

            def job_g(c):
                def fn(td):
                    xo = out_cols(edge(op_buf[...]), 24 * (j - 1), 24, c)
                    xacc_buf[:, 128 * c:128 * (c + 1)] += xo
                    gate(td + LATP, xo)
                return fn

            def job_a(c):
                def fn(td):
                    jn = j + 2 if isinstance(j, int) else jnp.minimum(j + 2, NP - 1)
                    qc = q_cols(edge(z_buf[...]), jn, c)
                    gate(td + LATP, qc)
                    qraw_buf[c] = qc
                return fn

            def job_x(par, t, tiles, key):
                def fn(td):
                    p = (p_buf0, p_buf1)[par][0, 8 * t:8 * t + 8, :]
                    rhs = v_tiles(h0 + par, tiles[0], tiles[1], t).reshape(8 * tiles[1], 128)
                    o = _dot_t(edge(_pack(p, p)), rhs)
                    env[key] = o if key not in env else env[key] + o
                    gate(td + LATP, env[key][:, 0:128] if tiles[1] >= 8 else
                         jnp.concatenate([env[key], env[key]], axis=1))
                return fn

            def job_xp(t):
                def fn(td):
                    assert j > 0
                    lhs = _pack(p_buf0[0, 8 * t:8 * t + 8, :], p_buf1[0, 8 * t:8 * t + 8, :])
                    rhs = v_tiles(h0, 0, 24, t).reshape(DH, 128)
                    o = _dot_t(edge(lhs), rhs)
                    env['xp'] = o if 'xp' not in env else env['xp'] + o
                    gate(td + LATP + 20, env['xp'][:, 256:384])
                    if t == xm(j) - 1:
                        xo_buf[0] = env['xp']
                return fn

            def finish(par, a0, a1, key, lhs_edge):
                r0 = par * (DH // 2)
                o = _dot_t(lhs_edge(ones32), accp_buf[slot(u), r0 + 8 * a0:r0 + 8 * a1, :])
                if key in env:
                    o = o + env[key]
                inv = get_inv(h0 + par)
                n = 16 * (a1 - a0)
                return o * (inv[:, 0:n] if n <= 128 else jnp.concatenate([inv, inv[:, 0:n - 128]], axis=1))

            env['finish'] = finish

            def job_fin(par, a0, a1, key):
                def fn(td):
                    o = finish(par, a0, a1, key, edge)
                    gate(td + LATP + 10, o[:, 0:128])
                    env['op' + key] = _pack(o, o)
                return fn

            def job_gfin(par, a0, a1, key, c):
                def fn(td):
                    xo = out_cols(edge(env['op' + key]), 12 * (h0 + par) + a0, a1 - a0, c)
                    xacc_buf[:, 128 * c:128 * (c + 1)] += xo
                    gate(td + LATP, xo)
                return fn

            jobs = []
            for g in range(0 if first else CA, ng):
                for c in range(4):
                    tail = 'sm1' if (c == 3 and g == ng - 1) else None
                    jobs.append((24, None, job_b(h0 + 1, 1, c, g, 's1', tail), 3))
            t_pair = t_step[inf['s0']] + EDEL if u > 0 else None
            groups = {
                'e': [] if first else [(EC, t_pair, job_e, 3)],
                'b': [(24, None, job_b(h0 + 2, 0, c, g, 's2',
                                       'sm2' if (c == 3 and g == ng - 1) else None), 3)
                      for g in range(ng) for c in range(4)],
                'a': [] if isinstance(j, int) and j + 2 >= NP else
                     [(40, None, job_a(c), 5) for c in range(3)],
                'x': [(EC, t_step[inf['s_odd'] + 1], job_xp(t), 3) for t in range(xm(j))],
                'g': [] if first else [(24, None, job_g(c), 3) for c in range(5)],
                'n': [(24, None, job_b(h0 + 3, 1, c, g, 's3', None), 3)
                      for g in range(CA) for c in range(4)],
            }
            if last:
                t_odd = t_step[inf['s_odd'] + 1]
                t_tail = t_step[inf['s_tail'] + 1]
                al, ah = (0, 8), (8, 4)
                jobs += groups['e'] + [(24, None, job_x(0, t, (0, 12), 'x0'), 2) for t in range(XE)]
                jobs += groups['g']
                jobs += [(32, t_odd, job_fin(0, 0, 12, 'x0'), 2)]
                jobs += [(16, None, job_x(1, t, al, 'x1a'), 1) for t in range(XO)]
                jobs += [(12, t_odd + LATP + 60, job_gfin(0, 0, 12, 'x0', c), 2) for c in range(5)]
                jobs += [(8, None, job_x(1, t, ah, 'x1b'), 1) for t in range(XB1)]
                jobs += [(16, t_tail, job_fin(1, 0, 8, 'x1a'), 1)]
                jobs += [(8, None, job_x(1, t, ah, 'x1b'), 1) for t in range(XB1, XB)]
            else:
                for ch in ORD:
                    jobs += groups[ch]
            return jobs

        pjobs = [pair_jobs(u) for u in range(len(kinds))]
        jobs = [job for pj in pjobs for job in pj]
        times = []
        tt = T0F if kinds[0] == 'first' else T0
        for u, pj in enumerate(pjobs):
            rho = RHO if 0 < u < len(kinds) - 1 else (RHO0 if u == 0 else RHOL)
            if RF and 0 < u < len(kinds) - 1:
                dur = t_step[info[u]['s_end']] - t_step[info[u]['s0']]
                rho = max(1.0, RF * dur / sum(job[0] for job in pj))
            if u > 0 and LEAD is not None:
                tt = max(tt, t_step[info[u]['s0']] - LEAD)
            for (cost, earliest, _, _) in pj:
                tt += cost * rho
                if earliest is not None:
                    tt = max(tt, earliest)
                times.append(tt)

        states = {}
        nj = 0
        for st, (u, par, tl, t, ts) in enumerate(steps):
            while nj < len(jobs) and times[nj] + EOFF <= t_step[st]:
                if times[nj] > 0 and 'j0' not in cur:
                    cur['j0'] = nj
                rel = nj - cur.get('j0', nj + 1)
                cur['edge'] = (0 <= rel < NE and rel % EE == EE - 1) or jobs[nj][1] == times[nj]
                jobs[nj][2](times[nj])
                nj += 1
            for (pv_, g_, rs_, po_) in stores.pop(st, ()):
                pv_ = pltpu.bitcast(edge(pltpu.bitcast(pv_, U32), SE, True), F32)
                if po_ is None:
                    l_buf[g_ & 3] = pv_
                else:
                    store_p(pv_, g_, rs_, po_)
            state = states.setdefault((u, par), dict(half=par, slot=slot(u)))
            pv_step(2 * (j0 + u) + par, tl, t, ts, (p_buf0, p_buf1)[par],
                    gates.get(st, ()), true_mask, state)
            cur['state'] = state
            cur['st'] = st
        cur['edge'] = False
        while nj < len(jobs):
            jobs[nj][2](times[nj])
            nj += 1
        assert not stores
        env = envs[-1]
        if kinds[-1] == 'last':
            o = env['finish'](1, 8, 12, 'x1b', lambda x: x)
            op = _pack(o, o)
            xa = [out_cols(env['opx1a'], 12 * (H - 1), 8, c) for c in range(5)]
            xb = [out_cols(op, 12 * (H - 1) + 8, 4, c) for c in range(5)]
            return (xacc_buf[...] + jnp.concatenate(xa, axis=1)) + jnp.concatenate(xb, axis=1), shift2
        return carry

    set_row(x2, shift2)
    xacc_buf[...] = x2
    z = z_buf[...]
    qx = [_dot(z, _bf(wx_buf[i].reshape(D // 2, 128))) * st_buf[0] - csq_buf[3 * NP + i] * st_buf[1]
          for i in range(3)]
    w0 = [_pack(jnp.where(evn, q_, zf), jnp.where(evn, zf, q_)) for q_ in qx]
    store_q([None, q_cols(z, 0, 1), q_cols(z, 0, 2)], 0, pars=(1,))
    sg = [None] * ng
    for g in range(ng):
        for c in range(4):
            lhs = jnp.concatenate([jnp.where(sub == c, w_, jnp.zeros_like(w_)) for w_ in w0], axis=1)
            s = score2(lhs, 0, 0, 4 * g + c)
            sg[g] = s if c == 0 else sg[g] + s
    q_pair(1)
    ps0, l0, c0 = softmax_lane(sg)
    for g in range(ng):
        store_p(ps0[g], g, range(8), p_buf0)
    l_buf[0] = l0
    if ALL:
        x3, shift3 = block(0, 0, ['first'] + ['mid'] * (NP - 2) + ['last'])
    else:
        carry = block(0, 0, ['first'] + ['mid'] * NF)
        n_mid = (NP - 2 - NF - NL) // U
        if n_mid:
            carry = lax.fori_loop(0, n_mid * REP, lambda i, c: block(1 + NF + U * (i if REP == 1 else lax.rem(i, n_mid)), c, ['mid'] * U, (1 + NF) & 1 if U % 2 == 0 and not DYN else None), carry)
        x3, shift3 = block(NP - 1 - NL, carry, ['mid'] * NL + ['last'])
    x4 = x3 + b2 + _dot(mlp_hidden(x3, shift3), w2_buf[...])
    o_ref[...] = x4[0:1, :].astype(o_ref.dtype)


@jax.jit
def pallas_interleave_layers__sliding_block_cached__dense_activation_gelu__decode_kernel(
    A_x: jax.Array,
    A_k_cache: jax.Array,
    A_v_cache: jax.Array,
    A_wq: jax.Array,
    A_wo: jax.Array,
    B_x: jax.Array,
    B_w1: jax.Array,
    B_b1: jax.Array,
    B_w2: jax.Array,
    B_b2: jax.Array,
):
    sk = A_k_cache.shape[2]
    w = min(4096, max(256, sk // 4))

    def tile_view(a):
        *lead, r, c = a.shape
        n = len(lead)
        a = a.reshape(*lead, r // 8, 8, c // 128, 128)
        a = a.transpose(*range(n), n, n + 2, n + 1, n + 3)
        return a.reshape(*lead, r // 16, 2, (c // 128) * 8, 128)

    kx = tile_view(jnp.swapaxes(A_k_cache, 2, 3)[0]).reshape(H * DH // 16, 2, sk // 16, 128)
    vx = tile_view(jnp.swapaxes(A_v_cache, 2, 3)[0]).reshape(H * DH // 16, 2, sk // 16, 128)
    wqx = tile_view(A_wq)
    wox = tile_view(A_wo).reshape(H * DH // 16, 80, 128)
    any_spec = pl.BlockSpec(memory_space=pl.ANY)
    out = pl.pallas_call(
        functools.partial(_kernel, sk=sk, w=w),
        out_shape=jax.ShapeDtypeStruct((1, D), A_x.dtype),
        in_specs=[any_spec] * 9,
        out_specs=pl.BlockSpec(memory_space=pltpu.VMEM),
        scratch_shapes=[
            pltpu.VMEM((H * DH // 16, 2, w // 32, 128), U32),
            pltpu.VMEM((H * DH // 16, 2, w // 32 - 4 * XF, 128), U32),
            pltpu.VMEM((H * DH // 16, 2, max(8 * XF, 8), 128), U32),
            pltpu.VMEM((D // 16, 2, H * DH // 32, 128), U32),
            pltpu.VMEM((H * DH // 16, 40, 128), U32),
            pltpu.VMEM((D, F), BF16),
            pltpu.VMEM((F, D), BF16),
            pltpu.VMEM((1, D), BF16),
            pltpu.VMEM((F // 128, 128), BF16),
            pltpu.VMEM((D // 128, 128), BF16),
            pltpu.VMEM((1, w // 16, 128), F32),
            pltpu.VMEM((1, w // 16, 128), F32),
            pltpu.VMEM((w // 1024, 8, 128), F32),
            pltpu.VMEM((2, DH, 128), U32),
            pltpu.VMEM((8, D), U32),
            pltpu.VMEM((8, D), F32),
            pltpu.VMEM((4, 4, 8, 2 * DH), U32),
            pltpu.VMEM((3, 8, 128), F32),
            pltpu.VMEM((3 * NP + 3, 8, 128), F32),
            pltpu.VMEM((8, F), F32),
            pltpu.VMEM((2, 8, 128), F32),
            pltpu.VMEM((3, 8, 128), jnp.int32),
            pltpu.SMEM((NS,), jnp.int32),
            pltpu.VMEM((w // 1024, 8, 128), F32),
            pltpu.VMEM((8, 2 * DH), U32),
            pltpu.VMEM((4, 8, 128), F32),
            pltpu.VMEM((3, D // 16, 8, 128), U32),
            pltpu.VMEM((8, 128), U32),
            pltpu.VMEM((1, 8, 2 * DH), F32),
            pltpu.SemaphoreType.DMA((2,)),
            pltpu.SemaphoreType.DMA((4,)),
            pltpu.SemaphoreType.DMA((6 + W2C,)),
        ],
        compiler_params=pltpu.CompilerParams(vmem_limit_bytes=int(OPT.get('VM', 127)) * 1024 * 1024,
                                             disable_semaphore_checks=bool(DSC), disable_bounds_checks=bool(DBC)),
    )(A_x.reshape(1, D), kx, vx, wqx, wox, B_w1, B_b1.reshape(F // 128, 128),
      B_w2, B_b2.reshape(D // 128, 128))
    return out.reshape(A_x.shape)
```

```python
import functools
import math

import jax
import jax.numpy as jnp
from jax import lax
import jax.experimental.pallas as pl
import jax.experimental.pallas.tpu as pltpu

F32 = jnp.float32
BF16 = jnp.bfloat16
U32 = jnp.uint32

D = 640
H = 32
DH = 192
F = 1536
EPS = 1e-5
NP = H // 2
OPT = {}
NS = int(OPT.get('NS', 4))
CA = int(OPT.get('CA', 2))
CU = float(OPT.get('CU', 0.263))
XF = int(OPT.get('XF', 6))
CHUNKS = [int(c) for c in OPT.get('CHUNKS', '44322 1').replace(' ', '')]
LATP = float(OPT.get('LATP', 160))
T0 = float(OPT.get('T0', -10))
T0F = float(OPT.get('T0F', -100))
RHO = float(OPT.get('RHO', 1.0))
BE = int(OPT.get('BE', 6))
MOFF = float(OPT.get('MOFF', 160))
MOFF2 = float(OPT.get('MOFF2', 240))
EC = float(OPT.get('EC', 48))
SG = int(OPT.get('SG', 4))
SDT = float(OPT.get('SDT', 12))
CHAIN = int(OPT.get('CHAIN', 0))
XE = int(OPT.get('XE', 7))
XO = int(OPT.get('XO', 7))
W2R = [128 * int(c) for c in OPT.get('W2R', '5421')]
W2C = len(W2R)
W2S = [sum(W2R[:i]) for i in range(W2C)]
ORD = OPT.get('ORD', 'ebxagn')
OPQ = int(OPT.get('OPQ', 0))
LA = int(OPT.get('LA', 1))
NE = int(OPT.get('NE', 7))
EE = int(OPT.get('EE', 2))
SE = int(OPT.get('SE', 1))
EOFF = float(OPT.get('EOFF', 0))
SM = int(OPT.get('SM', 1))
OM = int(OPT.get('OM', 1))
U = int(OPT.get('U', 2))
NF = int(OPT.get('NF', 0))
NL = int(OPT.get('NL', 0))
EDEL = float(OPT.get('EDEL', 70))
RHO0 = float(OPT.get('RHO0', 1.0))
RHOL = float(OPT.get('RHOL', 1.0))
BAR = int(OPT.get('BAR', 0))
IOFF = float(OPT.get('IOFF', 0))
DYN = int(OPT.get('DYN', 0))
MST = int(OPT.get('MST', 1))
DSC = int(OPT.get('DSC', 1))
DBC = int(OPT.get('DBC', 0))
REP = int(OPT.get('REP', 1))
PB = int(OPT.get('PB', 0))
ALL = int(OPT.get('ALL', 1))
LEAD = float(OPT.get('LEAD', 100))
OPQ2 = int(OPT.get('OPQ2', 1))
XB = int(OPT.get('XB', 16))
XB1 = int(OPT.get('XB1', 6))
NGT = int(OPT.get('NGT', 12))
MOFL = float(OPT.get('MOFL', 60))
XM = int(OPT.get('XM', 1))
XMP = int(OPT.get('XMP', 2))
RF = float(OPT.get('RF', 0))
GE = int(OPT.get('GE', 1))
RCP = int(OPT.get('RCP', 1))
XMS = [int(c) for c in OPT.get('XMS', '1111111111111110')]
SKIP2 = int(OPT.get('SKIP2', 0))
SKIP1 = int(OPT.get('SKIP1', 0))


def _gelu(x):
    c = math.sqrt(2.0 / math.pi)
    return 0.5 * x * (1.0 + jnp.tanh(c * (x + 0.044715 * (x * x * x))))


def _rows_to_lanes(b, n):
    return jnp.concatenate([b[i:i + 1, :] for i in range(n)], axis=1)


def _bf(x):
    return pltpu.bitcast(x, BF16)


def _pack(a, b):
    return pltpu.bitcast(pltpu.pack_elementwise([a, b], packed_dtype=BF16), U32)


def _unpack(x):
    return (pltpu.unpack_elementwise(x, index=0, packed_dtype=BF16, unpacked_dtype=F32),
            pltpu.unpack_elementwise(x, index=1, packed_dtype=BF16, unpacked_dtype=F32))


def _dot(lhs32, rhs):
    return jnp.dot(_bf(lhs32), rhs, preferred_element_type=F32)[0:8]


def _dot_t(lhs32, rhs32):
    return lax.dot_general(_bf(lhs32), _bf(rhs32), (((1,), (1,)), ((), ())),
                           preferred_element_type=F32)[0:8]


def _ln_stats(xp, shift):
    x = _unpack(xp)[0] - shift
    m = jnp.mean(x, axis=-1, keepdims=True)
    v = jnp.maximum(jnp.mean(x * x, axis=-1, keepdims=True) - m * m, 0.0)
    return m + shift, lax.rsqrt(v + EPS)


def _mean(x):
    return jnp.mean(x, axis=-1, keepdims=True)


def _kernel(x_hbm, kx_hbm, vx_hbm, wq_hbm, wo_hbm, w1_hbm, b1_hbm, w2_hbm, b2_hbm,
            o_ref,
            kbuf, vbuf, vf_buf, wq_buf, wo_buf, w1_buf, w2_buf, x_buf, b1_buf, b2_buf,
            p_buf0, p_buf1, sp_buf, accp_buf, z_buf, xacc_buf, qv_buf, qraw_buf,
            csq_buf, cs1_buf, st_buf, tm_buf, zs_ref, s2_buf, op_buf, l_buf, wx_buf, lhs0_buf, xo_buf,
            sem_k, sem_v, sem_w, *, sk, w):
    c_scale = (DH ** -0.5) * math.log2(math.e)
    nt = w // 128
    ng = nt // 8
    na = 12 // NS
    nst = NS * nt
    r0w = (sk - w) // 16
    nrw = w // 16

    ntb = nt - XF
    starts = [sum(CHUNKS[:c]) for c in range(len(CHUNKS))]
    assert sum(CHUNKS) == NP

    def k_copy(c):
        rows = pl.ds(24 * starts[c], 24 * CHUNKS[c])
        return [pltpu.make_async_copy(kx_hbm.at[rows, :, pl.ds(r0w, nrw), :],
                                      kbuf.bitcast(BF16).at[rows], sem_k.at[c & 1])]

    def v_copy(c):
        rows = pl.ds(24 * starts[c], 24 * CHUNKS[c])
        cps = [pltpu.make_async_copy(vx_hbm.at[rows, :, pl.ds(r0w, 8 * ntb), :],
                                     vbuf.bitcast(BF16).at[rows], sem_v.at[c & 1])]
        if XF:
            cps.append(pltpu.make_async_copy(
                vx_hbm.at[rows, :, pl.ds(r0w + 8 * ntb, 8 * XF), :],
                vf_buf.bitcast(BF16).at[rows, :, pl.ds(8 * XF, 8 * XF), :], sem_v.at[2 + (c & 1)]))
        return cps

    wq_cp = pltpu.make_async_copy(wq_hbm, wq_buf.bitcast(BF16), sem_w.at[0])
    wo_cp = pltpu.make_async_copy(wo_hbm, wo_buf.bitcast(BF16), sem_w.at[1])
    w1_cp = pltpu.make_async_copy(w1_hbm, w1_buf, sem_w.at[2])
    x_cp = pltpu.make_async_copy(x_hbm, x_buf, sem_w.at[3])
    b1_cp = pltpu.make_async_copy(b1_hbm, b1_buf, sem_w.at[4])
    b2_cp = pltpu.make_async_copy(b2_hbm, b2_buf, sem_w.at[5])
    w2_cps = [pltpu.make_async_copy(w2_hbm.at[pl.ds(W2S[i], W2R[i]), :],
                                    w2_buf.at[pl.ds(W2S[i], W2R[i]), :], sem_w.at[6 + i])
              for i in range(W2C)]

    if not SKIP1:
        wq_cp.start()
    x_cp.start()
    b1_cp.start()
    b2_cp.start()
    if not SKIP1:
        wo_cp.start()
        for cp in k_copy(0) + v_copy(0):
            cp.start()
    x_cp.wait()
    b1_cp.wait()
    b2_cp.wait()

    x0 = jnp.broadcast_to(x_buf[...].astype(F32), (8, D))
    b1 = _rows_to_lanes(b1_buf[...].astype(F32), F // 128)
    b2 = _rows_to_lanes(b2_buf[...].astype(F32), D // 128)

    lane = lax.broadcasted_iota(jnp.int32, (8, 128), 1)
    sub_lo = lax.broadcasted_iota(jnp.int32, (1, 8, 128), 1) < 4
    lo64 = lane < 64
    sub = lax.broadcasted_iota(jnp.int32, (8, 128), 0)
    evn = (lane & 8) == 0
    zf = jnp.zeros((8, 128), F32)
    ones32 = jnp.full((8, 128), 0x3F803F80, U32)
    k_order = (((0, 8, 0), (0, 8, 1), (8, 4, 0), (8, 4, 1)),
               ((4, 8, 0), (4, 8, 1), (0, 4, 1), (0, 4, 0)))

    def swap_halves(ref2):
        n = ref2.shape[1]
        a = ref2[0].reshape(n // 8, 8, 128)
        b = ref2[1].reshape(n // 8, 8, 128)
        ref2[0] = jnp.where(sub_lo, a, pltpu.roll(b, 4, 1)).reshape(n, 128)
        ref2[1] = jnp.where(sub_lo, pltpu.roll(a, 4, 1), b).reshape(n, 128)

    def fix_wq(a, carry):
        swap_halves(wq_buf.at[a])
        return carry

    def fix_wo(g8, carry):
        g0 = pl.multiple_of(g8 * 8, 8)
        v = [wo_buf[pl.ds(g0, 8), 8 * c:8 * c + 8, :] for c in range(5)]
        n = [jnp.where(sub_lo, v[0], v[2]),
             pltpu.roll(jnp.where(sub_lo, v[3], v[0]), 4, 1),
             jnp.where(sub_lo, v[1], v[3]),
             pltpu.roll(jnp.where(sub_lo, v[4], v[1]), 4, 1),
             jnp.where(sub_lo, v[2], v[4])]
        for c in range(5):
            wo_buf[pl.ds(g0, 8), 8 * c:8 * c + 8, :] = n[c]
        return carry

    def set_row(x, shift):
        xp = _pack(x, x)
        z_buf[...] = xp
        m, r = _ln_stats(xp, shift)
        rc = r * c_scale
        st_buf[0] = jnp.broadcast_to(rc, (8, 128))
        st_buf[1] = jnp.broadcast_to(m * rc, (8, 128))

    def wq_cols(ct):
        r0 = pl.multiple_of(lax.shift_right_logical(ct, 1) * 8, 8) if not isinstance(ct, int) else (ct // 2) * 8
        return _bf(wq_buf[:, ct & 1, pl.ds(r0, 8), :].reshape(D // 2, 128))

    def q_cols(z, j, c):
        ct = 3 * j + c
        return _dot(z, wq_cols(ct)) * st_buf[0] - csq_buf[ct] * st_buf[1]

    def store_lhs(hh, ww):
        for c in range(4):
            for i in range(3):
                pltpu.store(qv_buf.at[hh & 3, c, :, 128 * i:128 * (i + 1)], ww[i], mask=sub == c)

    def store_q(qs, j, pars=(0, 1)):
        q0, q1, q2 = qs
        r56, r64, r8 = (pltpu.roll(q1, s, 1) for s in (56, 64, 8))

        def lhs(qf, a2, b2):
            a0 = jnp.where(evn, qf, zf)
            b1_ = jnp.where(evn, zf, qf)
            return [_pack(a0, pltpu.roll(a0, 8, 1)), _pack(pltpu.roll(b1_, 120, 1), b1_),
                    _pack(jnp.where(evn, a2, zf), jnp.where(evn, zf, b2))]

        if 0 in pars:
            store_lhs(2 * j, lhs(q0, jnp.where(lo64, q1, r56), jnp.where(lo64, r8, r64)))
        if 1 in pars:
            store_lhs(2 * j + 1, lhs(q2, jnp.where(lo64, r56, q1), jnp.where(lo64, r64, r8)))

    def q_pair(j):
        z = z_buf[...]
        store_q([q_cols(z, j, c) for c in range(3)], j)

    def score2(lhs, h, par, k):
        rhs = jnp.concatenate([kbuf[pl.ds(12 * h + a, n), e, 8 * k:8 * k + 8, :]
                               for a, n, e in k_order[par]], axis=0)
        return _dot(lhs, _bf(rhs.reshape(DH, 128)))

    def scores_all(h, par):
        sg = [None] * ng
        for c in range(4):
            lhs = qv_buf[h & 3, c]
            for g in range(ng):
                s = score2(lhs, h, par, 4 * g + c)
                sg[g] = s if sg[g] is None else sg[g] + s
        return sg

    def store_p(p, g, rs, p_out):
        for r in rs:
            if PB:
                p_out[0, 64 * g + 8 * r:64 * g + 8 * r + 8, :] = jnp.broadcast_to(p[r:r + 1, :], (8, 128))
            else:
                p_out[0, pl.ds(64 * g + r, 8, stride=8), :] = p

    def inv_sum(l):
        l = jnp.sum(jnp.sum(l, axis=1, keepdims=True), axis=0, keepdims=True)
        l = jnp.broadcast_to(l, (8, 128))
        if RCP:
            r = pl.reciprocal(l, approx=True)
            r = r * (2.0 - l * r)
            return r * (2.0 - l * r) if RCP > 1 else r
        return 1.0 / l

    def softmax(sg, p_out):
        mx = sg[0]
        for s in sg[1:]:
            mx = jnp.maximum(mx, s)
        m = jnp.max(jnp.max(mx, axis=1, keepdims=True), axis=0, keepdims=True)
        l = None
        ps = []
        for g in range(ng):
            p = jnp.exp2(sg[g] - m)
            ps.append(p)
            if p_out is not None:
                store_p(p, g, range(8), p_out)
            l = p if l is None else l + p
        if p_out is None:
            return ps, l
        return ps, inv_sum(l)

    def softmax_lane(sg):
        mx = jnp.maximum(jnp.maximum(sg[0], sg[1]), jnp.maximum(sg[2], sg[3]))
        m = jnp.broadcast_to(jnp.max(mx, axis=0, keepdims=True), (8, 128))
        ps = [jnp.exp2(s - m) for s in sg]
        c = jnp.exp2(m - jnp.max(m, axis=1, keepdims=True))
        c = _unpack(_pack(c, c))[0]
        return ps, ((ps[0] + ps[1]) + (ps[2] + ps[3])) * c, c

    def v_tiles(h, a0, n, t):
        return vbuf[pl.ds(12 * h + a0, n), t % 2, 8 * (t // 2):8 * (t // 2) + 8, :]

    def pv_step(h, tiles, t, ts, p_in, gvals, true_mask, state):
        a0, n = tiles
        p = p_in[0, 8 * t:8 * t + 8, :]
        for i, gval in enumerate(gvals):
            p = jnp.where(true_mask[i], p, gval)
        if t < ntb:
            ys = _unpack(v_tiles(h, a0, n, t))
        else:
            r = 8 * (t - ntb)
            ys = [pltpu.bitcast(vf_buf[pl.ds(12 * h + a0, n), e, r:r + 8, :], F32) for e in range(2)]
        if t == ts[0]:
            state['accs'] = [y * p for y in ys]
        else:
            state['accs'] = [acc + y * p for acc, y in zip(state['accs'], ys)]
        if t == ts[-1]:
            r0 = state['half'] * (DH // 2) + 8 * a0
            accp_buf[state['slot'], r0:r0 + 8 * n, :] = _pack(*state['accs']).reshape(8 * n, 128)

    def o_pair(ones, accp, ie, io):
        inv = jnp.concatenate([ie, jnp.where(lo64, ie, io), io], axis=1)
        return _dot_t(ones, accp) * inv

    def out_cols(op, g0, ngrp, c):
        rhs = wo_buf[pl.ds(g0, ngrp), 8 * c:8 * c + 8, :].reshape(ngrp * 8, 128)
        return _dot(op, _bf(rhs))

    def mlp_hidden(x, shift):
        xp = _pack(x, x)
        m, r = _ln_stats(xp, shift)
        hh = (_dot(xp, w1_buf[...]) - cs1_buf[...] * m) * r + b1
        g = _gelu(hh)
        return _pack(g, g)

    def xm(j):
        return XMS[j]

    def transpose_v(j, t):
        y = _bf(v_tiles(2 * j, 0, 24, t).reshape(DH, 128)).astype(F32)
        yt = pltpu.bitcast(y.T.astype(BF16), U32)
        for ct in range(3):
            vbuf[pl.ds(24 * j + 8 * ct, 8), t % 2, 8 * (t // 2):8 * (t // 2) + 8, :] = (
                yt[:, 128 * ct:128 * (ct + 1)].reshape(8, 8, 128))

    def fix_v(r2, carry):
        swap_halves(vbuf.at[r2])
        if XF:
            n = 4 * XF
            a = vf_buf[r2, 0, n:2 * n, :].reshape(n // 8, 8, 128)
            b = vf_buf[r2, 1, n:2 * n, :].reshape(n // 8, 8, 128)
            t0 = _unpack(jnp.where(sub_lo, a, pltpu.roll(b, 4, 1)))
            t1 = _unpack(jnp.where(sub_lo, pltpu.roll(a, 4, 1), b))
            for e in range(2):
                for k in range(XF // 2):
                    vf_buf[r2, e, 16 * k:16 * k + 8, :] = pltpu.bitcast(t0[e][k], U32)
                    vf_buf[r2, e, 16 * k + 8:16 * k + 16, :] = pltpu.bitcast(t1[e][k], U32)
        return carry

    def next_copies(j, copy_fn, tail_cps):
        for c in range(len(CHUNKS)):
            @pl.when(j == starts[c])
            def _():
                for cp in copy_fn(c):
                    cp.wait()
                for cp in (copy_fn(c + 1) if c + 1 < len(CHUNKS) else tail_cps):
                    cp.start()

    def pair1(j, carry):
        q_pair(j)
        next_copies(j, k_copy, [w1_cp])
        invs = []
        for par in range(2):
            _, inv = softmax(scores_all(2 * j + par, par), (p_buf0, p_buf1)[par])
            invs.append(inv)
        next_copies(j, v_copy, w2_cps)
        lax.fori_loop(24 * j, 24 * (j + 1), fix_v, 0)
        for par in range(2):
            state = dict(half=par, slot=0)
            for sw in range(NS):
                for t in range(nt):
                    pv_step(2 * j + par, (sw * na, na), t, range(nt),
                            (p_buf0, p_buf1)[par], (), None, state)
        for t in range(max(XMS)):
            @pl.when(j < NP - 1)
            def _():
                transpose_v(j, t)
        o = o_pair(ones32, accp_buf[0], invs[0], invs[1])
        op = _pack(o, o)
        for c in range(5):
            xacc_buf[:, 128 * c:128 * (c + 1)] += out_cols(op, 24 * j, 24, c)
        return carry

    def expand(t0, t1):
        return [jnp.where(evn, t0, pltpu.roll(t0, 8, 1)),
                jnp.where(evn, pltpu.roll(t0, 120, 1), t0),
                jnp.where(evn, jnp.where(lo64, t1, pltpu.roll(t1, 56, 1)),
                          jnp.where(lo64, pltpu.roll(t1, 8, 1), pltpu.roll(t1, 64, 1)))]

    def expand_wq(a, carry):
        e = expand(wq_buf[a, 0, 0:8, :], wq_buf[a, 1, 0:8, :])
        for i in range(3):
            wx_buf[i, a] = e[i]
        return carry

    def colsum_q(ct, carry):
        ones = jnp.concatenate([ones32] * (D // 128), axis=1)
        csq_buf[ct] = _dot(ones, wq_cols(ct))
        return carry

    qv_buf[...] = jnp.zeros(qv_buf.shape, U32)
    for i in range(3):
        tm_buf[i] = lane
    for sw in range(NS):
        zs_ref[sw] = 0
    if not SKIP1:
        set_row(x0, _mean(x0))
        xacc_buf[...] = x0
        wq_cp.wait()
        lax.fori_loop(0, D // 16, fix_wq, 0)
        lax.fori_loop(0, 3 * NP, colsum_q, 0)
        lax.fori_loop(0, D // 16, expand_wq, 0)
        e = expand(csq_buf[0], csq_buf[1])
        for i in range(3):
            csq_buf[3 * NP + i] = e[i]
        wo_cp.wait()
        lax.fori_loop(0, H * DH // 128, fix_wo, 0)
        lax.fori_loop(0, NP, pair1, 0)
        x1 = xacc_buf[...]
        w1_cp.wait()
        cs1_buf[...] = _dot(jnp.concatenate([ones32] * (D // 128), axis=1), w1_buf[...])
        gp = mlp_hidden(x1, _mean(x1))
        x2 = x1 + b2
        for i in range(W2C):
            if i == W2C - 1:
                shift2 = _mean(x2)
            w2_cps[i].wait()
            x2 = x2 + _dot(gp[:, W2S[i]:W2S[i] + W2R[i]], w2_buf[W2S[i]:W2S[i] + W2R[i], :])
    else:
        x2 = lax.fori_loop(0, 2, lambda i, x: x + 1.0, x0)
        shift2 = _mean(x0)

    if SKIP2:
        o_ref[...] = x2[0:1, :].astype(o_ref.dtype)
        return

    def block(j0, carry, kinds, jpar=None):
        true_mask = [tm_buf[i] >= 0 for i in range(3)]
        zs = [0] + [zs_ref[sw] if OPQ else 0 for sw in range(1, NS)]
        steps = []
        info = []
        std = [(sw * na, na) for sw in range(NS)]
        for u, kind in enumerate(kinds):
            if kind == 'last':
                sweeps = [[(tl, list(range(XE, nt))) for tl in std],
                          [((5, 3), list(range(XO, nt))), ((2, 3), list(range(XO, nt))),
                           ((0, 2), list(range(XO, nt))), ((8, 4), list(range(XB, nt)))]]
            else:
                sweeps = [[(tl, list(range(xm(j0 + u), nt))) for tl in std]] * 2
            s0 = len(steps)
            steps += [(u, 0, tl, t, ts) for tl, ts in sweeps[0] for t in ts]
            s_odd = len(steps)
            steps += [(u, 1, tl, t, ts) for tl, ts in sweeps[1] for t in ts]
            info.append(dict(s0=s0, s_odd=s_odd, s_end=len(steps),
                             s_tail=len(steps) - len(sweeps[1][-1][1])))
        t_step = [0.0]
        for (_, _, tl, t, _) in steps:
            t_step.append(t_step[-1] + CU * tl[1] * (6 if t < ntb else 4))
        gates, stores = {}, {}
        cur = dict(state=None, st=-1, nedge=0)
        envs = [dict(s1=[None] * ng, s2=[None] * ng, s3=[None] * ng) for _ in kinds]

        zq = zs_ref[0] if OPQ2 else 0

        def get_inv(h):
            return inv_sum(l_buf[zq + (h & 3)])

        def slot(u):
            return (j0 + u) & 1 if jpar is None else (jpar + u) & 1

        def step_at(cyc):
            return next((i for i, tt_ in enumerate(t_step) if tt_ >= cyc), len(t_step))

        def gate(cyc, v):
            st = step_at(cyc)
            while len(gates.get(st, ())) >= 2:
                st += 1
            if st < len(steps) - NGT and st > cur['st']:
                gates.setdefault(st, []).append(v)

        def edge(x, n=BE, force=False):
            if cur['st'] < 0 or not (force or cur['edge']):
                return x
            accs = cur['state']['accs']
            cand = [(e, a) for e in range(2) for a in range(accs[0].shape[0])]
            ntile = -(-x.shape[1] // 128)
            parts = [x[:, 128 * i:min(128 * (i + 1), x.shape[1])] for i in range(ntile)]
            for e in range(min(n, 3 * ntile)):
                ce, ca = cand[cur['nedge'] % len(cand)]
                cur['nedge'] += 1
                i = e % ntile
                w_ = parts[i].shape[1]
                parts[i] = jnp.where(true_mask[e // ntile][:, 0:w_], parts[i],
                                     pltpu.bitcast(accs[ce][ca], U32)[:, 0:w_])
            return parts[0] if ntile == 1 else jnp.concatenate(parts, axis=1)

        def sched_stores(ps, lsum, h, p_out, t_ready, lo, hi, l_off=10):
            gate(t_ready, ps[-1])
            st_l = min(max(step_at(t_ready + l_off), cur['st'] + 1), len(steps) - 1)
            stores.setdefault(st_l, []).append((lsum, h, None, None))
            n = 8 // SG
            t_first = max(t_ready, t_step[lo])
            for i in range(ng * n):
                g, k = divmod(i, n)
                st = min(max(step_at(t_first + SDT * i) + 1, cur['st'] + 1), hi)
                stores.setdefault(st, []).append((ps[g], g, range(SG * k, SG * (k + 1)), p_out))

        def pair_jobs(u):
            kind, env, inf = kinds[u], envs[u], info[u]
            first, last = kind == 'first', kind == 'last'
            j = j0 + u
            h0 = 2 * j

            def job_b(h, par, c, g, key, tail):
                def fn(td):
                    s = score2(edge(qv_buf[h & 3, c]), h, par, 4 * g + c)
                    sg = env[key]
                    sg[g] = s if c == 0 else sg[g] + s
                    if c % GE == GE - 1:
                        gate(td + LATP, sg[g])
                    if c == 3:
                        (sp_buf if key != 's2' else s2_buf)[g] = sg[g]
                    if tail == 'sm1' and first:
                        ps, lsum, c1 = softmax_lane([sp_buf[zq + gg] for gg in range(ng)])
                        lhs0_buf[...] = _pack(c0, c1)
                        sched_stores(ps, lsum, h, p_buf1, td + LATP + MOFL, inf['s0'], inf['s_odd'], 130)
                    elif tail == 'sm1':
                        ps, lsum = softmax([sp_buf[zq + gg] for gg in range(ng)], None)
                        sched_stores(ps, lsum, h, p_buf1, td + LATP + MOFF, inf['s0'], inf['s_odd'])
                        if not first and not last:
                            store_q([qraw_buf[zq + i] for i in range(3)], j + 1)
                    elif tail == 'sm2':
                        ps, lsum = softmax([s2_buf[zq + gg] for gg in range(ng)], None)
                        sched_stores(ps, lsum, h, p_buf0, td + LATP + MOFF2, inf['s_odd'], inf['s_end'] - 1)
                return fn

            def job_e(td):
                if j == 1 or xm(j - 1):
                    x = _dot_t(edge(lhs0_buf[...] if j == 1 else ones32), accp_buf[1 - slot(u)])
                    if xm(j - 1):
                        x = x + xo_buf[zq]
                    row = lambda i, r: jnp.broadcast_to(x[r:r + 1, 128 * i:128 * (i + 1)], (8, 128))
                    ie, io = get_inv(h0 - 2), get_inv(h0 - 1)
                    o = jnp.concatenate([row(0, 0) * ie, jnp.where(lo64, row(1, 0) * ie, row(1, 1) * io),
                                         row(2, 1) * io], axis=1)
                else:
                    o = o_pair(edge(ones32), accp_buf[1 - slot(u)], get_inv(h0 - 2), get_inv(h0 - 1))
                gate(td + LATP + 10, o[:, 256:384])
                op_buf[...] = _pack(o, o)

            def job_g(c):
                def fn(td):
                    xo = out_cols(edge(op_buf[...]), 24 * (j - 1), 24, c)
                    xacc_buf[:, 128 * c:128 * (c + 1)] += xo
                    gate(td + LATP, xo)
                return fn

            def job_a(c):
                def fn(td):
                    jn = j + 2 if isinstance(j, int) else jnp.minimum(j + 2, NP - 1)
                    qc = q_cols(edge(z_buf[...]), jn, c)
                    gate(td + LATP, qc)
                    qraw_buf[c] = qc
                return fn

            def job_x(par, t, tiles, key):
                def fn(td):
                    p = (p_buf0, p_buf1)[par][0, 8 * t:8 * t + 8, :]
                    rhs = v_tiles(h0 + par, tiles[0], tiles[1], t).reshape(8 * tiles[1], 128)
                    o = _dot_t(edge(_pack(p, p)), rhs)
                    env[key] = o if key not in env else env[key] + o
                    gate(td + LATP, env[key][:, 0:128] if tiles[1] >= 8 else
                         jnp.concatenate([env[key], env[key]], axis=1))
                return fn

            def job_xp(t):
                def fn(td):
                    pe, po = p_buf0[0, 8 * t:8 * t + 8, :], p_buf1[0, 8 * t:8 * t + 8, :]
                    if j == 0:
                        ce, co = _unpack(lhs0_buf[...])
                        pe, po = pe * ce, po * co
                    lhs = _pack(pe, po)
                    lhs = edge(lhs)
                    o = jnp.concatenate([_dot(lhs, _bf(v_tiles(h0, 8 * ct, 8, t).reshape(64, 128)))
                                         for ct in range(3)], axis=1)
                    env['xp'] = o if 'xp' not in env else env['xp'] + o
                    gate(td + LATP + 20, env['xp'][:, 256:384])
                    if t == xm(j) - 1:
                        xo_buf[0] = env['xp']
                return fn

            def finish(par, a0, a1, key, lhs_edge):
                r0 = par * (DH // 2)
                o = _dot_t(lhs_edge(ones32), accp_buf[slot(u), r0 + 8 * a0:r0 + 8 * a1, :])
                if key in env:
                    o = o + env[key]
                inv = get_inv(h0 + par)
                n = 16 * (a1 - a0)
                return o * (inv[:, 0:n] if n <= 128 else jnp.concatenate([inv, inv[:, 0:n - 128]], axis=1))

            env['finish'] = finish

            def job_fin(par, a0, a1, key):
                def fn(td):
                    o = finish(par, a0, a1, key, edge)
                    gate(td + LATP + 10, o[:, 0:128])
                    env['op' + key] = _pack(o, o)
                return fn

            def job_gfin(par, a0, a1, key, c):
                def fn(td):
                    xo = out_cols(edge(env['op' + key]), 12 * (h0 + par) + a0, a1 - a0, c)
                    xacc_buf[:, 128 * c:128 * (c + 1)] += xo
                    gate(td + LATP, xo)
                return fn

            jobs = []
            for g in range(0 if first else CA, ng):
                for c in range(4):
                    tail = 'sm1' if (c == 3 and g == ng - 1) else None
                    jobs.append((24, None, job_b(h0 + 1, 1, c, g, 's1', tail), 3))
            t_pair = t_step[inf['s0']] + EDEL if u > 0 else None
            groups = {
                'e': [] if first else [(EC, t_pair, job_e, 3)],
                'b': [(24, None, job_b(h0 + 2, 0, c, g, 's2',
                                       'sm2' if (c == 3 and g == ng - 1) else None), 3)
                      for g in range(ng) for c in range(4)],
                'a': [] if isinstance(j, int) and j + 2 >= NP else
                     [(40, None, job_a(c), 5) for c in range(3)],
                'x': [(24, t_step[inf['s_odd'] + 1], job_xp(t), 3) for t in range(xm(j))],
                'g': [] if first else [(24, None, job_g(c), 3) for c in range(5)],
                'n': [(24, None, job_b(h0 + 3, 1, c, g, 's3', None), 3)
                      for g in range(CA) for c in range(4)],
            }
            if last:
                t_odd = t_step[inf['s_odd'] + 1]
                t_tail = t_step[inf['s_tail'] + 1]
                al, ah = (0, 8), (8, 4)
                jobs += groups['e'] + [(24, None, job_x(0, t, (0, 12), 'x0'), 2) for t in range(XE)]
                jobs += groups['g']
                jobs += [(32, t_odd, job_fin(0, 0, 12, 'x0'), 2)]
                jobs += [(16, None, job_x(1, t, al, 'x1a'), 1) for t in range(XO)]
                jobs += [(12, t_odd + LATP + 60, job_gfin(0, 0, 12, 'x0', c), 2) for c in range(5)]
                jobs += [(8, None, job_x(1, t, ah, 'x1b'), 1) for t in range(XB1)]
                jobs += [(16, t_tail, job_fin(1, 0, 8, 'x1a'), 1)]
                jobs += [(8, None, job_x(1, t, ah, 'x1b'), 1) for t in range(XB1, XB)]
            else:
                for ch in ORD:
                    jobs += groups[ch]
            return jobs

        pjobs = [pair_jobs(u) for u in range(len(kinds))]
        jobs = [job for pj in pjobs for job in pj]
        times = []
        tt = T0F if kinds[0] == 'first' else T0
        for u, pj in enumerate(pjobs):
            rho = RHO if 0 < u < len(kinds) - 1 else (RHO0 if u == 0 else RHOL)
            if RF and 0 < u < len(kinds) - 1:
                dur = t_step[info[u]['s_end']] - t_step[info[u]['s0']]
                rho = max(1.0, RF * dur / sum(job[0] for job in pj))
            if u > 0 and LEAD is not None:
                tt = max(tt, t_step[info[u]['s0']] - LEAD)
            for (cost, earliest, _, _) in pj:
                tt += cost * rho
                if earliest is not None:
                    tt = max(tt, earliest)
                times.append(tt)

        states = {}
        nj = 0
        for st, (u, par, tl, t, ts) in enumerate(steps):
            while nj < len(jobs) and times[nj] + EOFF <= t_step[st]:
                if times[nj] > 0 and 'j0' not in cur:
                    cur['j0'] = nj
                rel = nj - cur.get('j0', nj + 1)
                cur['edge'] = (0 <= rel < NE and rel % EE == EE - 1) or jobs[nj][1] == times[nj]
                jobs[nj][2](times[nj])
                nj += 1
            for (pv_, g_, rs_, po_) in stores.pop(st, ()):
                pv_ = pltpu.bitcast(edge(pltpu.bitcast(pv_, U32), SE, True), F32)
                if po_ is None:
                    l_buf[g_ & 3] = pv_
                else:
                    store_p(pv_, g_, rs_, po_)
            state = states.setdefault((u, par), dict(half=par, slot=slot(u)))
            pv_step(2 * (j0 + u) + par, tl, t, ts, (p_buf0, p_buf1)[par],
                    gates.get(st, ()), true_mask, state)
            cur['state'] = state
            cur['st'] = st
        cur['edge'] = False
        while nj < len(jobs):
            jobs[nj][2](times[nj])
            nj += 1
        assert not stores
        env = envs[-1]
        if kinds[-1] == 'last':
            o = env['finish'](1, 8, 12, 'x1b', lambda x: x)
            op = _pack(o, o)
            xa = [out_cols(env['opx1a'], 12 * (H - 1), 8, c) for c in range(5)]
            xb = [out_cols(op, 12 * (H - 1) + 8, 4, c) for c in range(5)]
            return (xacc_buf[...] + jnp.concatenate(xa, axis=1)) + jnp.concatenate(xb, axis=1), shift2
        return carry

    set_row(x2, shift2)
    xacc_buf[...] = x2
    z = z_buf[...]
    qx = [_dot(z, _bf(wx_buf[i].reshape(D // 2, 128))) * st_buf[0] - csq_buf[3 * NP + i] * st_buf[1]
          for i in range(3)]
    w0 = [_pack(jnp.where(evn, q_, zf), jnp.where(evn, zf, q_)) for q_ in qx]
    store_q([None, q_cols(z, 0, 1), q_cols(z, 0, 2)], 0, pars=(1,))
    sg = [None] * ng
    for g in range(ng):
        for c in range(4):
            lhs = jnp.concatenate([jnp.where(sub == c, w_, jnp.zeros_like(w_)) for w_ in w0], axis=1)
            s = score2(lhs, 0, 0, 4 * g + c)
            sg[g] = s if c == 0 else sg[g] + s
    q_pair(1)
    ps0, l0, c0 = softmax_lane(sg)
    for g in range(ng):
        store_p(ps0[g], g, range(8), p_buf0)
    l_buf[0] = l0
    if ALL:
        x3, shift3 = block(0, 0, ['first'] + ['mid'] * (NP - 2) + ['last'])
    else:
        carry = block(0, 0, ['first'] + ['mid'] * NF)
        n_mid = (NP - 2 - NF - NL) // U
        if n_mid:
            carry = lax.fori_loop(0, n_mid * REP, lambda i, c: block(1 + NF + U * (i if REP == 1 else lax.rem(i, n_mid)), c, ['mid'] * U, (1 + NF) & 1 if U % 2 == 0 and not DYN else None), carry)
        x3, shift3 = block(NP - 1 - NL, carry, ['mid'] * NL + ['last'])
    x4 = x3 + b2 + _dot(mlp_hidden(x3, shift3), w2_buf[...])
    o_ref[...] = x4[0:1, :].astype(o_ref.dtype)


@jax.jit
def pallas_interleave_layers__sliding_block_cached__dense_activation_gelu__decode_kernel(
    A_x: jax.Array,
    A_k_cache: jax.Array,
    A_v_cache: jax.Array,
    A_wq: jax.Array,
    A_wo: jax.Array,
    B_x: jax.Array,
    B_w1: jax.Array,
    B_b1: jax.Array,
    B_w2: jax.Array,
    B_b2: jax.Array,
):
    sk = A_k_cache.shape[2]
    w = min(4096, max(256, sk // 4))

    def tile_view(a):
        *lead, r, c = a.shape
        n = len(lead)
        a = a.reshape(*lead, r // 8, 8, c // 128, 128)
        a = a.transpose(*range(n), n, n + 2, n + 1, n + 3)
        return a.reshape(*lead, r // 16, 2, (c // 128) * 8, 128)

    kx = tile_view(jnp.swapaxes(A_k_cache, 2, 3)[0]).reshape(H * DH // 16, 2, sk // 16, 128)
    vx = tile_view(jnp.swapaxes(A_v_cache, 2, 3)[0]).reshape(H * DH // 16, 2, sk // 16, 128)
    wqx = tile_view(A_wq)
    wox = tile_view(A_wo).reshape(H * DH // 16, 80, 128)
    any_spec = pl.BlockSpec(memory_space=pl.ANY)
    out = pl.pallas_call(
        functools.partial(_kernel, sk=sk, w=w),
        out_shape=jax.ShapeDtypeStruct((1, D), A_x.dtype),
        in_specs=[any_spec] * 9,
        out_specs=pl.BlockSpec(memory_space=pltpu.VMEM),
        scratch_shapes=[
            pltpu.VMEM((H * DH // 16, 2, w // 32, 128), U32),
            pltpu.VMEM((H * DH // 16, 2, w // 32 - 4 * XF, 128), U32),
            pltpu.VMEM((H * DH // 16, 2, max(8 * XF, 8), 128), U32),
            pltpu.VMEM((D // 16, 2, H * DH // 32, 128), U32),
            pltpu.VMEM((H * DH // 16, 40, 128), U32),
            pltpu.VMEM((D, F), BF16),
            pltpu.VMEM((F, D), BF16),
            pltpu.VMEM((1, D), BF16),
            pltpu.VMEM((F // 128, 128), BF16),
            pltpu.VMEM((D // 128, 128), BF16),
            pltpu.VMEM((1, w // 16, 128), F32),
            pltpu.VMEM((1, w // 16, 128), F32),
            pltpu.VMEM((w // 1024, 8, 128), F32),
            pltpu.VMEM((2, DH, 128), U32),
            pltpu.VMEM((8, D), U32),
            pltpu.VMEM((8, D), F32),
            pltpu.VMEM((4, 4, 8, 2 * DH), U32),
            pltpu.VMEM((3, 8, 128), F32),
            pltpu.VMEM((3 * NP + 3, 8, 128), F32),
            pltpu.VMEM((8, F), F32),
            pltpu.VMEM((2, 8, 128), F32),
            pltpu.VMEM((3, 8, 128), jnp.int32),
            pltpu.SMEM((NS,), jnp.int32),
            pltpu.VMEM((w // 1024, 8, 128), F32),
            pltpu.VMEM((8, 2 * DH), U32),
            pltpu.VMEM((4, 8, 128), F32),
            pltpu.VMEM((3, D // 16, 8, 128), U32),
            pltpu.VMEM((8, 128), U32),
            pltpu.VMEM((1, 8, 2 * DH), F32),
            pltpu.SemaphoreType.DMA((2,)),
            pltpu.SemaphoreType.DMA((4,)),
            pltpu.SemaphoreType.DMA((6 + W2C,)),
        ],
        compiler_params=pltpu.CompilerParams(vmem_limit_bytes=int(OPT.get('VM', 127)) * 1024 * 1024,
                                             disable_semaphore_checks=bool(DSC), disable_bounds_checks=bool(DBC)),
    )(A_x.reshape(1, D), kx, vx, wqx, wox, B_w1, B_b1.reshape(F // 128, 128),
      B_w2, B_b2.reshape(D // 128, 128))
    return out.reshape(A_x.shape)
```

```python
import functools
import math

import jax
import jax.numpy as jnp
from jax import lax
import jax.experimental.pallas as pl
import jax.experimental.pallas.tpu as pltpu

F32 = jnp.float32
BF16 = jnp.bfloat16
U32 = jnp.uint32

D = 640
H = 32
DH = 192
F = 1536
EPS = 1e-5
NP = H // 2

CHUNKS = (4, 4, 3, 2, 2, 1)
W2_ROWS = (640, 512, 256, 128)
NS = 4
XF = 6
XM = 1
XE, XO, XB, XB1 = 7, 7, 16, 6

CU = 0.263
T0 = -100.0
LEAD = 100.0
LATP = 160.0
MOFF, MOFF2, MOFL = 160.0, 240.0, 60.0
EDEL = 70.0
SDT = 12.0
NE, BE, NGT = 7, 6, 12


def _gelu(x):
    c = math.sqrt(2.0 / math.pi)
    return 0.5 * x * (1.0 + jnp.tanh(c * (x + 0.044715 * (x * x * x))))


def _rows_to_lanes(b, n):
    return jnp.concatenate([b[i:i + 1, :] for i in range(n)], axis=1)


def _bf(x):
    return pltpu.bitcast(x, BF16)


def _pack(a, b):
    return pltpu.bitcast(pltpu.pack_elementwise([a, b], packed_dtype=BF16), U32)


def _unpack(x):
    return (pltpu.unpack_elementwise(x, index=0, packed_dtype=BF16, unpacked_dtype=F32),
            pltpu.unpack_elementwise(x, index=1, packed_dtype=BF16, unpacked_dtype=F32))


def _dot(lhs32, rhs):
    return jnp.dot(_bf(lhs32), rhs, preferred_element_type=F32)[0:8]


def _dot_t(lhs32, rhs32):
    return lax.dot_general(_bf(lhs32), _bf(rhs32), (((1,), (1,)), ((), ())),
                           preferred_element_type=F32)[0:8]


def _mean(x):
    return jnp.mean(x, axis=-1, keepdims=True)


def _ln_stats(xp, shift):
    x = _unpack(xp)[0] - shift
    m = _mean(x)
    v = jnp.maximum(_mean(x * x) - m * m, 0.0)
    return m + shift, lax.rsqrt(v + EPS)


def _kernel(x_hbm, kx_hbm, vx_hbm, wq_hbm, wo_hbm, w1_hbm, b1_hbm, w2_hbm, b2_hbm,
            o_ref,
            kbuf, vbuf, vf_buf, wq_buf, wo_buf, w1_buf, w2_buf, x_buf, b1_buf, b2_buf,
            p_buf0, p_buf1, so_buf, se_buf, l_buf, qraw_buf, xo_buf, accp_buf, z_buf,
            xacc_buf, qv_buf, csq_buf, cs1_buf, st_buf, op_buf, wx_buf, c01_buf,
            tm_buf, zero_ref, sem_k, sem_v, sem_w, *, sk, w):
    c_scale = (DH ** -0.5) * math.log2(math.e)
    nt = w // 128
    ng = nt // 8
    na = 12 // NS
    ntb = nt - XF
    r0w = (sk - w) // 16
    p_bufs = (p_buf0, p_buf1)
    starts = [sum(CHUNKS[:c]) for c in range(len(CHUNKS))]
    w2_at = [sum(W2_ROWS[:i]) for i in range(len(W2_ROWS))]

    def k_copy(c):
        rows = pl.ds(24 * starts[c], 24 * CHUNKS[c])
        return [pltpu.make_async_copy(kx_hbm.at[rows, :, pl.ds(r0w, 8 * nt), :],
                                      kbuf.bitcast(BF16).at[rows], sem_k.at[c & 1])]

    def v_copy(c):
        rows = pl.ds(24 * starts[c], 24 * CHUNKS[c])
        return [pltpu.make_async_copy(vx_hbm.at[rows, :, pl.ds(r0w, 8 * ntb), :],
                                      vbuf.bitcast(BF16).at[rows], sem_v.at[c & 1]),
                pltpu.make_async_copy(vx_hbm.at[rows, :, pl.ds(r0w + 8 * ntb, 8 * XF), :],
                                      vf_buf.bitcast(BF16).at[rows, :, pl.ds(8 * XF, 8 * XF), :],
                                      sem_v.at[2 + (c & 1)])]

    wq_cp = pltpu.make_async_copy(wq_hbm, wq_buf.bitcast(BF16), sem_w.at[0])
    wo_cp = pltpu.make_async_copy(wo_hbm, wo_buf.bitcast(BF16), sem_w.at[1])
    w1_cp = pltpu.make_async_copy(w1_hbm, w1_buf, sem_w.at[2])
    x_cp = pltpu.make_async_copy(x_hbm, x_buf, sem_w.at[3])
    b1_cp = pltpu.make_async_copy(b1_hbm, b1_buf, sem_w.at[4])
    b2_cp = pltpu.make_async_copy(b2_hbm, b2_buf, sem_w.at[5])
    w2_cps = [pltpu.make_async_copy(w2_hbm.at[pl.ds(r, n), :], w2_buf.at[pl.ds(r, n), :],
                                    sem_w.at[6 + i])
              for i, (r, n) in enumerate(zip(w2_at, W2_ROWS))]

    for cp in [wq_cp, x_cp, b1_cp, b2_cp, wo_cp] + k_copy(0) + v_copy(0):
        cp.start()
    x_cp.wait()
    b1_cp.wait()
    b2_cp.wait()

    x0 = jnp.broadcast_to(x_buf[...].astype(F32), (8, D))
    b1 = _rows_to_lanes(b1_buf[...].astype(F32), F // 128)
    b2 = _rows_to_lanes(b2_buf[...].astype(F32), D // 128)

    lane = lax.broadcasted_iota(jnp.int32, (8, 128), 1)
    sub = lax.broadcasted_iota(jnp.int32, (8, 128), 0)
    sub_lo = lax.broadcasted_iota(jnp.int32, (1, 8, 128), 1) < 4
    lo64 = lane < 64
    evn = (lane & 8) == 0
    zf = jnp.zeros((8, 128), F32)
    ones32 = jnp.full((8, 128), 0x3F803F80, U32)
    k_order = (((0, 8, 0), (0, 8, 1), (8, 4, 0), (8, 4, 1)),
               ((4, 8, 0), (4, 8, 1), (0, 4, 1), (0, 4, 0)))

    def regroup(a, b):
        return jnp.where(sub_lo, a, pltpu.roll(b, 4, 1)), jnp.where(sub_lo, pltpu.roll(a, 4, 1), b)

    def swap_halves(ref2):
        n = ref2.shape[1]
        a, b = regroup(ref2[0].reshape(n // 8, 8, 128), ref2[1].reshape(n // 8, 8, 128))
        ref2[0] = a.reshape(n, 128)
        ref2[1] = b.reshape(n, 128)

    def fix_wq(a, carry):
        swap_halves(wq_buf.at[a])
        return carry

    def fix_wo(g8, carry):
        g0 = pl.multiple_of(g8 * 8, 8)
        v = [wo_buf[pl.ds(g0, 8), 8 * c:8 * c + 8, :] for c in range(5)]
        n = [jnp.where(sub_lo, v[0], v[2]),
             pltpu.roll(jnp.where(sub_lo, v[3], v[0]), 4, 1),
             jnp.where(sub_lo, v[1], v[3]),
             pltpu.roll(jnp.where(sub_lo, v[4], v[1]), 4, 1),
             jnp.where(sub_lo, v[2], v[4])]
        for c in range(5):
            wo_buf[pl.ds(g0, 8), 8 * c:8 * c + 8, :] = n[c]
        return carry

    def fix_v(r2, carry):
        swap_halves(vbuf.at[r2])
        n = 4 * XF
        t0, t1 = regroup(vf_buf[r2, 0, n:2 * n, :].reshape(n // 8, 8, 128),
                         vf_buf[r2, 1, n:2 * n, :].reshape(n // 8, 8, 128))
        t0, t1 = _unpack(t0), _unpack(t1)
        for e in range(2):
            for k in range(XF // 2):
                vf_buf[r2, e, 16 * k:16 * k + 8, :] = pltpu.bitcast(t0[e][k], U32)
                vf_buf[r2, e, 16 * k + 8:16 * k + 16, :] = pltpu.bitcast(t1[e][k], U32)
        return carry

    def v_tiles(h, a0, n, t):
        return vbuf[pl.ds(12 * h + a0, n), t % 2, 8 * (t // 2):8 * (t // 2) + 8, :]

    def transpose_v(j, t):
        y = _bf(v_tiles(2 * j, 0, 24, t).reshape(DH, 128)).astype(F32)
        yt = pltpu.bitcast(y.T.astype(BF16), U32)
        for ct in range(3):
            vbuf[pl.ds(24 * j + 8 * ct, 8), t % 2, 8 * (t // 2):8 * (t // 2) + 8, :] = (
                yt[:, 128 * ct:128 * (ct + 1)].reshape(8, 8, 128))

    def set_row(x, shift):
        xp = _pack(x, x)
        z_buf[...] = xp
        m, r = _ln_stats(xp, shift)
        rc = r * c_scale
        st_buf[0] = jnp.broadcast_to(rc, (8, 128))
        st_buf[1] = jnp.broadcast_to(m * rc, (8, 128))

    def wq_cols(ct):
        if isinstance(ct, int):
            r0 = (ct // 2) * 8
        else:
            r0 = pl.multiple_of(lax.shift_right_logical(ct, 1) * 8, 8)
        return _bf(wq_buf[:, ct & 1, pl.ds(r0, 8), :].reshape(D // 2, 128))

    def q_cols(z, j, c):
        ct = 3 * j + c
        return _dot(z, wq_cols(ct)) * st_buf[0] - csq_buf[ct] * st_buf[1]

    def store_q(qs, j, pars=(0, 1)):
        q0, q1, q2 = qs
        r56, r64, r8 = (pltpu.roll(q1, s, 1) for s in (56, 64, 8))

        def put(h, qf, a2, b2):
            a0 = jnp.where(evn, qf, zf)
            b1_ = jnp.where(evn, zf, qf)
            ww = [_pack(a0, pltpu.roll(a0, 8, 1)), _pack(pltpu.roll(b1_, 120, 1), b1_),
                  _pack(jnp.where(evn, a2, zf), jnp.where(evn, zf, b2))]
            for c in range(4):
                for i in range(3):
                    pltpu.store(qv_buf.at[h & 3, c, :, 128 * i:128 * (i + 1)], ww[i],
                                mask=sub == c)

        if 0 in pars:
            put(2 * j, q0, jnp.where(lo64, q1, r56), jnp.where(lo64, r8, r64))
        if 1 in pars:
            put(2 * j + 1, q2, jnp.where(lo64, r56, q1), jnp.where(lo64, r64, r8))

    def q_pair(j):
        z = z_buf[...]
        store_q([q_cols(z, j, c) for c in range(3)], j)

    def score2(lhs, h, par, k):
        rhs = jnp.concatenate([kbuf[pl.ds(12 * h + a, n), e, 8 * k:8 * k + 8, :]
                               for a, n, e in k_order[par]], axis=0)
        return _dot(lhs, _bf(rhs.reshape(DH, 128)))

    def store_p(p, g, rs, p_out):
        for r in rs:
            p_out[pl.ds(64 * g + r, 8, stride=8), :] = p

    def inv_sum(l):
        l = jnp.sum(jnp.sum(l, axis=1, keepdims=True), axis=0, keepdims=True)
        l = jnp.broadcast_to(l, (8, 128))
        r = pl.reciprocal(l, approx=True)
        return r * (2.0 - l * r)

    def softmax(sg):
        mx = sg[0]
        for s in sg[1:]:
            mx = jnp.maximum(mx, s)
        m = jnp.max(jnp.max(mx, axis=1, keepdims=True), axis=0, keepdims=True)
        ps, l = [], None
        for s in sg:
            ps.append(jnp.exp2(s - m))
            l = ps[-1] if l is None else l + ps[-1]
        return ps, l

    def softmax_lane(sg):
        mx = jnp.maximum(jnp.maximum(sg[0], sg[1]), jnp.maximum(sg[2], sg[3]))
        m = jnp.broadcast_to(jnp.max(mx, axis=0, keepdims=True), (8, 128))
        ps = [jnp.exp2(s - m) for s in sg]
        c = jnp.exp2(m - jnp.max(m, axis=1, keepdims=True))
        c = _unpack(_pack(c, c))[0]
        return ps, ((ps[0] + ps[1]) + (ps[2] + ps[3])) * c, c

    def pv_step(h, tiles, t, ts, gated, state):
        a0, n = tiles
        p = p_bufs[state['par']][8 * t:8 * t + 8, :]
        for mask, val in gated:
            p = jnp.where(mask, p, val)
        if t < ntb:
            ys = _unpack(v_tiles(h, a0, n, t))
        else:
            r = 8 * (t - ntb)
            ys = [pltpu.bitcast(vf_buf[pl.ds(12 * h + a0, n), e, r:r + 8, :], F32)
                  for e in range(2)]
        if t == ts[0]:
            state['accs'] = [y * p for y in ys]
        else:
            state['accs'] = [acc + y * p for acc, y in zip(state['accs'], ys)]
        if t == ts[-1]:
            r0 = state['par'] * (DH // 2) + 8 * a0
            accp_buf[state['slot'], r0:r0 + 8 * n, :] = _pack(*state['accs']).reshape(8 * n, 128)

    def out_cols(op, g0, ngrp, c):
        rhs = wo_buf[pl.ds(g0, ngrp), 8 * c:8 * c + 8, :].reshape(ngrp * 8, 128)
        return _dot(op, _bf(rhs))

    def mlp_hidden(x, shift):
        xp = _pack(x, x)
        m, r = _ln_stats(xp, shift)
        g = _gelu((_dot(xp, w1_buf[...]) - cs1_buf[...] * m) * r + b1)
        return _pack(g, g)

    def next_copies(j, copy_fn, tail_cps):
        for c in range(len(CHUNKS)):
            @pl.when(j == starts[c])
            def _():
                for cp in copy_fn(c):
                    cp.wait()
                for cp in (copy_fn(c + 1) if c + 1 < len(CHUNKS) else tail_cps):
                    cp.start()

    def pair1(j, carry):
        q_pair(j)
        next_copies(j, k_copy, [w1_cp])
        invs = []
        for par in range(2):
            h = 2 * j + par
            sg = [None] * ng
            for c in range(4):
                lhs = qv_buf[h & 3, c]
                for g in range(ng):
                    s = score2(lhs, h, par, 4 * g + c)
                    sg[g] = s if c == 0 else sg[g] + s
            ps, l = softmax(sg)
            for g in range(ng):
                store_p(ps[g], g, range(8), p_bufs[par])
            invs.append(inv_sum(l))
        next_copies(j, v_copy, w2_cps)
        lax.fori_loop(24 * j, 24 * (j + 1), fix_v, 0)
        for par in range(2):
            state = dict(par=par, slot=0)
            for sw in range(NS):
                for t in range(nt):
                    pv_step(2 * j + par, (sw * na, na), t, range(nt), (), state)

        @pl.when(j < NP - 1)
        def _():
            for t in range(XM):
                transpose_v(j, t)

        ie, io = invs
        o = _dot_t(ones32, accp_buf[0]) * jnp.concatenate([ie, jnp.where(lo64, ie, io), io], axis=1)
        op = _pack(o, o)
        for c in range(5):
            xacc_buf[:, 128 * c:128 * (c + 1)] += out_cols(op, 24 * j, 24, c)
        return carry

    def expand(t0, t1):
        return [jnp.where(evn, t0, pltpu.roll(t0, 8, 1)),
                jnp.where(evn, pltpu.roll(t0, 120, 1), t0),
                jnp.where(evn, jnp.where(lo64, t1, pltpu.roll(t1, 56, 1)),
                          jnp.where(lo64, pltpu.roll(t1, 8, 1), pltpu.roll(t1, 64, 1)))]

    def expand_wq(a, carry):
        e = expand(wq_buf[a, 0, 0:8, :], wq_buf[a, 1, 0:8, :])
        for i in range(3):
            wx_buf[i, a] = e[i]
        return carry

    ones_row = jnp.concatenate([ones32] * (D // 128), axis=1)

    def colsum_q(ct, carry):
        csq_buf[ct] = _dot(ones_row, wq_cols(ct))
        return carry

    for ref in (qv_buf, so_buf, se_buf, l_buf, qraw_buf, xo_buf):
        ref[...] = jnp.zeros(ref.shape, ref.dtype)
    for i in range(3):
        tm_buf[i] = lane
    zero_ref[0] = 0

    set_row(x0, _mean(x0))
    xacc_buf[...] = x0
    wq_cp.wait()
    lax.fori_loop(0, D // 16, fix_wq, 0)
    lax.fori_loop(0, 3 * NP, colsum_q, 0)
    lax.fori_loop(0, D // 16, expand_wq, 0)
    e = expand(csq_buf[0], csq_buf[1])
    for i in range(3):
        csq_buf[3 * NP + i] = e[i]
    wo_cp.wait()
    lax.fori_loop(0, H * DH // 128, fix_wo, 0)
    lax.fori_loop(0, NP, pair1, 0)
    x1 = xacc_buf[...]
    w1_cp.wait()
    cs1_buf[...] = _dot(ones_row, w1_buf[...])
    gp = mlp_hidden(x1, _mean(x1))
    x2 = x1 + b2
    for cp, r, n in zip(w2_cps, w2_at, W2_ROWS):
        shift = _mean(x2) if cp is w2_cps[-1] else None
        cp.wait()
        x2 = x2 + _dot(gp[:, r:r + n], w2_buf[r:r + n, :])

    set_row(x2, shift)
    xacc_buf[...] = x2
    z = z_buf[...]
    qx = [_dot(z, _bf(wx_buf[i].reshape(D // 2, 128))) * st_buf[0]
          - csq_buf[3 * NP + i] * st_buf[1] for i in range(3)]
    w0 = [_pack(jnp.where(evn, q_, zf), jnp.where(evn, zf, q_)) for q_ in qx]
    store_q([None, q_cols(z, 0, 1), q_cols(z, 0, 2)], 0, pars=(1,))
    sg = [None] * ng
    for g in range(ng):
        for c in range(4):
            lhs = jnp.concatenate([jnp.where(sub == c, w_, jnp.zeros_like(w_)) for w_ in w0],
                                  axis=1)
            s = score2(lhs, 0, 0, 4 * g + c)
            sg[g] = s if c == 0 else sg[g] + s
    q_pair(1)
    ps0, l0, c0 = softmax_lane(sg)
    for g in range(ng):
        store_p(ps0[g], g, range(8), p_buf0)
    l_buf[0] = l0

    true_mask = [tm_buf[i] >= 0 for i in range(3)]
    zq = jnp.clip(zero_ref[0], 0, 1)
    std = [(sw * na, na) for sw in range(NS)]
    steps, info = [], []
    for j in range(NP):
        if j == NP - 1:
            sweeps = [[(tl, range(XE, nt)) for tl in std],
                      [((5, 3), range(XO, nt)), ((2, 3), range(XO, nt)),
                       ((0, 2), range(XO, nt)), ((8, 4), range(XB, nt))]]
        else:
            sweeps = [[(tl, range(XM, nt)) for tl in std]] * 2
        s0 = len(steps)
        steps += [(j, 0, tl, t, ts) for tl, ts in sweeps[0] for t in ts]
        s_odd = len(steps)
        steps += [(j, 1, tl, t, ts) for tl, ts in sweeps[1] for t in ts]
        info.append(dict(s0=s0, s_odd=s_odd, s_end=len(steps),
                         s_tail=len(steps) - len(sweeps[1][-1][1])))
    t_step = [0.0]
    for (_, _, tl, t, _) in steps:
        t_step.append(t_step[-1] + CU * tl[1] * (6 if t < ntb else 4))
    gates, stores, env = {}, {}, {}
    cur = dict(state=None, st=-1, nedge=0, edge=False, p_head=[0, None])

    def get_inv(h):
        return inv_sum(l_buf[zq + (h & 3)])

    def step_at(cyc):
        return next((i for i, tt_ in enumerate(t_step) if tt_ >= cyc), len(t_step))

    def gate(cyc, v):
        st = step_at(cyc)
        while len(gates.get(st, ())) >= 2:
            st += 1
        if cur['st'] < st < len(steps) - NGT:
            gates.setdefault(st, []).append(v)

    def edge(x, n=BE, force=False):
        if cur['st'] < 0 or not (force or cur['edge']):
            return x
        accs = cur['state']['accs']
        cand = [(e_, a) for e_ in range(2) for a in range(accs[0].shape[0])]
        ntile = -(-x.shape[1] // 128)
        parts = [x[:, 128 * i:min(128 * (i + 1), x.shape[1])] for i in range(ntile)]
        for k in range(min(n, 3 * ntile)):
            ce, ca = cand[cur['nedge'] % len(cand)]
            cur['nedge'] += 1
            i = k % ntile
            w_ = parts[i].shape[1]
            parts[i] = jnp.where(true_mask[k // ntile][:, 0:w_], parts[i],
                                 pltpu.bitcast(accs[ce][ca], U32)[:, 0:w_])
        return parts[0] if ntile == 1 else jnp.concatenate(parts, axis=1)

    def sched_stores(ps, lsum, h, t_ready, lo, hi, l_off=10):
        gate(t_ready, ps[-1])
        st_l = min(max(step_at(t_ready + l_off), cur['st'] + 1), len(steps) - 1)
        stores.setdefault(st_l, []).append((lsum, h, None, None))
        t_first = max(t_ready, t_step[lo])
        for i in range(2 * ng):
            g, k = divmod(i, 2)
            st = min(max(step_at(t_first + SDT * i) + 1, cur['st'] + 1), hi)
            assert lo <= st <= hi
            stores.setdefault(st, []).append((ps[g], h, g, range(4 * k, 4 * k + 4)))

    def p_block(h, t):
        assert cur['p_head'][h & 1] == h and not any(
            s_[1] == h and s_[2] is not None for ss in stores.values() for s_ in ss)
        return p_bufs[h & 1][8 * t:8 * t + 8, :]

    def pair_jobs(j):
        inf = info[j]
        first, last = j == 0, j == NP - 1
        h0 = 2 * j

        def job_b(h, c, g):
            s_buf = (se_buf, so_buf)[h & 1]

            def fn(td):
                s = score2(edge(qv_buf[h & 3, c]), h, h & 1, 4 * g + c)
                env['s'] = s if c == 0 else env['s'] + s
                gate(td + LATP, env['s'])
                if c == 3:
                    s_buf[g] = env['s']
                if c == 3 and g == ng - 1:
                    sg_ = [s_buf[zq + gg] for gg in range(ng)]
                    if h == 1:
                        ps, lsum, c1 = softmax_lane(sg_)
                        c01_buf[...] = _pack(c0, c1)
                        sched_stores(ps, lsum, h, td + LATP + MOFL, inf['s0'], inf['s_odd'], 130)
                    elif h & 1:
                        ps, lsum = softmax(sg_)
                        sched_stores(ps, lsum, h, td + LATP + MOFF, inf['s0'], inf['s_odd'])
                        if not last:
                            store_q([qraw_buf[zq + i] for i in range(3)], j + 1)
                    else:
                        ps, lsum = softmax(sg_)
                        sched_stores(ps, lsum, h, td + LATP + MOFF2, inf['s_odd'],
                                     inf['s_end'] - 1)
            return fn

        def job_e(td):
            x = _dot_t(edge(c01_buf[...] if j == 1 else ones32), accp_buf[(j - 1) & 1])
            x = x + xo_buf[zq]

            def row(i, r):
                return jnp.broadcast_to(x[r:r + 1, 128 * i:128 * (i + 1)], (8, 128))

            ie, io = get_inv(h0 - 2), get_inv(h0 - 1)
            o = jnp.concatenate([row(0, 0) * ie, jnp.where(lo64, row(1, 0) * ie, row(1, 1) * io),
                                 row(2, 1) * io], axis=1)
            gate(td + LATP + 10, o[:, 256:384])
            op_buf[...] = _pack(o, o)

        def job_g(c):
            def fn(td):
                xo = out_cols(edge(op_buf[...]), 24 * (j - 1), 24, c)
                xacc_buf[:, 128 * c:128 * (c + 1)] += xo
                gate(td + LATP, xo)
            return fn

        def job_a(c):
            def fn(td):
                qc = q_cols(edge(z_buf[...]), j + 2, c)
                gate(td + LATP, qc)
                qraw_buf[c] = qc
            return fn

        def job_xp(t):
            def fn(td):
                pe, po = p_block(h0, t), p_block(h0 + 1, t)
                if first:
                    ce, co = _unpack(c01_buf[...])
                    pe, po = pe * ce, po * co
                lhs = edge(_pack(pe, po))
                o = jnp.concatenate([_dot(lhs, _bf(v_tiles(h0, 8 * ct, 8, t).reshape(64, 128)))
                                     for ct in range(3)], axis=1)
                env['xp'] = o if t == 0 else env['xp'] + o
                gate(td + LATP + 20, env['xp'][:, 256:384])
                if t == XM - 1:
                    xo_buf[0] = env['xp']
            return fn

        def job_x(par, t, tiles, key):
            def fn(td):
                p = p_block(h0 + par, t)
                rhs = v_tiles(h0 + par, tiles[0], tiles[1], t).reshape(8 * tiles[1], 128)
                o = _dot_t(edge(_pack(p, p)), rhs)
                env[key] = o if key not in env else env[key] + o
                gate(td + LATP, env[key][:, 0:128] if tiles[1] >= 8 else
                     jnp.concatenate([env[key], env[key]], axis=1))
            return fn

        def finish(par, a0, a1, key):
            r0 = par * (DH // 2)
            o = _dot_t(edge(ones32), accp_buf[j & 1, r0 + 8 * a0:r0 + 8 * a1, :]) + env[key]
            inv = get_inv(h0 + par)
            n = 16 * (a1 - a0)
            return o * (inv[:, 0:n] if n <= 128 else
                        jnp.concatenate([inv, inv[:, 0:n - 128]], axis=1))

        env['finish'] = finish

        def job_fin(par, a0, a1, key):
            def fn(td):
                o = finish(par, a0, a1, key)
                gate(td + LATP + 10, o[:, 0:128])
                env['op' + key] = _pack(o, o)
            return fn

        def job_gfin(c):
            def fn(td):
                xo = out_cols(edge(env['opx0']), 12 * h0, 12, c)
                xacc_buf[:, 128 * c:128 * (c + 1)] += xo
                gate(td + LATP, xo)
            return fn

        t_odd = t_step[inf['s_odd'] + 1]
        jobs = [(24, None, job_b(h0 + 1, c, g))
                for g in range(0 if first else ng // 2, ng) for c in range(4)]
        if not first:
            jobs += [(48, t_step[inf['s0']] + EDEL, job_e)]
        out_jobs = [] if first else [(24, None, job_g(c)) for c in range(5)]
        if last:
            t_tail = t_step[inf['s_tail'] + 1]
            jobs += [(24, None, job_x(0, t, (0, 12), 'x0')) for t in range(XE)]
            jobs += out_jobs
            jobs += [(32, t_odd, job_fin(0, 0, 12, 'x0'))]
            jobs += [(16, None, job_x(1, t, (0, 8), 'x1a')) for t in range(XO)]
            jobs += [(12, t_odd + LATP + 60, job_gfin(c)) for c in range(5)]
            jobs += [(8, None, job_x(1, t, (8, 4), 'x1b')) for t in range(XB1)]
            jobs += [(16, t_tail, job_fin(1, 0, 8, 'x1a'))]
            jobs += [(8, None, job_x(1, t, (8, 4), 'x1b')) for t in range(XB1, XB)]
        else:
            jobs += [(24, None, job_b(h0 + 2, c, g)) for g in range(ng) for c in range(4)]
            jobs += [(24, t_odd, job_xp(t)) for t in range(XM)]
            if j + 2 < NP:
                jobs += [(40, None, job_a(c)) for c in range(3)]
            jobs += out_jobs
            jobs += [(24, None, job_b(h0 + 3, c, g)) for g in range(ng // 2) for c in range(4)]
        return jobs

    jobs, times = [], []
    tt = T0
    for j in range(NP):
        if j > 0:
            tt = max(tt, t_step[info[j]['s0']] - LEAD)
        for job in pair_jobs(j):
            tt = tt + job[0] if job[1] is None else max(tt + job[0], job[1])
            jobs.append(job)
            times.append(tt)
    j_first = next(i for i, tt_ in enumerate(times) if tt_ > 0)

    nj = 0
    for st, (j, par, tl, t, ts) in enumerate(steps):
        while nj < len(jobs) and times[nj] <= t_step[st]:
            rel = nj - j_first
            cur['edge'] = (0 <= rel < NE and rel % 2 == 1) or jobs[nj][1] == times[nj]
            jobs[nj][2](times[nj])
            nj += 1
        for val, h, g, rs in stores.pop(st, ()):
            val = pltpu.bitcast(edge(pltpu.bitcast(val, U32), 1, True), F32)
            if g is None:
                l_buf[h & 3] = val
            else:
                store_p(val, g, rs, p_bufs[h & 1])
                cur['p_head'][h & 1] = h
        if st in (info[j]['s0'], info[j]['s_odd']):
            state = dict(par=par, slot=j & 1)
        assert cur['p_head'][par] == 2 * j + par
        pv_step(2 * j + par, tl, t, ts, zip(true_mask, gates.get(st, ())), state)
        cur['state'] = state
        cur['st'] = st
    cur['edge'] = False
    for job, tt in zip(jobs[nj:], times[nj:]):
        job[2](tt)
    assert not stores

    o = env['finish'](1, 8, 12, 'x1b')
    op = _pack(o, o)
    xa = [out_cols(env['opx1a'], 12 * (H - 1), 8, c) for c in range(5)]
    xb = [out_cols(op, 12 * (H - 1) + 8, 4, c) for c in range(5)]
    x3 = (xacc_buf[...] + jnp.concatenate(xa, axis=1)) + jnp.concatenate(xb, axis=1)
    x4 = x3 + b2 + _dot(mlp_hidden(x3, shift), w2_buf[...])
    o_ref[...] = x4[0:1, :].astype(o_ref.dtype)


@jax.jit
def pallas_interleave_layers__sliding_block_cached__dense_activation_gelu__decode_kernel(
    A_x: jax.Array,
    A_k_cache: jax.Array,
    A_v_cache: jax.Array,
    A_wq: jax.Array,
    A_wo: jax.Array,
    B_x: jax.Array,
    B_w1: jax.Array,
    B_b1: jax.Array,
    B_w2: jax.Array,
    B_b2: jax.Array,
):
    sk = A_k_cache.shape[2]
    w = min(4096, max(256, sk // 4))
    ng = w // 1024

    def tile_view(a):
        *lead, r, c = a.shape
        n = len(lead)
        a = a.reshape(*lead, r // 8, 8, c // 128, 128)
        a = a.transpose(*range(n), n, n + 2, n + 1, n + 3)
        return a.reshape(*lead, r // 16, 2, (c // 128) * 8, 128)

    kx = tile_view(jnp.swapaxes(A_k_cache, 2, 3)[0]).reshape(H * DH // 16, 2, sk // 16, 128)
    vx = tile_view(jnp.swapaxes(A_v_cache, 2, 3)[0]).reshape(H * DH // 16, 2, sk // 16, 128)
    wqx = tile_view(A_wq)
    wox = tile_view(A_wo).reshape(H * DH // 16, 80, 128)
    out = pl.pallas_call(
        functools.partial(_kernel, sk=sk, w=w),
        out_shape=jax.ShapeDtypeStruct((1, D), A_x.dtype),
        in_specs=[pl.BlockSpec(memory_space=pl.ANY)] * 9,
        out_specs=pl.BlockSpec(memory_space=pltpu.VMEM),
        scratch_shapes=[
            pltpu.VMEM((H * DH // 16, 2, w // 32, 128), U32),
            pltpu.VMEM((H * DH // 16, 2, w // 32 - 4 * XF, 128), U32),
            pltpu.VMEM((H * DH // 16, 2, 8 * XF, 128), U32),
            pltpu.VMEM((D // 16, 2, H * DH // 32, 128), U32),
            pltpu.VMEM((H * DH // 16, 40, 128), U32),
            pltpu.VMEM((D, F), BF16),
            pltpu.VMEM((F, D), BF16),
            pltpu.VMEM((1, D), BF16),
            pltpu.VMEM((F // 128, 128), BF16),
            pltpu.VMEM((D // 128, 128), BF16),
            pltpu.VMEM((w // 16, 128), F32),
            pltpu.VMEM((w // 16, 128), F32),
            pltpu.VMEM((ng + 1, 8, 128), F32),
            pltpu.VMEM((ng + 1, 8, 128), F32),
            pltpu.VMEM((5, 8, 128), F32),
            pltpu.VMEM((4, 8, 128), F32),
            pltpu.VMEM((2, 8, 2 * DH), F32),
            pltpu.VMEM((2, DH, 128), U32),
            pltpu.VMEM((8, D), U32),
            pltpu.VMEM((8, D), F32),
            pltpu.VMEM((4, 4, 8, 2 * DH), U32),
            pltpu.VMEM((3 * NP + 3, 8, 128), F32),
            pltpu.VMEM((8, F), F32),
            pltpu.VMEM((2, 8, 128), F32),
            pltpu.VMEM((8, 2 * DH), U32),
            pltpu.VMEM((3, D // 16, 8, 128), U32),
            pltpu.VMEM((8, 128), U32),
            pltpu.VMEM((3, 8, 128), jnp.int32),
            pltpu.SMEM((1,), jnp.int32),
            pltpu.SemaphoreType.DMA((2,)),
            pltpu.SemaphoreType.DMA((4,)),
            pltpu.SemaphoreType.DMA((6 + len(W2_ROWS),)),
        ],
        compiler_params=pltpu.CompilerParams(vmem_limit_bytes=127 * 1024 * 1024,
                                             disable_semaphore_checks=True),
    )(A_x.reshape(1, D), kx, vx, wqx, wox, B_w1, B_b1.reshape(F // 128, 128),
      B_w2, B_b2.reshape(D // 128, 128))
    return out.reshape(A_x.shape)
```

```python
import functools
import math

import jax
import jax.numpy as jnp
from jax import lax
import jax.experimental.pallas as pl
import jax.experimental.pallas.tpu as pltpu

F32 = jnp.float32
BF16 = jnp.bfloat16
U32 = jnp.uint32

D = 640
H = 32
DH = 192
F = 1536
EPS = 1e-5
NP = H // 2

CHUNKS = (4, 4, 3, 2, 2, 1)
W2_ROWS = (640, 512, 256, 128)
NS = 4
XF = 6
XM = 1
XE, XO, XB, XB1 = 7, 7, 16, 6

CU = 0.263
T0 = -100.0
LEAD = 100.0
LATP = 160.0
MOFF, MOFF2, MOFL = 160.0, 240.0, 60.0
EDEL = 70.0
SDT = 12.0
NE, BE, NGT = 7, 6, 12


def _gelu(x):
    c = math.sqrt(2.0 / math.pi)
    return 0.5 * x * (1.0 + jnp.tanh(c * (x + 0.044715 * (x * x * x))))


def _rows_to_lanes(b, n):
    return jnp.concatenate([b[i:i + 1, :] for i in range(n)], axis=1)


def _bf(x):
    return pltpu.bitcast(x, BF16)


def _pack(a, b):
    return pltpu.bitcast(pltpu.pack_elementwise([a, b], packed_dtype=BF16), U32)


def _unpack(x):
    return (pltpu.unpack_elementwise(x, index=0, packed_dtype=BF16, unpacked_dtype=F32),
            pltpu.unpack_elementwise(x, index=1, packed_dtype=BF16, unpacked_dtype=F32))


def _dot(lhs32, rhs):
    return jnp.dot(_bf(lhs32), rhs, preferred_element_type=F32)[0:8]


def _dot_t(lhs32, rhs32):
    return lax.dot_general(_bf(lhs32), _bf(rhs32), (((1,), (1,)), ((), ())),
                           preferred_element_type=F32)[0:8]


def _mean(x):
    return jnp.mean(x, axis=-1, keepdims=True)


def _ln_stats(xp, shift):
    x = _unpack(xp)[0] - shift
    m = _mean(x)
    v = jnp.maximum(_mean(x * x) - m * m, 0.0)
    return m + shift, lax.rsqrt(v + EPS)


def _kernel(x_hbm, kx_hbm, vx_hbm, wq_hbm, wo_hbm, w1_hbm, b1_hbm, w2_hbm, b2_hbm,
            o_ref,
            kbuf, vbuf, vf_buf, wq_buf, wo_buf, w1_buf, w2_buf, x_buf, b1_buf, b2_buf,
            p_buf0, p_buf1, so_buf, se_buf, l_buf, qraw_buf, xo_buf, accp_buf, z_buf,
            xacc_buf, qw_buf, csq_buf, cs1_buf, st_buf, op_buf, wx_buf, c01_buf,
            tm_buf, zero_ref, sem_k, sem_v, sem_w, *, sk, w):
    c_scale = (DH ** -0.5) * math.log2(math.e)
    nt = w // 128
    ng = nt // 8
    na = 12 // NS
    ntb = nt - XF
    r0w = (sk - w) // 16
    p_bufs = (p_buf0, p_buf1)
    starts = [sum(CHUNKS[:c]) for c in range(len(CHUNKS))]
    w2_at = [sum(W2_ROWS[:i]) for i in range(len(W2_ROWS))]

    def k_copy(c):
        rows = pl.ds(24 * starts[c], 24 * CHUNKS[c])
        return [pltpu.make_async_copy(kx_hbm.at[rows, :, pl.ds(r0w, 8 * nt), :],
                                      kbuf.bitcast(BF16).at[rows], sem_k.at[c & 1])]

    def v_copy(c):
        rows = pl.ds(24 * starts[c], 24 * CHUNKS[c])
        return [pltpu.make_async_copy(vx_hbm.at[rows, :, pl.ds(r0w, 8 * ntb), :],
                                      vbuf.bitcast(BF16).at[rows], sem_v.at[c & 1]),
                pltpu.make_async_copy(vx_hbm.at[rows, :, pl.ds(r0w + 8 * ntb, 8 * XF), :],
                                      vf_buf.bitcast(BF16).at[rows, :, pl.ds(8 * XF, 8 * XF), :],
                                      sem_v.at[2 + (c & 1)])]

    wq_cp = pltpu.make_async_copy(wq_hbm, wq_buf.bitcast(BF16), sem_w.at[0])
    wo_cp = pltpu.make_async_copy(wo_hbm, wo_buf.bitcast(BF16), sem_w.at[1])
    w1_cp = pltpu.make_async_copy(w1_hbm, w1_buf, sem_w.at[2])
    x_cp = pltpu.make_async_copy(x_hbm, x_buf, sem_w.at[3])
    b1_cp = pltpu.make_async_copy(b1_hbm, b1_buf, sem_w.at[4])
    b2_cp = pltpu.make_async_copy(b2_hbm, b2_buf, sem_w.at[5])
    w2_cps = [pltpu.make_async_copy(w2_hbm.at[pl.ds(r, n), :], w2_buf.at[pl.ds(r, n), :],
                                    sem_w.at[6 + i])
              for i, (r, n) in enumerate(zip(w2_at, W2_ROWS))]

    for cp in [wq_cp, x_cp, b1_cp, b2_cp, wo_cp] + k_copy(0) + v_copy(0):
        cp.start()
    x_cp.wait()
    b1_cp.wait()
    b2_cp.wait()

    x0 = jnp.broadcast_to(x_buf[...].astype(F32), (8, D))
    b1 = _rows_to_lanes(b1_buf[...].astype(F32), F // 128)
    b2 = _rows_to_lanes(b2_buf[...].astype(F32), D // 128)

    lane = lax.broadcasted_iota(jnp.int32, (8, 128), 1)
    sub3 = lax.broadcasted_iota(jnp.int32, (8, 2 * DH), 0)
    sub_lo = lax.broadcasted_iota(jnp.int32, (1, 8, 128), 1) < 4
    lo64 = lane < 64
    evn = (lane & 8) == 0
    zf = jnp.zeros((8, 128), F32)
    ones32 = jnp.full((8, 128), 0x3F803F80, U32)
    k_order = (((0, 8, 0), (0, 8, 1), (8, 4, 0), (8, 4, 1)),
               ((4, 8, 0), (4, 8, 1), (0, 4, 1), (0, 4, 0)))

    def regroup(a, b):
        return jnp.where(sub_lo, a, pltpu.roll(b, 4, 1)), jnp.where(sub_lo, pltpu.roll(a, 4, 1), b)

    def swap_halves(ref2):
        n = ref2.shape[1]
        a, b = regroup(ref2[0].reshape(n // 8, 8, 128), ref2[1].reshape(n // 8, 8, 128))
        ref2[0] = a.reshape(n, 128)
        ref2[1] = b.reshape(n, 128)

    def fix_wq(a, carry):
        swap_halves(wq_buf.at[a])
        return carry

    def fix_wo(g8, carry):
        g0 = pl.multiple_of(g8 * 8, 8)
        v = [wo_buf[pl.ds(g0, 8), 8 * c:8 * c + 8, :] for c in range(5)]
        n = [jnp.where(sub_lo, v[0], v[2]),
             pltpu.roll(jnp.where(sub_lo, v[3], v[0]), 4, 1),
             jnp.where(sub_lo, v[1], v[3]),
             pltpu.roll(jnp.where(sub_lo, v[4], v[1]), 4, 1),
             jnp.where(sub_lo, v[2], v[4])]
        for c in range(5):
            wo_buf[pl.ds(g0, 8), 8 * c:8 * c + 8, :] = n[c]
        return carry

    def fix_v(r2, carry):
        swap_halves(vbuf.at[r2])
        n = 4 * XF
        t0, t1 = regroup(vf_buf[r2, 0, n:2 * n, :].reshape(n // 8, 8, 128),
                         vf_buf[r2, 1, n:2 * n, :].reshape(n // 8, 8, 128))
        t0, t1 = _unpack(t0), _unpack(t1)
        for e in range(2):
            for k in range(XF // 2):
                vf_buf[r2, e, 16 * k:16 * k + 8, :] = pltpu.bitcast(t0[e][k], U32)
                vf_buf[r2, e, 16 * k + 8:16 * k + 16, :] = pltpu.bitcast(t1[e][k], U32)
        return carry

    def v_tiles(h, a0, n, t):
        return vbuf[pl.ds(12 * h + a0, n), t % 2, 8 * (t // 2):8 * (t // 2) + 8, :]

    def transpose_v(j, t):
        y = _bf(v_tiles(2 * j, 0, 24, t).reshape(DH, 128)).astype(F32)
        yt = pltpu.bitcast(y.T.astype(BF16), U32)
        for ct in range(3):
            vbuf[pl.ds(24 * j + 8 * ct, 8), t % 2, 8 * (t // 2):8 * (t // 2) + 8, :] = (
                yt[:, 128 * ct:128 * (ct + 1)].reshape(8, 8, 128))

    def set_row(x, shift):
        xp = _pack(x, x)
        z_buf[...] = xp
        m, r = _ln_stats(xp, shift)
        rc = r * c_scale
        st_buf[0] = jnp.broadcast_to(rc, (8, 128))
        st_buf[1] = jnp.broadcast_to(m * rc, (8, 128))

    def wq_cols(ct):
        if isinstance(ct, int):
            r0 = (ct // 2) * 8
        else:
            r0 = pl.multiple_of(lax.shift_right_logical(ct, 1) * 8, 8)
        return _bf(wq_buf[:, ct & 1, pl.ds(r0, 8), :].reshape(D // 2, 128))

    def q_cols(z, j, c):
        ct = 3 * j + c
        return _dot(z, wq_cols(ct)) * st_buf[0] - csq_buf[ct] * st_buf[1]

    def store_q(qs, j, pars=(0, 1)):
        q0, q1, q2 = qs
        r56, r64, r8 = (pltpu.roll(q1, s, 1) for s in (56, 64, 8))

        def put(h, qf, a2, b2):
            a0 = jnp.where(evn, qf, zf)
            b1_ = jnp.where(evn, zf, qf)
            ww = [_pack(a0, pltpu.roll(a0, 8, 1)), _pack(pltpu.roll(b1_, 120, 1), b1_),
                  _pack(jnp.where(evn, a2, zf), jnp.where(evn, zf, b2))]
            qw_buf[h & 3] = jnp.concatenate(ww, axis=1)

        if 0 in pars:
            put(2 * j, q0, jnp.where(lo64, q1, r56), jnp.where(lo64, r8, r64))
        if 1 in pars:
            put(2 * j + 1, q2, jnp.where(lo64, r56, q1), jnp.where(lo64, r64, r8))

    def q_pair(j):
        z = z_buf[...]
        store_q([q_cols(z, j, c) for c in range(3)], j)

    def score2(lhs, h, par, k):
        lhs = jnp.where(sub3 == k % 4, lhs, jnp.zeros_like(lhs))
        rhs = jnp.concatenate([kbuf[pl.ds(12 * h + a, n), e, 8 * k:8 * k + 8, :]
                               for a, n, e in k_order[par]], axis=0)
        return _dot(lhs, _bf(rhs.reshape(DH, 128)))

    def store_p(p, g, rs, p_out):
        for r in rs:
            p_out[pl.ds(64 * g + r, 8, stride=8), :] = p

    def inv_sum(l):
        l = jnp.sum(jnp.sum(l, axis=1, keepdims=True), axis=0, keepdims=True)
        l = jnp.broadcast_to(l, (8, 128))
        r = pl.reciprocal(l, approx=True)
        return r * (2.0 - l * r)

    def softmax(sg):
        mx = sg[0]
        for s in sg[1:]:
            mx = jnp.maximum(mx, s)
        m = jnp.max(jnp.max(mx, axis=1, keepdims=True), axis=0, keepdims=True)
        ps, l = [], None
        for s in sg:
            ps.append(jnp.exp2(s - m))
            l = ps[-1] if l is None else l + ps[-1]
        return ps, l

    def softmax_lane(sg):
        mx = jnp.maximum(jnp.maximum(sg[0], sg[1]), jnp.maximum(sg[2], sg[3]))
        m = jnp.broadcast_to(jnp.max(mx, axis=0, keepdims=True), (8, 128))
        ps = [jnp.exp2(s - m) for s in sg]
        c = jnp.exp2(m - jnp.max(m, axis=1, keepdims=True))
        c = _unpack(_pack(c, c))[0]
        return ps, ((ps[0] + ps[1]) + (ps[2] + ps[3])) * c, c

    def pv_step(h, tiles, t, ts, gated, state):
        a0, n = tiles
        p = p_bufs[state['par']][8 * t:8 * t + 8, :]
        for mask, val in gated:
            p = jnp.where(mask, p, val)
        if t < ntb:
            ys = _unpack(v_tiles(h, a0, n, t))
        else:
            r = 8 * (t - ntb)
            ys = [pltpu.bitcast(vf_buf[pl.ds(12 * h + a0, n), e, r:r + 8, :], F32)
                  for e in range(2)]
        if t == ts[0]:
            state['accs'] = [y * p for y in ys]
        else:
            state['accs'] = [acc + y * p for acc, y in zip(state['accs'], ys)]
        if t == ts[-1]:
            r0 = state['par'] * (DH // 2) + 8 * a0
            accp_buf[state['slot'], r0:r0 + 8 * n, :] = _pack(*state['accs']).reshape(8 * n, 128)

    def out_cols(op, g0, ngrp, c):
        rhs = wo_buf[pl.ds(g0, ngrp), 8 * c:8 * c + 8, :].reshape(ngrp * 8, 128)
        return _dot(op, _bf(rhs))

    def mlp_hidden(x, shift):
        xp = _pack(x, x)
        m, r = _ln_stats(xp, shift)
        g = _gelu((_dot(xp, w1_buf[...]) - cs1_buf[...] * m) * r + b1)
        return _pack(g, g)

    def next_copies(j, copy_fn, tail_cps):
        for c in range(len(CHUNKS)):
            @pl.when(j == starts[c])
            def _():
                for cp in copy_fn(c):
                    cp.wait()
                for cp in (copy_fn(c + 1) if c + 1 < len(CHUNKS) else tail_cps):
                    cp.start()

    def pair1(j, carry):
        q_pair(j)
        next_copies(j, k_copy, [w1_cp])
        invs = []
        for par in range(2):
            h = 2 * j + par
            sg = [None] * ng
            lhs = qw_buf[h & 3]
            for c in range(4):
                for g in range(ng):
                    s = score2(lhs, h, par, 4 * g + c)
                    sg[g] = s if c == 0 else sg[g] + s
            ps, l = softmax(sg)
            for g in range(ng):
                store_p(ps[g], g, range(8), p_bufs[par])
            invs.append(inv_sum(l))
        next_copies(j, v_copy, w2_cps)
        lax.fori_loop(24 * j, 24 * (j + 1), fix_v, 0)
        for par in range(2):
            state = dict(par=par, slot=0)
            for sw in range(NS):
                for t in range(nt):
                    pv_step(2 * j + par, (sw * na, na), t, range(nt), (), state)

        @pl.when(j < NP - 1)
        def _():
            for t in range(XM):
                transpose_v(j, t)

        ie, io = invs
        o = _dot_t(ones32, accp_buf[0]) * jnp.concatenate([ie, jnp.where(lo64, ie, io), io], axis=1)
        op = _pack(o, o)
        for c in range(5):
            xacc_buf[:, 128 * c:128 * (c + 1)] += out_cols(op, 24 * j, 24, c)
        return carry

    def expand(t0, t1):
        return [jnp.where(evn, t0, pltpu.roll(t0, 8, 1)),
                jnp.where(evn, pltpu.roll(t0, 120, 1), t0),
                jnp.where(evn, jnp.where(lo64, t1, pltpu.roll(t1, 56, 1)),
                          jnp.where(lo64, pltpu.roll(t1, 8, 1), pltpu.roll(t1, 64, 1)))]

    def expand_wq(a, carry):
        e = expand(wq_buf[a, 0, 0:8, :], wq_buf[a, 1, 0:8, :])
        for i in range(3):
            wx_buf[i, a] = e[i]
        return carry

    ones_row = jnp.concatenate([ones32] * (D // 128), axis=1)

    def colsum_q(ct, carry):
        csq_buf[ct] = _dot(ones_row, wq_cols(ct))
        return carry

    for ref in (so_buf, se_buf, l_buf, qraw_buf, xo_buf):
        ref[...] = jnp.zeros(ref.shape, ref.dtype)
    for i in range(3):
        tm_buf[i] = lane
    zero_ref[0] = 0

    set_row(x0, _mean(x0))
    xacc_buf[...] = x0
    wq_cp.wait()
    lax.fori_loop(0, D // 16, fix_wq, 0)
    lax.fori_loop(0, 3 * NP, colsum_q, 0)
    lax.fori_loop(0, D // 16, expand_wq, 0)
    e = expand(csq_buf[0], csq_buf[1])
    for i in range(3):
        csq_buf[3 * NP + i] = e[i]
    wo_cp.wait()
    lax.fori_loop(0, H * DH // 128, fix_wo, 0)
    lax.fori_loop(0, NP, pair1, 0)
    x1 = xacc_buf[...]
    w1_cp.wait()
    cs1_buf[...] = _dot(ones_row, w1_buf[...])
    gp = mlp_hidden(x1, _mean(x1))
    x2 = x1 + b2
    for cp, r, n in zip(w2_cps, w2_at, W2_ROWS):
        shift = _mean(x2) if cp is w2_cps[-1] else None
        cp.wait()
        x2 = x2 + _dot(gp[:, r:r + n], w2_buf[r:r + n, :])

    set_row(x2, shift)
    xacc_buf[...] = x2
    z = z_buf[...]
    qx = [_dot(z, _bf(wx_buf[i].reshape(D // 2, 128))) * st_buf[0]
          - csq_buf[3 * NP + i] * st_buf[1] for i in range(3)]
    w0 = jnp.concatenate([_pack(jnp.where(evn, q_, zf), jnp.where(evn, zf, q_)) for q_ in qx],
                         axis=1)
    store_q([None, q_cols(z, 0, 1), q_cols(z, 0, 2)], 0, pars=(1,))
    sg = [None] * ng
    for g in range(ng):
        for c in range(4):
            s = score2(w0, 0, 0, 4 * g + c)
            sg[g] = s if c == 0 else sg[g] + s
    q_pair(1)
    ps0, l0, c0 = softmax_lane(sg)
    for g in range(ng):
        store_p(ps0[g], g, range(8), p_buf0)
    l_buf[0] = l0

    true_mask = [tm_buf[i] >= 0 for i in range(3)]
    zq = jnp.clip(zero_ref[0], 0, 1)
    std = [(sw * na, na) for sw in range(NS)]
    steps, info = [], []
    for j in range(NP):
        if j == NP - 1:
            sweeps = [[(tl, range(XE, nt)) for tl in std],
                      [((5, 3), range(XO, nt)), ((2, 3), range(XO, nt)),
                       ((0, 2), range(XO, nt)), ((8, 4), range(XB, nt))]]
        else:
            sweeps = [[(tl, range(XM, nt)) for tl in std]] * 2
        s0 = len(steps)
        steps += [(j, 0, tl, t, ts) for tl, ts in sweeps[0] for t in ts]
        s_odd = len(steps)
        steps += [(j, 1, tl, t, ts) for tl, ts in sweeps[1] for t in ts]
        info.append(dict(s0=s0, s_odd=s_odd, s_end=len(steps),
                         s_tail=len(steps) - len(sweeps[1][-1][1])))
    t_step = [0.0]
    for (_, _, tl, t, _) in steps:
        t_step.append(t_step[-1] + CU * tl[1] * (6 if t < ntb else 4))
    gates, stores, env = {}, {}, {}
    cur = dict(state=None, st=-1, nedge=0, edge=False, p_head=[0, None])

    def get_inv(h):
        return inv_sum(l_buf[zq + (h & 3)])

    def step_at(cyc):
        return next((i for i, tt_ in enumerate(t_step) if tt_ >= cyc), len(t_step))

    def gate(cyc, v):
        st = step_at(cyc)
        while len(gates.get(st, ())) >= 2:
            st += 1
        if cur['st'] < st < len(steps) - NGT:
            gates.setdefault(st, []).append(v)

    def edge(x, n=BE, force=False):
        if cur['st'] < 0 or not (force or cur['edge']):
            return x
        accs = cur['state']['accs']
        cand = [(e_, a) for e_ in range(2) for a in range(accs[0].shape[0])]
        ntile = -(-x.shape[1] // 128)
        parts = [x[:, 128 * i:min(128 * (i + 1), x.shape[1])] for i in range(ntile)]
        for k in range(min(n, 3 * ntile)):
            ce, ca = cand[cur['nedge'] % len(cand)]
            cur['nedge'] += 1
            i = k % ntile
            w_ = parts[i].shape[1]
            parts[i] = jnp.where(true_mask[k // ntile][:, 0:w_], parts[i],
                                 pltpu.bitcast(accs[ce][ca], U32)[:, 0:w_])
        return parts[0] if ntile == 1 else jnp.concatenate(parts, axis=1)

    def sched_stores(ps, lsum, h, t_ready, lo, hi, l_off=10):
        gate(t_ready, ps[-1])
        st_l = min(max(step_at(t_ready + l_off), cur['st'] + 1), len(steps) - 1)
        stores.setdefault(st_l, []).append((lsum, h, None, None))
        t_first = max(t_ready, t_step[lo])
        for i in range(2 * ng):
            g, k = divmod(i, 2)
            st = min(max(step_at(t_first + SDT * i) + 1, cur['st'] + 1), hi)
            assert lo <= st <= hi
            stores.setdefault(st, []).append((ps[g], h, g, range(4 * k, 4 * k + 4)))

    def p_block(h, t):
        assert cur['p_head'][h & 1] == h and not any(
            s_[1] == h and s_[2] is not None for ss in stores.values() for s_ in ss)
        return p_bufs[h & 1][8 * t:8 * t + 8, :]

    def pair_jobs(j):
        inf = info[j]
        first, last = j == 0, j == NP - 1
        h0 = 2 * j

        def job_b(h, c, g):
            s_buf = (se_buf, so_buf)[h & 1]

            def fn(td):
                s = score2(edge(qw_buf[h & 3]), h, h & 1, 4 * g + c)
                env['s'] = s if c == 0 else env['s'] + s
                gate(td + LATP, env['s'])
                if c == 3:
                    s_buf[g] = env['s']
                if c == 3 and g == ng - 1:
                    sg_ = [s_buf[zq + gg] for gg in range(ng)]
                    if h == 1:
                        ps, lsum, c1 = softmax_lane(sg_)
                        c01_buf[...] = _pack(c0, c1)
                        sched_stores(ps, lsum, h, td + LATP + MOFL, inf['s0'], inf['s_odd'], 130)
                    elif h & 1:
                        ps, lsum = softmax(sg_)
                        sched_stores(ps, lsum, h, td + LATP + MOFF, inf['s0'], inf['s_odd'])
                        if not last:
                            store_q([qraw_buf[zq + i] for i in range(3)], j + 1)
                    else:
                        ps, lsum = softmax(sg_)
                        sched_stores(ps, lsum, h, td + LATP + MOFF2, inf['s_odd'],
                                     inf['s_end'] - 1)
            return fn

        def job_e(td):
            x = _dot_t(edge(c01_buf[...] if j == 1 else ones32), accp_buf[(j - 1) & 1])
            x = x + xo_buf[zq]

            def row(i, r):
                return jnp.broadcast_to(x[r:r + 1, 128 * i:128 * (i + 1)], (8, 128))

            ie, io = get_inv(h0 - 2), get_inv(h0 - 1)
            o = jnp.concatenate([row(0, 0) * ie, jnp.where(lo64, row(1, 0) * ie, row(1, 1) * io),
                                 row(2, 1) * io], axis=1)
            gate(td + LATP + 10, o[:, 256:384])
            op_buf[...] = _pack(o, o)

        def job_g(c):
            def fn(td):
                xo = out_cols(edge(op_buf[...]), 24 * (j - 1), 24, c)
                xacc_buf[:, 128 * c:128 * (c + 1)] += xo
                gate(td + LATP, xo)
            return fn

        def job_a(c):
            def fn(td):
                qc = q_cols(edge(z_buf[...]), j + 2, c)
                gate(td + LATP, qc)
                qraw_buf[c] = qc
            return fn

        def job_xp(t):
            def fn(td):
                pe, po = p_block(h0, t), p_block(h0 + 1, t)
                if first:
                    ce, co = _unpack(c01_buf[...])
                    pe, po = pe * ce, po * co
                lhs = edge(_pack(pe, po))
                o = jnp.concatenate([_dot(lhs, _bf(v_tiles(h0, 8 * ct, 8, t).reshape(64, 128)))
                                     for ct in range(3)], axis=1)
                env['xp'] = o if t == 0 else env['xp'] + o
                gate(td + LATP + 20, env['xp'][:, 256:384])
                if t == XM - 1:
                    xo_buf[0] = env['xp']
            return fn

        def job_x(par, t, tiles, key):
            def fn(td):
                p = p_block(h0 + par, t)
                rhs = v_tiles(h0 + par, tiles[0], tiles[1], t).reshape(8 * tiles[1], 128)
                o = _dot_t(edge(_pack(p, p)), rhs)
                env[key] = o if key not in env else env[key] + o
                gate(td + LATP, env[key][:, 0:128] if tiles[1] >= 8 else
                     jnp.concatenate([env[key], env[key]], axis=1))
            return fn

        def finish(par, a0, a1, key):
            r0 = par * (DH // 2)
            o = _dot_t(edge(ones32), accp_buf[j & 1, r0 + 8 * a0:r0 + 8 * a1, :]) + env[key]
            inv = get_inv(h0 + par)
            n = 16 * (a1 - a0)
            return o * (inv[:, 0:n] if n <= 128 else
                        jnp.concatenate([inv, inv[:, 0:n - 128]], axis=1))

        env['finish'] = finish

        def job_fin(par, a0, a1, key):
            def fn(td):
                o = finish(par, a0, a1, key)
                gate(td + LATP + 10, o[:, 0:128])
                env['op' + key] = _pack(o, o)
            return fn

        def job_gfin(c):
            def fn(td):
                xo = out_cols(edge(env['opx0']), 12 * h0, 12, c)
                xacc_buf[:, 128 * c:128 * (c + 1)] += xo
                gate(td + LATP, xo)
            return fn

        t_odd = t_step[inf['s_odd'] + 1]
        jobs = [(24, None, job_b(h0 + 1, c, g))
                for g in range(0 if first else ng // 2, ng) for c in range(4)]
        if not first:
            jobs += [(48, t_step[inf['s0']] + EDEL, job_e)]
        out_jobs = [] if first else [(24, None, job_g(c)) for c in range(5)]
        if last:
            t_tail = t_step[inf['s_tail'] + 1]
            jobs += [(24, None, job_x(0, t, (0, 12), 'x0')) for t in range(XE)]
            jobs += out_jobs
            jobs += [(32, t_odd, job_fin(0, 0, 12, 'x0'))]
            jobs += [(16, None, job_x(1, t, (0, 8), 'x1a')) for t in range(XO)]
            jobs += [(12, t_odd + LATP + 60, job_gfin(c)) for c in range(5)]
            jobs += [(8, None, job_x(1, t, (8, 4), 'x1b')) for t in range(XB1)]
            jobs += [(16, t_tail, job_fin(1, 0, 8, 'x1a'))]
            jobs += [(8, None, job_x(1, t, (8, 4), 'x1b')) for t in range(XB1, XB)]
        else:
            jobs += [(24, None, job_b(h0 + 2, c, g)) for g in range(ng) for c in range(4)]
            jobs += [(24, t_odd, job_xp(t)) for t in range(XM)]
            if j + 2 < NP:
                jobs += [(40, None, job_a(c)) for c in range(3)]
            jobs += out_jobs
            jobs += [(24, None, job_b(h0 + 3, c, g)) for g in range(ng // 2) for c in range(4)]
        return jobs

    jobs, times = [], []
    tt = T0
    for j in range(NP):
        if j > 0:
            tt = max(tt, t_step[info[j]['s0']] - LEAD)
        for job in pair_jobs(j):
            tt = tt + job[0] if job[1] is None else max(tt + job[0], job[1])
            jobs.append(job)
            times.append(tt)
    j_first = next(i for i, tt_ in enumerate(times) if tt_ > 0)

    nj = 0
    for st, (j, par, tl, t, ts) in enumerate(steps):
        while nj < len(jobs) and times[nj] <= t_step[st]:
            rel = nj - j_first
            cur['edge'] = (0 <= rel < NE and rel % 2 == 1) or jobs[nj][1] == times[nj]
            jobs[nj][2](times[nj])
            nj += 1
        for val, h, g, rs in stores.pop(st, ()):
            val = pltpu.bitcast(edge(pltpu.bitcast(val, U32), 1, True), F32)
            if g is None:
                l_buf[h & 3] = val
            else:
                store_p(val, g, rs, p_bufs[h & 1])
                cur['p_head'][h & 1] = h
        if st in (info[j]['s0'], info[j]['s_odd']):
            state = dict(par=par, slot=j & 1)
        assert cur['p_head'][par] == 2 * j + par
        pv_step(2 * j + par, tl, t, ts, zip(true_mask, gates.get(st, ())), state)
        cur['state'] = state
        cur['st'] = st
    cur['edge'] = False
    for job, tt in zip(jobs[nj:], times[nj:]):
        job[2](tt)
    assert not stores

    o = env['finish'](1, 8, 12, 'x1b')
    op = _pack(o, o)
    xa = [out_cols(env['opx1a'], 12 * (H - 1), 8, c) for c in range(5)]
    xb = [out_cols(op, 12 * (H - 1) + 8, 4, c) for c in range(5)]
    x3 = (xacc_buf[...] + jnp.concatenate(xa, axis=1)) + jnp.concatenate(xb, axis=1)
    x4 = x3 + b2 + _dot(mlp_hidden(x3, shift), w2_buf[...])
    o_ref[...] = x4[0:1, :].astype(o_ref.dtype)


@jax.jit
def pallas_interleave_layers__sliding_block_cached__dense_activation_gelu__decode_kernel(
    A_x: jax.Array,
    A_k_cache: jax.Array,
    A_v_cache: jax.Array,
    A_wq: jax.Array,
    A_wo: jax.Array,
    B_x: jax.Array,
    B_w1: jax.Array,
    B_b1: jax.Array,
    B_w2: jax.Array,
    B_b2: jax.Array,
):
    sk = A_k_cache.shape[2]
    w = min(4096, max(256, sk // 4))
    ng = w // 1024

    def tile_view(a):
        *lead, r, c = a.shape
        n = len(lead)
        a = a.reshape(*lead, r // 8, 8, c // 128, 128)
        a = a.transpose(*range(n), n, n + 2, n + 1, n + 3)
        return a.reshape(*lead, r // 16, 2, (c // 128) * 8, 128)

    kx = tile_view(jnp.swapaxes(A_k_cache, 2, 3)[0]).reshape(H * DH // 16, 2, sk // 16, 128)
    vx = tile_view(jnp.swapaxes(A_v_cache, 2, 3)[0]).reshape(H * DH // 16, 2, sk // 16, 128)
    wqx = tile_view(A_wq)
    wox = tile_view(A_wo).reshape(H * DH // 16, 80, 128)
    out = pl.pallas_call(
        functools.partial(_kernel, sk=sk, w=w),
        out_shape=jax.ShapeDtypeStruct((1, D), A_x.dtype),
        in_specs=[pl.BlockSpec(memory_space=pl.ANY)] * 9,
        out_specs=pl.BlockSpec(memory_space=pltpu.VMEM),
        scratch_shapes=[
            pltpu.VMEM((H * DH // 16, 2, w // 32, 128), U32),
            pltpu.VMEM((H * DH // 16, 2, w // 32 - 4 * XF, 128), U32),
            pltpu.VMEM((H * DH // 16, 2, 8 * XF, 128), U32),
            pltpu.VMEM((D // 16, 2, H * DH // 32, 128), U32),
            pltpu.VMEM((H * DH // 16, 40, 128), U32),
            pltpu.VMEM((D, F), BF16),
            pltpu.VMEM((F, D), BF16),
            pltpu.VMEM((1, D), BF16),
            pltpu.VMEM((F // 128, 128), BF16),
            pltpu.VMEM((D // 128, 128), BF16),
            pltpu.VMEM((w // 16, 128), F32),
            pltpu.VMEM((w // 16, 128), F32),
            pltpu.VMEM((ng + 1, 8, 128), F32),
            pltpu.VMEM((ng + 1, 8, 128), F32),
            pltpu.VMEM((5, 8, 128), F32),
            pltpu.VMEM((4, 8, 128), F32),
            pltpu.VMEM((2, 8, 2 * DH), F32),
            pltpu.VMEM((2, DH, 128), U32),
            pltpu.VMEM((8, D), U32),
            pltpu.VMEM((8, D), F32),
            pltpu.VMEM((4, 8, 2 * DH), U32),
            pltpu.VMEM((3 * NP + 3, 8, 128), F32),
            pltpu.VMEM((8, F), F32),
            pltpu.VMEM((2, 8, 128), F32),
            pltpu.VMEM((8, 2 * DH), U32),
            pltpu.VMEM((3, D // 16, 8, 128), U32),
            pltpu.VMEM((8, 128), U32),
            pltpu.VMEM((3, 8, 128), jnp.int32),
            pltpu.SMEM((1,), jnp.int32),
            pltpu.SemaphoreType.DMA((2,)),
            pltpu.SemaphoreType.DMA((4,)),
            pltpu.SemaphoreType.DMA((6 + len(W2_ROWS),)),
        ],
        compiler_params=pltpu.CompilerParams(vmem_limit_bytes=127 * 1024 * 1024,
                                             disable_semaphore_checks=True),
    )(A_x.reshape(1, D), kx, vx, wqx, wox, B_w1, B_b1.reshape(F // 128, 128),
      B_w2, B_b2.reshape(D // 128, 128))
    return out.reshape(A_x.shape)
```

```python
import functools
import math

import jax
import jax.numpy as jnp
from jax import lax
import jax.experimental.pallas as pl
import jax.experimental.pallas.tpu as pltpu

F32 = jnp.float32
BF16 = jnp.bfloat16
U32 = jnp.uint32

D = 640
H = 32
DH = 192
F = 1536
EPS = 1e-5
NP = H // 2

CHUNKS = (4, 4, 3, 2, 2, 1)
W2_ROWS = (640, 512, 256, 128)
NS = 4
XF = 6
XM = 1
XE, XO, XB, XB1 = 7, 7, 16, 6

CU = 0.263
T0 = -100.0
LEAD = 100.0
LATP = 160.0
MOFF, MOFF2, MOFL = 160.0, 240.0, 60.0
EDEL = 70.0
SDT = 12.0
NE, BE, NGT = 7, 6, 12
W2K = 128


def _gelu(x):
    c = math.sqrt(2.0 / math.pi)
    return 0.5 * x * (1.0 + jnp.tanh(c * (x + 0.044715 * (x * x * x))))


def _rows_to_lanes(b, n):
    return jnp.concatenate([b[i:i + 1, :] for i in range(n)], axis=1)


def _bf(x):
    return pltpu.bitcast(x, BF16)


def _pack(a, b):
    return pltpu.bitcast(pltpu.pack_elementwise([a, b], packed_dtype=BF16), U32)


def _unpack(x):
    return (pltpu.unpack_elementwise(x, index=0, packed_dtype=BF16, unpacked_dtype=F32),
            pltpu.unpack_elementwise(x, index=1, packed_dtype=BF16, unpacked_dtype=F32))


def _dot(lhs32, rhs):
    return jnp.dot(_bf(lhs32), rhs, preferred_element_type=F32)[0:8]


def _dot_t(lhs32, rhs32):
    return lax.dot_general(_bf(lhs32), _bf(rhs32), (((1,), (1,)), ((), ())),
                           preferred_element_type=F32)[0:8]


def _mean(x):
    return jnp.mean(x, axis=-1, keepdims=True)


def _ln_stats(xp, shift):
    x = _unpack(xp)[0] - shift
    m = _mean(x)
    v = jnp.maximum(_mean(x * x) - m * m, 0.0)
    return m + shift, lax.rsqrt(v + EPS)


def _kernel(x_hbm, kx_hbm, vx_hbm, wq_hbm, wo_hbm, w1_hbm, b1_hbm, w2_hbm, b2_hbm,
            o_ref,
            kbuf, vbuf, vf_buf, wq_buf, wo_buf, w1_buf, w2_buf, x_buf, b1_buf, b2_buf,
            p_buf0, p_buf1, so_buf, se_buf, l_buf, qraw_buf, xo_buf, accp_buf, z_buf,
            xacc_buf, qw_buf, csq_buf, cs1_buf, st_buf, op_buf, wx_buf, c01_buf,
            tm_buf, zero_ref, sem_k, sem_v, sem_w, *, sk, w):
    c_scale = (DH ** -0.5) * math.log2(math.e)
    nt = w // 128
    ng = nt // 8
    na = 12 // NS
    ntb = nt - XF
    r0w = (sk - w) // 16
    p_bufs = (p_buf0, p_buf1)
    starts = [sum(CHUNKS[:c]) for c in range(len(CHUNKS))]
    w2_at = [sum(W2_ROWS[:i]) for i in range(len(W2_ROWS))]

    def k_copy(c):
        rows = pl.ds(24 * starts[c], 24 * CHUNKS[c])
        return [pltpu.make_async_copy(kx_hbm.at[rows, :, pl.ds(r0w, 8 * nt), :],
                                      kbuf.bitcast(BF16).at[rows], sem_k.at[c & 1])]

    def v_copy(c):
        rows = pl.ds(24 * starts[c], 24 * CHUNKS[c])
        return [pltpu.make_async_copy(vx_hbm.at[rows, :, pl.ds(r0w, 8 * ntb), :],
                                      vbuf.bitcast(BF16).at[rows], sem_v.at[c & 1]),
                pltpu.make_async_copy(vx_hbm.at[rows, :, pl.ds(r0w + 8 * ntb, 8 * XF), :],
                                      vf_buf.bitcast(BF16).at[rows, :, pl.ds(8 * XF, 8 * XF), :],
                                      sem_v.at[2 + (c & 1)])]

    wq_cp = pltpu.make_async_copy(wq_hbm, wq_buf.bitcast(BF16), sem_w.at[0])
    wo_cp = pltpu.make_async_copy(wo_hbm, wo_buf.bitcast(BF16), sem_w.at[1])
    w1_cp = pltpu.make_async_copy(w1_hbm, w1_buf, sem_w.at[2])
    x_cp = pltpu.make_async_copy(x_hbm, x_buf, sem_w.at[3])
    b1_cp = pltpu.make_async_copy(b1_hbm, b1_buf, sem_w.at[4])
    b2_cp = pltpu.make_async_copy(b2_hbm, b2_buf, sem_w.at[5])
    w2_cps = [pltpu.make_async_copy(w2_hbm.at[pl.ds(r, n), :], w2_buf.at[pl.ds(r, n), :],
                                    sem_w.at[6 + i])
              for i, (r, n) in enumerate(zip(w2_at, W2_ROWS))]

    for cp in [wq_cp, x_cp, b1_cp, b2_cp, wo_cp] + k_copy(0) + v_copy(0):
        cp.start()
    x_cp.wait()
    b1_cp.wait()
    b2_cp.wait()

    x0 = jnp.broadcast_to(x_buf[...].astype(F32), (8, D))
    b1 = _rows_to_lanes(b1_buf[...].astype(F32), F // 128)
    b2 = _rows_to_lanes(b2_buf[...].astype(F32), D // 128)

    lane = lax.broadcasted_iota(jnp.int32, (8, 128), 1)
    sub3 = lax.broadcasted_iota(jnp.int32, (8, 2 * DH), 0)
    sub_lo = lax.broadcasted_iota(jnp.int32, (1, 8, 128), 1) < 4
    lo64 = lane < 64
    evn = (lane & 8) == 0
    zf = jnp.zeros((8, 128), F32)
    ones32 = jnp.full((8, 128), 0x3F803F80, U32)
    k_order = (((0, 8, 0), (0, 8, 1), (8, 4, 0), (8, 4, 1)),
               ((4, 8, 0), (4, 8, 1), (0, 4, 1), (0, 4, 0)))

    def regroup(a, b):
        return jnp.where(sub_lo, a, pltpu.roll(b, 4, 1)), jnp.where(sub_lo, pltpu.roll(a, 4, 1), b)

    def swap_halves(ref2):
        n = ref2.shape[1]
        a, b = regroup(ref2[0].reshape(n // 8, 8, 128), ref2[1].reshape(n // 8, 8, 128))
        ref2[0] = a.reshape(n, 128)
        ref2[1] = b.reshape(n, 128)

    def fix_wq(a, carry):
        swap_halves(wq_buf.at[a])
        return carry

    def fix_wo(g8, carry):
        g0 = pl.multiple_of(g8 * 8, 8)
        v = [wo_buf[pl.ds(g0, 8), 8 * c:8 * c + 8, :] for c in range(5)]
        n = [jnp.where(sub_lo, v[0], v[2]),
             pltpu.roll(jnp.where(sub_lo, v[3], v[0]), 4, 1),
             jnp.where(sub_lo, v[1], v[3]),
             pltpu.roll(jnp.where(sub_lo, v[4], v[1]), 4, 1),
             jnp.where(sub_lo, v[2], v[4])]
        for c in range(5):
            wo_buf[pl.ds(g0, 8), 8 * c:8 * c + 8, :] = n[c]
        return carry

    def fix_v(r2, carry):
        swap_halves(vbuf.at[r2])
        n = 4 * XF
        t0, t1 = regroup(vf_buf[r2, 0, n:2 * n, :].reshape(n // 8, 8, 128),
                         vf_buf[r2, 1, n:2 * n, :].reshape(n // 8, 8, 128))
        t0, t1 = _unpack(t0), _unpack(t1)
        for e in range(2):
            for k in range(XF // 2):
                vf_buf[r2, e, 16 * k:16 * k + 8, :] = pltpu.bitcast(t0[e][k], U32)
                vf_buf[r2, e, 16 * k + 8:16 * k + 16, :] = pltpu.bitcast(t1[e][k], U32)
        return carry

    def v_tiles(h, a0, n, t):
        return vbuf[pl.ds(12 * h + a0, n), t % 2, 8 * (t // 2):8 * (t // 2) + 8, :]

    def transpose_v(j, t):
        y = _bf(v_tiles(2 * j, 0, 24, t).reshape(DH, 128)).astype(F32)
        yt = pltpu.bitcast(y.T.astype(BF16), U32)
        for ct in range(3):
            vbuf[pl.ds(24 * j + 8 * ct, 8), t % 2, 8 * (t // 2):8 * (t // 2) + 8, :] = (
                yt[:, 128 * ct:128 * (ct + 1)].reshape(8, 8, 128))

    def set_row(x, shift):
        xp = _pack(x, x)
        z_buf[...] = xp
        m, r = _ln_stats(xp, shift)
        rc = r * c_scale
        st_buf[0] = jnp.broadcast_to(rc, (8, 128))
        st_buf[1] = jnp.broadcast_to(m * rc, (8, 128))

    def wq_cols(ct):
        if isinstance(ct, int):
            r0 = (ct // 2) * 8
        else:
            r0 = pl.multiple_of(lax.shift_right_logical(ct, 1) * 8, 8)
        return _bf(wq_buf[:, ct & 1, pl.ds(r0, 8), :].reshape(D // 2, 128))

    def q_cols(z, j, c):
        ct = 3 * j + c
        return _dot(z, wq_cols(ct)) * st_buf[0] - csq_buf[ct] * st_buf[1]

    def store_q(qs, j, pars=(0, 1)):
        q0, q1, q2 = qs
        r56, r64, r8 = (pltpu.roll(q1, s, 1) for s in (56, 64, 8))

        def put(h, qf, a2, b2):
            a0 = jnp.where(evn, qf, zf)
            b1_ = jnp.where(evn, zf, qf)
            ww = [_pack(a0, pltpu.roll(a0, 8, 1)), _pack(pltpu.roll(b1_, 120, 1), b1_),
                  _pack(jnp.where(evn, a2, zf), jnp.where(evn, zf, b2))]
            qw_buf[h & 3] = jnp.concatenate(ww, axis=1)

        if 0 in pars:
            put(2 * j, q0, jnp.where(lo64, q1, r56), jnp.where(lo64, r8, r64))
        if 1 in pars:
            put(2 * j + 1, q2, jnp.where(lo64, r56, q1), jnp.where(lo64, r64, r8))

    def q_pair(j):
        z = z_buf[...]
        store_q([q_cols(z, j, c) for c in range(3)], j)

    def score2(lhs, h, par, k):
        lhs = jnp.where(sub3 == k % 4, lhs, jnp.zeros_like(lhs))
        rhs = jnp.concatenate([kbuf[pl.ds(12 * h + a, n), e, 8 * k:8 * k + 8, :]
                               for a, n, e in k_order[par]], axis=0)
        return _dot(lhs, _bf(rhs.reshape(DH, 128)))

    def store_p(p, g, rs, p_out):
        for r in rs:
            p_out[pl.ds(64 * g + r, 8, stride=8), :] = p

    def inv_sum(l):
        l = jnp.sum(jnp.sum(l, axis=1, keepdims=True), axis=0, keepdims=True)
        l = jnp.broadcast_to(l, (8, 128))
        r = pl.reciprocal(l, approx=True)
        return r * (2.0 - l * r)

    def softmax(sg):
        mx = sg[0]
        for s in sg[1:]:
            mx = jnp.maximum(mx, s)
        m = jnp.max(jnp.max(mx, axis=1, keepdims=True), axis=0, keepdims=True)
        ps, l = [], None
        for s in sg:
            ps.append(jnp.exp2(s - m))
            l = ps[-1] if l is None else l + ps[-1]
        return ps, l

    def softmax_lane(sg):
        mx = jnp.maximum(jnp.maximum(sg[0], sg[1]), jnp.maximum(sg[2], sg[3]))
        m = jnp.broadcast_to(jnp.max(mx, axis=0, keepdims=True), (8, 128))
        ps = [jnp.exp2(s - m) for s in sg]
        c = jnp.exp2(m - jnp.max(m, axis=1, keepdims=True))
        c = _unpack(_pack(c, c))[0]
        return ps, ((ps[0] + ps[1]) + (ps[2] + ps[3])) * c, c

    def pv_step(h, tiles, t, ts, gated, state):
        a0, n = tiles
        p = p_bufs[state['par']][8 * t:8 * t + 8, :]
        for mask, val in gated:
            p = jnp.where(mask, p, val)
        if t < ntb:
            ys = _unpack(v_tiles(h, a0, n, t))
        else:
            r = 8 * (t - ntb)
            ys = [pltpu.bitcast(vf_buf[pl.ds(12 * h + a0, n), e, r:r + 8, :], F32)
                  for e in range(2)]
        if t == ts[0]:
            state['accs'] = [y * p for y in ys]
        else:
            state['accs'] = [acc + y * p for acc, y in zip(state['accs'], ys)]
        if t == ts[-1]:
            r0 = state['par'] * (DH // 2) + 8 * a0
            accp_buf[state['slot'], r0:r0 + 8 * n, :] = _pack(*state['accs']).reshape(8 * n, 128)

    def out_cols(op, g0, ngrp, c):
        rhs = wo_buf[pl.ds(g0, ngrp), 8 * c:8 * c + 8, :].reshape(ngrp * 8, 128)
        return _dot(op, _bf(rhs))

    def mlp_hidden(x, shift):
        xp = _pack(x, x)
        m, r = _ln_stats(xp, shift)
        g = _gelu((_dot(xp, w1_buf[...]) - cs1_buf[...] * m) * r + b1)
        return _pack(g, g)

    def next_copies(j, copy_fn, tail_cps):
        for c in range(len(CHUNKS)):
            @pl.when(j == starts[c])
            def _():
                for cp in copy_fn(c):
                    cp.wait()
                for cp in (copy_fn(c + 1) if c + 1 < len(CHUNKS) else tail_cps):
                    cp.start()

    def pair1(j, carry):
        q_pair(j)
        next_copies(j, k_copy, [w1_cp])
        invs = []
        for par in range(2):
            h = 2 * j + par
            sg = [None] * ng
            lhs = qw_buf[h & 3]
            for c in range(4):
                for g in range(ng):
                    s = score2(lhs, h, par, 4 * g + c)
                    sg[g] = s if c == 0 else sg[g] + s
            ps, l = softmax(sg)
            for g in range(ng):
                store_p(ps[g], g, range(8), p_bufs[par])
            invs.append(inv_sum(l))
        next_copies(j, v_copy, w2_cps)
        lax.fori_loop(24 * j, 24 * (j + 1), fix_v, 0)
        for par in range(2):
            state = dict(par=par, slot=0)
            for sw in range(NS):
                for t in range(nt):
                    pv_step(2 * j + par, (sw * na, na), t, range(nt), (), state)

        @pl.when(j < NP - 1)
        def _():
            for t in range(XM):
                transpose_v(j, t)

        ie, io = invs
        o = _dot_t(ones32, accp_buf[0]) * jnp.concatenate([ie, jnp.where(lo64, ie, io), io], axis=1)
        op = _pack(o, o)
        for c in range(5):
            xacc_buf[:, 128 * c:128 * (c + 1)] += out_cols(op, 24 * j, 24, c)
        return carry

    def expand(t0, t1):
        return [jnp.where(evn, t0, pltpu.roll(t0, 8, 1)),
                jnp.where(evn, pltpu.roll(t0, 120, 1), t0),
                jnp.where(evn, jnp.where(lo64, t1, pltpu.roll(t1, 56, 1)),
                          jnp.where(lo64, pltpu.roll(t1, 8, 1), pltpu.roll(t1, 64, 1)))]

    def expand_wq(a, carry):
        e = expand(wq_buf[a, 0, 0:8, :], wq_buf[a, 1, 0:8, :])
        for i in range(3):
            wx_buf[i, a] = e[i]
        return carry

    ones_row = jnp.concatenate([ones32] * (D // 128), axis=1)

    def colsum_q(ct, carry):
        csq_buf[ct] = _dot(ones_row, wq_cols(ct))
        return carry

    for ref in (so_buf, se_buf, l_buf, qraw_buf, xo_buf):
        ref[...] = jnp.zeros(ref.shape, ref.dtype)
    for i in range(3):
        tm_buf[i] = lane
    zero_ref[0] = 0

    set_row(x0, _mean(x0))
    xacc_buf[...] = x0
    wq_cp.wait()
    lax.fori_loop(0, D // 16, fix_wq, 0)
    lax.fori_loop(0, 3 * NP, colsum_q, 0)
    lax.fori_loop(0, D // 16, expand_wq, 0)
    e = expand(csq_buf[0], csq_buf[1])
    for i in range(3):
        csq_buf[3 * NP + i] = e[i]
    wo_cp.wait()
    lax.fori_loop(0, H * DH // 128, fix_wo, 0)
    lax.fori_loop(0, NP, pair1, 0)
    x1 = xacc_buf[...]
    w1_cp.wait()
    cs1_buf[...] = _dot(ones_row, w1_buf[...])
    gp = mlp_hidden(x1, _mean(x1))
    x2 = x1 + b2
    for cp, r, n in zip(w2_cps, w2_at, W2_ROWS):
        shift = _mean(x2) if cp is w2_cps[-1] else None
        cp.wait()
        x2 = x2 + _dot(gp[:, r:r + n], w2_buf[r:r + n, :])

    set_row(x2, shift)
    xacc_buf[...] = x2
    z = z_buf[...]
    qx = [_dot(z, _bf(wx_buf[i].reshape(D // 2, 128))) * st_buf[0]
          - csq_buf[3 * NP + i] * st_buf[1] for i in range(3)]
    w0 = jnp.concatenate([_pack(jnp.where(evn, q_, zf), jnp.where(evn, zf, q_)) for q_ in qx],
                         axis=1)
    store_q([None, q_cols(z, 0, 1), q_cols(z, 0, 2)], 0, pars=(1,))
    sg = [None] * ng
    for g in range(ng):
        for c in range(4):
            s = score2(w0, 0, 0, 4 * g + c)
            sg[g] = s if c == 0 else sg[g] + s
    q_pair(1)
    ps0, l0, c0 = softmax_lane(sg)
    for g in range(ng):
        store_p(ps0[g], g, range(8), p_buf0)
    l_buf[0] = l0

    true_mask = [tm_buf[i] >= 0 for i in range(3)]
    zq = jnp.clip(zero_ref[0], 0, 1)
    std = [(sw * na, na) for sw in range(NS)]
    steps, info = [], []
    for j in range(NP):
        if j == NP - 1:
            sweeps = [[(tl, range(XE, nt)) for tl in std],
                      [((5, 3), range(XO, nt)), ((2, 3), range(XO, nt)),
                       ((0, 2), range(XO, nt)), ((8, 4), range(XB, nt))]]
        else:
            sweeps = [[(tl, range(XM, nt)) for tl in std]] * 2
        s0 = len(steps)
        steps += [(j, 0, tl, t, ts) for tl, ts in sweeps[0] for t in ts]
        s_odd = len(steps)
        steps += [(j, 1, tl, t, ts) for tl, ts in sweeps[1] for t in ts]
        info.append(dict(s0=s0, s_odd=s_odd, s_end=len(steps),
                         s_tail=len(steps) - len(sweeps[1][-1][1])))
    t_step = [0.0]
    for (_, _, tl, t, _) in steps:
        t_step.append(t_step[-1] + CU * tl[1] * (6 if t < ntb else 4))
    gates, stores, env = {}, {}, {}
    cur = dict(state=None, st=-1, nedge=0, edge=False, p_head=[0, None])

    def get_inv(h):
        return inv_sum(l_buf[zq + (h & 3)])

    def step_at(cyc):
        return next((i for i, tt_ in enumerate(t_step) if tt_ >= cyc), len(t_step))

    def gate(cyc, v):
        st = step_at(cyc)
        while len(gates.get(st, ())) >= 2:
            st += 1
        if cur['st'] < st < len(steps) - NGT:
            gates.setdefault(st, []).append(v)

    def edge(x, n=BE, force=False):
        if cur['st'] < 0 or not (force or cur['edge']):
            return x
        accs = cur['state']['accs']
        cand = [(e_, a) for e_ in range(2) for a in range(accs[0].shape[0])]
        ntile = -(-x.shape[1] // 128)
        parts = [x[:, 128 * i:min(128 * (i + 1), x.shape[1])] for i in range(ntile)]
        for k in range(min(n, 3 * ntile)):
            ce, ca = cand[cur['nedge'] % len(cand)]
            cur['nedge'] += 1
            i = k % ntile
            w_ = parts[i].shape[1]
            parts[i] = jnp.where(true_mask[k // ntile][:, 0:w_], parts[i],
                                 pltpu.bitcast(accs[ce][ca], U32)[:, 0:w_])
        return parts[0] if ntile == 1 else jnp.concatenate(parts, axis=1)

    def sched_stores(ps, lsum, h, t_ready, lo, hi, l_off=10):
        gate(t_ready, ps[-1])
        st_l = min(max(step_at(t_ready + l_off), cur['st'] + 1), len(steps) - 1)
        stores.setdefault(st_l, []).append((lsum, h, None, None))
        t_first = max(t_ready, t_step[lo])
        for i in range(2 * ng):
            g, k = divmod(i, 2)
            st = min(max(step_at(t_first + SDT * i) + 1, cur['st'] + 1), hi)
            assert lo <= st <= hi
            stores.setdefault(st, []).append((ps[g], h, g, range(4 * k, 4 * k + 4)))

    def p_block(h, t):
        assert cur['p_head'][h & 1] == h and not any(
            s_[1] == h and s_[2] is not None for ss in stores.values() for s_ in ss)
        return p_bufs[h & 1][8 * t:8 * t + 8, :]

    def pair_jobs(j):
        inf = info[j]
        first, last = j == 0, j == NP - 1
        h0 = 2 * j

        def job_b(h, c, g):
            s_buf = (se_buf, so_buf)[h & 1]

            def fn(td):
                s = score2(edge(qw_buf[h & 3]), h, h & 1, 4 * g + c)
                env['s'] = s if c == 0 else env['s'] + s
                gate(td + LATP, env['s'])
                if c == 3:
                    s_buf[g] = env['s']
                if c == 3 and g == ng - 1:
                    sg_ = [s_buf[zq + gg] for gg in range(ng)]
                    if h == 1:
                        ps, lsum, c1 = softmax_lane(sg_)
                        c01_buf[...] = _pack(c0, c1)
                        sched_stores(ps, lsum, h, td + LATP + MOFL, inf['s0'], inf['s_odd'], 130)
                    elif h & 1:
                        ps, lsum = softmax(sg_)
                        sched_stores(ps, lsum, h, td + LATP + MOFF, inf['s0'], inf['s_odd'])
                        if not last:
                            store_q([qraw_buf[zq + i] for i in range(3)], j + 1)
                    else:
                        ps, lsum = softmax(sg_)
                        sched_stores(ps, lsum, h, td + LATP + MOFF2, inf['s_odd'],
                                     inf['s_end'] - 1)
            return fn

        def job_e(td):
            x = _dot_t(edge(c01_buf[...] if j == 1 else ones32), accp_buf[(j - 1) & 1])
            x = x + xo_buf[zq]

            def row(i, r):
                return jnp.broadcast_to(x[r:r + 1, 128 * i:128 * (i + 1)], (8, 128))

            ie, io = get_inv(h0 - 2), get_inv(h0 - 1)
            o = jnp.concatenate([row(0, 0) * ie, jnp.where(lo64, row(1, 0) * ie, row(1, 1) * io),
                                 row(2, 1) * io], axis=1)
            gate(td + LATP + 10, o[:, 256:384])
            op_buf[...] = _pack(o, o)

        def job_g(c):
            def fn(td):
                xo = out_cols(edge(op_buf[...]), 24 * (j - 1), 24, c)
                xacc_buf[:, 128 * c:128 * (c + 1)] += xo
                gate(td + LATP, xo)
            return fn

        def job_a(c):
            def fn(td):
                qc = q_cols(edge(z_buf[...]), j + 2, c)
                gate(td + LATP, qc)
                qraw_buf[c] = qc
            return fn

        def job_xp(t):
            def fn(td):
                pe, po = p_block(h0, t), p_block(h0 + 1, t)
                if first:
                    ce, co = _unpack(c01_buf[...])
                    pe, po = pe * ce, po * co
                lhs = edge(_pack(pe, po))
                o = jnp.concatenate([_dot(lhs, _bf(v_tiles(h0, 8 * ct, 8, t).reshape(64, 128)))
                                     for ct in range(3)], axis=1)
                env['xp'] = o if t == 0 else env['xp'] + o
                gate(td + LATP + 20, env['xp'][:, 256:384])
                if t == XM - 1:
                    xo_buf[0] = env['xp']
            return fn

        def job_x(par, t, tiles, key):
            def fn(td):
                p = p_block(h0 + par, t)
                rhs = v_tiles(h0 + par, tiles[0], tiles[1], t).reshape(8 * tiles[1], 128)
                o = _dot_t(edge(_pack(p, p)), rhs)
                env[key] = o if key not in env else env[key] + o
                gate(td + LATP, env[key][:, 0:128] if tiles[1] >= 8 else
                     jnp.concatenate([env[key], env[key]], axis=1))
            return fn

        def finish(par, a0, a1, key):
            r0 = par * (DH // 2)
            o = _dot_t(edge(ones32), accp_buf[j & 1, r0 + 8 * a0:r0 + 8 * a1, :]) + env[key]
            inv = get_inv(h0 + par)
            n = 16 * (a1 - a0)
            return o * (inv[:, 0:n] if n <= 128 else
                        jnp.concatenate([inv, inv[:, 0:n - 128]], axis=1))

        env['finish'] = finish

        def job_fin(par, a0, a1, key):
            def fn(td):
                o = finish(par, a0, a1, key)
                gate(td + LATP + 10, o[:, 0:128])
                env['op' + key] = _pack(o, o)
            return fn

        def job_gfin(c):
            def fn(td):
                xo = out_cols(edge(env['opx0']), 12 * h0, 12, c)
                xacc_buf[:, 128 * c:128 * (c + 1)] += xo
                gate(td + LATP, xo)
            return fn

        t_odd = t_step[inf['s_odd'] + 1]
        jobs = [(24, None, job_b(h0 + 1, c, g))
                for g in range(0 if first else ng // 2, ng) for c in range(4)]
        if not first:
            jobs += [(48, t_step[inf['s0']] + EDEL, job_e)]
        out_jobs = [] if first else [(24, None, job_g(c)) for c in range(5)]
        if last:
            t_tail = t_step[inf['s_tail'] + 1]
            jobs += [(24, None, job_x(0, t, (0, 12), 'x0')) for t in range(XE)]
            jobs += out_jobs
            jobs += [(32, t_odd, job_fin(0, 0, 12, 'x0'))]
            jobs += [(16, None, job_x(1, t, (0, 8), 'x1a')) for t in range(XO)]
            jobs += [(12, t_odd + LATP + 60, job_gfin(c)) for c in range(5)]
            jobs += [(8, None, job_x(1, t, (8, 4), 'x1b')) for t in range(XB1)]
            jobs += [(16, t_tail, job_fin(1, 0, 8, 'x1a'))]
            jobs += [(8, None, job_x(1, t, (8, 4), 'x1b')) for t in range(XB1, XB)]
        else:
            jobs += [(24, None, job_b(h0 + 2, c, g)) for g in range(ng) for c in range(4)]
            jobs += [(24, t_odd, job_xp(t)) for t in range(XM)]
            if j + 2 < NP:
                jobs += [(40, None, job_a(c)) for c in range(3)]
            jobs += out_jobs
            jobs += [(24, None, job_b(h0 + 3, c, g)) for g in range(ng // 2) for c in range(4)]
        return jobs

    jobs, times = [], []
    tt = T0
    for j in range(NP):
        if j > 0:
            tt = max(tt, t_step[info[j]['s0']] - LEAD)
        for job in pair_jobs(j):
            tt = tt + job[0] if job[1] is None else max(tt + job[0], job[1])
            jobs.append(job)
            times.append(tt)
    j_first = next(i for i, tt_ in enumerate(times) if tt_ > 0)

    nj = 0
    for st, (j, par, tl, t, ts) in enumerate(steps):
        while nj < len(jobs) and times[nj] <= t_step[st]:
            rel = nj - j_first
            cur['edge'] = (0 <= rel < NE and rel % 2 == 1) or jobs[nj][1] == times[nj]
            jobs[nj][2](times[nj])
            nj += 1
        for val, h, g, rs in stores.pop(st, ()):
            val = pltpu.bitcast(edge(pltpu.bitcast(val, U32), 1, True), F32)
            if g is None:
                l_buf[h & 3] = val
            else:
                store_p(val, g, rs, p_bufs[h & 1])
                cur['p_head'][h & 1] = h
        if st in (info[j]['s0'], info[j]['s_odd']):
            state = dict(par=par, slot=j & 1)
        assert cur['p_head'][par] == 2 * j + par
        pv_step(2 * j + par, tl, t, ts, zip(true_mask, gates.get(st, ())), state)
        cur['state'] = state
        cur['st'] = st
    cur['edge'] = False
    for job, tt in zip(jobs[nj:], times[nj:]):
        job[2](tt)
    assert not stores

    o = env['finish'](1, 8, 12, 'x1b')
    op = _pack(o, o)
    xa = [out_cols(env['opx1a'], 12 * (H - 1), 8, c) for c in range(5)]
    xb = [out_cols(op, 12 * (H - 1) + 8, 4, c) for c in range(5)]
    x3 = (xacc_buf[...] + jnp.concatenate(xa, axis=1)) + jnp.concatenate(xb, axis=1)
    gp = mlp_hidden(x3, shift)
    x4 = x3 + b2
    for r in range(0, F, W2K):
        x4 = x4 + _dot(gp[:, r:r + W2K], w2_buf[r:r + W2K, :])
    o_ref[...] = x4[0:1, :].astype(o_ref.dtype)


@jax.jit
def pallas_interleave_layers__sliding_block_cached__dense_activation_gelu__decode_kernel(
    A_x: jax.Array,
    A_k_cache: jax.Array,
    A_v_cache: jax.Array,
    A_wq: jax.Array,
    A_wo: jax.Array,
    B_x: jax.Array,
    B_w1: jax.Array,
    B_b1: jax.Array,
    B_w2: jax.Array,
    B_b2: jax.Array,
):
    sk = A_k_cache.shape[2]
    w = min(4096, max(256, sk // 4))
    ng = w // 1024

    def tile_view(a):
        *lead, r, c = a.shape
        n = len(lead)
        a = a.reshape(*lead, r // 8, 8, c // 128, 128)
        a = a.transpose(*range(n), n, n + 2, n + 1, n + 3)
        return a.reshape(*lead, r // 16, 2, (c // 128) * 8, 128)

    kx = tile_view(jnp.swapaxes(A_k_cache, 2, 3)[0]).reshape(H * DH // 16, 2, sk // 16, 128)
    vx = tile_view(jnp.swapaxes(A_v_cache, 2, 3)[0]).reshape(H * DH // 16, 2, sk // 16, 128)
    wqx = tile_view(A_wq)
    wox = tile_view(A_wo).reshape(H * DH // 16, 80, 128)
    out = pl.pallas_call(
        functools.partial(_kernel, sk=sk, w=w),
        out_shape=jax.ShapeDtypeStruct((1, D), A_x.dtype),
        in_specs=[pl.BlockSpec(memory_space=pl.ANY)] * 9,
        out_specs=pl.BlockSpec(memory_space=pltpu.VMEM),
        scratch_shapes=[
            pltpu.VMEM((H * DH // 16, 2, w // 32, 128), U32),
            pltpu.VMEM((H * DH // 16, 2, w // 32 - 4 * XF, 128), U32),
            pltpu.VMEM((H * DH // 16, 2, 8 * XF, 128), U32),
            pltpu.VMEM((D // 16, 2, H * DH // 32, 128), U32),
            pltpu.VMEM((H * DH // 16, 40, 128), U32),
            pltpu.VMEM((D, F), BF16),
            pltpu.VMEM((F, D), BF16),
            pltpu.VMEM((1, D), BF16),
            pltpu.VMEM((F // 128, 128), BF16),
            pltpu.VMEM((D // 128, 128), BF16),
            pltpu.VMEM((w // 16, 128), F32),
            pltpu.VMEM((w // 16, 128), F32),
            pltpu.VMEM((ng + 1, 8, 128), F32),
            pltpu.VMEM((ng + 1, 8, 128), F32),
            pltpu.VMEM((5, 8, 128), F32),
            pltpu.VMEM((4, 8, 128), F32),
            pltpu.VMEM((2, 8, 2 * DH), F32),
            pltpu.VMEM((2, DH, 128), U32),
            pltpu.VMEM((8, D), U32),
            pltpu.VMEM((8, D), F32),
            pltpu.VMEM((4, 8, 2 * DH), U32),
            pltpu.VMEM((3 * NP + 3, 8, 128), F32),
            pltpu.VMEM((8, F), F32),
            pltpu.VMEM((2, 8, 128), F32),
            pltpu.VMEM((8, 2 * DH), U32),
            pltpu.VMEM((3, D // 16, 8, 128), U32),
            pltpu.VMEM((8, 128), U32),
            pltpu.VMEM((3, 8, 128), jnp.int32),
            pltpu.SMEM((1,), jnp.int32),
            pltpu.SemaphoreType.DMA((2,)),
            pltpu.SemaphoreType.DMA((4,)),
            pltpu.SemaphoreType.DMA((6 + len(W2_ROWS),)),
        ],
        compiler_params=pltpu.CompilerParams(vmem_limit_bytes=127 * 1024 * 1024,
                                             disable_semaphore_checks=True),
    )(A_x.reshape(1, D), kx, vx, wqx, wox, B_w1, B_b1.reshape(F // 128, 128),
      B_w2, B_b2.reshape(D // 128, 128))
    return out.reshape(A_x.shape)
```

```python
import functools
import math

import jax
import jax.numpy as jnp
from jax import lax
import jax.experimental.pallas as pl
import jax.experimental.pallas.tpu as pltpu

F32 = jnp.float32
BF16 = jnp.bfloat16
U32 = jnp.uint32

D = 640
H = 32
DH = 192
F = 1536
EPS = 1e-5
NP = H // 2

CHUNKS = (4, 4, 3, 2, 2, 1)
W2_ROWS = (640, 512, 256, 128)
NS = 4
XF = 6
XM = 1
XE, XO, XB, XB1 = 7, 7, 16, 6

CU = 0.261
T0 = -100.0
LEAD = 100.0
LATP = 160.0
MOFF, MOFF2, MOFL = 160.0, 240.0, 60.0
EDEL = 70.0
SDT = 12.0
NE, BE, NGT = 7, 6, 12
W2K = 128


def _gelu(x):
    c = math.sqrt(2.0 / math.pi)
    return 0.5 * x * (1.0 + jnp.tanh(c * (x + 0.044715 * (x * x * x))))


def _rows_to_lanes(b, n):
    return jnp.concatenate([b[i:i + 1, :] for i in range(n)], axis=1)


def _bf(x):
    return pltpu.bitcast(x, BF16)


def _pack(a, b):
    return pltpu.bitcast(pltpu.pack_elementwise([a, b], packed_dtype=BF16), U32)


def _unpack(x):
    return (pltpu.unpack_elementwise(x, index=0, packed_dtype=BF16, unpacked_dtype=F32),
            pltpu.unpack_elementwise(x, index=1, packed_dtype=BF16, unpacked_dtype=F32))


def _dot(lhs32, rhs):
    return jnp.dot(_bf(lhs32), rhs, preferred_element_type=F32)[0:8]


def _dot_t(lhs32, rhs32):
    return lax.dot_general(_bf(lhs32), _bf(rhs32), (((1,), (1,)), ((), ())),
                           preferred_element_type=F32)[0:8]


def _mean(x):
    return jnp.mean(x, axis=-1, keepdims=True)


def _ln_stats(xp, shift):
    x = _unpack(xp)[0] - shift
    m = _mean(x)
    v = jnp.maximum(_mean(x * x) - m * m, 0.0)
    return m + shift, lax.rsqrt(v + EPS)


def _kernel(x_hbm, kx_hbm, vx_hbm, wq_hbm, wo_hbm, w1_hbm, b1_hbm, w2_hbm, b2_hbm,
            o_ref,
            kbuf, vbuf, vf_buf, wq_buf, wo_buf, w1_buf, w2_buf, x_buf, b1_buf, b2_buf,
            p_buf0, p_buf1, so_buf, se_buf, l_buf, qraw_buf, xo_buf, accp_buf, z_buf,
            xacc_buf, qw_buf, csq_buf, cs1_buf, st_buf, op_buf, wx_buf, c01_buf,
            tm_buf, zero_ref, sem_k, sem_v, sem_w, *, sk, w):
    c_scale = (DH ** -0.5) * math.log2(math.e)
    nt = w // 128
    ng = nt // 8
    na = 12 // NS
    ntb = nt - XF
    r0w = (sk - w) // 16
    p_bufs = (p_buf0, p_buf1)
    starts = [sum(CHUNKS[:c]) for c in range(len(CHUNKS))]
    w2_at = [sum(W2_ROWS[:i]) for i in range(len(W2_ROWS))]

    def k_copy(c):
        rows = pl.ds(24 * starts[c], 24 * CHUNKS[c])
        return [pltpu.make_async_copy(kx_hbm.at[rows, :, pl.ds(r0w, 8 * nt), :],
                                      kbuf.bitcast(BF16).at[rows], sem_k.at[c & 1])]

    def v_copy(c):
        rows = pl.ds(24 * starts[c], 24 * CHUNKS[c])
        return [pltpu.make_async_copy(vx_hbm.at[rows, :, pl.ds(r0w, 8 * ntb), :],
                                      vbuf.bitcast(BF16).at[rows], sem_v.at[c & 1]),
                pltpu.make_async_copy(vx_hbm.at[rows, :, pl.ds(r0w + 8 * ntb, 8 * XF), :],
                                      vf_buf.bitcast(BF16).at[rows, :, pl.ds(8 * XF, 8 * XF), :],
                                      sem_v.at[2 + (c & 1)])]

    wq_cp = pltpu.make_async_copy(wq_hbm, wq_buf.bitcast(BF16), sem_w.at[0])
    wo_cp = pltpu.make_async_copy(wo_hbm, wo_buf.bitcast(BF16), sem_w.at[1])
    w1_cp = pltpu.make_async_copy(w1_hbm, w1_buf, sem_w.at[2])
    x_cp = pltpu.make_async_copy(x_hbm, x_buf, sem_w.at[3])
    b1_cp = pltpu.make_async_copy(b1_hbm, b1_buf, sem_w.at[4])
    b2_cp = pltpu.make_async_copy(b2_hbm, b2_buf, sem_w.at[5])
    w2_cps = [pltpu.make_async_copy(w2_hbm.at[pl.ds(r, n), :], w2_buf.at[pl.ds(r, n), :],
                                    sem_w.at[6 + i])
              for i, (r, n) in enumerate(zip(w2_at, W2_ROWS))]

    for cp in [wq_cp, x_cp, b1_cp, b2_cp, wo_cp] + k_copy(0) + v_copy(0):
        cp.start()
    x_cp.wait()
    b1_cp.wait()
    b2_cp.wait()

    x0 = jnp.broadcast_to(x_buf[...].astype(F32), (8, D))
    b1 = _rows_to_lanes(b1_buf[...].astype(F32), F // 128)
    b2 = _rows_to_lanes(b2_buf[...].astype(F32), D // 128)

    lane = lax.broadcasted_iota(jnp.int32, (8, 128), 1)
    sub3 = lax.broadcasted_iota(jnp.int32, (8, 2 * DH), 0)
    sub2 = lax.broadcasted_iota(jnp.int32, (8, 128), 0) // 2
    sub_lo = lax.broadcasted_iota(jnp.int32, (1, 8, 128), 1) < 4
    lo64 = lane < 64
    evn = (lane & 8) == 0
    zf = jnp.zeros((8, 128), F32)
    ones32 = jnp.full((8, 128), 0x3F803F80, U32)
    k_order = (((0, 8, 0), (0, 8, 1), (8, 4, 0), (8, 4, 1)),
               ((4, 8, 0), (4, 8, 1), (0, 4, 1), (0, 4, 0)))

    def regroup(a, b):
        return jnp.where(sub_lo, a, pltpu.roll(b, 4, 1)), jnp.where(sub_lo, pltpu.roll(a, 4, 1), b)

    def swap_halves(ref2):
        n = ref2.shape[1]
        a, b = regroup(ref2[0].reshape(n // 8, 8, 128), ref2[1].reshape(n // 8, 8, 128))
        ref2[0] = a.reshape(n, 128)
        ref2[1] = b.reshape(n, 128)

    def fix_wq(a, carry):
        swap_halves(wq_buf.at[a])
        return carry

    def fix_wo(g8, carry):
        g0 = pl.multiple_of(g8 * 8, 8)
        v = [wo_buf[pl.ds(g0, 8), 8 * c:8 * c + 8, :] for c in range(5)]
        n = [jnp.where(sub_lo, v[0], v[2]),
             pltpu.roll(jnp.where(sub_lo, v[3], v[0]), 4, 1),
             jnp.where(sub_lo, v[1], v[3]),
             pltpu.roll(jnp.where(sub_lo, v[4], v[1]), 4, 1),
             jnp.where(sub_lo, v[2], v[4])]
        for c in range(5):
            wo_buf[pl.ds(g0, 8), 8 * c:8 * c + 8, :] = n[c]
        return carry

    def fix_v(r2, carry):
        swap_halves(vbuf.at[r2])
        n = 4 * XF
        t0, t1 = regroup(vf_buf[r2, 0, n:2 * n, :].reshape(n // 8, 8, 128),
                         vf_buf[r2, 1, n:2 * n, :].reshape(n // 8, 8, 128))
        t0, t1 = _unpack(t0), _unpack(t1)
        for e in range(2):
            for k in range(XF // 2):
                vf_buf[r2, e, 16 * k:16 * k + 8, :] = pltpu.bitcast(t0[e][k], U32)
                vf_buf[r2, e, 16 * k + 8:16 * k + 16, :] = pltpu.bitcast(t1[e][k], U32)
        return carry

    def v_tiles(h, a0, n, t):
        return vbuf[pl.ds(12 * h + a0, n), t % 2, 8 * (t // 2):8 * (t // 2) + 8, :]

    def transpose_v(j, t):
        y = _bf(v_tiles(2 * j, 0, 24, t).reshape(DH, 128)).astype(F32)
        yt = pltpu.bitcast(y.T.astype(BF16), U32)
        for ct in range(3):
            vbuf[pl.ds(24 * j + 8 * ct, 8), t % 2, 8 * (t // 2):8 * (t // 2) + 8, :] = (
                yt[:, 128 * ct:128 * (ct + 1)].reshape(8, 8, 128))

    def set_row(x, shift):
        xp = _pack(x, x)
        z_buf[...] = xp
        m, r = _ln_stats(xp, shift)
        rc = r * c_scale
        st_buf[0] = jnp.broadcast_to(rc, (8, 128))
        st_buf[1] = jnp.broadcast_to(m * rc, (8, 128))

    def wq_cols(ct):
        if isinstance(ct, int):
            r0 = (ct // 2) * 8
        else:
            r0 = pl.multiple_of(lax.shift_right_logical(ct, 1) * 8, 8)
        return _bf(wq_buf[:, ct & 1, pl.ds(r0, 8), :].reshape(D // 2, 128))

    def q_cols(z, j, c):
        ct = 3 * j + c
        return _dot(z, wq_cols(ct)) * st_buf[0] - csq_buf[ct] * st_buf[1]

    def store_q(qs, j, pars=(0, 1)):
        q0, q1, q2 = qs
        r56, r64, r8 = (pltpu.roll(q1, s, 1) for s in (56, 64, 8))

        def put(h, qf, a2, b2):
            a0 = jnp.where(evn, qf, zf)
            b1_ = jnp.where(evn, zf, qf)
            ww = [_pack(a0, pltpu.roll(a0, 8, 1)), _pack(pltpu.roll(b1_, 120, 1), b1_),
                  _pack(jnp.where(evn, a2, zf), jnp.where(evn, zf, b2))]
            qw_buf[h & 3] = jnp.concatenate(ww, axis=1)

        if 0 in pars:
            put(2 * j, q0, jnp.where(lo64, q1, r56), jnp.where(lo64, r8, r64))
        if 1 in pars:
            put(2 * j + 1, q2, jnp.where(lo64, r56, q1), jnp.where(lo64, r64, r8))

    def q_pair(j):
        z = z_buf[...]
        store_q([q_cols(z, j, c) for c in range(3)], j)

    def score2(lhs, h, par, k):
        lhs = jnp.where(sub3 == k % 4, lhs, jnp.zeros_like(lhs))
        rhs = jnp.concatenate([kbuf[pl.ds(12 * h + a, n), e, 8 * k:8 * k + 8, :]
                               for a, n, e in k_order[par]], axis=0)
        return _dot(lhs, _bf(rhs.reshape(DH, 128)))

    def store_p(p, g, rs, p_out):
        for r in rs:
            p_out[pl.ds(64 * g + r, 8, stride=8), :] = p

    def inv_sum(l):
        l = jnp.sum(jnp.sum(l, axis=1, keepdims=True), axis=0, keepdims=True)
        l = jnp.broadcast_to(l, (8, 128))
        r = pl.reciprocal(l, approx=True)
        return r * (2.0 - l * r)

    def softmax(sg):
        mx = sg[0]
        for s in sg[1:]:
            mx = jnp.maximum(mx, s)
        m = jnp.max(jnp.max(mx, axis=1, keepdims=True), axis=0, keepdims=True)
        ps, l = [], None
        for s in sg:
            ps.append(jnp.exp2(s - m))
            l = ps[-1] if l is None else l + ps[-1]
        return ps, l

    def softmax_lane(sg):
        mx = jnp.maximum(jnp.maximum(sg[0], sg[1]), jnp.maximum(sg[2], sg[3]))
        m = jnp.broadcast_to(jnp.max(mx, axis=0, keepdims=True), (8, 128))
        ps = [jnp.exp2(s - m) for s in sg]
        c = jnp.exp2(m - jnp.max(m, axis=1, keepdims=True))
        c = _unpack(_pack(c, c))[0]
        return ps, ((ps[0] + ps[1]) + (ps[2] + ps[3])) * c, c

    def pv_step(h, tiles, t, ts, gated, state):
        a0, n = tiles
        p = p_bufs[state['par']][8 * t:8 * t + 8, :]
        for mask, val in gated:
            p = jnp.where(mask, p, val)
        if t < ntb:
            ys = _unpack(v_tiles(h, a0, n, t))
        else:
            r = 8 * (t - ntb)
            ys = [pltpu.bitcast(vf_buf[pl.ds(12 * h + a0, n), e, r:r + 8, :], F32)
                  for e in range(2)]
        if t == ts[0]:
            state['accs'] = [y * p for y in ys]
        else:
            state['accs'] = [acc + y * p for acc, y in zip(state['accs'], ys)]
        if t == ts[-1]:
            r0 = state['par'] * (DH // 2) + 8 * a0
            accp_buf[state['slot'], r0:r0 + 8 * n, :] = _pack(*state['accs']).reshape(8 * n, 128)

    def out_cols(op, g0, ngrp, c):
        rhs = wo_buf[pl.ds(g0, ngrp), 8 * c:8 * c + 8, :].reshape(ngrp * 8, 128)
        return _dot(op, _bf(rhs))

    def mlp_hidden(x, shift):
        xp = _pack(x, x)
        m, r = _ln_stats(xp, shift)
        g = _gelu((_dot(xp, w1_buf[...]) - cs1_buf[...] * m) * r + b1)
        return _pack(g, g)

    def next_copies(j, copy_fn, tail_cps):
        for c in range(len(CHUNKS)):
            @pl.when(j == starts[c])
            def _():
                for cp in copy_fn(c):
                    cp.wait()
                for cp in (copy_fn(c + 1) if c + 1 < len(CHUNKS) else tail_cps):
                    cp.start()

    def pair1(j, carry):
        q_pair(j)
        next_copies(j, k_copy, [w1_cp])
        invs = []
        for par in range(2):
            h = 2 * j + par
            sg = [None] * ng
            lhs = qw_buf[h & 3]
            for c in range(4):
                for g in range(ng):
                    s = score2(lhs, h, par, 4 * g + c)
                    sg[g] = s if c == 0 else sg[g] + s
            ps, l = softmax(sg)
            for g in range(ng):
                store_p(ps[g], g, range(8), p_bufs[par])
            invs.append(inv_sum(l))
        next_copies(j, v_copy, w2_cps)
        lax.fori_loop(24 * j, 24 * (j + 1), fix_v, 0)
        for par in range(2):
            state = dict(par=par, slot=0)
            for sw in range(NS):
                for t in range(nt):
                    pv_step(2 * j + par, (sw * na, na), t, range(nt), (), state)

        @pl.when(j < NP - 1)
        def _():
            for t in range(XM):
                transpose_v(j, t)

        ie, io = invs
        o = _dot_t(ones32, accp_buf[0]) * jnp.concatenate([ie, jnp.where(lo64, ie, io), io], axis=1)
        op = _pack(o, o)
        for c in range(5):
            xacc_buf[:, 128 * c:128 * (c + 1)] += out_cols(op, 24 * j, 24, c)
        return carry

    def expand(t0, t1):
        return [jnp.where(evn, t0, pltpu.roll(t0, 8, 1)),
                jnp.where(evn, pltpu.roll(t0, 120, 1), t0),
                jnp.where(evn, jnp.where(lo64, t1, pltpu.roll(t1, 56, 1)),
                          jnp.where(lo64, pltpu.roll(t1, 8, 1), pltpu.roll(t1, 64, 1)))]

    def expand_wq(a, carry):
        e = expand(wq_buf[a, 0, 0:8, :], wq_buf[a, 1, 0:8, :])
        for i in range(3):
            wx_buf[i, a] = e[i]
        return carry

    ones_row = jnp.concatenate([ones32] * (D // 128), axis=1)

    def colsum_q(ct, carry):
        csq_buf[ct] = _dot(ones_row, wq_cols(ct))
        return carry

    for ref in (so_buf, se_buf, l_buf, qraw_buf, xo_buf):
        ref[...] = jnp.zeros(ref.shape, ref.dtype)
    for i in range(3):
        tm_buf[i] = lane
    zero_ref[0] = 0

    set_row(x0, _mean(x0))
    xacc_buf[...] = x0
    wq_cp.wait()
    lax.fori_loop(0, D // 16, fix_wq, 0)
    lax.fori_loop(0, 3 * NP, colsum_q, 0)
    lax.fori_loop(0, D // 16, expand_wq, 0)
    e = expand(csq_buf[0], csq_buf[1])
    for i in range(3):
        csq_buf[3 * NP + i] = e[i]
    wo_cp.wait()
    lax.fori_loop(0, H * DH // 128, fix_wo, 0)
    lax.fori_loop(0, NP, pair1, 0)
    x1 = xacc_buf[...]
    w1_cp.wait()
    cs1_buf[...] = _dot(ones_row, w1_buf[...])
    gp = mlp_hidden(x1, _mean(x1))
    x2 = x1 + b2
    for cp, r, n in zip(w2_cps, w2_at, W2_ROWS):
        shift = _mean(x2) if cp is w2_cps[-1] else None
        cp.wait()
        x2 = x2 + _dot(gp[:, r:r + n], w2_buf[r:r + n, :])

    set_row(x2, shift)
    xacc_buf[...] = x2
    z = z_buf[...]
    qx = [_dot(z, _bf(wx_buf[i].reshape(D // 2, 128))) * st_buf[0]
          - csq_buf[3 * NP + i] * st_buf[1] for i in range(3)]
    w0 = jnp.concatenate([_pack(jnp.where(evn, q_, zf), jnp.where(evn, zf, q_)) for q_ in qx],
                         axis=1)
    store_q([None, q_cols(z, 0, 1), q_cols(z, 0, 2)], 0, pars=(1,))
    sg = [None] * ng
    for g in range(ng):
        for c in range(4):
            s = score2(w0, 0, 0, 4 * g + c)
            sg[g] = s if c == 0 else sg[g] + s
    q_pair(1)
    ps0, l0, c0 = softmax_lane(sg)
    for g in range(ng):
        store_p(ps0[g], g, range(8), p_buf0)
    l_buf[0] = l0

    true_mask = [tm_buf[i] >= 0 for i in range(3)]
    zq = jnp.clip(zero_ref[0], 0, 1)
    std = [(sw * na, na) for sw in range(NS)]
    steps, info = [], []
    for j in range(NP):
        if j == NP - 1:
            sweeps = [[(tl, range(XE, nt)) for tl in std],
                      [((5, 3), range(XO, nt)), ((2, 3), range(XO, nt)),
                       ((0, 2), range(XO, nt)), ((8, 4), range(XB, nt))]]
        else:
            sweeps = [[(tl, range(XM, nt)) for tl in std]] * 2
        s0 = len(steps)
        steps += [(j, 0, tl, t, ts) for tl, ts in sweeps[0] for t in ts]
        s_odd = len(steps)
        steps += [(j, 1, tl, t, ts) for tl, ts in sweeps[1] for t in ts]
        info.append(dict(s0=s0, s_odd=s_odd, s_end=len(steps),
                         s_tail=len(steps) - len(sweeps[1][-1][1])))
    t_step = [0.0]
    for (_, _, tl, t, _) in steps:
        t_step.append(t_step[-1] + CU * tl[1] * (6 if t < ntb else 4))
    gates, stores, env = {}, {}, {}
    cur = dict(state=None, st=-1, nedge=0, edge=False, p_head=[0, None])

    def get_inv(h):
        return inv_sum(l_buf[zq + (h & 3)])

    def step_at(cyc):
        return next((i for i, tt_ in enumerate(t_step) if tt_ >= cyc), len(t_step))

    def gate(cyc, v):
        st = step_at(cyc)
        while len(gates.get(st, ())) >= 2:
            st += 1
        if cur['st'] < st < len(steps) - NGT:
            gates.setdefault(st, []).append(v)

    def edge(x, n=BE, force=False):
        if cur['st'] < 0 or not (force or cur['edge']):
            return x
        accs = cur['state']['accs']
        cand = [(e_, a) for e_ in range(2) for a in range(accs[0].shape[0])]
        ntile = -(-x.shape[1] // 128)
        parts = [x[:, 128 * i:min(128 * (i + 1), x.shape[1])] for i in range(ntile)]
        for k in range(min(n, 3 * ntile)):
            ce, ca = cand[cur['nedge'] % len(cand)]
            cur['nedge'] += 1
            i = k % ntile
            w_ = parts[i].shape[1]
            parts[i] = jnp.where(true_mask[k // ntile][:, 0:w_], parts[i],
                                 pltpu.bitcast(accs[ce][ca], U32)[:, 0:w_])
        return parts[0] if ntile == 1 else jnp.concatenate(parts, axis=1)

    def sched_stores(ps, lsum, h, t_ready, lo, hi, l_off=10):
        gate(t_ready, ps[-1])
        st_l = min(max(step_at(t_ready + l_off), cur['st'] + 1), len(steps) - 1)
        stores.setdefault(st_l, []).append((lsum, h, None, None))
        t_first = max(t_ready, t_step[lo])
        for i in range(2 * ng):
            g, k = divmod(i, 2)
            st = min(max(step_at(t_first + SDT * i) + 1, cur['st'] + 1), hi)
            assert lo <= st <= hi
            stores.setdefault(st, []).append((ps[g], h, g, range(4 * k, 4 * k + 4)))

    def p_block(h, t):
        assert cur['p_head'][h & 1] == h and not any(
            s_[1] == h and s_[2] is not None for ss in stores.values() for s_ in ss)
        return p_bufs[h & 1][8 * t:8 * t + 8, :]

    def pair_jobs(j):
        inf = info[j]
        first, last = j == 0, j == NP - 1
        h0 = 2 * j

        def job_b(h, c, g):
            s_buf = (se_buf, so_buf)[h & 1]

            def fn(td):
                s = score2(edge(qw_buf[h & 3]), h, h & 1, 4 * g + c)
                gate(td + LATP, s)
                pltpu.store(s_buf.at[g], s, mask=sub2 == c)
                if c == 3 and g == ng - 1:
                    sg_ = [s_buf[zq + gg] for gg in range(ng)]
                    if h == 1:
                        ps, lsum, c1 = softmax_lane(sg_)
                        c01_buf[...] = _pack(c0, c1)
                        sched_stores(ps, lsum, h, td + LATP + MOFL, inf['s0'], inf['s_odd'], 130)
                    elif h & 1:
                        ps, lsum = softmax(sg_)
                        sched_stores(ps, lsum, h, td + LATP + MOFF, inf['s0'], inf['s_odd'])
                        if not last:
                            store_q([qraw_buf[zq + i] for i in range(3)], j + 1)
                    else:
                        ps, lsum = softmax(sg_)
                        sched_stores(ps, lsum, h, td + LATP + MOFF2, inf['s_odd'],
                                     inf['s_end'] - 1)
            return fn

        def job_e(td):
            x = _dot_t(edge(c01_buf[...] if j == 1 else ones32), accp_buf[(j - 1) & 1])
            x = x + xo_buf[zq]

            def row(i, r):
                return jnp.broadcast_to(x[r:r + 1, 128 * i:128 * (i + 1)], (8, 128))

            ie, io = get_inv(h0 - 2), get_inv(h0 - 1)
            o = jnp.concatenate([row(0, 0) * ie, jnp.where(lo64, row(1, 0) * ie, row(1, 1) * io),
                                 row(2, 1) * io], axis=1)
            gate(td + LATP + 10, o[:, 256:384])
            op_buf[...] = _pack(o, o)

        def job_g(c):
            def fn(td):
                xo = out_cols(edge(op_buf[...]), 24 * (j - 1), 24, c)
                xacc_buf[:, 128 * c:128 * (c + 1)] += xo
                gate(td + LATP, xo)
            return fn

        def job_a(c):
            def fn(td):
                qc = q_cols(edge(z_buf[...]), j + 2, c)
                gate(td + LATP, qc)
                qraw_buf[c] = qc
            return fn

        def job_xp(t):
            def fn(td):
                pe, po = p_block(h0, t), p_block(h0 + 1, t)
                if first:
                    ce, co = _unpack(c01_buf[...])
                    pe, po = pe * ce, po * co
                lhs = edge(_pack(pe, po))
                o = jnp.concatenate([_dot(lhs, _bf(v_tiles(h0, 8 * ct, 8, t).reshape(64, 128)))
                                     for ct in range(3)], axis=1)
                env['xp'] = o if t == 0 else env['xp'] + o
                gate(td + LATP + 20, env['xp'][:, 256:384])
                if t == XM - 1:
                    xo_buf[0] = env['xp']
            return fn

        def job_x(par, t, tiles, key):
            def fn(td):
                p = p_block(h0 + par, t)
                rhs = v_tiles(h0 + par, tiles[0], tiles[1], t).reshape(8 * tiles[1], 128)
                o = _dot_t(edge(_pack(p, p)), rhs)
                env[key] = o if key not in env else env[key] + o
                gate(td + LATP, env[key][:, 0:128] if tiles[1] >= 8 else
                     jnp.concatenate([env[key], env[key]], axis=1))
            return fn

        def finish(par, a0, a1, key):
            r0 = par * (DH // 2)
            o = _dot_t(edge(ones32), accp_buf[j & 1, r0 + 8 * a0:r0 + 8 * a1, :]) + env[key]
            inv = get_inv(h0 + par)
            n = 16 * (a1 - a0)
            return o * (inv[:, 0:n] if n <= 128 else
                        jnp.concatenate([inv, inv[:, 0:n - 128]], axis=1))

        env['finish'] = finish

        def job_fin(par, a0, a1, key):
            def fn(td):
                o = finish(par, a0, a1, key)
                gate(td + LATP + 10, o[:, 0:128])
                env['op' + key] = _pack(o, o)
            return fn

        def job_gfin(c):
            def fn(td):
                xo = out_cols(edge(env['opx0']), 12 * h0, 12, c)
                xacc_buf[:, 128 * c:128 * (c + 1)] += xo
                gate(td + LATP, xo)
            return fn

        t_odd = t_step[inf['s_odd'] + 1]
        jobs = [(24, None, job_b(h0 + 1, c, g))
                for g in range(0 if first else ng // 2, ng) for c in range(4)]
        if not first:
            jobs += [(48, t_step[inf['s0']] + EDEL, job_e)]
        out_jobs = [] if first else [(24, None, job_g(c)) for c in range(5)]
        if last:
            t_tail = t_step[inf['s_tail'] + 1]
            jobs += [(24, None, job_x(0, t, (0, 12), 'x0')) for t in range(XE)]
            jobs += out_jobs
            jobs += [(32, t_odd, job_fin(0, 0, 12, 'x0'))]
            jobs += [(16, None, job_x(1, t, (0, 8), 'x1a')) for t in range(XO)]
            jobs += [(12, t_odd + LATP + 60, job_gfin(c)) for c in range(5)]
            jobs += [(8, None, job_x(1, t, (8, 4), 'x1b')) for t in range(XB1)]
            jobs += [(16, t_tail, job_fin(1, 0, 8, 'x1a'))]
            jobs += [(8, None, job_x(1, t, (8, 4), 'x1b')) for t in range(XB1, XB)]
        else:
            jobs += [(24, None, job_b(h0 + 2, c, g)) for g in range(ng) for c in range(4)]
            jobs += [(24, t_odd, job_xp(t)) for t in range(XM)]
            if j + 2 < NP:
                jobs += [(40, None, job_a(c)) for c in range(3)]
            jobs += out_jobs
            jobs += [(24, None, job_b(h0 + 3, c, g)) for g in range(ng // 2) for c in range(4)]
        return jobs

    jobs, times = [], []
    tt = T0
    for j in range(NP):
        if j > 0:
            tt = max(tt, t_step[info[j]['s0']] - LEAD)
        for job in pair_jobs(j):
            tt = tt + job[0] if job[1] is None else max(tt + job[0], job[1])
            jobs.append(job)
            times.append(tt)
    j_first = next(i for i, tt_ in enumerate(times) if tt_ > 0)

    nj = 0
    for st, (j, par, tl, t, ts) in enumerate(steps):
        while nj < len(jobs) and times[nj] <= t_step[st]:
            rel = nj - j_first
            cur['edge'] = (0 <= rel < NE and rel % 2 == 1) or jobs[nj][1] == times[nj]
            jobs[nj][2](times[nj])
            nj += 1
        for val, h, g, rs in stores.pop(st, ()):
            val = pltpu.bitcast(edge(pltpu.bitcast(val, U32), 1, True), F32)
            if g is None:
                l_buf[h & 3] = val
            else:
                store_p(val, g, rs, p_bufs[h & 1])
                cur['p_head'][h & 1] = h
        if st in (info[j]['s0'], info[j]['s_odd']):
            state = dict(par=par, slot=j & 1)
        assert cur['p_head'][par] == 2 * j + par
        pv_step(2 * j + par, tl, t, ts, zip(true_mask, gates.get(st, ())), state)
        cur['state'] = state
        cur['st'] = st
    cur['edge'] = False
    for job, tt in zip(jobs[nj:], times[nj:]):
        job[2](tt)
    assert not stores

    o = env['finish'](1, 8, 12, 'x1b')
    op = _pack(o, o)
    xa = [out_cols(env['opx1a'], 12 * (H - 1), 8, c) for c in range(5)]
    xb = [out_cols(op, 12 * (H - 1) + 8, 4, c) for c in range(5)]
    x3 = (xacc_buf[...] + jnp.concatenate(xa, axis=1)) + jnp.concatenate(xb, axis=1)
    gp = mlp_hidden(x3, shift)
    x4 = x3 + b2
    for r in range(0, F, W2K):
        x4 = x4 + _dot(gp[:, r:r + W2K], w2_buf[r:r + W2K, :])
    o_ref[...] = x4[0:1, :].astype(o_ref.dtype)


@jax.jit
def pallas_interleave_layers__sliding_block_cached__dense_activation_gelu__decode_kernel(
    A_x: jax.Array,
    A_k_cache: jax.Array,
    A_v_cache: jax.Array,
    A_wq: jax.Array,
    A_wo: jax.Array,
    B_x: jax.Array,
    B_w1: jax.Array,
    B_b1: jax.Array,
    B_w2: jax.Array,
    B_b2: jax.Array,
):
    sk = A_k_cache.shape[2]
    w = min(4096, max(256, sk // 4))
    ng = w // 1024

    def tile_view(a):
        *lead, r, c = a.shape
        n = len(lead)
        a = a.reshape(*lead, r // 8, 8, c // 128, 128)
        a = a.transpose(*range(n), n, n + 2, n + 1, n + 3)
        return a.reshape(*lead, r // 16, 2, (c // 128) * 8, 128)

    kx = tile_view(jnp.swapaxes(A_k_cache, 2, 3)[0]).reshape(H * DH // 16, 2, sk // 16, 128)
    vx = tile_view(jnp.swapaxes(A_v_cache, 2, 3)[0]).reshape(H * DH // 16, 2, sk // 16, 128)
    wqx = tile_view(A_wq)
    wox = tile_view(A_wo).reshape(H * DH // 16, 80, 128)
    out = pl.pallas_call(
        functools.partial(_kernel, sk=sk, w=w),
        out_shape=jax.ShapeDtypeStruct((1, D), A_x.dtype),
        in_specs=[pl.BlockSpec(memory_space=pl.ANY)] * 9,
        out_specs=pl.BlockSpec(memory_space=pltpu.VMEM),
        scratch_shapes=[
            pltpu.VMEM((H * DH // 16, 2, w // 32, 128), U32),
            pltpu.VMEM((H * DH // 16, 2, w // 32 - 4 * XF, 128), U32),
            pltpu.VMEM((H * DH // 16, 2, 8 * XF, 128), U32),
            pltpu.VMEM((D // 16, 2, H * DH // 32, 128), U32),
            pltpu.VMEM((H * DH // 16, 40, 128), U32),
            pltpu.VMEM((D, F), BF16),
            pltpu.VMEM((F, D), BF16),
            pltpu.VMEM((1, D), BF16),
            pltpu.VMEM((F // 128, 128), BF16),
            pltpu.VMEM((D // 128, 128), BF16),
            pltpu.VMEM((w // 16, 128), F32),
            pltpu.VMEM((w // 16, 128), F32),
            pltpu.VMEM((ng + 1, 8, 128), F32),
            pltpu.VMEM((ng + 1, 8, 128), F32),
            pltpu.VMEM((5, 8, 128), F32),
            pltpu.VMEM((4, 8, 128), F32),
            pltpu.VMEM((2, 8, 2 * DH), F32),
            pltpu.VMEM((2, DH, 128), U32),
            pltpu.VMEM((8, D), U32),
            pltpu.VMEM((8, D), F32),
            pltpu.VMEM((4, 8, 2 * DH), U32),
            pltpu.VMEM((3 * NP + 3, 8, 128), F32),
            pltpu.VMEM((8, F), F32),
            pltpu.VMEM((2, 8, 128), F32),
            pltpu.VMEM((8, 2 * DH), U32),
            pltpu.VMEM((3, D // 16, 8, 128), U32),
            pltpu.VMEM((8, 128), U32),
            pltpu.VMEM((3, 8, 128), jnp.int32),
            pltpu.SMEM((1,), jnp.int32),
            pltpu.SemaphoreType.DMA((2,)),
            pltpu.SemaphoreType.DMA((4,)),
            pltpu.SemaphoreType.DMA((6 + len(W2_ROWS),)),
        ],
        compiler_params=pltpu.CompilerParams(vmem_limit_bytes=127 * 1024 * 1024,
                                             disable_semaphore_checks=True),
    )(A_x.reshape(1, D), kx, vx, wqx, wox, B_w1, B_b1.reshape(F // 128, 128),
      B_w2, B_b2.reshape(D // 128, 128))
    return out.reshape(A_x.shape)
```

```python
import functools
import math

import jax
import jax.numpy as jnp
from jax import lax
import jax.experimental.pallas as pl
import jax.experimental.pallas.tpu as pltpu

F32 = jnp.float32
BF16 = jnp.bfloat16
U32 = jnp.uint32

D = 640
H = 32
DH = 192
F = 1536
EPS = 1e-5
NP = H // 2

CHUNKS = (4, 4, 3, 2, 2, 1)
W2_ROWS = (640, 512, 256, 128)
NS = 4
XF = 6
XM = 1
XE, XO, XB, XB1 = 7, 7, 16, 6

CU = 0.261
T0 = -100.0
LEAD = 100.0
LATP = 160.0
MOFF, MOFF2, MOFL = 160.0, 240.0, 60.0
EDEL = 70.0
SDT = 12.0
NE, BE, NGT = 7, 6, 12
W2K = 128


def _gelu(x):
    c = math.sqrt(2.0 / math.pi)
    return 0.5 * x * (1.0 + jnp.tanh(c * (x + 0.044715 * (x * x * x))))


def _rows_to_lanes(b, n):
    return jnp.concatenate([b[i:i + 1, :] for i in range(n)], axis=1)


def _bf(x):
    return pltpu.bitcast(x, BF16)


def _pack(a, b):
    return pltpu.bitcast(pltpu.pack_elementwise([a, b], packed_dtype=BF16), U32)


def _unpack(x):
    return (pltpu.unpack_elementwise(x, index=0, packed_dtype=BF16, unpacked_dtype=F32),
            pltpu.unpack_elementwise(x, index=1, packed_dtype=BF16, unpacked_dtype=F32))


def _dot(lhs32, rhs):
    return jnp.dot(_bf(lhs32), rhs, preferred_element_type=F32)[0:8]


def _dot_t(lhs32, rhs32):
    return lax.dot_general(_bf(lhs32), _bf(rhs32), (((1,), (1,)), ((), ())),
                           preferred_element_type=F32)[0:8]


def _mean(x):
    return jnp.mean(x, axis=-1, keepdims=True)


def _ln_stats(xp, shift):
    x = _unpack(xp)[0] - shift
    m = _mean(x)
    v = jnp.maximum(_mean(x * x) - m * m, 0.0)
    return m + shift, lax.rsqrt(v + EPS)


def _kernel(x_hbm, kx_hbm, vx_hbm, wq_hbm, wo_hbm, w1_hbm, b1_hbm, w2_hbm, b2_hbm,
            o_ref,
            kbuf, vbuf, vf_buf, wq_buf, wo_buf, w1_buf, w2_buf, x_buf, b1_buf, b2_buf,
            p_buf0, p_buf1, so_buf, se_buf, l_buf, qraw_buf, xo_buf, accp_buf, z_buf,
            xacc_buf, qw_buf, csq_buf, cs1_buf, st_buf, op_buf, wx_buf, c01_buf,
            tm_buf, zero_ref, sem_k, sem_v, sem_w, *, sk, w):
    c_scale = (DH ** -0.5) * math.log2(math.e)
    nt = w // 128
    ng = nt // 8
    na = 12 // NS
    ntb = nt - XF
    r0w = (sk - w) // 32
    p_bufs = (p_buf0, p_buf1)
    starts = [sum(CHUNKS[:c]) for c in range(len(CHUNKS))]
    w2_at = [sum(W2_ROWS[:i]) for i in range(len(W2_ROWS))]

    kx32, vx32 = kx_hbm.bitcast(U32), vx_hbm.bitcast(U32)

    def k_copy(c):
        rows = pl.ds(24 * starts[c], 24 * CHUNKS[c])
        return [pltpu.make_async_copy(kx32.at[rows, :, pl.ds(r0w, 4 * nt), :],
                                      kbuf.at[rows], sem_k.at[c & 1])]

    def v_copy(c):
        rows = pl.ds(24 * starts[c], 24 * CHUNKS[c])
        return [pltpu.make_async_copy(vx32.at[rows, :, pl.ds(r0w, 4 * ntb), :],
                                      vbuf.at[rows], sem_v.at[c & 1]),
                pltpu.make_async_copy(vx32.at[rows, :, pl.ds(r0w + 4 * ntb, 4 * XF), :],
                                      vf_buf.at[rows, :, pl.ds(4 * XF, 4 * XF), :],
                                      sem_v.at[2 + (c & 1)])]

    wq_cp = pltpu.make_async_copy(wq_hbm.bitcast(U32), wq_buf, sem_w.at[0])
    wo_cp = pltpu.make_async_copy(wo_hbm.bitcast(U32), wo_buf, sem_w.at[1])
    w1_cp = pltpu.make_async_copy(w1_hbm, w1_buf, sem_w.at[2])
    x_cp = pltpu.make_async_copy(x_hbm, x_buf, sem_w.at[3])
    b1_cp = pltpu.make_async_copy(b1_hbm, b1_buf, sem_w.at[4])
    b2_cp = pltpu.make_async_copy(b2_hbm, b2_buf, sem_w.at[5])
    w2_cps = [pltpu.make_async_copy(w2_hbm.at[pl.ds(r, n), :], w2_buf.at[pl.ds(r, n), :],
                                    sem_w.at[6 + i])
              for i, (r, n) in enumerate(zip(w2_at, W2_ROWS))]

    for cp in [wq_cp, x_cp, b1_cp, b2_cp, wo_cp] + k_copy(0) + v_copy(0):
        cp.start()
    x_cp.wait()
    b1_cp.wait()
    b2_cp.wait()

    x0 = jnp.broadcast_to(x_buf[...].astype(F32), (8, D))
    b1 = _rows_to_lanes(b1_buf[...].astype(F32), F // 128)
    b2 = _rows_to_lanes(b2_buf[...].astype(F32), D // 128)

    lane = lax.broadcasted_iota(jnp.int32, (8, 128), 1)
    sub3 = lax.broadcasted_iota(jnp.int32, (8, 2 * DH), 0)
    sub2 = lax.broadcasted_iota(jnp.int32, (8, 128), 0) // 2
    sub_lo = lax.broadcasted_iota(jnp.int32, (1, 8, 128), 1) < 4
    lo64 = lane < 64
    evn = (lane & 8) == 0
    zf = jnp.zeros((8, 128), F32)
    ones32 = jnp.full((8, 128), 0x3F803F80, U32)
    k_order = (((0, 8, 0), (0, 8, 1), (8, 4, 0), (8, 4, 1)),
               ((4, 8, 0), (4, 8, 1), (0, 4, 1), (0, 4, 0)))

    def regroup(a, b):
        return jnp.where(sub_lo, a, pltpu.roll(b, 4, 1)), jnp.where(sub_lo, pltpu.roll(a, 4, 1), b)

    def swap_halves(ref2):
        n = ref2.shape[1]
        a, b = regroup(ref2[0].reshape(n // 8, 8, 128), ref2[1].reshape(n // 8, 8, 128))
        ref2[0] = a.reshape(n, 128)
        ref2[1] = b.reshape(n, 128)

    def fix_wq(a, carry):
        swap_halves(wq_buf.at[a])
        return carry

    def fix_wo(g8, carry):
        g0 = pl.multiple_of(g8 * 8, 8)
        v = [wo_buf[pl.ds(g0, 8), 8 * c:8 * c + 8, :] for c in range(5)]
        n = [jnp.where(sub_lo, v[0], v[2]),
             pltpu.roll(jnp.where(sub_lo, v[3], v[0]), 4, 1),
             jnp.where(sub_lo, v[1], v[3]),
             pltpu.roll(jnp.where(sub_lo, v[4], v[1]), 4, 1),
             jnp.where(sub_lo, v[2], v[4])]
        for c in range(5):
            wo_buf[pl.ds(g0, 8), 8 * c:8 * c + 8, :] = n[c]
        return carry

    def fix_v(r2, carry):
        swap_halves(vbuf.at[r2])
        n = 4 * XF
        t0, t1 = regroup(vf_buf[r2, 0, n:2 * n, :].reshape(n // 8, 8, 128),
                         vf_buf[r2, 1, n:2 * n, :].reshape(n // 8, 8, 128))
        t0, t1 = _unpack(t0), _unpack(t1)
        for e in range(2):
            for k in range(XF // 2):
                vf_buf[r2, e, 16 * k:16 * k + 8, :] = pltpu.bitcast(t0[e][k], U32)
                vf_buf[r2, e, 16 * k + 8:16 * k + 16, :] = pltpu.bitcast(t1[e][k], U32)
        return carry

    def v_tiles(h, a0, n, t):
        return vbuf[pl.ds(12 * h + a0, n), t % 2, 8 * (t // 2):8 * (t // 2) + 8, :]

    def transpose_v(j, t):
        y = _bf(v_tiles(2 * j, 0, 24, t).reshape(DH, 128)).astype(F32)
        yt = pltpu.bitcast(y.T.astype(BF16), U32)
        for ct in range(3):
            vbuf[pl.ds(24 * j + 8 * ct, 8), t % 2, 8 * (t // 2):8 * (t // 2) + 8, :] = (
                yt[:, 128 * ct:128 * (ct + 1)].reshape(8, 8, 128))

    def set_row(x, shift):
        xp = _pack(x, x)
        z_buf[...] = xp
        m, r = _ln_stats(xp, shift)
        rc = r * c_scale
        st_buf[0] = jnp.broadcast_to(rc, (8, 128))
        st_buf[1] = jnp.broadcast_to(m * rc, (8, 128))

    def wq_cols(ct):
        if isinstance(ct, int):
            r0 = (ct // 2) * 8
        else:
            r0 = pl.multiple_of(lax.shift_right_logical(ct, 1) * 8, 8)
        return _bf(wq_buf[:, ct & 1, pl.ds(r0, 8), :].reshape(D // 2, 128))

    def q_cols(z, j, c):
        ct = 3 * j + c
        return _dot(z, wq_cols(ct)) * st_buf[0] - csq_buf[ct] * st_buf[1]

    def store_q(qs, j, pars=(0, 1)):
        q0, q1, q2 = qs
        r56, r64, r8 = (pltpu.roll(q1, s, 1) for s in (56, 64, 8))

        def put(h, qf, a2, b2):
            a0 = jnp.where(evn, qf, zf)
            b1_ = jnp.where(evn, zf, qf)
            ww = [_pack(a0, pltpu.roll(a0, 8, 1)), _pack(pltpu.roll(b1_, 120, 1), b1_),
                  _pack(jnp.where(evn, a2, zf), jnp.where(evn, zf, b2))]
            qw_buf[h & 3] = jnp.concatenate(ww, axis=1)

        if 0 in pars:
            put(2 * j, q0, jnp.where(lo64, q1, r56), jnp.where(lo64, r8, r64))
        if 1 in pars:
            put(2 * j + 1, q2, jnp.where(lo64, r56, q1), jnp.where(lo64, r64, r8))

    def q_pair(j):
        z = z_buf[...]
        store_q([q_cols(z, j, c) for c in range(3)], j)

    def score2(lhs, h, par, k):
        lhs = jnp.where(sub3 == k % 4, lhs, jnp.zeros_like(lhs))
        rhs = jnp.concatenate([kbuf[pl.ds(12 * h + a, n), e, 8 * k:8 * k + 8, :]
                               for a, n, e in k_order[par]], axis=0)
        return _dot(lhs, _bf(rhs.reshape(DH, 128)))

    def store_p(p, g, rs, p_out):
        for r in rs:
            p_out[pl.ds(64 * g + r, 8, stride=8), :] = p

    def inv_sum(l):
        l = jnp.sum(jnp.sum(l, axis=1, keepdims=True), axis=0, keepdims=True)
        l = jnp.broadcast_to(l, (8, 128))
        r = pl.reciprocal(l, approx=True)
        return r * (2.0 - l * r)

    def softmax(sg):
        mx = sg[0]
        for s in sg[1:]:
            mx = jnp.maximum(mx, s)
        m = jnp.max(jnp.max(mx, axis=1, keepdims=True), axis=0, keepdims=True)
        ps, l = [], None
        for s in sg:
            ps.append(jnp.exp2(s - m))
            l = ps[-1] if l is None else l + ps[-1]
        return ps, l

    def softmax_lane(sg):
        mx = jnp.maximum(jnp.maximum(sg[0], sg[1]), jnp.maximum(sg[2], sg[3]))
        m = jnp.broadcast_to(jnp.max(mx, axis=0, keepdims=True), (8, 128))
        ps = [jnp.exp2(s - m) for s in sg]
        c = jnp.exp2(m - jnp.max(m, axis=1, keepdims=True))
        c = _unpack(_pack(c, c))[0]
        return ps, ((ps[0] + ps[1]) + (ps[2] + ps[3])) * c, c

    def pv_step(h, tiles, t, ts, gated, state):
        a0, n = tiles
        p = p_bufs[state['par']][8 * t:8 * t + 8, :]
        for mask, val in gated:
            p = jnp.where(mask, p, val)
        if t < ntb:
            ys = _unpack(v_tiles(h, a0, n, t))
        else:
            r = 8 * (t - ntb)
            ys = [pltpu.bitcast(vf_buf[pl.ds(12 * h + a0, n), e, r:r + 8, :], F32)
                  for e in range(2)]
        if t == ts[0]:
            state['accs'] = [y * p for y in ys]
        else:
            state['accs'] = [acc + y * p for acc, y in zip(state['accs'], ys)]
        if t == ts[-1]:
            r0 = state['par'] * (DH // 2) + 8 * a0
            accp_buf[state['slot'], r0:r0 + 8 * n, :] = _pack(*state['accs']).reshape(8 * n, 128)

    def out_cols(op, g0, ngrp, c):
        rhs = wo_buf[pl.ds(g0, ngrp), 8 * c:8 * c + 8, :].reshape(ngrp * 8, 128)
        return _dot(op, _bf(rhs))

    def mlp_hidden(x, shift):
        xp = _pack(x, x)
        m, r = _ln_stats(xp, shift)
        g = _gelu((_dot(xp, w1_buf[...]) - cs1_buf[...] * m) * r + b1)
        return _pack(g, g)

    def next_copies(j, copy_fn, tail_cps):
        for c in range(len(CHUNKS)):
            @pl.when(j == starts[c])
            def _():
                for cp in copy_fn(c):
                    cp.wait()
                for cp in (copy_fn(c + 1) if c + 1 < len(CHUNKS) else tail_cps):
                    cp.start()

    def pair1(j, carry):
        q_pair(j)
        next_copies(j, k_copy, [w1_cp])
        invs = []
        for par in range(2):
            h = 2 * j + par
            sg = [None] * ng
            lhs = qw_buf[h & 3]
            for c in range(4):
                for g in range(ng):
                    s = score2(lhs, h, par, 4 * g + c)
                    sg[g] = s if c == 0 else sg[g] + s
            ps, l = softmax(sg)
            for g in range(ng):
                store_p(ps[g], g, range(8), p_bufs[par])
            invs.append(inv_sum(l))
        next_copies(j, v_copy, w2_cps)
        lax.fori_loop(24 * j, 24 * (j + 1), fix_v, 0)
        for par in range(2):
            state = dict(par=par, slot=0)
            for sw in range(NS):
                for t in range(nt):
                    pv_step(2 * j + par, (sw * na, na), t, range(nt), (), state)

        @pl.when(j < NP - 1)
        def _():
            for t in range(XM):
                transpose_v(j, t)

        ie, io = invs
        o = _dot_t(ones32, accp_buf[0]) * jnp.concatenate([ie, jnp.where(lo64, ie, io), io], axis=1)
        op = _pack(o, o)
        for c in range(5):
            xacc_buf[:, 128 * c:128 * (c + 1)] += out_cols(op, 24 * j, 24, c)
        return carry

    def expand(t0, t1):
        return [jnp.where(evn, t0, pltpu.roll(t0, 8, 1)),
                jnp.where(evn, pltpu.roll(t0, 120, 1), t0),
                jnp.where(evn, jnp.where(lo64, t1, pltpu.roll(t1, 56, 1)),
                          jnp.where(lo64, pltpu.roll(t1, 8, 1), pltpu.roll(t1, 64, 1)))]

    def expand_wq(a, carry):
        e = expand(wq_buf[a, 0, 0:8, :], wq_buf[a, 1, 0:8, :])
        for i in range(3):
            wx_buf[i, a] = e[i]
        return carry

    ones_row = jnp.concatenate([ones32] * (D // 128), axis=1)

    def colsum_q(ct, carry):
        csq_buf[ct] = _dot(ones_row, wq_cols(ct))
        return carry

    for ref in (so_buf, se_buf, l_buf, qraw_buf, xo_buf):
        ref[...] = jnp.zeros(ref.shape, ref.dtype)
    for i in range(3):
        tm_buf[i] = lane
    zero_ref[0] = 0

    set_row(x0, _mean(x0))
    xacc_buf[...] = x0
    wq_cp.wait()
    lax.fori_loop(0, D // 16, fix_wq, 0)
    lax.fori_loop(0, 3 * NP, colsum_q, 0)
    lax.fori_loop(0, D // 16, expand_wq, 0)
    e = expand(csq_buf[0], csq_buf[1])
    for i in range(3):
        csq_buf[3 * NP + i] = e[i]
    wo_cp.wait()
    lax.fori_loop(0, H * DH // 128, fix_wo, 0)
    lax.fori_loop(0, NP, pair1, 0)
    x1 = xacc_buf[...]
    w1_cp.wait()
    cs1_buf[...] = _dot(ones_row, w1_buf[...])
    gp = mlp_hidden(x1, _mean(x1))
    x2 = x1 + b2
    for cp, r, n in zip(w2_cps, w2_at, W2_ROWS):
        shift = _mean(x2) if cp is w2_cps[-1] else None
        cp.wait()
        x2 = x2 + _dot(gp[:, r:r + n], w2_buf[r:r + n, :])

    set_row(x2, shift)
    xacc_buf[...] = x2
    z = z_buf[...]
    qx = [_dot(z, _bf(wx_buf[i].reshape(D // 2, 128))) * st_buf[0]
          - csq_buf[3 * NP + i] * st_buf[1] for i in range(3)]
    w0 = jnp.concatenate([_pack(jnp.where(evn, q_, zf), jnp.where(evn, zf, q_)) for q_ in qx],
                         axis=1)
    store_q([None, q_cols(z, 0, 1), q_cols(z, 0, 2)], 0, pars=(1,))
    sg = [None] * ng
    for g in range(ng):
        for c in range(4):
            s = score2(w0, 0, 0, 4 * g + c)
            sg[g] = s if c == 0 else sg[g] + s
    q_pair(1)
    ps0, l0, c0 = softmax_lane(sg)
    for g in range(ng):
        store_p(ps0[g], g, range(8), p_buf0)
    l_buf[0] = l0

    true_mask = [tm_buf[i] >= 0 for i in range(3)]
    zq = jnp.clip(zero_ref[0], 0, 1)
    std = [(sw * na, na) for sw in range(NS)]
    steps, info = [], []
    for j in range(NP):
        if j == NP - 1:
            sweeps = [[(tl, range(XE, nt)) for tl in std],
                      [((5, 3), range(XO, nt)), ((2, 3), range(XO, nt)),
                       ((0, 2), range(XO, nt)), ((8, 4), range(XB, nt))]]
        else:
            sweeps = [[(tl, range(XM, nt)) for tl in std]] * 2
        s0 = len(steps)
        steps += [(j, 0, tl, t, ts) for tl, ts in sweeps[0] for t in ts]
        s_odd = len(steps)
        steps += [(j, 1, tl, t, ts) for tl, ts in sweeps[1] for t in ts]
        info.append(dict(s0=s0, s_odd=s_odd, s_end=len(steps),
                         s_tail=len(steps) - len(sweeps[1][-1][1])))
    t_step = [0.0]
    for (_, _, tl, t, _) in steps:
        t_step.append(t_step[-1] + CU * tl[1] * (6 if t < ntb else 4))
    gates, stores, env = {}, {}, {}
    cur = dict(state=None, st=-1, nedge=0, edge=False, p_head=[0, None])

    def get_inv(h):
        return inv_sum(l_buf[zq + (h & 3)])

    def step_at(cyc):
        return next((i for i, tt_ in enumerate(t_step) if tt_ >= cyc), len(t_step))

    def gate(cyc, v):
        st = step_at(cyc)
        while len(gates.get(st, ())) >= 2:
            st += 1
        if cur['st'] < st < len(steps) - NGT:
            gates.setdefault(st, []).append(v)

    def edge(x, n=BE, force=False):
        if cur['st'] < 0 or not (force or cur['edge']):
            return x
        accs = cur['state']['accs']
        cand = [(e_, a) for e_ in range(2) for a in range(accs[0].shape[0])]
        ntile = -(-x.shape[1] // 128)
        parts = [x[:, 128 * i:min(128 * (i + 1), x.shape[1])] for i in range(ntile)]
        for k in range(min(n, 3 * ntile)):
            ce, ca = cand[cur['nedge'] % len(cand)]
            cur['nedge'] += 1
            i = k % ntile
            w_ = parts[i].shape[1]
            parts[i] = jnp.where(true_mask[k // ntile][:, 0:w_], parts[i],
                                 pltpu.bitcast(accs[ce][ca], U32)[:, 0:w_])
        return parts[0] if ntile == 1 else jnp.concatenate(parts, axis=1)

    def sched_stores(ps, lsum, h, t_ready, lo, hi, l_off=10):
        gate(t_ready, ps[-1])
        st_l = min(max(step_at(t_ready + l_off), cur['st'] + 1), len(steps) - 1)
        stores.setdefault(st_l, []).append((lsum, h, None, None))
        t_first = max(t_ready, t_step[lo])
        for i in range(2 * ng):
            g, k = divmod(i, 2)
            st = min(max(step_at(t_first + SDT * i) + 1, cur['st'] + 1), hi)
            assert lo <= st <= hi
            stores.setdefault(st, []).append((ps[g], h, g, range(4 * k, 4 * k + 4)))

    def p_block(h, t):
        assert cur['p_head'][h & 1] == h and not any(
            s_[1] == h and s_[2] is not None for ss in stores.values() for s_ in ss)
        return p_bufs[h & 1][8 * t:8 * t + 8, :]

    def pair_jobs(j):
        inf = info[j]
        first, last = j == 0, j == NP - 1
        h0 = 2 * j

        def job_b(h, c, g):
            s_buf = (se_buf, so_buf)[h & 1]

            def fn(td):
                s = score2(edge(qw_buf[h & 3]), h, h & 1, 4 * g + c)
                gate(td + LATP, s)
                pltpu.store(s_buf.at[g], s, mask=sub2 == c)
                if c == 3 and g == ng - 1:
                    sg_ = [s_buf[zq + gg] for gg in range(ng)]
                    if h == 1:
                        ps, lsum, c1 = softmax_lane(sg_)
                        c01_buf[...] = _pack(c0, c1)
                        sched_stores(ps, lsum, h, td + LATP + MOFL, inf['s0'], inf['s_odd'], 130)
                    elif h & 1:
                        ps, lsum = softmax(sg_)
                        sched_stores(ps, lsum, h, td + LATP + MOFF, inf['s0'], inf['s_odd'])
                        if not last:
                            store_q([qraw_buf[zq + i] for i in range(3)], j + 1)
                    else:
                        ps, lsum = softmax(sg_)
                        sched_stores(ps, lsum, h, td + LATP + MOFF2, inf['s_odd'],
                                     inf['s_end'] - 1)
            return fn

        def job_e(td):
            x = _dot_t(edge(c01_buf[...] if j == 1 else ones32), accp_buf[(j - 1) & 1])
            x = x + xo_buf[zq]

            def row(i, r):
                return jnp.broadcast_to(x[r:r + 1, 128 * i:128 * (i + 1)], (8, 128))

            ie, io = get_inv(h0 - 2), get_inv(h0 - 1)
            o = jnp.concatenate([row(0, 0) * ie, jnp.where(lo64, row(1, 0) * ie, row(1, 1) * io),
                                 row(2, 1) * io], axis=1)
            gate(td + LATP + 10, o[:, 256:384])
            op_buf[...] = _pack(o, o)

        def job_g(c):
            def fn(td):
                xo = out_cols(edge(op_buf[...]), 24 * (j - 1), 24, c)
                xacc_buf[:, 128 * c:128 * (c + 1)] += xo
                gate(td + LATP, xo)
            return fn

        def job_a(c):
            def fn(td):
                qc = q_cols(edge(z_buf[...]), j + 2, c)
                gate(td + LATP, qc)
                qraw_buf[c] = qc
            return fn

        def job_xp(t):
            def fn(td):
                pe, po = p_block(h0, t), p_block(h0 + 1, t)
                if first:
                    ce, co = _unpack(c01_buf[...])
                    pe, po = pe * ce, po * co
                lhs = edge(_pack(pe, po))
                o = jnp.concatenate([_dot(lhs, _bf(v_tiles(h0, 8 * ct, 8, t).reshape(64, 128)))
                                     for ct in range(3)], axis=1)
                env['xp'] = o if t == 0 else env['xp'] + o
                gate(td + LATP + 20, env['xp'][:, 256:384])
                if t == XM - 1:
                    xo_buf[0] = env['xp']
            return fn

        def job_x(par, t, tiles, key):
            def fn(td):
                p = p_block(h0 + par, t)
                rhs = v_tiles(h0 + par, tiles[0], tiles[1], t).reshape(8 * tiles[1], 128)
                o = _dot_t(edge(_pack(p, p)), rhs)
                env[key] = o if key not in env else env[key] + o
                gate(td + LATP, env[key][:, 0:128] if tiles[1] >= 8 else
                     jnp.concatenate([env[key], env[key]], axis=1))
            return fn

        def finish(par, a0, a1, key):
            r0 = par * (DH // 2)
            o = _dot_t(edge(ones32), accp_buf[j & 1, r0 + 8 * a0:r0 + 8 * a1, :]) + env[key]
            inv = get_inv(h0 + par)
            n = 16 * (a1 - a0)
            return o * (inv[:, 0:n] if n <= 128 else
                        jnp.concatenate([inv, inv[:, 0:n - 128]], axis=1))

        env['finish'] = finish

        def job_fin(par, a0, a1, key):
            def fn(td):
                o = finish(par, a0, a1, key)
                gate(td + LATP + 10, o[:, 0:128])
                env['op' + key] = _pack(o, o)
            return fn

        def job_gfin(c):
            def fn(td):
                xo = out_cols(edge(env['opx0']), 12 * h0, 12, c)
                xacc_buf[:, 128 * c:128 * (c + 1)] += xo
                gate(td + LATP, xo)
            return fn

        t_odd = t_step[inf['s_odd'] + 1]
        jobs = [(24, None, job_b(h0 + 1, c, g))
                for g in range(0 if first else ng // 2, ng) for c in range(4)]
        if not first:
            jobs += [(48, t_step[inf['s0']] + EDEL, job_e)]
        out_jobs = [] if first else [(24, None, job_g(c)) for c in range(5)]
        if last:
            t_tail = t_step[inf['s_tail'] + 1]
            jobs += [(24, None, job_x(0, t, (0, 12), 'x0')) for t in range(XE)]
            jobs += out_jobs
            jobs += [(32, t_odd, job_fin(0, 0, 12, 'x0'))]
            jobs += [(16, None, job_x(1, t, (0, 8), 'x1a')) for t in range(XO)]
            jobs += [(12, t_odd + LATP + 60, job_gfin(c)) for c in range(5)]
            jobs += [(8, None, job_x(1, t, (8, 4), 'x1b')) for t in range(XB1)]
            jobs += [(16, t_tail, job_fin(1, 0, 8, 'x1a'))]
            jobs += [(8, None, job_x(1, t, (8, 4), 'x1b')) for t in range(XB1, XB)]
        else:
            jobs += [(24, None, job_b(h0 + 2, c, g)) for g in range(ng) for c in range(4)]
            jobs += [(24, t_odd, job_xp(t)) for t in range(XM)]
            if j + 2 < NP:
                jobs += [(40, None, job_a(c)) for c in range(3)]
            jobs += out_jobs
            jobs += [(24, None, job_b(h0 + 3, c, g)) for g in range(ng // 2) for c in range(4)]
        return jobs

    jobs, times = [], []
    tt = T0
    for j in range(NP):
        if j > 0:
            tt = max(tt, t_step[info[j]['s0']] - LEAD)
        for job in pair_jobs(j):
            tt = tt + job[0] if job[1] is None else max(tt + job[0], job[1])
            jobs.append(job)
            times.append(tt)
    j_first = next(i for i, tt_ in enumerate(times) if tt_ > 0)

    nj = 0
    for st, (j, par, tl, t, ts) in enumerate(steps):
        while nj < len(jobs) and times[nj] <= t_step[st]:
            rel = nj - j_first
            cur['edge'] = (0 <= rel < NE and rel % 2 == 1) or jobs[nj][1] == times[nj]
            jobs[nj][2](times[nj])
            nj += 1
        for val, h, g, rs in stores.pop(st, ()):
            val = pltpu.bitcast(edge(pltpu.bitcast(val, U32), 1, True), F32)
            if g is None:
                l_buf[h & 3] = val
            else:
                store_p(val, g, rs, p_bufs[h & 1])
                cur['p_head'][h & 1] = h
        if st in (info[j]['s0'], info[j]['s_odd']):
            state = dict(par=par, slot=j & 1)
        assert cur['p_head'][par] == 2 * j + par
        pv_step(2 * j + par, tl, t, ts, zip(true_mask, gates.get(st, ())), state)
        cur['state'] = state
        cur['st'] = st
    cur['edge'] = False
    for job, tt in zip(jobs[nj:], times[nj:]):
        job[2](tt)
    assert not stores

    o = env['finish'](1, 8, 12, 'x1b')
    op = _pack(o, o)
    xa = [out_cols(env['opx1a'], 12 * (H - 1), 8, c) for c in range(5)]
    xb = [out_cols(op, 12 * (H - 1) + 8, 4, c) for c in range(5)]
    x3 = (xacc_buf[...] + jnp.concatenate(xa, axis=1)) + jnp.concatenate(xb, axis=1)
    gp = mlp_hidden(x3, shift)
    x4 = x3 + b2
    for r in range(0, F, W2K):
        x4 = x4 + _dot(gp[:, r:r + W2K], w2_buf[r:r + W2K, :])
    o_ref[...] = x4[0:1, :].astype(o_ref.dtype)


@jax.jit
def pallas_interleave_layers__sliding_block_cached__dense_activation_gelu__decode_kernel(
    A_x: jax.Array,
    A_k_cache: jax.Array,
    A_v_cache: jax.Array,
    A_wq: jax.Array,
    A_wo: jax.Array,
    B_x: jax.Array,
    B_w1: jax.Array,
    B_b1: jax.Array,
    B_w2: jax.Array,
    B_b2: jax.Array,
):
    sk = A_k_cache.shape[2]
    w = min(4096, max(256, sk // 4))
    ng = w // 1024

    def tile_view(a):
        *lead, r, c = a.shape
        n = len(lead)
        a = a.reshape(*lead, r // 8, 8, c // 128, 128)
        a = a.transpose(*range(n), n, n + 2, n + 1, n + 3)
        return a.reshape(*lead, r // 16, 2, (c // 128) * 8, 128)

    kx = tile_view(jnp.swapaxes(A_k_cache, 2, 3)[0]).reshape(H * DH // 16, 2, sk // 16, 128)
    vx = tile_view(jnp.swapaxes(A_v_cache, 2, 3)[0]).reshape(H * DH // 16, 2, sk // 16, 128)
    wqx = tile_view(A_wq)
    wox = tile_view(A_wo).reshape(H * DH // 16, 80, 128)
    out = pl.pallas_call(
        functools.partial(_kernel, sk=sk, w=w),
        out_shape=jax.ShapeDtypeStruct((1, D), A_x.dtype),
        in_specs=[pl.BlockSpec(memory_space=pl.ANY)] * 9,
        out_specs=pl.BlockSpec(memory_space=pltpu.VMEM),
        scratch_shapes=[
            pltpu.VMEM((H * DH // 16, 2, w // 32, 128), U32),
            pltpu.VMEM((H * DH // 16, 2, w // 32 - 4 * XF, 128), U32),
            pltpu.VMEM((H * DH // 16, 2, 8 * XF, 128), U32),
            pltpu.VMEM((D // 16, 2, H * DH // 32, 128), U32),
            pltpu.VMEM((H * DH // 16, 40, 128), U32),
            pltpu.VMEM((D, F), BF16),
            pltpu.VMEM((F, D), BF16),
            pltpu.VMEM((1, D), BF16),
            pltpu.VMEM((F // 128, 128), BF16),
            pltpu.VMEM((D // 128, 128), BF16),
            pltpu.VMEM((w // 16, 128), F32),
            pltpu.VMEM((w // 16, 128), F32),
            pltpu.VMEM((ng + 1, 8, 128), F32),
            pltpu.VMEM((ng + 1, 8, 128), F32),
            pltpu.VMEM((5, 8, 128), F32),
            pltpu.VMEM((4, 8, 128), F32),
            pltpu.VMEM((2, 8, 2 * DH), F32),
            pltpu.VMEM((2, DH, 128), U32),
            pltpu.VMEM((8, D), U32),
            pltpu.VMEM((8, D), F32),
            pltpu.VMEM((4, 8, 2 * DH), U32),
            pltpu.VMEM((3 * NP + 3, 8, 128), F32),
            pltpu.VMEM((8, F), F32),
            pltpu.VMEM((2, 8, 128), F32),
            pltpu.VMEM((8, 2 * DH), U32),
            pltpu.VMEM((3, D // 16, 8, 128), U32),
            pltpu.VMEM((8, 128), U32),
            pltpu.VMEM((3, 8, 128), jnp.int32),
            pltpu.SMEM((1,), jnp.int32),
            pltpu.SemaphoreType.DMA((2,)),
            pltpu.SemaphoreType.DMA((4,)),
            pltpu.SemaphoreType.DMA((6 + len(W2_ROWS),)),
        ],
        compiler_params=pltpu.CompilerParams(vmem_limit_bytes=127 * 1024 * 1024,
                                             disable_semaphore_checks=True),
    )(A_x.reshape(1, D), kx, vx, wqx, wox, B_w1, B_b1.reshape(F // 128, 128),
      B_w2, B_b2.reshape(D // 128, 128))
    return out.reshape(A_x.shape)
```

```python
import functools
import math

import jax
import jax.numpy as jnp
from jax import lax
import jax.experimental.pallas as pl
import jax.experimental.pallas.tpu as pltpu

F32 = jnp.float32
BF16 = jnp.bfloat16
U32 = jnp.uint32

D = 640
H = 32
DH = 192
F = 1536
EPS = 1e-5
NP = H // 2

CHUNKS = (4, 4, 3, 2, 2, 1)
W2_ROWS = (640, 512, 256, 128)
NS = 4
XF = 6
XM = 1
XE, XO, XB, XB1 = 7, 7, 16, 8

CU = 0.263
T0 = -100.0
LEAD = 100.0
LATP = 160.0
MOFF, MOFF2, MOFL = 160.0, 200.0, 40.0
EDEL = 70.0
SDT = 12.0
NE, BE, NGT = 7, 6, 12
NV, GV0, GVS = 5, -16, 4


def _gelu(x):
    c = math.sqrt(2.0 / math.pi)
    return 0.5 * x * (1.0 + jnp.tanh(c * (x + 0.044715 * (x * x * x))))


def _rows_to_lanes(b, n):
    return jnp.concatenate([b[i:i + 1, :] for i in range(n)], axis=1)


def _bf(x):
    return pltpu.bitcast(x, BF16)


def _pack(a, b):
    return pltpu.bitcast(pltpu.pack_elementwise([a, b], packed_dtype=BF16), U32)


def _unpack(x):
    return (pltpu.unpack_elementwise(x, index=0, packed_dtype=BF16, unpacked_dtype=F32),
            pltpu.unpack_elementwise(x, index=1, packed_dtype=BF16, unpacked_dtype=F32))


def _dot(lhs32, rhs):
    return jnp.dot(_bf(lhs32), rhs, preferred_element_type=F32)[0:8]


def _dot_t(lhs32, rhs32):
    return lax.dot_general(_bf(lhs32), _bf(rhs32), (((1,), (1,)), ((), ())),
                           preferred_element_type=F32)[0:8]


def _mean(x):
    return jnp.mean(x, axis=-1, keepdims=True)


def _ln_stats(xp, shift):
    x = _unpack(xp)[0] - shift
    m = _mean(x)
    v = jnp.maximum(_mean(x * x) - m * m, 0.0)
    return m + shift, lax.rsqrt(v + EPS)


def _kernel(x_hbm, kx_hbm, vx_hbm, wq_hbm, wo_hbm, w1_hbm, b1_hbm, w2_hbm, b2_hbm,
            o_ref,
            kbuf, vbuf, vf_buf, wq_buf, wo_buf, w1_buf, w2_buf, x_buf, b1_buf, b2_buf,
            p_buf0, p_buf1, so_buf, se_buf, l_buf, qraw_buf, xo_buf, accp_buf, z_buf,
            xacc_buf, qw_buf, csq_buf, cs1_buf, st_buf, op_buf, wx_buf, c01_buf,
            tm_buf, zero_ref, sem_k, sem_v, sem_w, *, sk, w):
    c_scale = (DH ** -0.5) * math.log2(math.e)
    nt = w // 128
    ng = nt // 8
    na = 12 // NS
    ntb = nt - XF
    r0w = (sk - w) // 32
    p_bufs = (p_buf0, p_buf1)
    starts = [sum(CHUNKS[:c]) for c in range(len(CHUNKS))]
    w2_at = [sum(W2_ROWS[:i]) for i in range(len(W2_ROWS))]

    kx32, vx32 = kx_hbm.bitcast(U32), vx_hbm.bitcast(U32)

    def k_copy(c):
        rows = pl.ds(24 * starts[c], 24 * CHUNKS[c])
        return [pltpu.make_async_copy(kx32.at[rows, :, pl.ds(r0w, 4 * nt), :],
                                      kbuf.at[rows], sem_k.at[c & 1])]

    def v_copy(c):
        rows = pl.ds(24 * starts[c], 24 * CHUNKS[c])
        return [pltpu.make_async_copy(vx32.at[rows, :, pl.ds(r0w, 4 * ntb), :],
                                      vbuf.at[rows], sem_v.at[c & 1]),
                pltpu.make_async_copy(vx32.at[rows, :, pl.ds(r0w + 4 * ntb, 4 * XF), :],
                                      vf_buf.at[rows, :, pl.ds(4 * XF, 4 * XF), :],
                                      sem_v.at[2 + (c & 1)])]

    wq_cp = pltpu.make_async_copy(wq_hbm.bitcast(U32), wq_buf, sem_w.at[0])
    wo_cp = pltpu.make_async_copy(wo_hbm.bitcast(U32), wo_buf, sem_w.at[1])
    w1_cp = pltpu.make_async_copy(w1_hbm.bitcast(U32), w1_buf, sem_w.at[2])
    x_cp = pltpu.make_async_copy(x_hbm, x_buf, sem_w.at[3])
    b1_cp = pltpu.make_async_copy(b1_hbm, b1_buf, sem_w.at[4])
    b2_cp = pltpu.make_async_copy(b2_hbm, b2_buf, sem_w.at[5])
    w2_cps = [pltpu.make_async_copy(w2_hbm.bitcast(U32).at[pl.ds(r // 16, n // 16)],
                                    w2_buf.at[pl.ds(r // 16, n // 16)], sem_w.at[6 + i])
              for i, (r, n) in enumerate(zip(w2_at, W2_ROWS))]

    for cp in [wq_cp, x_cp, b1_cp, b2_cp, wo_cp] + k_copy(0) + v_copy(0):
        cp.start()
    x_cp.wait()
    b1_cp.wait()
    b2_cp.wait()

    x0 = jnp.broadcast_to(x_buf[...].astype(F32), (8, D))
    b1 = _rows_to_lanes(b1_buf[...].astype(F32), F // 128)
    b2 = _rows_to_lanes(b2_buf[...].astype(F32), D // 128)

    lane = lax.broadcasted_iota(jnp.int32, (8, 128), 1)
    sub3 = lax.broadcasted_iota(jnp.int32, (8, 2 * DH), 0)
    sub2 = lax.broadcasted_iota(jnp.int32, (8, 128), 0) // 2
    sub_lo = lax.broadcasted_iota(jnp.int32, (1, 8, 128), 1) < 4
    lo64 = lane < 64
    evn = (lane & 8) == 0
    zf = jnp.zeros((8, 128), F32)
    ones32 = jnp.full((8, 128), 0x3F803F80, U32)
    k_order = (((0, 8, 0), (0, 8, 1), (8, 4, 0), (8, 4, 1)),
               ((4, 8, 0), (4, 8, 1), (0, 4, 1), (0, 4, 0)))

    def regroup(a, b):
        return jnp.where(sub_lo, a, pltpu.roll(b, 4, 1)), jnp.where(sub_lo, pltpu.roll(a, 4, 1), b)

    def swap_halves(ref2):
        n = ref2.shape[1]
        a, b = regroup(ref2[0].reshape(n // 8, 8, 128), ref2[1].reshape(n // 8, 8, 128))
        ref2[0] = a.reshape(n, 128)
        ref2[1] = b.reshape(n, 128)

    def fix_wq(a, carry):
        swap_halves(wq_buf.at[a])
        return carry

    def fix5(buf, g0):
        v = [buf[pl.ds(g0, 8), 8 * c:8 * c + 8, :] for c in range(5)]
        n = [jnp.where(sub_lo, v[0], v[2]),
             pltpu.roll(jnp.where(sub_lo, v[3], v[0]), 4, 1),
             jnp.where(sub_lo, v[1], v[3]),
             pltpu.roll(jnp.where(sub_lo, v[4], v[1]), 4, 1),
             jnp.where(sub_lo, v[2], v[4])]
        for c in range(5):
            buf[pl.ds(g0, 8), 8 * c:8 * c + 8, :] = n[c]
        return n

    def fix_wo(g8, carry):
        fix5(wo_buf, pl.multiple_of(g8 * 8, 8))
        return carry

    def fix_w1(a, carry):
        swap_halves(w1_buf.at[a])
        return carry

    def fix_v(r2, carry):
        swap_halves(vbuf.at[r2])
        n = 4 * XF
        t0, t1 = regroup(vf_buf[r2, 0, n:2 * n, :].reshape(n // 8, 8, 128),
                         vf_buf[r2, 1, n:2 * n, :].reshape(n // 8, 8, 128))
        t0, t1 = _unpack(t0), _unpack(t1)
        for e in range(2):
            for k in range(XF // 2):
                vf_buf[r2, e, 16 * k:16 * k + 8, :] = pltpu.bitcast(t0[e][k], U32)
                vf_buf[r2, e, 16 * k + 8:16 * k + 16, :] = pltpu.bitcast(t1[e][k], U32)
        return carry

    def v_tiles(h, a0, n, t):
        return vbuf[pl.ds(12 * h + a0, n), t % 2, 8 * (t // 2):8 * (t // 2) + 8, :]

    def transpose_v(j, t):
        y = _bf(v_tiles(2 * j, 0, 24, t).reshape(DH, 128)).astype(F32)
        yt = pltpu.bitcast(y.T.astype(BF16), U32)
        for ct in range(3):
            vbuf[pl.ds(24 * j + 8 * ct, 8), t % 2, 8 * (t // 2):8 * (t // 2) + 8, :] = (
                yt[:, 128 * ct:128 * (ct + 1)].reshape(8, 8, 128))

    def set_row(x, shift):
        xp = _pack(x, x)
        z_buf[...] = xp
        m, r = _ln_stats(xp, shift)
        rc = r * c_scale
        st_buf[0] = jnp.broadcast_to(rc, (8, 128))
        st_buf[1] = jnp.broadcast_to(m * rc, (8, 128))

    def wq_cols(ct):
        if isinstance(ct, int):
            r0 = (ct // 2) * 8
        else:
            r0 = pl.multiple_of(lax.shift_right_logical(ct, 1) * 8, 8)
        return _bf(wq_buf[:, ct & 1, pl.ds(r0, 8), :].reshape(D // 2, 128))

    def q_cols(z, j, c):
        ct = 3 * j + c
        return _dot(z, wq_cols(ct)) * st_buf[0] - csq_buf[ct] * st_buf[1]

    def store_q(qs, j, pars=(0, 1)):
        q0, q1, q2 = qs
        r56, r64, r8 = (pltpu.roll(q1, s, 1) for s in (56, 64, 8))

        def put(h, qf, a2, b2):
            a0 = jnp.where(evn, qf, zf)
            b1_ = jnp.where(evn, zf, qf)
            ww = [_pack(a0, pltpu.roll(a0, 8, 1)), _pack(pltpu.roll(b1_, 120, 1), b1_),
                  _pack(jnp.where(evn, a2, zf), jnp.where(evn, zf, b2))]
            qw_buf[h & 3] = jnp.concatenate(ww, axis=1)

        if 0 in pars:
            put(2 * j, q0, jnp.where(lo64, q1, r56), jnp.where(lo64, r8, r64))
        if 1 in pars:
            put(2 * j + 1, q2, jnp.where(lo64, r56, q1), jnp.where(lo64, r64, r8))

    def q_pair(j):
        z = z_buf[...]
        store_q([q_cols(z, j, c) for c in range(3)], j)

    def score2(lhs, h, par, k):
        lhs = jnp.where(sub3 == k % 4, lhs, jnp.zeros_like(lhs))
        rhs = jnp.concatenate([kbuf[pl.ds(12 * h + a, n), e, 8 * k:8 * k + 8, :]
                               for a, n, e in k_order[par]], axis=0)
        return _dot(lhs, _bf(rhs.reshape(DH, 128)))

    def store_p(p, g, rs, p_out):
        for r in rs:
            p_out[pl.ds(64 * g + r, 8, stride=8), :] = p

    def inv_sum(l):
        l = jnp.sum(jnp.sum(l, axis=1, keepdims=True), axis=0, keepdims=True)
        l = jnp.broadcast_to(l, (8, 128))
        r = pl.reciprocal(l, approx=True)
        return r * (2.0 - l * r)

    def softmax(sg):
        mx = sg[0]
        for s in sg[1:]:
            mx = jnp.maximum(mx, s)
        m = jnp.max(jnp.max(mx, axis=1, keepdims=True), axis=0, keepdims=True)
        ps, l = [], None
        for s in sg:
            ps.append(jnp.exp2(s - m))
            l = ps[-1] if l is None else l + ps[-1]
        return ps, l

    def softmax_lane(sg):
        mx = jnp.maximum(jnp.maximum(sg[0], sg[1]), jnp.maximum(sg[2], sg[3]))
        m = jnp.broadcast_to(jnp.max(mx, axis=0, keepdims=True), (8, 128))
        ps = [jnp.exp2(s - m) for s in sg]
        c = jnp.exp2(m - jnp.max(m, axis=1, keepdims=True))
        c = _unpack(_pack(c, c))[0]
        return ps, ((ps[0] + ps[1]) + (ps[2] + ps[3])) * c, c

    def pv_step(h, tiles, t, ts, gated, state):
        a0, n = tiles
        p = p_bufs[state['par']][8 * t:8 * t + 8, :]
        for mask, val in gated:
            p = jnp.where(mask, p, val)
        if t < ntb:
            ys = _unpack(v_tiles(h, a0, n, t))
        else:
            r = 8 * (t - ntb)
            ys = [pltpu.bitcast(vf_buf[pl.ds(12 * h + a0, n), e, r:r + 8, :], F32)
                  for e in range(2)]
        if t == ts[0]:
            state['accs'] = [y * p for y in ys]
        else:
            state['accs'] = [acc + y * p for acc, y in zip(state['accs'], ys)]
        if t == ts[-1]:
            r0 = state['par'] * (DH // 2) + 8 * a0
            accp_buf[state['slot'], r0:r0 + 8 * n, :] = _pack(*state['accs']).reshape(8 * n, 128)

    def out_cols(op, g0, ngrp, c):
        rhs = wo_buf[pl.ds(g0, ngrp), 8 * c:8 * c + 8, :].reshape(ngrp * 8, 128)
        return _dot(op, _bf(rhs))

    def w1_cols(k):
        return _bf(w1_buf[:, k % 2, 8 * (k // 2):8 * (k // 2) + 8, :].reshape(D // 2, 128))

    def mlp_hidden(x, shift):
        xp = _pack(x, x)
        m, r = _ln_stats(xp, shift)
        return [_gelu((_dot(xp, w1_cols(k)) - cs1_buf[k] * m) * r + b1[:, 128 * k:128 * (k + 1)])
                for k in range(F // 128)]

    def w2_dot(g, tiles):
        gp = _pack(g, g)
        return jnp.concatenate([_dot(gp, _bf(t.reshape(64, 128))) for t in tiles], axis=1)

    def next_copies(j, copy_fn, tail_cps):
        for c in range(len(CHUNKS)):
            @pl.when(j == starts[c])
            def _():
                for cp in copy_fn(c):
                    cp.wait()
                for cp in (copy_fn(c + 1) if c + 1 < len(CHUNKS) else tail_cps):
                    cp.start()

    def pair1(j, carry):
        q_pair(j)
        next_copies(j, k_copy, [w1_cp])
        invs = []
        for par in range(2):
            h = 2 * j + par
            sg = [None] * ng
            lhs = qw_buf[h & 3]
            for c in range(4):
                for g in range(ng):
                    s = score2(lhs, h, par, 4 * g + c)
                    sg[g] = s if c == 0 else sg[g] + s
            ps, l = softmax(sg)
            for g in range(ng):
                store_p(ps[g], g, range(8), p_bufs[par])
            invs.append(inv_sum(l))
        next_copies(j, v_copy, w2_cps)
        lax.fori_loop(24 * j, 24 * (j + 1), fix_v, 0)
        for par in range(2):
            state = dict(par=par, slot=0)
            for sw in range(NS):
                for t in range(nt):
                    pv_step(2 * j + par, (sw * na, na), t, range(nt), (), state)

        @pl.when(j < NP - 1)
        def _():
            for t in range(XM):
                transpose_v(j, t)

        ie, io = invs
        o = _dot_t(ones32, accp_buf[0]) * jnp.concatenate([ie, jnp.where(lo64, ie, io), io], axis=1)
        op = _pack(o, o)
        for c in range(5):
            xacc_buf[:, 128 * c:128 * (c + 1)] += out_cols(op, 24 * j, 24, c)
        return carry

    def expand(t0, t1):
        return [jnp.where(evn, t0, pltpu.roll(t0, 8, 1)),
                jnp.where(evn, pltpu.roll(t0, 120, 1), t0),
                jnp.where(evn, jnp.where(lo64, t1, pltpu.roll(t1, 56, 1)),
                          jnp.where(lo64, pltpu.roll(t1, 8, 1), pltpu.roll(t1, 64, 1)))]

    def expand_wq(a, carry):
        e = expand(wq_buf[a, 0, 0:8, :], wq_buf[a, 1, 0:8, :])
        for i in range(3):
            wx_buf[i, a] = e[i]
        return carry

    ones_row = jnp.concatenate([ones32] * (D // 128), axis=1)

    def colsum_q(ct, carry):
        csq_buf[ct] = _dot(ones_row, wq_cols(ct))
        return carry

    for ref in (so_buf, se_buf, l_buf, qraw_buf, xo_buf):
        ref[...] = jnp.zeros(ref.shape, ref.dtype)
    for i in range(3):
        tm_buf[i] = lane
    zero_ref[0] = 0

    set_row(x0, _mean(x0))
    xacc_buf[...] = x0
    wq_cp.wait()
    lax.fori_loop(0, D // 16, fix_wq, 0)
    lax.fori_loop(0, 3 * NP, colsum_q, 0)
    lax.fori_loop(0, D // 16, expand_wq, 0)
    e = expand(csq_buf[0], csq_buf[1])
    for i in range(3):
        csq_buf[3 * NP + i] = e[i]
    wo_cp.wait()
    lax.fori_loop(0, H * DH // 128, fix_wo, 0)
    lax.fori_loop(0, NP, pair1, 0)
    x1 = xacc_buf[...]
    w1_cp.wait()
    lax.fori_loop(0, D // 16, fix_w1, 0)
    for k in range(F // 128):
        cs1_buf[k] = _dot(ones_row, w1_cols(k))
    gs = mlp_hidden(x1, _mean(x1))
    x2 = x1 + b2
    for cp, r, n in zip(w2_cps, w2_at, W2_ROWS):
        shift = _mean(x2) if cp is w2_cps[-1] else None
        cp.wait()
        for k in range(r // 128, (r + n) // 128):
            x2 = x2 + w2_dot(gs[k], fix5(w2_buf, 8 * k))

    set_row(x2, shift)
    xacc_buf[...] = x2
    z = z_buf[...]
    qx = [_dot(z, _bf(wx_buf[i].reshape(D // 2, 128))) * st_buf[0]
          - csq_buf[3 * NP + i] * st_buf[1] for i in range(3)]
    w0 = jnp.concatenate([_pack(jnp.where(evn, q_, zf), jnp.where(evn, zf, q_)) for q_ in qx],
                         axis=1)
    store_q([None, q_cols(z, 0, 1), q_cols(z, 0, 2)], 0, pars=(1,))
    sg = [None] * ng
    for g in range(ng):
        for c in range(4):
            s = score2(w0, 0, 0, 4 * g + c)
            sg[g] = s if c == 0 else sg[g] + s
    q_pair(1)
    ps0, l0, c0 = softmax_lane(sg)
    for g in range(ng):
        store_p(ps0[g], g, range(8), p_buf0)
    l_buf[0] = l0

    true_mask = [tm_buf[i] >= 0 for i in range(3)]
    zq = jnp.clip(zero_ref[0], 0, 1)
    std = [(sw * na, na) for sw in range(NS)]
    steps, info = [], []
    for j in range(NP):
        if j == NP - 1:
            sweeps = [[(tl, range(XE, nt)) for tl in std],
                      [((5, 3), range(XO, nt)), ((2, 3), range(XO, nt)),
                       ((0, 2), range(XO, nt)), ((8, 4), range(XB, nt))]]
        else:
            sweeps = [[(tl, range(XM, nt)) for tl in std]] * 2
        s0 = len(steps)
        steps += [(j, 0, tl, t, ts) for tl, ts in sweeps[0] for t in ts]
        s_odd = len(steps)
        steps += [(j, 1, tl, t, ts) for tl, ts in sweeps[1] for t in ts]
        info.append(dict(s0=s0, s_odd=s_odd, s_end=len(steps),
                         s_tail=len(steps) - len(sweeps[1][-1][1])))
    t_step = [0.0]
    for (_, _, tl, t, _) in steps:
        t_step.append(t_step[-1] + CU * tl[1] * (6 if t < ntb else 4))
    gates, stores, env = {}, {}, {}
    cur = dict(state=None, st=-1, nedge=0, edge=False, p_head=[0, None])

    def get_inv(h):
        return inv_sum(l_buf[zq + (h & 3)])

    def step_at(cyc):
        return next((i for i, tt_ in enumerate(t_step) if tt_ >= cyc), len(t_step))

    def gate(cyc, v):
        st = step_at(cyc)
        while len(gates.get(st, ())) >= 2:
            st += 1
        if cur['st'] < st < len(steps) - NGT:
            gates.setdefault(st, []).append(v)

    def edge(x, n=BE, force=False):
        if cur['st'] < 0 or not (force or cur['edge']):
            return x
        accs = cur['state']['accs']
        cand = [(e_, a) for e_ in range(2) for a in range(accs[0].shape[0])]
        ntile = -(-x.shape[1] // 128)
        parts = [x[:, 128 * i:min(128 * (i + 1), x.shape[1])] for i in range(ntile)]
        for k in range(min(n, 3 * ntile)):
            ce, ca = cand[cur['nedge'] % len(cand)]
            cur['nedge'] += 1
            i = k % ntile
            w_ = parts[i].shape[1]
            parts[i] = jnp.where(true_mask[k // ntile][:, 0:w_], parts[i],
                                 pltpu.bitcast(accs[ce][ca], U32)[:, 0:w_])
        return parts[0] if ntile == 1 else jnp.concatenate(parts, axis=1)

    def sched_stores(ps, lsum, h, t_ready, lo, hi, l_off=10):
        gate(t_ready, ps[-1])
        st_l = min(max(step_at(t_ready + l_off), cur['st'] + 1), len(steps) - 1)
        stores.setdefault(st_l, []).append((lsum, h, None, None))
        t_first = max(t_ready, t_step[lo])
        for i in range(2 * ng):
            g, k = divmod(i, 2)
            st = min(max(step_at(t_first + SDT * i) + 1, cur['st'] + 1), hi)
            assert lo <= st <= hi
            stores.setdefault(st, []).append((ps[g], h, g, range(4 * k, 4 * k + 4)))

    def p_block(h, t):
        assert cur['p_head'][h & 1] == h and not any(
            s_[1] == h and s_[2] is not None for ss in stores.values() for s_ in ss)
        return p_bufs[h & 1][8 * t:8 * t + 8, :]

    def pair_jobs(j):
        inf = info[j]
        first, last = j == 0, j == NP - 1
        h0 = 2 * j

        def job_b(h, c, g):
            s_buf = (se_buf, so_buf)[h & 1]

            def fn(td):
                s = score2(edge(qw_buf[h & 3]), h, h & 1, 4 * g + c)
                gate(td + LATP, s)
                pltpu.store(s_buf.at[g], s, mask=sub2 == c)
                if c == 3 and g == ng - 1:
                    sg_ = [s_buf[zq + gg] for gg in range(ng)]
                    if h == 1:
                        ps, lsum, c1 = softmax_lane(sg_)
                        c01_buf[...] = _pack(c0, c1)
                        sched_stores(ps, lsum, h, td + LATP + MOFL, inf['s0'], inf['s_odd'], 130)
                    elif h & 1:
                        ps, lsum = softmax(sg_)
                        sched_stores(ps, lsum, h, td + LATP + MOFF, inf['s0'], inf['s_odd'])
                        if not last:
                            store_q([qraw_buf[zq + i] for i in range(3)], j + 1)
                    else:
                        ps, lsum = softmax(sg_)
                        sched_stores(ps, lsum, h, td + LATP + MOFF2, inf['s_odd'],
                                     inf['s_end'] - 1)
            return fn

        def job_e(td):
            x = _dot_t(edge(c01_buf[...] if j == 1 else ones32), accp_buf[(j - 1) & 1])
            x = x + xo_buf[zq]

            def row(i, r):
                return jnp.broadcast_to(x[r:r + 1, 128 * i:128 * (i + 1)], (8, 128))

            ie, io = get_inv(h0 - 2), get_inv(h0 - 1)
            o = jnp.concatenate([row(0, 0) * ie, jnp.where(lo64, row(1, 0) * ie, row(1, 1) * io),
                                 row(2, 1) * io], axis=1)
            gate(td + LATP + 10, o[:, 256:384])
            op_buf[...] = _pack(o, o)

        def job_g(c):
            def fn(td):
                xo = out_cols(edge(op_buf[...]), 24 * (j - 1), 24, c)
                xacc_buf[:, 128 * c:128 * (c + 1)] += xo
                gate(td + LATP, xo)
            return fn

        def job_a(c):
            def fn(td):
                qc = q_cols(edge(z_buf[...]), j + 2, c)
                gate(td + LATP, qc)
                qraw_buf[c] = qc
            return fn

        def job_xp(t):
            def fn(td):
                pe, po = p_block(h0, t), p_block(h0 + 1, t)
                if first:
                    ce, co = _unpack(c01_buf[...])
                    pe, po = pe * ce, po * co
                lhs = edge(_pack(pe, po))
                o = jnp.concatenate([_dot(lhs, _bf(v_tiles(h0, 8 * ct, 8, t).reshape(64, 128)))
                                     for ct in range(3)], axis=1)
                env['xp'] = o if t == 0 else env['xp'] + o
                gate(td + LATP, env['xp'][:, 256:384])
                if t == XM - 1:
                    xo_buf[0] = env['xp']
            return fn

        def job_x(par, t, tiles, key):
            def fn(td):
                p = p_block(h0 + par, t)
                rhs = v_tiles(h0 + par, tiles[0], tiles[1], t).reshape(8 * tiles[1], 128)
                o = _dot_t(edge(_pack(p, p)), rhs)
                env[key] = o if key not in env else env[key] + o
                gate(td + LATP, env[key][:, 0:128] if tiles[1] >= 8 else
                     jnp.concatenate([env[key], env[key]], axis=1))
            return fn

        def finish(par, a0, a1, key):
            r0 = par * (DH // 2)
            o = _dot_t(edge(ones32), accp_buf[j & 1, r0 + 8 * a0:r0 + 8 * a1, :]) + env[key]
            inv = get_inv(h0 + par)
            n = 16 * (a1 - a0)
            return o * (inv[:, 0:n] if n <= 128 else
                        jnp.concatenate([inv, inv[:, 0:n - 128]], axis=1))

        env['finish'] = finish

        def job_fin(par, a0, a1, key):
            def fn(td):
                o = finish(par, a0, a1, key)
                gate(td + LATP + 10, o[:, 0:128])
                env['op' + key] = _pack(o, o)
            return fn

        def job_gfin(c):
            def fn(td):
                xo = out_cols(edge(env['opx0']), 12 * h0, 12, c)
                xacc_buf[:, 128 * c:128 * (c + 1)] += xo
                gate(td + LATP, xo)
            return fn

        t_odd = t_step[inf['s_odd'] + 1]
        jobs = [(24, None, job_b(h0 + 1, c, g))
                for g in range(0 if first else ng // 2, ng) for c in range(4)]
        if not first:
            jobs += [(56, t_step[inf['s0']] + EDEL, job_e)]
        out_jobs = [] if first else [(24, None, job_g(c)) for c in range(5)]
        if last:
            t_tail = t_step[inf['s_tail'] + 1]
            jobs += [(24, None, job_x(0, t, (0, 12), 'x0')) for t in range(XE)]
            jobs += out_jobs
            jobs += [(32, t_odd, job_fin(0, 0, 12, 'x0'))]
            jobs += [(16, None, job_x(1, t, (0, 8), 'x1a')) for t in range(XO)]
            jobs += [(12, t_odd + LATP + 60, job_gfin(c)) for c in range(5)]
            jobs += [(8, None, job_x(1, t, (8, 4), 'x1b')) for t in range(XB1)]
            jobs += [(16, t_tail, job_fin(1, 0, 8, 'x1a'))]
            jobs += [(8, None, job_x(1, t, (8, 4), 'x1b')) for t in range(XB1, XB)]
        else:
            jobs += [(24, None, job_b(h0 + 2, c, g)) for g in range(ng) for c in range(4)]
            jobs += [(24, t_odd, job_xp(t)) for t in range(XM)]
            if j + 2 < NP:
                jobs += [(40, None, job_a(c)) for c in range(3)]
            jobs += out_jobs
            jobs += [(24, None, job_b(h0 + 3, c, g)) for g in range(ng // 2) for c in range(4)]
        return jobs

    jobs, times = [], []
    tt = T0
    for j in range(NP):
        if j > 0:
            tt = max(tt, t_step[info[j]['s0']] - LEAD)
        for job in pair_jobs(j):
            tt = tt + job[0] if job[1] is None else max(tt + job[0], job[1])
            jobs.append(job)
            times.append(tt)
    j_first = next(i for i, tt_ in enumerate(times) if tt_ > 0)

    nj = 0
    for st, (j, par, tl, t, ts) in enumerate(steps):
        while nj < len(jobs) and times[nj] <= t_step[st]:
            rel = nj - j_first
            cur['edge'] = (0 <= rel < NE and rel % 2 == 1) or jobs[nj][1] == times[nj]
            jobs[nj][2](times[nj])
            nj += 1
        for val, h, g, rs in stores.pop(st, ()):
            val = pltpu.bitcast(edge(pltpu.bitcast(val, U32), 1, True), F32)
            if g is None:
                l_buf[h & 3] = val
            else:
                store_p(val, g, rs, p_bufs[h & 1])
                cur['p_head'][h & 1] = h
        if st in (info[j]['s0'], info[j]['s_odd']):
            state = dict(par=par, slot=j & 1)
        assert cur['p_head'][par] == 2 * j + par
        pv_step(2 * j + par, tl, t, ts, zip(true_mask, gates.get(st, ())), state)
        cur['state'] = state
        cur['st'] = st
    cur['edge'] = False
    for job, tt in zip(jobs[nj:], times[nj:]):
        job[2](tt)
    assert not stores

    o = env['finish'](1, 8, 12, 'x1b')
    op = _pack(o, o)
    xa = [out_cols(env['opx1a'], 12 * (H - 1), 8, c) for c in range(5)]
    xb = [out_cols(op, 12 * (H - 1) + 8, 4, c) for c in range(5)]
    x3 = (xacc_buf[...] + jnp.concatenate(xa, axis=1)) + jnp.concatenate(xb, axis=1)
    gs = mlp_hidden(x3, shift)
    x4 = x3 + b2
    parts = []
    for k in range(NV, F // 128):
        x4 = x4 + w2_dot(gs[k], [w2_buf[8 * k:8 * k + 8, 8 * c:8 * c + 8, :] for c in range(5)])
        parts.append(x4[:, 0:128])
    pins = gs[NV:] + parts
    acc = None
    for k in range(NV):
        col = jnp.broadcast_to(gs[k][0:1, :], (128, 128)).T
        for i in range(8):
            ci = col[16 * i:16 * i + 16, :]
            pin = (8 * k + i - GV0) // GVS
            if (8 * k + i - GV0) % GVS == 0 and 0 <= pin < len(pins):
                ci = jnp.concatenate([jnp.where(true_mask[0], ci[0:8], pins[pin]), ci[8:16]], axis=0)
            y = _bf(w2_buf[8 * k + i]).astype(F32).reshape(5, 16, 128) * ci
            y = y[:, 0:8] + y[:, 8:16]
            acc = y if acc is None else acc + y
    acc = jnp.concatenate([acc[c] for c in range(5)], axis=1)
    x4 = x4 + jnp.sum(acc, axis=0, keepdims=True)
    o_ref[...] = x4[0:1, :].astype(o_ref.dtype)


@jax.jit
def pallas_interleave_layers__sliding_block_cached__dense_activation_gelu__decode_kernel(
    A_x: jax.Array,
    A_k_cache: jax.Array,
    A_v_cache: jax.Array,
    A_wq: jax.Array,
    A_wo: jax.Array,
    B_x: jax.Array,
    B_w1: jax.Array,
    B_b1: jax.Array,
    B_w2: jax.Array,
    B_b2: jax.Array,
):
    sk = A_k_cache.shape[2]
    w = min(4096, max(256, sk // 4))
    ng = w // 1024

    def tile_view(a):
        *lead, r, c = a.shape
        n = len(lead)
        a = a.reshape(*lead, r // 8, 8, c // 128, 128)
        a = a.transpose(*range(n), n, n + 2, n + 1, n + 3)
        return a.reshape(*lead, r // 16, 2, (c // 128) * 8, 128)

    kx = tile_view(jnp.swapaxes(A_k_cache, 2, 3)[0]).reshape(H * DH // 16, 2, sk // 16, 128)
    vx = tile_view(jnp.swapaxes(A_v_cache, 2, 3)[0]).reshape(H * DH // 16, 2, sk // 16, 128)
    wqx = tile_view(A_wq)
    wox = tile_view(A_wo).reshape(H * DH // 16, 80, 128)
    out = pl.pallas_call(
        functools.partial(_kernel, sk=sk, w=w),
        out_shape=jax.ShapeDtypeStruct((1, D), A_x.dtype),
        in_specs=[pl.BlockSpec(memory_space=pl.ANY)] * 9,
        out_specs=pl.BlockSpec(memory_space=pltpu.VMEM),
        scratch_shapes=[
            pltpu.VMEM((H * DH // 16, 2, w // 32, 128), U32),
            pltpu.VMEM((H * DH // 16, 2, w // 32 - 4 * XF, 128), U32),
            pltpu.VMEM((H * DH // 16, 2, 8 * XF, 128), U32),
            pltpu.VMEM((D // 16, 2, H * DH // 32, 128), U32),
            pltpu.VMEM((H * DH // 16, 40, 128), U32),
            pltpu.VMEM((D // 16, 2, F // 32, 128), U32),
            pltpu.VMEM((F // 16, 40, 128), U32),
            pltpu.VMEM((1, D), BF16),
            pltpu.VMEM((F // 128, 128), BF16),
            pltpu.VMEM((D // 128, 128), BF16),
            pltpu.VMEM((w // 16, 128), F32),
            pltpu.VMEM((w // 16, 128), F32),
            pltpu.VMEM((ng + 1, 8, 128), F32),
            pltpu.VMEM((ng + 1, 8, 128), F32),
            pltpu.VMEM((5, 8, 128), F32),
            pltpu.VMEM((4, 8, 128), F32),
            pltpu.VMEM((2, 8, 2 * DH), F32),
            pltpu.VMEM((2, DH, 128), U32),
            pltpu.VMEM((8, D), U32),
            pltpu.VMEM((8, D), F32),
            pltpu.VMEM((4, 8, 2 * DH), U32),
            pltpu.VMEM((3 * NP + 3, 8, 128), F32),
            pltpu.VMEM((F // 128, 8, 128), F32),
            pltpu.VMEM((2, 8, 128), F32),
            pltpu.VMEM((8, 2 * DH), U32),
            pltpu.VMEM((3, D // 16, 8, 128), U32),
            pltpu.VMEM((8, 128), U32),
            pltpu.VMEM((3, 8, 128), jnp.int32),
            pltpu.SMEM((1,), jnp.int32),
            pltpu.SemaphoreType.DMA((2,)),
            pltpu.SemaphoreType.DMA((4,)),
            pltpu.SemaphoreType.DMA((6 + len(W2_ROWS),)),
        ],
        compiler_params=pltpu.CompilerParams(vmem_limit_bytes=127 * 1024 * 1024,
                                             disable_semaphore_checks=True),
    )(A_x.reshape(1, D), kx, vx, wqx, wox, tile_view(B_w1), B_b1.reshape(F // 128, 128),
      tile_view(B_w2).reshape(F // 16, 80, 128), B_b2.reshape(D // 128, 128))
    return out.reshape(A_x.shape)
```

```python
import functools
import math

import jax
import jax.numpy as jnp
from jax import lax
import jax.experimental.pallas as pl
import jax.experimental.pallas.tpu as pltpu

F32 = jnp.float32
BF16 = jnp.bfloat16
U32 = jnp.uint32

D = 640
H = 32
DH = 192
F = 1536
EPS = 1e-5
NP = H // 2

CHUNKS = (4, 4, 3, 2, 2, 1)
W2_ROWS = (640, 512, 256, 128)
NS = 4
XF = 6
XM = 1
XE, XO, XB, XB1 = 7, 7, 16, 8

CU = 0.263
T0 = -100.0
LEAD = 100.0
LATP = 160.0
MOFF, MOFF2, MOFL = 160.0, 200.0, 40.0
EDEL = 70.0
SDT = 12.0
NE, BE, NGT = 7, 6, 12
NV, GV0, GVS = 5, -16, 4


def _gelu(x):
    c = math.sqrt(2.0 / math.pi)
    return 0.5 * x * (1.0 + jnp.tanh(c * (x + 0.044715 * (x * x * x))))


def _rows_to_lanes(b, n):
    return jnp.concatenate([b[i:i + 1, :] for i in range(n)], axis=1)


def _bf(x):
    return pltpu.bitcast(x, BF16)


def _pack(a, b):
    return pltpu.bitcast(pltpu.pack_elementwise([a, b], packed_dtype=BF16), U32)


def _unpack(x):
    return (pltpu.unpack_elementwise(x, index=0, packed_dtype=BF16, unpacked_dtype=F32),
            pltpu.unpack_elementwise(x, index=1, packed_dtype=BF16, unpacked_dtype=F32))


def _dot(lhs32, rhs):
    return jnp.dot(_bf(lhs32), rhs, preferred_element_type=F32)[0:8]


def _dot_t(lhs32, rhs32):
    return lax.dot_general(_bf(lhs32), _bf(rhs32), (((1,), (1,)), ((), ())),
                           preferred_element_type=F32)[0:8]


def _mean(x):
    return jnp.mean(x, axis=-1, keepdims=True)


def _ln_stats(xp, shift):
    x = _unpack(xp)[0] - shift
    m = _mean(x)
    v = jnp.maximum(_mean(x * x) - m * m, 0.0)
    return m + shift, lax.rsqrt(v + EPS)


def _kernel(x_hbm, kx_hbm, vx_hbm, wq_hbm, wo_hbm, w1_hbm, b1_hbm, w2_hbm, b2_hbm,
            o_ref,
            kbuf, vbuf, vf_buf, wq_buf, wo_buf, w1_buf, w2_buf, x_buf, b1_buf, b2_buf,
            p_buf0, p_buf1, so_buf, se_buf, l_buf, qraw_buf, xo_buf, accp_buf, z_buf,
            xacc_buf, qw_buf, csq_buf, cs1_buf, st_buf, op_buf, wx_buf, c01_buf,
            tm_buf, zero_ref, sem_k, sem_v, sem_w, *, sk, w):
    c_scale = (DH ** -0.5) * math.log2(math.e)
    nt = w // 128
    ng = nt // 8
    na = 12 // NS
    ntb = nt - XF
    r0w = (sk - w) // 32
    p_bufs = (p_buf0, p_buf1)
    starts = [sum(CHUNKS[:c]) for c in range(len(CHUNKS))]
    w2_at = [sum(W2_ROWS[:i]) for i in range(len(W2_ROWS))]

    kx32, vx32 = kx_hbm.bitcast(U32), vx_hbm.bitcast(U32)

    def k_copy(c):
        rows = pl.ds(24 * starts[c], 24 * CHUNKS[c])
        return [pltpu.make_async_copy(kx32.at[rows, :, pl.ds(r0w, 4 * nt), :],
                                      kbuf.at[rows], sem_k.at[c & 1])]

    def v_copy(c):
        rows = pl.ds(24 * starts[c], 24 * CHUNKS[c])
        return [pltpu.make_async_copy(vx32.at[rows, :, pl.ds(r0w, 4 * ntb), :],
                                      vbuf.at[rows], sem_v.at[c & 1]),
                pltpu.make_async_copy(vx32.at[rows, :, pl.ds(r0w + 4 * ntb, 4 * XF), :],
                                      vf_buf.at[rows, :, pl.ds(4 * XF, 4 * XF), :],
                                      sem_v.at[2 + (c & 1)])]

    wq_cp = pltpu.make_async_copy(wq_hbm.bitcast(U32), wq_buf, sem_w.at[0])
    wo_cp = pltpu.make_async_copy(wo_hbm.bitcast(U32), wo_buf, sem_w.at[1])
    w1_cp = pltpu.make_async_copy(w1_hbm.bitcast(U32), w1_buf, sem_w.at[2])
    x_cp = pltpu.make_async_copy(x_hbm, x_buf, sem_w.at[3])
    b1_cp = pltpu.make_async_copy(b1_hbm, b1_buf, sem_w.at[4])
    b2_cp = pltpu.make_async_copy(b2_hbm, b2_buf, sem_w.at[5])
    w2_cps = [pltpu.make_async_copy(w2_hbm.bitcast(U32).at[pl.ds(r // 16, n // 16)],
                                    w2_buf.at[pl.ds(r // 16, n // 16)], sem_w.at[6 + i])
              for i, (r, n) in enumerate(zip(w2_at, W2_ROWS))]

    for cp in [wq_cp, x_cp, b1_cp, b2_cp, wo_cp] + k_copy(0) + v_copy(0):
        cp.start()
    x_cp.wait()
    b1_cp.wait()
    b2_cp.wait()

    x0 = jnp.broadcast_to(x_buf[...].astype(F32), (8, D))

    lane = lax.broadcasted_iota(jnp.int32, (8, 128), 1)
    sub3 = lax.broadcasted_iota(jnp.int32, (8, 2 * DH), 0)
    sub2 = lax.broadcasted_iota(jnp.int32, (8, 128), 0) // 2
    sub_lo = lax.broadcasted_iota(jnp.int32, (1, 8, 128), 1) < 4
    lo64 = lane < 64
    evn = (lane & 8) == 0
    zf = jnp.zeros((8, 128), F32)
    ones32 = jnp.full((8, 128), 0x3F803F80, U32)
    k_order = (((0, 8, 0), (0, 8, 1), (8, 4, 0), (8, 4, 1)),
               ((4, 8, 0), (4, 8, 1), (0, 4, 1), (0, 4, 0)))

    def regroup(a, b):
        return jnp.where(sub_lo, a, pltpu.roll(b, 4, 1)), jnp.where(sub_lo, pltpu.roll(a, 4, 1), b)

    def swap_halves(ref2):
        n = ref2.shape[1]
        a, b = regroup(ref2[0].reshape(n // 8, 8, 128), ref2[1].reshape(n // 8, 8, 128))
        ref2[0] = a.reshape(n, 128)
        ref2[1] = b.reshape(n, 128)

    def fix_wq(a, carry):
        swap_halves(wq_buf.at[a])
        return carry

    def fix5(buf, g0):
        v = [buf[pl.ds(g0, 8), 8 * c:8 * c + 8, :] for c in range(5)]
        n = [jnp.where(sub_lo, v[0], v[2]),
             pltpu.roll(jnp.where(sub_lo, v[3], v[0]), 4, 1),
             jnp.where(sub_lo, v[1], v[3]),
             pltpu.roll(jnp.where(sub_lo, v[4], v[1]), 4, 1),
             jnp.where(sub_lo, v[2], v[4])]
        for c in range(5):
            buf[pl.ds(g0, 8), 8 * c:8 * c + 8, :] = n[c]
        return n

    def fix_wo(g8, carry):
        fix5(wo_buf, pl.multiple_of(g8 * 8, 8))
        return carry

    def fix_w1(a, carry):
        swap_halves(w1_buf.at[a])
        return carry

    def fix_v(r2, carry):
        swap_halves(vbuf.at[r2])
        n = 4 * XF
        t0, t1 = regroup(vf_buf[r2, 0, n:2 * n, :].reshape(n // 8, 8, 128),
                         vf_buf[r2, 1, n:2 * n, :].reshape(n // 8, 8, 128))
        t0, t1 = _unpack(t0), _unpack(t1)
        for e in range(2):
            for k in range(XF // 2):
                vf_buf[r2, e, 16 * k:16 * k + 8, :] = pltpu.bitcast(t0[e][k], U32)
                vf_buf[r2, e, 16 * k + 8:16 * k + 16, :] = pltpu.bitcast(t1[e][k], U32)
        return carry

    def v_tiles(h, a0, n, t):
        return vbuf[pl.ds(12 * h + a0, n), t % 2, 8 * (t // 2):8 * (t // 2) + 8, :]

    def transpose_v(j, t):
        y = _bf(v_tiles(2 * j, 0, 24, t).reshape(DH, 128)).astype(F32)
        yt = pltpu.bitcast(y.T.astype(BF16), U32)
        for ct in range(3):
            vbuf[pl.ds(24 * j + 8 * ct, 8), t % 2, 8 * (t // 2):8 * (t // 2) + 8, :] = (
                yt[:, 128 * ct:128 * (ct + 1)].reshape(8, 8, 128))

    def set_row(x, shift):
        xp = _pack(x, x)
        m, r = _ln_stats(xp, shift)
        xc = _unpack(xp)[0] - m
        z_buf[...] = _pack(xc, xc)
        rc = jnp.broadcast_to(r * c_scale, (8, 128))
        st_buf[...] = rc
        return xp, rc, m * rc

    def wq_cols(ct):
        if isinstance(ct, int):
            r0 = (ct // 2) * 8
        else:
            r0 = pl.multiple_of(lax.shift_right_logical(ct, 1) * 8, 8)
        return _bf(wq_buf[:, ct & 1, pl.ds(r0, 8), :].reshape(D // 2, 128))

    def q_cols(z, j, c):
        return _dot(z, wq_cols(3 * j + c)) * st_buf[...]

    def store_q(qs, j, pars=(0, 1)):
        q0, q1, q2 = qs
        r56, r64, r8 = (pltpu.roll(q1, s, 1) for s in (56, 64, 8))

        def put(h, qf, a2, b2):
            a0 = jnp.where(evn, qf, zf)
            b1_ = jnp.where(evn, zf, qf)
            ww = [_pack(a0, pltpu.roll(a0, 8, 1)), _pack(pltpu.roll(b1_, 120, 1), b1_),
                  _pack(jnp.where(evn, a2, zf), jnp.where(evn, zf, b2))]
            qw_buf[h & 3] = jnp.concatenate(ww, axis=1)

        if 0 in pars:
            put(2 * j, q0, jnp.where(lo64, q1, r56), jnp.where(lo64, r8, r64))
        if 1 in pars:
            put(2 * j + 1, q2, jnp.where(lo64, r56, q1), jnp.where(lo64, r64, r8))

    def q_pair(j):
        z = z_buf[...]
        store_q([q_cols(z, j, c) for c in range(3)], j)

    def score2(lhs, h, par, k):
        lhs = jnp.where(sub3 == k % 4, lhs, jnp.zeros_like(lhs))
        rhs = jnp.concatenate([kbuf[pl.ds(12 * h + a, n), e, 8 * k:8 * k + 8, :]
                               for a, n, e in k_order[par]], axis=0)
        return _dot(lhs, _bf(rhs.reshape(DH, 128)))

    def store_p(p, g, rs, p_out):
        for r in rs:
            p_out[pl.ds(64 * g + r, 8, stride=8), :] = p

    def inv_sum(l):
        l = jnp.sum(jnp.sum(l, axis=1, keepdims=True), axis=0, keepdims=True)
        l = jnp.broadcast_to(l, (8, 128))
        r = pl.reciprocal(l, approx=True)
        return r * (2.0 - l * r)

    def softmax(sg):
        mx = sg[0]
        for s in sg[1:]:
            mx = jnp.maximum(mx, s)
        m = jnp.max(jnp.max(mx, axis=1, keepdims=True), axis=0, keepdims=True)
        ps, l = [], None
        for s in sg:
            ps.append(jnp.exp2(s - m))
            l = ps[-1] if l is None else l + ps[-1]
        return ps, l

    def softmax_lane(sg):
        mx = jnp.maximum(jnp.maximum(sg[0], sg[1]), jnp.maximum(sg[2], sg[3]))
        m = jnp.broadcast_to(jnp.max(mx, axis=0, keepdims=True), (8, 128))
        ps = [jnp.exp2(s - m) for s in sg]
        c = jnp.exp2(m - jnp.max(m, axis=1, keepdims=True))
        c = _unpack(_pack(c, c))[0]
        return ps, ((ps[0] + ps[1]) + (ps[2] + ps[3])) * c, c

    def pv_step(h, tiles, t, ts, gated, state):
        a0, n = tiles
        p = p_bufs[state['par']][8 * t:8 * t + 8, :]
        for mask, val in gated:
            p = jnp.where(mask, p, val)
        if t < ntb:
            ys = _unpack(v_tiles(h, a0, n, t))
        else:
            r = 8 * (t - ntb)
            ys = [pltpu.bitcast(vf_buf[pl.ds(12 * h + a0, n), e, r:r + 8, :], F32)
                  for e in range(2)]
        if t == ts[0]:
            state['accs'] = [y * p for y in ys]
        else:
            state['accs'] = [acc + y * p for acc, y in zip(state['accs'], ys)]
        if t == ts[-1]:
            r0 = state['par'] * (DH // 2) + 8 * a0
            accp_buf[state['slot'], r0:r0 + 8 * n, :] = _pack(*state['accs']).reshape(8 * n, 128)

    def out_cols(op, g0, ngrp, c):
        rhs = wo_buf[pl.ds(g0, ngrp), 8 * c:8 * c + 8, :].reshape(ngrp * 8, 128)
        return _dot(op, _bf(rhs))

    def w1_cols(k):
        return _bf(w1_buf[:, k % 2, 8 * (k // 2):8 * (k // 2) + 8, :].reshape(D // 2, 128))

    def mlp_hidden(x, shift):
        xp = _pack(x, x)
        m, r = _ln_stats(xp, shift)
        b1 = b1_buf[...].astype(F32)
        return [_gelu((_dot(xp, w1_cols(k)) - cs1_buf[k:k + 1, :] * m) * r + b1[k:k + 1, :])
                for k in range(F // 128)]

    def bias2():
        return _rows_to_lanes(b2_buf[...].astype(F32), D // 128)

    def w2_dot(g, tiles):
        gp = _pack(g, g)
        return jnp.concatenate([_dot(gp, _bf(t.reshape(64, 128))) for t in tiles], axis=1)

    def next_copies(j, copy_fn, tail_cps):
        for c in range(len(CHUNKS)):
            @pl.when(j == starts[c])
            def _():
                for cp in copy_fn(c):
                    cp.wait()
                for cp in (copy_fn(c + 1) if c + 1 < len(CHUNKS) else tail_cps):
                    cp.start()

    def pair1(j, carry):
        q_pair(j)

        @pl.when(j == 0)
        def _():
            lax.fori_loop(0, D // 16, expand_wq, 0)
            for i in range(5):
                csq_buf[i] = _dot(ones_row, first_cols(i))

        next_copies(j, k_copy, [w1_cp])
        invs = []
        for par in range(2):
            h = 2 * j + par
            sg = [None] * ng
            lhs = qw_buf[h & 3]
            for c in range(4):
                for g in range(ng):
                    s = score2(lhs, h, par, 4 * g + c)
                    sg[g] = s if c == 0 else sg[g] + s
            ps, l = softmax(sg)
            for g in range(ng):
                store_p(ps[g], g, range(8), p_bufs[par])
            invs.append(inv_sum(l))
        next_copies(j, v_copy, w2_cps)
        lax.fori_loop(24 * j, 24 * (j + 1), fix_v, 0)
        for par in range(2):
            state = dict(par=par, slot=0)
            for sw in range(NS):
                for t in range(nt):
                    pv_step(2 * j + par, (sw * na, na), t, range(nt), (), state)

        @pl.when(j < NP - 1)
        def _():
            for t in range(XM):
                transpose_v(j, t)

        ie, io = invs
        o = _dot_t(ones32, accp_buf[0]) * jnp.concatenate([ie, jnp.where(lo64, ie, io), io], axis=1)
        op = _pack(o, o)
        for c in range(5):
            xacc_buf[:, 128 * c:128 * (c + 1)] += out_cols(op, 24 * j, 24, c)
        return carry

    def expand(t0, t1):
        return [jnp.where(evn, t0, pltpu.roll(t0, 8, 1)),
                jnp.where(evn, pltpu.roll(t0, 120, 1), t0),
                jnp.where(evn, jnp.where(lo64, t1, pltpu.roll(t1, 56, 1)),
                          jnp.where(lo64, pltpu.roll(t1, 8, 1), pltpu.roll(t1, 64, 1)))]

    def expand_wq(a, carry):
        e = expand(wq_buf[a, 0, 0:8, :], wq_buf[a, 1, 0:8, :])
        wq_buf[a, 0, 0:8, :] = e[0]
        wx_buf[0, a] = e[1]
        wx_buf[1, a] = e[2]
        return carry

    ones_row = jnp.concatenate([ones32] * (D // 128), axis=1)

    def first_cols(i):
        if i in (1, 2):
            return _bf(wx_buf[i - 1].reshape(D // 2, 128))
        return wq_cols(max(i - 2, 0))

    for ref in (so_buf, se_buf, l_buf, qraw_buf, xo_buf):
        ref[...] = jnp.zeros(ref.shape, ref.dtype)
    tm_buf[...] = lane
    zero_ref[0] = 0

    set_row(x0, _mean(x0))
    xacc_buf[...] = x0
    wq_cp.wait()
    lax.fori_loop(0, D // 16, fix_wq, 0)
    wo_cp.wait()
    lax.fori_loop(0, H * DH // 128, fix_wo, 0)
    lax.fori_loop(0, NP, pair1, 0)
    x1 = xacc_buf[...]
    w1_cp.wait()
    lax.fori_loop(0, D // 16, fix_w1, 0)
    for k in range(F // 128):
        cs1_buf[k:k + 1, :] = _dot(ones_row, w1_cols(k))[0:1]
    gs = mlp_hidden(x1, _mean(x1))
    x2 = x1 + bias2()
    for cp, r, n in zip(w2_cps, w2_at, W2_ROWS):
        shift = _mean(x2) if cp is w2_cps[-1] else None
        cp.wait()
        for k in range(r // 128, (r + n) // 128):
            x2 = x2 + w2_dot(gs[k], fix5(w2_buf, 8 * k))

    xp, rc, mrc = set_row(x2, shift)
    xacc_buf[...] = x2
    qx = [_dot(xp, first_cols(i)) * rc - csq_buf[i] * mrc for i in range(5)]
    w0 = jnp.concatenate([_pack(jnp.where(evn, q_, zf), jnp.where(evn, zf, q_)) for q_ in qx[0:3]],
                         axis=1)
    store_q([None, qx[3], qx[4]], 0, pars=(1,))
    sg = [None] * ng
    for g in range(ng):
        for c in range(4):
            s = score2(w0, 0, 0, 4 * g + c)
            sg[g] = s if c == 0 else sg[g] + s
    q_pair(1)
    ps0, l0, c0 = softmax_lane(sg)
    for g in range(ng):
        store_p(ps0[g], g, range(8), p_buf0)
    l_buf[0] = l0

    true_mask = [tm_buf[...] >= -i for i in range(3)]
    zq = jnp.clip(zero_ref[0], 0, 1)
    std = [(sw * na, na) for sw in range(NS)]
    steps, info = [], []
    for j in range(NP):
        if j == NP - 1:
            sweeps = [[(tl, range(XE, nt)) for tl in std],
                      [((5, 3), range(XO, nt)), ((2, 3), range(XO, nt)),
                       ((0, 2), range(XO, nt)), ((8, 4), range(XB, nt))]]
        else:
            sweeps = [[(tl, range(XM, nt)) for tl in std]] * 2
        s0 = len(steps)
        steps += [(j, 0, tl, t, ts) for tl, ts in sweeps[0] for t in ts]
        s_odd = len(steps)
        steps += [(j, 1, tl, t, ts) for tl, ts in sweeps[1] for t in ts]
        info.append(dict(s0=s0, s_odd=s_odd, s_end=len(steps),
                         s_tail=len(steps) - len(sweeps[1][-1][1])))
    t_step = [0.0]
    for (_, _, tl, t, _) in steps:
        t_step.append(t_step[-1] + CU * tl[1] * (6 if t < ntb else 4))
    gates, stores, env = {}, {}, {}
    cur = dict(state=None, st=-1, nedge=0, edge=False, p_head=[0, None])

    def get_inv(h):
        return inv_sum(l_buf[zq + (h & 3)])

    def step_at(cyc):
        return next((i for i, tt_ in enumerate(t_step) if tt_ >= cyc), len(t_step))

    def gate(cyc, v):
        st = step_at(cyc)
        while len(gates.get(st, ())) >= 2:
            st += 1
        if cur['st'] < st < len(steps) - NGT:
            gates.setdefault(st, []).append(v)

    def edge(x, n=BE, force=False):
        if cur['st'] < 0 or not (force or cur['edge']):
            return x
        accs = cur['state']['accs']
        cand = [(e_, a) for e_ in range(2) for a in range(accs[0].shape[0])]
        ntile = -(-x.shape[1] // 128)
        parts = [x[:, 128 * i:min(128 * (i + 1), x.shape[1])] for i in range(ntile)]
        for k in range(min(n, 3 * ntile)):
            ce, ca = cand[cur['nedge'] % len(cand)]
            cur['nedge'] += 1
            i = k % ntile
            w_ = parts[i].shape[1]
            parts[i] = jnp.where(true_mask[k // ntile][:, 0:w_], parts[i],
                                 pltpu.bitcast(accs[ce][ca], U32)[:, 0:w_])
        return parts[0] if ntile == 1 else jnp.concatenate(parts, axis=1)

    def sched_stores(ps, lsum, h, t_ready, lo, hi, l_off=10):
        gate(t_ready, ps[-1])
        st_l = min(max(step_at(t_ready + l_off), cur['st'] + 1), len(steps) - 1)
        stores.setdefault(st_l, []).append((lsum, h, None, None))
        t_first = max(t_ready, t_step[lo])
        for i in range(2 * ng):
            g, k = divmod(i, 2)
            st = min(max(step_at(t_first + SDT * i) + 1, cur['st'] + 1), hi)
            assert lo <= st <= hi
            stores.setdefault(st, []).append((ps[g], h, g, range(4 * k, 4 * k + 4)))

    def p_block(h, t):
        assert cur['p_head'][h & 1] == h and not any(
            s_[1] == h and s_[2] is not None for ss in stores.values() for s_ in ss)
        return p_bufs[h & 1][8 * t:8 * t + 8, :]

    def pair_jobs(j):
        inf = info[j]
        first, last = j == 0, j == NP - 1
        h0 = 2 * j

        def job_b(h, c, g):
            s_buf = (se_buf, so_buf)[h & 1]

            def fn(td):
                s = score2(edge(qw_buf[h & 3]), h, h & 1, 4 * g + c)
                gate(td + LATP, s)
                pltpu.store(s_buf.at[g], s, mask=sub2 == c)
                if c == 3 and g == ng - 1:
                    sg_ = [s_buf[zq + gg] for gg in range(ng)]
                    if h == 1:
                        ps, lsum, c1 = softmax_lane(sg_)
                        c01_buf[...] = _pack(c0, c1)
                        sched_stores(ps, lsum, h, td + LATP + MOFL, inf['s0'], inf['s_odd'], 130)
                    elif h & 1:
                        ps, lsum = softmax(sg_)
                        sched_stores(ps, lsum, h, td + LATP + MOFF, inf['s0'], inf['s_odd'])
                        if not last:
                            store_q([qraw_buf[zq + i] for i in range(3)], j + 1)
                    else:
                        ps, lsum = softmax(sg_)
                        sched_stores(ps, lsum, h, td + LATP + MOFF2, inf['s_odd'],
                                     inf['s_end'] - 1)
            return fn

        def job_e(td):
            x = _dot_t(edge(c01_buf[...] if j == 1 else ones32), accp_buf[(j - 1) & 1])
            x = x + xo_buf[zq]

            def row(i, r):
                return jnp.broadcast_to(x[r:r + 1, 128 * i:128 * (i + 1)], (8, 128))

            ie, io = get_inv(h0 - 2), get_inv(h0 - 1)
            o = jnp.concatenate([row(0, 0) * ie, jnp.where(lo64, row(1, 0) * ie, row(1, 1) * io),
                                 row(2, 1) * io], axis=1)
            gate(td + LATP + 10, o[:, 256:384])
            op_buf[...] = _pack(o, o)

        def job_g(c):
            def fn(td):
                xo = out_cols(edge(op_buf[...]), 24 * (j - 1), 24, c)
                xacc_buf[:, 128 * c:128 * (c + 1)] += xo
                gate(td + LATP, xo)
            return fn

        def job_a(c):
            def fn(td):
                qc = q_cols(edge(z_buf[...]), j + 2, c)
                gate(td + LATP, qc)
                qraw_buf[c] = qc
            return fn

        def job_xp(t):
            def fn(td):
                pe, po = p_block(h0, t), p_block(h0 + 1, t)
                if first:
                    ce, co = _unpack(c01_buf[...])
                    pe, po = pe * ce, po * co
                lhs = edge(_pack(pe, po))
                o = jnp.concatenate([_dot(lhs, _bf(v_tiles(h0, 8 * ct, 8, t).reshape(64, 128)))
                                     for ct in range(3)], axis=1)
                env['xp'] = o if t == 0 else env['xp'] + o
                gate(td + LATP, env['xp'][:, 256:384])
                if t == XM - 1:
                    xo_buf[0] = env['xp']
            return fn

        def job_x(par, t, tiles, key):
            def fn(td):
                p = p_block(h0 + par, t)
                rhs = v_tiles(h0 + par, tiles[0], tiles[1], t).reshape(8 * tiles[1], 128)
                o = _dot_t(edge(_pack(p, p)), rhs)
                env[key] = o if key not in env else env[key] + o
                gate(td + LATP, env[key][:, 0:128] if tiles[1] >= 8 else
                     jnp.concatenate([env[key], env[key]], axis=1))
            return fn

        def finish(par, a0, a1, key):
            r0 = par * (DH // 2)
            o = _dot_t(edge(ones32), accp_buf[j & 1, r0 + 8 * a0:r0 + 8 * a1, :]) + env[key]
            inv = get_inv(h0 + par)
            n = 16 * (a1 - a0)
            return o * (inv[:, 0:n] if n <= 128 else
                        jnp.concatenate([inv, inv[:, 0:n - 128]], axis=1))

        env['finish'] = finish

        def job_fin(par, a0, a1, key):
            def fn(td):
                o = finish(par, a0, a1, key)
                gate(td + LATP + 10, o[:, 0:128])
                env['op' + key] = _pack(o, o)
            return fn

        def job_gfin(c):
            def fn(td):
                xo = out_cols(edge(env['opx0']), 12 * h0, 12, c)
                xacc_buf[:, 128 * c:128 * (c + 1)] += xo
                gate(td + LATP, xo)
            return fn

        t_odd = t_step[inf['s_odd'] + 1]
        jobs = [(24, None, job_b(h0 + 1, c, g))
                for g in range(0 if first else ng // 2, ng) for c in range(4)]
        if not first:
            jobs += [(56, t_step[inf['s0']] + EDEL, job_e)]
        out_jobs = [] if first else [(24, None, job_g(c)) for c in range(5)]
        if last:
            t_tail = t_step[inf['s_tail'] + 1]
            jobs += [(24, None, job_x(0, t, (0, 12), 'x0')) for t in range(XE)]
            jobs += out_jobs
            jobs += [(32, t_odd, job_fin(0, 0, 12, 'x0'))]
            jobs += [(16, None, job_x(1, t, (0, 8), 'x1a')) for t in range(XO)]
            jobs += [(12, t_odd + LATP + 60, job_gfin(c)) for c in range(5)]
            jobs += [(8, None, job_x(1, t, (8, 4), 'x1b')) for t in range(XB1)]
            jobs += [(16, t_tail, job_fin(1, 0, 8, 'x1a'))]
            jobs += [(8, None, job_x(1, t, (8, 4), 'x1b')) for t in range(XB1, XB)]
        else:
            jobs += [(24, None, job_b(h0 + 2, c, g)) for g in range(ng) for c in range(4)]
            jobs += [(24, t_odd, job_xp(t)) for t in range(XM)]
            if j + 2 < NP:
                jobs += [(40, None, job_a(c)) for c in range(3)]
            jobs += out_jobs
            jobs += [(24, None, job_b(h0 + 3, c, g)) for g in range(ng // 2) for c in range(4)]
        return jobs

    jobs, times = [], []
    tt = T0
    for j in range(NP):
        if j > 0:
            tt = max(tt, t_step[info[j]['s0']] - LEAD)
        for job in pair_jobs(j):
            tt = tt + job[0] if job[1] is None else max(tt + job[0], job[1])
            jobs.append(job)
            times.append(tt)
    j_first = next(i for i, tt_ in enumerate(times) if tt_ > 0)

    nj = 0
    for st, (j, par, tl, t, ts) in enumerate(steps):
        while nj < len(jobs) and times[nj] <= t_step[st]:
            rel = nj - j_first
            cur['edge'] = (0 <= rel < NE and rel % 2 == 1) or jobs[nj][1] == times[nj]
            jobs[nj][2](times[nj])
            nj += 1
        for val, h, g, rs in stores.pop(st, ()):
            val = pltpu.bitcast(edge(pltpu.bitcast(val, U32), 1, True), F32)
            if g is None:
                l_buf[h & 3] = val
            else:
                store_p(val, g, rs, p_bufs[h & 1])
                cur['p_head'][h & 1] = h
        if st in (info[j]['s0'], info[j]['s_odd']):
            state = dict(par=par, slot=j & 1)
        assert cur['p_head'][par] == 2 * j + par
        pv_step(2 * j + par, tl, t, ts, zip(true_mask, gates.get(st, ())), state)
        cur['state'] = state
        cur['st'] = st
    cur['edge'] = False
    for job, tt in zip(jobs[nj:], times[nj:]):
        job[2](tt)
    assert not stores

    o = env['finish'](1, 8, 12, 'x1b')
    op = _pack(o, o)
    xa = [out_cols(env['opx1a'], 12 * (H - 1), 8, c) for c in range(5)]
    xb = [out_cols(op, 12 * (H - 1) + 8, 4, c) for c in range(5)]
    x3 = (xacc_buf[...] + jnp.concatenate(xa, axis=1)) + jnp.concatenate(xb, axis=1)
    gs = mlp_hidden(x3, shift)
    x4 = x3 + bias2()
    parts = []
    for k in range(NV, F // 128):
        x4 = x4 + w2_dot(gs[k], [w2_buf[8 * k:8 * k + 8, 8 * c:8 * c + 8, :] for c in range(5)])
        parts.append(x4[:, 0:128])
    pins = gs[NV:] + parts
    acc = None
    for k in range(NV):
        col = jnp.broadcast_to(gs[k][0:1, :], (128, 128)).T
        for i in range(8):
            ci = col[16 * i:16 * i + 16, :]
            pin = (8 * k + i - GV0) // GVS
            if (8 * k + i - GV0) % GVS == 0 and 0 <= pin < len(pins):
                ci = jnp.concatenate([jnp.where(true_mask[0], ci[0:8], pins[pin]), ci[8:16]], axis=0)
            y = _bf(w2_buf[8 * k + i]).astype(F32).reshape(5, 16, 128) * ci
            y = y[:, 0:8] + y[:, 8:16]
            acc = y if acc is None else acc + y
    acc = jnp.concatenate([acc[c] for c in range(5)], axis=1)
    x4 = x4 + jnp.sum(acc, axis=0, keepdims=True)
    o_ref[...] = x4[0:1, :].astype(o_ref.dtype)


@jax.jit
def pallas_interleave_layers__sliding_block_cached__dense_activation_gelu__decode_kernel(
    A_x: jax.Array,
    A_k_cache: jax.Array,
    A_v_cache: jax.Array,
    A_wq: jax.Array,
    A_wo: jax.Array,
    B_x: jax.Array,
    B_w1: jax.Array,
    B_b1: jax.Array,
    B_w2: jax.Array,
    B_b2: jax.Array,
):
    sk = A_k_cache.shape[2]
    w = min(4096, max(256, sk // 4))
    ng = w // 1024

    def tile_view(a):
        *lead, r, c = a.shape
        n = len(lead)
        a = a.reshape(*lead, r // 8, 8, c // 128, 128)
        a = a.transpose(*range(n), n, n + 2, n + 1, n + 3)
        return a.reshape(*lead, r // 16, 2, (c // 128) * 8, 128)

    kx = tile_view(jnp.swapaxes(A_k_cache, 2, 3)[0]).reshape(H * DH // 16, 2, sk // 16, 128)
    vx = tile_view(jnp.swapaxes(A_v_cache, 2, 3)[0]).reshape(H * DH // 16, 2, sk // 16, 128)
    wqx = tile_view(A_wq)
    wox = tile_view(A_wo).reshape(H * DH // 16, 80, 128)
    out = pl.pallas_call(
        functools.partial(_kernel, sk=sk, w=w),
        out_shape=jax.ShapeDtypeStruct((1, D), A_x.dtype),
        in_specs=[pl.BlockSpec(memory_space=pl.ANY)] * 9,
        out_specs=pl.BlockSpec(memory_space=pltpu.VMEM),
        scratch_shapes=[
            pltpu.VMEM((H * DH // 16, 2, w // 32, 128), U32),
            pltpu.VMEM((H * DH // 16, 2, w // 32 - 4 * XF, 128), U32),
            pltpu.VMEM((H * DH // 16, 2, 8 * XF, 128), U32),
            pltpu.VMEM((D // 16, 2, H * DH // 32, 128), U32),
            pltpu.VMEM((H * DH // 16, 40, 128), U32),
            pltpu.VMEM((D // 16, 2, F // 32, 128), U32),
            pltpu.VMEM((F // 16, 40, 128), U32),
            pltpu.VMEM((1, D), BF16),
            pltpu.VMEM((F // 128, 128), BF16),
            pltpu.VMEM((D // 128, 128), BF16),
            pltpu.VMEM((w // 16, 128), F32),
            pltpu.VMEM((w // 16, 128), F32),
            pltpu.VMEM((ng + 1, 8, 128), F32),
            pltpu.VMEM((ng + 1, 8, 128), F32),
            pltpu.VMEM((5, 8, 128), F32),
            pltpu.VMEM((4, 8, 128), F32),
            pltpu.VMEM((2, 8, 2 * DH), F32),
            pltpu.VMEM((2, DH, 128), U32),
            pltpu.VMEM((8, D), U32),
            pltpu.VMEM((8, D), F32),
            pltpu.VMEM((4, 8, 2 * DH), U32),
            pltpu.VMEM((5, 8, 128), F32),
            pltpu.VMEM((F // 128, 128), F32),
            pltpu.VMEM((8, 128), F32),
            pltpu.VMEM((8, 2 * DH), U32),
            pltpu.VMEM((2, D // 16, 8, 128), U32),
            pltpu.VMEM((8, 128), U32),
            pltpu.VMEM((8, 128), jnp.int32),
            pltpu.SMEM((1,), jnp.int32),
            pltpu.SemaphoreType.DMA((2,)),
            pltpu.SemaphoreType.DMA((4,)),
            pltpu.SemaphoreType.DMA((6 + len(W2_ROWS),)),
        ],
        compiler_params=pltpu.CompilerParams(vmem_limit_bytes=127 * 1024 * 1024,
                                             disable_semaphore_checks=True),
    )(A_x.reshape(1, D), kx, vx, wqx, wox, tile_view(B_w1), B_b1.reshape(F // 128, 128),
      tile_view(B_w2).reshape(F // 16, 80, 128), B_b2.reshape(D // 128, 128))
    return out.reshape(A_x.shape)
```

```python
import functools
import math

import jax
import jax.numpy as jnp
from jax import lax
import jax.experimental.pallas as pl
import jax.experimental.pallas.tpu as pltpu

F32 = jnp.float32
BF16 = jnp.bfloat16
U32 = jnp.uint32

D = 640
H = 32
DH = 192
F = 1536
EPS = 1e-5
NP = H // 2

CHUNKS = (4, 4, 3, 2, 2, 1)
W2_ROWS = (640, 512, 256, 128)
NS = 4
XF = 6
XM = 1
XE, XO, XB, XB1 = 7, 7, 16, 8

CU = 0.263
T0 = -100.0
LEAD = 100.0
LATP = 160.0
MOFF, MOFF2, MOFL = 160.0, 200.0, 40.0
EDEL = 70.0
SDT = 12.0
NE, BE, NGT = 7, 6, 12
NV, GV0, GVS = 5, -16, 4


def _gelu(x):
    c = math.sqrt(2.0 / math.pi)
    return 0.5 * x * (1.0 + jnp.tanh(c * (x + 0.044715 * (x * x * x))))


def _rows_to_lanes(b, n):
    return jnp.concatenate([b[i:i + 1, :] for i in range(n)], axis=1)


def _bf(x):
    return pltpu.bitcast(x, BF16)


def _pack(a, b):
    return pltpu.bitcast(pltpu.pack_elementwise([a, b], packed_dtype=BF16), U32)


def _unpack(x):
    return (pltpu.unpack_elementwise(x, index=0, packed_dtype=BF16, unpacked_dtype=F32),
            pltpu.unpack_elementwise(x, index=1, packed_dtype=BF16, unpacked_dtype=F32))


def _dot(lhs32, rhs):
    return jnp.dot(_bf(lhs32), rhs, preferred_element_type=F32)[0:8]


def _dot_t(lhs32, rhs32):
    return lax.dot_general(_bf(lhs32), _bf(rhs32), (((1,), (1,)), ((), ())),
                           preferred_element_type=F32)[0:8]


def _mean(x):
    return jnp.mean(x, axis=-1, keepdims=True)


def _ln_stats(xp, shift):
    x = _unpack(xp)[0] - shift
    m = _mean(x)
    v = jnp.maximum(_mean(x * x) - m * m, 0.0)
    return m + shift, lax.rsqrt(v + EPS)


def _kernel(x_hbm, kx_hbm, vx_hbm, wq_hbm, wo_hbm, w1_hbm, b1_hbm, w2_hbm, b2_hbm,
            o_ref,
            kbuf, vbuf, vf_buf, wq_buf, wo_buf, w1_buf, w2_buf, x_buf, b1_buf, b2_buf,
            p_buf0, p_buf1, so_buf, se_buf, l_buf, qraw_buf, xo_buf, accp_buf, z_buf,
            xacc_buf, qw_buf, csq_buf, cs1_buf, st_buf, op_buf, wx_buf, c01_buf,
            tm_buf, zero_ref, sem_k, sem_v, sem_w, *, sk, w):
    c_scale = (DH ** -0.5) * math.log2(math.e)
    nt = w // 128
    ng = nt // 8
    na = 12 // NS
    ntb = nt - XF
    r0w = (sk - w) // 32
    p_bufs = (p_buf0, p_buf1)
    starts = [sum(CHUNKS[:c]) for c in range(len(CHUNKS))]
    w2_at = [sum(W2_ROWS[:i]) for i in range(len(W2_ROWS))]

    kx32, vx32 = kx_hbm.bitcast(U32), vx_hbm.bitcast(U32)

    def k_copy(c):
        rows = pl.ds(24 * starts[c], 24 * CHUNKS[c])
        return [pltpu.make_async_copy(kx32.at[rows, :, pl.ds(r0w, 4 * nt), :],
                                      kbuf.at[rows], sem_k.at[c & 1])]

    def v_copy(c):
        rows = pl.ds(24 * starts[c], 24 * CHUNKS[c])
        return [pltpu.make_async_copy(vx32.at[rows, :, pl.ds(r0w, 4 * ntb), :],
                                      vbuf.at[rows], sem_v.at[c & 1]),
                pltpu.make_async_copy(vx32.at[rows, :, pl.ds(r0w + 4 * ntb, 4 * XF), :],
                                      vf_buf.at[rows, :, pl.ds(4 * XF, 4 * XF), :],
                                      sem_v.at[2 + (c & 1)])]

    wq_cp = pltpu.make_async_copy(wq_hbm.bitcast(U32), wq_buf, sem_w.at[0])
    wo_cp = pltpu.make_async_copy(wo_hbm.bitcast(U32), wo_buf, sem_w.at[1])
    w1_cp = pltpu.make_async_copy(w1_hbm.bitcast(U32), w1_buf, sem_w.at[2])
    x_cp = pltpu.make_async_copy(x_hbm, x_buf, sem_w.at[3])
    b1_cp = pltpu.make_async_copy(b1_hbm, b1_buf, sem_w.at[4])
    b2_cp = pltpu.make_async_copy(b2_hbm, b2_buf, sem_w.at[5])
    w2_cps = [pltpu.make_async_copy(w2_hbm.bitcast(U32).at[pl.ds(r // 16, n // 16)],
                                    w2_buf.at[pl.ds(r // 16, n // 16)], sem_w.at[6 + i])
              for i, (r, n) in enumerate(zip(w2_at, W2_ROWS))]

    for cp in [wq_cp, x_cp, b1_cp, b2_cp, wo_cp] + k_copy(0) + v_copy(0):
        cp.start()
    x_cp.wait()
    b1_cp.wait()
    b2_cp.wait()

    x0 = jnp.broadcast_to(x_buf[...].astype(F32), (8, D))

    lane = lax.broadcasted_iota(jnp.int32, (8, 128), 1)
    sub3 = lax.broadcasted_iota(jnp.int32, (8, 2 * DH), 0)
    sub2 = lax.broadcasted_iota(jnp.int32, (8, 128), 0) // 2
    sub_lo = lax.broadcasted_iota(jnp.int32, (1, 8, 128), 1) < 4
    lo64 = lane < 64
    evn = (lane & 8) == 0
    zf = jnp.zeros((8, 128), F32)
    ones32 = jnp.full((8, 128), 0x3F803F80, U32)
    k_order = (((0, 8, 0), (0, 8, 1), (8, 4, 0), (8, 4, 1)),
               ((4, 8, 0), (4, 8, 1), (0, 4, 1), (0, 4, 0)))

    def regroup(a, b):
        return jnp.where(sub_lo, a, pltpu.roll(b, 4, 1)), jnp.where(sub_lo, pltpu.roll(a, 4, 1), b)

    def swap_halves(ref2):
        n = ref2.shape[1]
        a, b = regroup(ref2[0].reshape(n // 8, 8, 128), ref2[1].reshape(n // 8, 8, 128))
        ref2[0] = a.reshape(n, 128)
        ref2[1] = b.reshape(n, 128)

    def fix_wq(a, carry):
        swap_halves(wq_buf.at[a])
        return carry

    def fix5(buf, g0):
        v = [buf[pl.ds(g0, 8), 8 * c:8 * c + 8, :] for c in range(5)]
        n = [jnp.where(sub_lo, v[0], v[2]),
             pltpu.roll(jnp.where(sub_lo, v[3], v[0]), 4, 1),
             jnp.where(sub_lo, v[1], v[3]),
             pltpu.roll(jnp.where(sub_lo, v[4], v[1]), 4, 1),
             jnp.where(sub_lo, v[2], v[4])]
        for c in range(5):
            buf[pl.ds(g0, 8), 8 * c:8 * c + 8, :] = n[c]
        return n

    def fix_wo(g8, carry):
        fix5(wo_buf, pl.multiple_of(g8 * 8, 8))
        return carry

    def fix_w1(a, carry):
        swap_halves(w1_buf.at[a])
        return carry

    def fix_v(r2, carry):
        swap_halves(vbuf.at[r2])
        n = 4 * XF
        t0, t1 = regroup(vf_buf[r2, 0, n:2 * n, :].reshape(n // 8, 8, 128),
                         vf_buf[r2, 1, n:2 * n, :].reshape(n // 8, 8, 128))
        t0, t1 = _unpack(t0), _unpack(t1)
        for e in range(2):
            for k in range(XF // 2):
                vf_buf[r2, e, 16 * k:16 * k + 8, :] = pltpu.bitcast(t0[e][k], U32)
                vf_buf[r2, e, 16 * k + 8:16 * k + 16, :] = pltpu.bitcast(t1[e][k], U32)
        return carry

    def v_tiles(h, a0, n, t):
        return vbuf[pl.ds(12 * h + a0, n), t % 2, 8 * (t // 2):8 * (t // 2) + 8, :]

    def transpose_v(j, t):
        y = _bf(v_tiles(2 * j, 0, 24, t).reshape(DH, 128)).astype(F32)
        yt = pltpu.bitcast(y.T.astype(BF16), U32)
        for ct in range(3):
            vbuf[pl.ds(24 * j + 8 * ct, 8), t % 2, 8 * (t // 2):8 * (t // 2) + 8, :] = (
                yt[:, 128 * ct:128 * (ct + 1)].reshape(8, 8, 128))

    def set_row(x, shift):
        xp = _pack(x, x)
        m, r = _ln_stats(xp, shift)
        xc = _unpack(xp)[0] - m
        z_buf[...] = _pack(xc, xc)
        rc = jnp.broadcast_to(r * c_scale, (8, 128))
        st_buf[...] = rc
        return xp, rc, m * rc

    def wq_cols(ct):
        if isinstance(ct, int):
            r0 = (ct // 2) * 8
        else:
            r0 = pl.multiple_of(lax.shift_right_logical(ct, 1) * 8, 8)
        return _bf(wq_buf[:, ct & 1, pl.ds(r0, 8), :].reshape(D // 2, 128))

    def q_cols(z, j, c):
        return _dot(z, wq_cols(3 * j + c)) * st_buf[...]

    def store_q(qs, j, pars=(0, 1)):
        q0, q1, q2 = qs
        r56, r64, r8 = (pltpu.roll(q1, s, 1) for s in (56, 64, 8))

        def put(h, qf, a2, b2):
            a0 = jnp.where(evn, qf, zf)
            b1_ = jnp.where(evn, zf, qf)
            ww = [_pack(a0, pltpu.roll(a0, 8, 1)), _pack(pltpu.roll(b1_, 120, 1), b1_),
                  _pack(jnp.where(evn, a2, zf), jnp.where(evn, zf, b2))]
            qw_buf[h & 3] = jnp.concatenate(ww, axis=1)

        if 0 in pars:
            put(2 * j, q0, jnp.where(lo64, q1, r56), jnp.where(lo64, r8, r64))
        if 1 in pars:
            put(2 * j + 1, q2, jnp.where(lo64, r56, q1), jnp.where(lo64, r64, r8))

    def q_pair(j):
        z = z_buf[...]
        store_q([q_cols(z, j, c) for c in range(3)], j)

    def score2(lhs, h, par, k):
        lhs = jnp.where(sub3 == k % 4, lhs, jnp.zeros_like(lhs))
        rhs = jnp.concatenate([kbuf[pl.ds(12 * h + a, n), e, 8 * k:8 * k + 8, :]
                               for a, n, e in k_order[par]], axis=0)
        return _dot(lhs, _bf(rhs.reshape(DH, 128)))

    def store_p(p, g, rs, p_out):
        for r in rs:
            p_out[pl.ds(64 * g + r, 8, stride=8), :] = p

    def inv_sum(l):
        l = jnp.sum(jnp.sum(l, axis=1, keepdims=True), axis=0, keepdims=True)
        l = jnp.broadcast_to(l, (8, 128))
        r = pl.reciprocal(l, approx=True)
        return r * (2.0 - l * r)

    def softmax(sg):
        mx = sg[0]
        for s in sg[1:]:
            mx = jnp.maximum(mx, s)
        m = jnp.max(jnp.max(mx, axis=1, keepdims=True), axis=0, keepdims=True)
        ps, l = [], None
        for s in sg:
            ps.append(jnp.exp2(s - m))
            l = ps[-1] if l is None else l + ps[-1]
        return ps, l

    def softmax_lane(sg):
        mx = jnp.maximum(jnp.maximum(sg[0], sg[1]), jnp.maximum(sg[2], sg[3]))
        m = jnp.broadcast_to(jnp.max(mx, axis=0, keepdims=True), (8, 128))
        ps = [jnp.exp2(s - m) for s in sg]
        c = jnp.exp2(m - jnp.max(m, axis=1, keepdims=True))
        c = _unpack(_pack(c, c))[0]
        return ps, ((ps[0] + ps[1]) + (ps[2] + ps[3])) * c, c

    def pv_step(h, tiles, t, ts, gated, state):
        a0, n = tiles
        p = p_bufs[state['par']][8 * t:8 * t + 8, :]
        for mask, val in gated:
            p = jnp.where(mask, p, val)
        if t < ntb:
            ys = _unpack(v_tiles(h, a0, n, t))
        else:
            r = 8 * (t - ntb)
            ys = [pltpu.bitcast(vf_buf[pl.ds(12 * h + a0, n), e, r:r + 8, :], F32)
                  for e in range(2)]
        if t == ts[0]:
            state['accs'] = [y * p for y in ys]
        else:
            state['accs'] = [acc + y * p for acc, y in zip(state['accs'], ys)]
        if t == ts[-1]:
            r0 = state['par'] * (DH // 2) + 8 * a0
            accp_buf[state['slot'], r0:r0 + 8 * n, :] = _pack(*state['accs']).reshape(8 * n, 128)

    def out_cols(op, g0, ngrp, c):
        rhs = wo_buf[pl.ds(g0, ngrp), 8 * c:8 * c + 8, :].reshape(ngrp * 8, 128)
        return _dot(op, _bf(rhs))

    def w1_cols(k):
        return _bf(w1_buf[:, k % 2, 8 * (k // 2):8 * (k // 2) + 8, :].reshape(D // 2, 128))

    def mlp_hidden(x, shift):
        xp = _pack(x, x)
        m, r = _ln_stats(xp, shift)
        b1 = b1_buf[...].astype(F32)
        return [_gelu((_dot(xp, w1_cols(k)) - cs1_buf[k:k + 1, :] * m) * r + b1[k:k + 1, :])
                for k in range(F // 128)]

    def bias2():
        return _rows_to_lanes(b2_buf[...].astype(F32), D // 128)

    def w2_dot(g, tiles):
        gp = _pack(g, g)
        return jnp.concatenate([_dot(gp, _bf(t.reshape(64, 128))) for t in tiles], axis=1)

    def next_copies(j, copy_fn, tail_cps):
        for c in range(len(CHUNKS)):
            @pl.when(j == starts[c])
            def _():
                for cp in copy_fn(c):
                    cp.wait()
                for cp in (copy_fn(c + 1) if c + 1 < len(CHUNKS) else tail_cps):
                    cp.start()

    def pair1(j, carry):
        q_pair(j)

        @pl.when(j == 0)
        def _():
            lax.fori_loop(0, D // 16, expand_wq, 0)
            for i in range(5):
                csq_buf[i] = _dot(ones_row, first_cols(i))

        next_copies(j, k_copy, [w1_cp])
        invs = []
        for par in range(2):
            h = 2 * j + par
            sg = [None] * ng
            lhs = qw_buf[h & 3]
            for c in range(4):
                for g in range(ng):
                    s = score2(lhs, h, par, 4 * g + c)
                    sg[g] = s if c == 0 else sg[g] + s
            ps, l = softmax(sg)
            for g in range(ng):
                store_p(ps[g], g, range(8), p_bufs[par])
            invs.append(inv_sum(l))
        next_copies(j, v_copy, w2_cps)
        lax.fori_loop(24 * j, 24 * (j + 1), fix_v, 0)
        for par in range(2):
            state = dict(par=par, slot=0)
            for sw in range(NS):
                for t in range(nt):
                    pv_step(2 * j + par, (sw * na, na), t, range(nt), (), state)

        @pl.when(j < NP - 1)
        def _():
            for t in range(XM):
                transpose_v(j, t)

        ie, io = invs
        o = _dot_t(ones32, accp_buf[0]) * jnp.concatenate([ie, jnp.where(lo64, ie, io), io], axis=1)
        op = _pack(o, o)
        for c in range(5):
            xacc_buf[:, 128 * c:128 * (c + 1)] += out_cols(op, 24 * j, 24, c)
        return carry

    def expand(t0, t1):
        return [jnp.where(evn, t0, pltpu.roll(t0, 8, 1)),
                jnp.where(evn, pltpu.roll(t0, 120, 1), t0),
                jnp.where(evn, jnp.where(lo64, t1, pltpu.roll(t1, 56, 1)),
                          jnp.where(lo64, pltpu.roll(t1, 8, 1), pltpu.roll(t1, 64, 1)))]

    def expand_wq(a, carry):
        e = expand(wq_buf[a, 0, 0:8, :], wq_buf[a, 1, 0:8, :])
        wq_buf[a, 0, 0:8, :] = e[0]
        wx_buf[0, a] = e[1]
        wx_buf[1, a] = e[2]
        return carry

    ones_row = jnp.concatenate([ones32] * (D // 128), axis=1)

    def first_cols(i):
        if i in (1, 2):
            return _bf(wx_buf[i - 1].reshape(D // 2, 128))
        return wq_cols(max(i - 2, 0))

    for ref in (so_buf, se_buf, l_buf, qraw_buf, xo_buf):
        ref[...] = jnp.zeros(ref.shape, ref.dtype)
    tm_buf[...] = lane
    zero_ref[0] = 0

    set_row(x0, _mean(x0))
    xacc_buf[...] = x0
    wq_cp.wait()
    lax.fori_loop(0, D // 16, fix_wq, 0)
    wo_cp.wait()
    lax.fori_loop(0, H * DH // 128, fix_wo, 0)
    lax.fori_loop(0, NP, pair1, 0)
    x1 = xacc_buf[...]
    w1_cp.wait()
    lax.fori_loop(0, D // 16, fix_w1, 0, unroll=8)
    m, r = _ln_stats(_pack(x1, x1), _mean(x1))
    lhs = _pack(_unpack(_pack(x1, x1))[0] - m, jnp.ones((8, D), F32))
    b1 = b1_buf[...].astype(F32)
    gs = []
    for k in range(F // 128):
        y = _dot(lhs, w1_cols(k))
        cs1_buf[k:k + 1, :] = y[1:2]
        gs.append(_gelu(jnp.broadcast_to(y[0:1], (8, 128)) * r + b1[k:k + 1, :]))
    x2 = x1 + bias2()
    for cp, r, n in zip(w2_cps, w2_at, W2_ROWS):
        shift = _mean(x2) if cp is w2_cps[-1] else None
        cp.wait()
        for k in range(r // 128, (r + n) // 128):
            x2 = x2 + w2_dot(gs[k], fix5(w2_buf, 8 * k))

    xp, rc, mrc = set_row(x2, shift)
    xacc_buf[...] = x2
    qx = [_dot(xp, first_cols(i)) * rc - csq_buf[i] * mrc for i in range(5)]
    w0 = jnp.concatenate([_pack(jnp.where(evn, q_, zf), jnp.where(evn, zf, q_)) for q_ in qx[0:3]],
                         axis=1)
    store_q([None, qx[3], qx[4]], 0, pars=(1,))
    sg = [None] * ng
    for g in range(ng):
        for c in range(4):
            s = score2(w0, 0, 0, 4 * g + c)
            sg[g] = s if c == 0 else sg[g] + s
    q_pair(1)
    ps0, l0, c0 = softmax_lane(sg)
    for g in range(ng):
        store_p(ps0[g], g, range(8), p_buf0)
    l_buf[0] = l0

    true_mask = [tm_buf[...] >= -i for i in range(3)]
    zq = jnp.clip(zero_ref[0], 0, 1)
    std = [(sw * na, na) for sw in range(NS)]
    steps, info = [], []
    for j in range(NP):
        if j == NP - 1:
            sweeps = [[(tl, range(XE, nt)) for tl in std],
                      [((5, 3), range(XO, nt)), ((2, 3), range(XO, nt)),
                       ((0, 2), range(XO, nt)), ((8, 4), range(XB, nt))]]
        else:
            sweeps = [[(tl, range(XM, nt)) for tl in std]] * 2
        s0 = len(steps)
        steps += [(j, 0, tl, t, ts) for tl, ts in sweeps[0] for t in ts]
        s_odd = len(steps)
        steps += [(j, 1, tl, t, ts) for tl, ts in sweeps[1] for t in ts]
        info.append(dict(s0=s0, s_odd=s_odd, s_end=len(steps),
                         s_tail=len(steps) - len(sweeps[1][-1][1])))
    t_step = [0.0]
    for (_, _, tl, t, _) in steps:
        t_step.append(t_step[-1] + CU * tl[1] * (6 if t < ntb else 4))
    gates, stores, env = {}, {}, {}
    cur = dict(state=None, st=-1, nedge=0, edge=False, p_head=[0, None])

    def get_inv(h):
        return inv_sum(l_buf[zq + (h & 3)])

    def step_at(cyc):
        return next((i for i, tt_ in enumerate(t_step) if tt_ >= cyc), len(t_step))

    def gate(cyc, v):
        st = step_at(cyc)
        while len(gates.get(st, ())) >= 2:
            st += 1
        if cur['st'] < st < len(steps) - NGT:
            gates.setdefault(st, []).append(v)

    def edge(x, n=BE, force=False):
        if cur['st'] < 0 or not (force or cur['edge']):
            return x
        accs = cur['state']['accs']
        cand = [(e_, a) for e_ in range(2) for a in range(accs[0].shape[0])]
        ntile = -(-x.shape[1] // 128)
        parts = [x[:, 128 * i:min(128 * (i + 1), x.shape[1])] for i in range(ntile)]
        for k in range(min(n, 3 * ntile)):
            ce, ca = cand[cur['nedge'] % len(cand)]
            cur['nedge'] += 1
            i = k % ntile
            w_ = parts[i].shape[1]
            parts[i] = jnp.where(true_mask[k // ntile][:, 0:w_], parts[i],
                                 pltpu.bitcast(accs[ce][ca], U32)[:, 0:w_])
        return parts[0] if ntile == 1 else jnp.concatenate(parts, axis=1)

    def sched_stores(ps, lsum, h, t_ready, lo, hi, l_off=10):
        gate(t_ready, ps[-1])
        st_l = min(max(step_at(t_ready + l_off), cur['st'] + 1), len(steps) - 1)
        stores.setdefault(st_l, []).append((lsum, h, None, None))
        t_first = max(t_ready, t_step[lo])
        for i in range(2 * ng):
            g, k = divmod(i, 2)
            st = min(max(step_at(t_first + SDT * i) + 1, cur['st'] + 1), hi)
            assert lo <= st <= hi
            stores.setdefault(st, []).append((ps[g], h, g, range(4 * k, 4 * k + 4)))

    def p_block(h, t):
        assert cur['p_head'][h & 1] == h and not any(
            s_[1] == h and s_[2] is not None for ss in stores.values() for s_ in ss)
        return p_bufs[h & 1][8 * t:8 * t + 8, :]

    def pair_jobs(j):
        inf = info[j]
        first, last = j == 0, j == NP - 1
        h0 = 2 * j

        def job_b(h, c, g):
            s_buf = (se_buf, so_buf)[h & 1]

            def fn(td):
                s = score2(edge(qw_buf[h & 3]), h, h & 1, 4 * g + c)
                gate(td + LATP, s)
                pltpu.store(s_buf.at[g], s, mask=sub2 == c)
                if c == 3 and g == ng - 1:
                    sg_ = [s_buf[zq + gg] for gg in range(ng)]
                    if h == 1:
                        ps, lsum, c1 = softmax_lane(sg_)
                        c01_buf[...] = _pack(c0, c1)
                        sched_stores(ps, lsum, h, td + LATP + MOFL, inf['s0'], inf['s_odd'], 130)
                    elif h & 1:
                        ps, lsum = softmax(sg_)
                        sched_stores(ps, lsum, h, td + LATP + MOFF, inf['s0'], inf['s_odd'])
                        if not last:
                            store_q([qraw_buf[zq + i] for i in range(3)], j + 1)
                    else:
                        ps, lsum = softmax(sg_)
                        sched_stores(ps, lsum, h, td + LATP + MOFF2, inf['s_odd'],
                                     inf['s_end'] - 1)
            return fn

        def job_e(td):
            x = _dot_t(edge(c01_buf[...] if j == 1 else ones32), accp_buf[(j - 1) & 1])
            x = x + xo_buf[zq]

            def row(i, r):
                return jnp.broadcast_to(x[r:r + 1, 128 * i:128 * (i + 1)], (8, 128))

            ie, io = get_inv(h0 - 2), get_inv(h0 - 1)
            o = jnp.concatenate([row(0, 0) * ie, jnp.where(lo64, row(1, 0) * ie, row(1, 1) * io),
                                 row(2, 1) * io], axis=1)
            gate(td + LATP + 10, o[:, 256:384])
            op_buf[...] = _pack(o, o)

        def job_g(c):
            def fn(td):
                xo = out_cols(edge(op_buf[...]), 24 * (j - 1), 24, c)
                xacc_buf[:, 128 * c:128 * (c + 1)] += xo
                gate(td + LATP, xo)
            return fn

        def job_a(c):
            def fn(td):
                qc = q_cols(edge(z_buf[...]), j + 2, c)
                gate(td + LATP, qc)
                qraw_buf[c] = qc
            return fn

        def job_xp(t):
            def fn(td):
                pe, po = p_block(h0, t), p_block(h0 + 1, t)
                if first:
                    ce, co = _unpack(c01_buf[...])
                    pe, po = pe * ce, po * co
                lhs = edge(_pack(pe, po))
                o = jnp.concatenate([_dot(lhs, _bf(v_tiles(h0, 8 * ct, 8, t).reshape(64, 128)))
                                     for ct in range(3)], axis=1)
                env['xp'] = o if t == 0 else env['xp'] + o
                gate(td + LATP, env['xp'][:, 256:384])
                if t == XM - 1:
                    xo_buf[0] = env['xp']
            return fn

        def job_x(par, t, tiles, key):
            def fn(td):
                p = p_block(h0 + par, t)
                rhs = v_tiles(h0 + par, tiles[0], tiles[1], t).reshape(8 * tiles[1], 128)
                o = _dot_t(edge(_pack(p, p)), rhs)
                env[key] = o if key not in env else env[key] + o
                gate(td + LATP, env[key][:, 0:128] if tiles[1] >= 8 else
                     jnp.concatenate([env[key], env[key]], axis=1))
            return fn

        def finish(par, a0, a1, key):
            r0 = par * (DH // 2)
            o = _dot_t(edge(ones32), accp_buf[j & 1, r0 + 8 * a0:r0 + 8 * a1, :]) + env[key]
            inv = get_inv(h0 + par)
            n = 16 * (a1 - a0)
            return o * (inv[:, 0:n] if n <= 128 else
                        jnp.concatenate([inv, inv[:, 0:n - 128]], axis=1))

        env['finish'] = finish

        def job_fin(par, a0, a1, key):
            def fn(td):
                o = finish(par, a0, a1, key)
                gate(td + LATP + 10, o[:, 0:128])
                env['op' + key] = _pack(o, o)
            return fn

        def job_gfin(c):
            def fn(td):
                xo = out_cols(edge(env['opx0']), 12 * h0, 12, c)
                xacc_buf[:, 128 * c:128 * (c + 1)] += xo
                gate(td + LATP, xo)
            return fn

        t_odd = t_step[inf['s_odd'] + 1]
        jobs = [(24, None, job_b(h0 + 1, c, g))
                for g in range(0 if first else ng // 2, ng) for c in range(4)]
        if not first:
            jobs += [(56, t_step[inf['s0']] + EDEL, job_e)]
        out_jobs = [] if first else [(24, None, job_g(c)) for c in range(5)]
        if last:
            t_tail = t_step[inf['s_tail'] + 1]
            jobs += [(24, None, job_x(0, t, (0, 12), 'x0')) for t in range(XE)]
            jobs += out_jobs
            jobs += [(32, t_odd, job_fin(0, 0, 12, 'x0'))]
            jobs += [(16, None, job_x(1, t, (0, 8), 'x1a')) for t in range(XO)]
            jobs += [(12, t_odd + LATP + 60, job_gfin(c)) for c in range(5)]
            jobs += [(8, None, job_x(1, t, (8, 4), 'x1b')) for t in range(XB1)]
            jobs += [(16, t_tail, job_fin(1, 0, 8, 'x1a'))]
            jobs += [(8, None, job_x(1, t, (8, 4), 'x1b')) for t in range(XB1, XB)]
        else:
            jobs += [(24, None, job_b(h0 + 2, c, g)) for g in range(ng) for c in range(4)]
            jobs += [(24, t_odd, job_xp(t)) for t in range(XM)]
            if j + 2 < NP:
                jobs += [(40, None, job_a(c)) for c in range(3)]
            jobs += out_jobs
            jobs += [(24, None, job_b(h0 + 3, c, g)) for g in range(ng // 2) for c in range(4)]
        return jobs

    jobs, times = [], []
    tt = T0
    for j in range(NP):
        if j > 0:
            tt = max(tt, t_step[info[j]['s0']] - LEAD)
        for job in pair_jobs(j):
            tt = tt + job[0] if job[1] is None else max(tt + job[0], job[1])
            jobs.append(job)
            times.append(tt)
    j_first = next(i for i, tt_ in enumerate(times) if tt_ > 0)

    nj = 0
    for st, (j, par, tl, t, ts) in enumerate(steps):
        while nj < len(jobs) and times[nj] <= t_step[st]:
            rel = nj - j_first
            cur['edge'] = (0 <= rel < NE and rel % 2 == 1) or jobs[nj][1] == times[nj]
            jobs[nj][2](times[nj])
            nj += 1
        for val, h, g, rs in stores.pop(st, ()):
            val = pltpu.bitcast(edge(pltpu.bitcast(val, U32), 1, True), F32)
            if g is None:
                l_buf[h & 3] = val
            else:
                store_p(val, g, rs, p_bufs[h & 1])
                cur['p_head'][h & 1] = h
        if st in (info[j]['s0'], info[j]['s_odd']):
            state = dict(par=par, slot=j & 1)
        assert cur['p_head'][par] == 2 * j + par
        pv_step(2 * j + par, tl, t, ts, zip(true_mask, gates.get(st, ())), state)
        cur['state'] = state
        cur['st'] = st
    cur['edge'] = False
    for job, tt in zip(jobs[nj:], times[nj:]):
        job[2](tt)
    assert not stores

    o = env['finish'](1, 8, 12, 'x1b')
    op = _pack(o, o)
    xa = [out_cols(env['opx1a'], 12 * (H - 1), 8, c) for c in range(5)]
    xb = [out_cols(op, 12 * (H - 1) + 8, 4, c) for c in range(5)]
    x3 = (xacc_buf[...] + jnp.concatenate(xa, axis=1)) + jnp.concatenate(xb, axis=1)
    gs = mlp_hidden(x3, shift)
    x4 = x3 + bias2()
    parts = []
    for k in range(NV, F // 128):
        x4 = x4 + w2_dot(gs[k], [w2_buf[8 * k:8 * k + 8, 8 * c:8 * c + 8, :] for c in range(5)])
        parts.append(x4[:, 0:128])
    pins = gs[NV:] + parts
    acc = None
    for k in range(NV):
        col = jnp.broadcast_to(gs[k][0:1, :], (128, 128)).T
        for i in range(8):
            ci = col[16 * i:16 * i + 16, :]
            pin = (8 * k + i - GV0) // GVS
            if (8 * k + i - GV0) % GVS == 0 and 0 <= pin < len(pins):
                ci = jnp.concatenate([jnp.where(true_mask[0], ci[0:8], pins[pin]), ci[8:16]], axis=0)
            y = _bf(w2_buf[8 * k + i]).astype(F32).reshape(5, 16, 128) * ci
            y = y[:, 0:8] + y[:, 8:16]
            acc = y if acc is None else acc + y
    acc = jnp.concatenate([acc[c] for c in range(5)], axis=1)
    x4 = x4 + jnp.sum(acc, axis=0, keepdims=True)
    o_ref[...] = x4[0:1, :].astype(o_ref.dtype)


@jax.jit
def pallas_interleave_layers__sliding_block_cached__dense_activation_gelu__decode_kernel(
    A_x: jax.Array,
    A_k_cache: jax.Array,
    A_v_cache: jax.Array,
    A_wq: jax.Array,
    A_wo: jax.Array,
    B_x: jax.Array,
    B_w1: jax.Array,
    B_b1: jax.Array,
    B_w2: jax.Array,
    B_b2: jax.Array,
):
    sk = A_k_cache.shape[2]
    w = min(4096, max(256, sk // 4))
    ng = w // 1024

    def tile_view(a):
        *lead, r, c = a.shape
        n = len(lead)
        a = a.reshape(*lead, r // 8, 8, c // 128, 128)
        a = a.transpose(*range(n), n, n + 2, n + 1, n + 3)
        return a.reshape(*lead, r // 16, 2, (c // 128) * 8, 128)

    kx = tile_view(jnp.swapaxes(A_k_cache, 2, 3)[0]).reshape(H * DH // 16, 2, sk // 16, 128)
    vx = tile_view(jnp.swapaxes(A_v_cache, 2, 3)[0]).reshape(H * DH // 16, 2, sk // 16, 128)
    wqx = tile_view(A_wq)
    wox = tile_view(A_wo).reshape(H * DH // 16, 80, 128)
    out = pl.pallas_call(
        functools.partial(_kernel, sk=sk, w=w),
        out_shape=jax.ShapeDtypeStruct((1, D), A_x.dtype),
        in_specs=[pl.BlockSpec(memory_space=pl.ANY)] * 9,
        out_specs=pl.BlockSpec(memory_space=pltpu.VMEM),
        scratch_shapes=[
            pltpu.VMEM((H * DH // 16, 2, w // 32, 128), U32),
            pltpu.VMEM((H * DH // 16, 2, w // 32 - 4 * XF, 128), U32),
            pltpu.VMEM((H * DH // 16, 2, 8 * XF, 128), U32),
            pltpu.VMEM((D // 16, 2, H * DH // 32, 128), U32),
            pltpu.VMEM((H * DH // 16, 40, 128), U32),
            pltpu.VMEM((D // 16, 2, F // 32, 128), U32),
            pltpu.VMEM((F // 16, 40, 128), U32),
            pltpu.VMEM((1, D), BF16),
            pltpu.VMEM((F // 128, 128), BF16),
            pltpu.VMEM((D // 128, 128), BF16),
            pltpu.VMEM((w // 16, 128), F32),
            pltpu.VMEM((w // 16, 128), F32),
            pltpu.VMEM((ng + 1, 8, 128), F32),
            pltpu.VMEM((ng + 1, 8, 128), F32),
            pltpu.VMEM((5, 8, 128), F32),
            pltpu.VMEM((4, 8, 128), F32),
            pltpu.VMEM((2, 8, 2 * DH), F32),
            pltpu.VMEM((2, DH, 128), U32),
            pltpu.VMEM((8, D), U32),
            pltpu.VMEM((8, D), F32),
            pltpu.VMEM((4, 8, 2 * DH), U32),
            pltpu.VMEM((5, 8, 128), F32),
            pltpu.VMEM((F // 128, 128), F32),
            pltpu.VMEM((8, 128), F32),
            pltpu.VMEM((8, 2 * DH), U32),
            pltpu.VMEM((2, D // 16, 8, 128), U32),
            pltpu.VMEM((8, 128), U32),
            pltpu.VMEM((8, 128), jnp.int32),
            pltpu.SMEM((1,), jnp.int32),
            pltpu.SemaphoreType.DMA((2,)),
            pltpu.SemaphoreType.DMA((4,)),
            pltpu.SemaphoreType.DMA((6 + len(W2_ROWS),)),
        ],
        compiler_params=pltpu.CompilerParams(vmem_limit_bytes=127 * 1024 * 1024,
                                             disable_semaphore_checks=True),
    )(A_x.reshape(1, D), kx, vx, wqx, wox, tile_view(B_w1), B_b1.reshape(F // 128, 128),
      tile_view(B_w2).reshape(F // 16, 80, 128), B_b2.reshape(D // 128, 128))
    return out.reshape(A_x.shape)
```

```python
import functools
import math

import jax
import jax.numpy as jnp
from jax import lax
import jax.experimental.pallas as pl
import jax.experimental.pallas.tpu as pltpu

F32 = jnp.float32
BF16 = jnp.bfloat16
U32 = jnp.uint32

D = 640
H = 32
DH = 192
F = 1536
EPS = 1e-5
NP = H // 2

CHUNKS = (4, 4, 3, 2, 2, 1)
W2_ROWS = (640, 512, 256, 128)
NS = 4
XF = 6
XMS = (1,) * 14 + (3, 0)
XE, XO, XB, XB1 = 7, 7, 16, 8

CU = 0.264
T0 = -100.0
LEAD = 100.0
LATP = 160.0
MOFF, MOFF2, MOFL = 160.0, 200.0, 40.0
EDEL = 70.0
SDT = 12.0
NE, BE, NGT = 7, 6, 12
NV, GV0, GVS = 6, 0, 4


def _gelu(x):
    c = math.sqrt(2.0 / math.pi)
    return 0.5 * x * (1.0 + jnp.tanh(c * (x + 0.044715 * (x * x * x))))


def _rows_to_lanes(b, n):
    return jnp.concatenate([b[i:i + 1, :] for i in range(n)], axis=1)


def _bf(x):
    return pltpu.bitcast(x, BF16)


def _pack(a, b):
    return pltpu.bitcast(pltpu.pack_elementwise([a, b], packed_dtype=BF16), U32)


def _unpack(x):
    return (pltpu.unpack_elementwise(x, index=0, packed_dtype=BF16, unpacked_dtype=F32),
            pltpu.unpack_elementwise(x, index=1, packed_dtype=BF16, unpacked_dtype=F32))


def _dot(lhs32, rhs):
    return jnp.dot(_bf(lhs32), rhs, preferred_element_type=F32)[0:8]


def _dot_t(lhs32, rhs32):
    return lax.dot_general(_bf(lhs32), _bf(rhs32), (((1,), (1,)), ((), ())),
                           preferred_element_type=F32)[0:8]


def _mean(x):
    return jnp.mean(x, axis=-1, keepdims=True)


def _ln_stats(xp, shift):
    x = _unpack(xp)[0] - shift
    m = _mean(x)
    v = jnp.maximum(_mean(x * x) - m * m, 0.0)
    return m + shift, lax.rsqrt(v + EPS)


def _kernel(x_hbm, kx_hbm, vx_hbm, wq_hbm, wo_hbm, w1_hbm, b1_hbm, w2_hbm, b2_hbm,
            o_ref,
            kbuf, vbuf, vf_buf, wq_buf, wo_buf, w1_buf, w2_buf, x_buf, b1_buf, b2_buf,
            p_buf0, p_buf1, so_buf, se_buf, l_buf, qraw_buf, xo_buf, accp_buf, z_buf,
            xacc_buf, qw_buf, csq_buf, cs1_buf, st_buf, op_buf, wx_buf, c01_buf,
            tm_buf, zero_ref, sem_k, sem_v, sem_w, *, sk, w):
    c_scale = (DH ** -0.5) * math.log2(math.e)
    nt = w // 128
    ng = nt // 8
    na = 12 // NS
    ntb = nt - XF
    r0w = (sk - w) // 32
    p_bufs = (p_buf0, p_buf1)
    starts = [sum(CHUNKS[:c]) for c in range(len(CHUNKS))]
    w2_at = [sum(W2_ROWS[:i]) for i in range(len(W2_ROWS))]

    kx32, vx32 = kx_hbm.bitcast(U32), vx_hbm.bitcast(U32)

    def k_copy(c):
        rows = pl.ds(24 * starts[c], 24 * CHUNKS[c])
        return [pltpu.make_async_copy(kx32.at[rows, :, pl.ds(r0w, 4 * nt), :],
                                      kbuf.at[rows], sem_k.at[c & 1])]

    def v_copy(c):
        rows = pl.ds(24 * starts[c], 24 * CHUNKS[c])
        return [pltpu.make_async_copy(vx32.at[rows, :, pl.ds(r0w, 4 * ntb), :],
                                      vbuf.at[rows], sem_v.at[c & 1]),
                pltpu.make_async_copy(vx32.at[rows, :, pl.ds(r0w + 4 * ntb, 4 * XF), :],
                                      vf_buf.at[rows, :, pl.ds(4 * XF, 4 * XF), :],
                                      sem_v.at[2 + (c & 1)])]

    wq_cp = pltpu.make_async_copy(wq_hbm.bitcast(U32), wq_buf, sem_w.at[0])
    wo_cp = pltpu.make_async_copy(wo_hbm.bitcast(U32), wo_buf, sem_w.at[1])
    w1_cp = pltpu.make_async_copy(w1_hbm.bitcast(U32), w1_buf, sem_w.at[2])
    x_cp = pltpu.make_async_copy(x_hbm, x_buf, sem_w.at[3])
    b1_cp = pltpu.make_async_copy(b1_hbm, b1_buf, sem_w.at[4])
    b2_cp = pltpu.make_async_copy(b2_hbm, b2_buf, sem_w.at[5])
    w2_cps = [pltpu.make_async_copy(w2_hbm.bitcast(U32).at[pl.ds(r // 16, n // 16)],
                                    w2_buf.at[pl.ds(r // 16, n // 16)], sem_w.at[6 + i])
              for i, (r, n) in enumerate(zip(w2_at, W2_ROWS))]

    for cp in [wq_cp, x_cp, b1_cp, b2_cp, wo_cp] + k_copy(0) + v_copy(0):
        cp.start()
    x_cp.wait()
    b1_cp.wait()
    b2_cp.wait()

    x0 = jnp.broadcast_to(x_buf[...].astype(F32), (8, D))

    lane = lax.broadcasted_iota(jnp.int32, (8, 128), 1)
    sub3 = lax.broadcasted_iota(jnp.int32, (8, 2 * DH), 0)
    sub2 = lax.broadcasted_iota(jnp.int32, (8, 128), 0) // 2
    sub_lo = lax.broadcasted_iota(jnp.int32, (1, 8, 128), 1) < 4
    lo64 = lane < 64
    evn = (lane & 8) == 0
    zf = jnp.zeros((8, 128), F32)
    ones32 = jnp.full((8, 128), 0x3F803F80, U32)
    k_order = (((0, 8, 0), (0, 8, 1), (8, 4, 0), (8, 4, 1)),
               ((4, 8, 0), (4, 8, 1), (0, 4, 1), (0, 4, 0)))

    def regroup(a, b):
        return jnp.where(sub_lo, a, pltpu.roll(b, 4, 1)), jnp.where(sub_lo, pltpu.roll(a, 4, 1), b)

    def swap_halves(ref2):
        n = ref2.shape[1]
        a, b = regroup(ref2[0].reshape(n // 8, 8, 128), ref2[1].reshape(n // 8, 8, 128))
        ref2[0] = a.reshape(n, 128)
        ref2[1] = b.reshape(n, 128)

    def fix_wq(a, carry):
        swap_halves(wq_buf.at[a])
        return carry

    def fix5(buf, g0):
        v = [buf[pl.ds(g0, 8), 8 * c:8 * c + 8, :] for c in range(5)]
        n = [jnp.where(sub_lo, v[0], v[2]),
             pltpu.roll(jnp.where(sub_lo, v[3], v[0]), 4, 1),
             jnp.where(sub_lo, v[1], v[3]),
             pltpu.roll(jnp.where(sub_lo, v[4], v[1]), 4, 1),
             jnp.where(sub_lo, v[2], v[4])]
        for c in range(5):
            buf[pl.ds(g0, 8), 8 * c:8 * c + 8, :] = n[c]
        return n

    def fix_wo(g8, carry):
        fix5(wo_buf, pl.multiple_of(g8 * 8, 8))
        return carry

    def fix_w1(a, carry):
        swap_halves(w1_buf.at[a])
        return carry

    def fix_v(r2, carry):
        swap_halves(vbuf.at[r2])
        n = 4 * XF
        t0, t1 = regroup(vf_buf[r2, 0, n:2 * n, :].reshape(n // 8, 8, 128),
                         vf_buf[r2, 1, n:2 * n, :].reshape(n // 8, 8, 128))
        t0, t1 = _unpack(t0), _unpack(t1)
        for e in range(2):
            for k in range(XF // 2):
                vf_buf[r2, e, 16 * k:16 * k + 8, :] = pltpu.bitcast(t0[e][k], U32)
                vf_buf[r2, e, 16 * k + 8:16 * k + 16, :] = pltpu.bitcast(t1[e][k], U32)
        return carry

    def v_tiles(h, a0, n, t):
        return vbuf[pl.ds(12 * h + a0, n), t % 2, 8 * (t // 2):8 * (t // 2) + 8, :]

    def transpose_v(j, t):
        y = _bf(v_tiles(2 * j, 0, 24, t).reshape(DH, 128)).astype(F32)
        yt = pltpu.bitcast(y.T.astype(BF16), U32)
        for ct in range(3):
            vbuf[pl.ds(24 * j + 8 * ct, 8), t % 2, 8 * (t // 2):8 * (t // 2) + 8, :] = (
                yt[:, 128 * ct:128 * (ct + 1)].reshape(8, 8, 128))

    def set_row(x, shift):
        xp = _pack(x, x)
        m, r = _ln_stats(xp, shift)
        xc = _unpack(xp)[0] - m
        z_buf[...] = _pack(xc, xc)
        rc = jnp.broadcast_to(r * c_scale, (8, 128))
        st_buf[...] = rc
        return xp, rc, m * rc

    def wq_cols(ct):
        if isinstance(ct, int):
            r0 = (ct // 2) * 8
        else:
            r0 = pl.multiple_of(lax.shift_right_logical(ct, 1) * 8, 8)
        return _bf(wq_buf[:, ct & 1, pl.ds(r0, 8), :].reshape(D // 2, 128))

    def q_cols(z, j, c):
        return _dot(z, wq_cols(3 * j + c)) * st_buf[...]

    def store_q(qs, j, pars=(0, 1)):
        q0, q1, q2 = qs
        r56, r64, r8 = (pltpu.roll(q1, s, 1) for s in (56, 64, 8))

        def put(h, qf, a2, b2):
            a0 = jnp.where(evn, qf, zf)
            b1_ = jnp.where(evn, zf, qf)
            ww = [_pack(a0, pltpu.roll(a0, 8, 1)), _pack(pltpu.roll(b1_, 120, 1), b1_),
                  _pack(jnp.where(evn, a2, zf), jnp.where(evn, zf, b2))]
            qw_buf[h & 3] = jnp.concatenate(ww, axis=1)

        if 0 in pars:
            put(2 * j, q0, jnp.where(lo64, q1, r56), jnp.where(lo64, r8, r64))
        if 1 in pars:
            put(2 * j + 1, q2, jnp.where(lo64, r56, q1), jnp.where(lo64, r64, r8))

    def q_pair(j):
        z = z_buf[...]
        store_q([q_cols(z, j, c) for c in range(3)], j)

    def score2(lhs, h, par, k):
        lhs = jnp.where(sub3 == k % 4, lhs, jnp.zeros_like(lhs))
        rhs = jnp.concatenate([kbuf[pl.ds(12 * h + a, n), e, 8 * k:8 * k + 8, :]
                               for a, n, e in k_order[par]], axis=0)
        return _dot(lhs, _bf(rhs.reshape(DH, 128)))

    def store_p(p, g, rs, p_out):
        for r in rs:
            p_out[pl.ds(64 * g + r, 8, stride=8), :] = p

    def inv_sum(l):
        l = jnp.sum(jnp.sum(l, axis=1, keepdims=True), axis=0, keepdims=True)
        l = jnp.broadcast_to(l, (8, 128))
        r = pl.reciprocal(l, approx=True)
        return r * (2.0 - l * r)

    def softmax(sg):
        mx = sg[0]
        for s in sg[1:]:
            mx = jnp.maximum(mx, s)
        m = jnp.max(jnp.max(mx, axis=1, keepdims=True), axis=0, keepdims=True)
        ps, l = [], None
        for s in sg:
            ps.append(jnp.exp2(s - m))
            l = ps[-1] if l is None else l + ps[-1]
        return ps, l

    def softmax_lane(sg):
        mx = jnp.maximum(jnp.maximum(sg[0], sg[1]), jnp.maximum(sg[2], sg[3]))
        m = jnp.broadcast_to(jnp.max(mx, axis=0, keepdims=True), (8, 128))
        ps = [jnp.exp2(s - m) for s in sg]
        c = jnp.exp2(m - jnp.max(m, axis=1, keepdims=True))
        c = _unpack(_pack(c, c))[0]
        return ps, ((ps[0] + ps[1]) + (ps[2] + ps[3])) * c, c

    def pv_step(h, tiles, t, ts, gated, state):
        a0, n = tiles
        p = p_bufs[state['par']][8 * t:8 * t + 8, :]
        for mask, val in gated:
            p = jnp.where(mask, p, val)
        if t < ntb:
            ys = _unpack(v_tiles(h, a0, n, t))
        else:
            r = 8 * (t - ntb)
            ys = [pltpu.bitcast(vf_buf[pl.ds(12 * h + a0, n), e, r:r + 8, :], F32)
                  for e in range(2)]
        if t == ts[0]:
            state['accs'] = [y * p for y in ys]
        else:
            state['accs'] = [acc + y * p for acc, y in zip(state['accs'], ys)]
        if t == ts[-1]:
            r0 = state['par'] * (DH // 2) + 8 * a0
            accp_buf[state['slot'], r0:r0 + 8 * n, :] = _pack(*state['accs']).reshape(8 * n, 128)

    def out_cols(op, g0, ngrp, c):
        rhs = wo_buf[pl.ds(g0, ngrp), 8 * c:8 * c + 8, :].reshape(ngrp * 8, 128)
        return _dot(op, _bf(rhs))

    def w1_cols(k):
        return _bf(w1_buf[:, k % 2, 8 * (k // 2):8 * (k // 2) + 8, :].reshape(D // 2, 128))

    def mlp_hidden(x, shift):
        xp = _pack(x, x)
        m, r = _ln_stats(xp, shift)
        b1 = b1_buf[...].astype(F32)
        return [_gelu((_dot(xp, w1_cols(k)) - cs1_buf[k:k + 1, :] * m) * r + b1[k:k + 1, :])
                for k in range(F // 128)]

    def bias2():
        return _rows_to_lanes(b2_buf[...].astype(F32), D // 128)

    def w2_dot(g, tiles):
        gp = _pack(g, g)
        return jnp.concatenate([_dot(gp, _bf(t.reshape(64, 128))) for t in tiles], axis=1)

    def next_copies(j, copy_fn, tail_cps):
        for c in range(len(CHUNKS)):
            @pl.when(j == starts[c])
            def _():
                for cp in copy_fn(c):
                    cp.wait()
                for cp in (copy_fn(c + 1) if c + 1 < len(CHUNKS) else tail_cps):
                    cp.start()

    def pair1(j, carry):
        q_pair(j)

        @pl.when(j == 0)
        def _():
            lax.fori_loop(0, D // 16, expand_wq, 0)
            for i in range(5):
                csq_buf[i] = _dot(ones_row, first_cols(i))

        next_copies(j, k_copy, [w1_cp])
        invs = []
        for par in range(2):
            h = 2 * j + par
            sg = [None] * ng
            lhs = qw_buf[h & 3]
            for c in range(4):
                for g in range(ng):
                    s = score2(lhs, h, par, 4 * g + c)
                    sg[g] = s if c == 0 else sg[g] + s
            ps, l = softmax(sg)
            for g in range(ng):
                store_p(ps[g], g, range(8), p_bufs[par])
            invs.append(inv_sum(l))
        next_copies(j, v_copy, w2_cps)
        lax.fori_loop(0, 24, lambda r, c_: fix_v(24 * j + r, c_), 0)
        for par in range(2):
            state = dict(par=par, slot=0)
            for sw in range(NS):
                for t in range(nt):
                    pv_step(2 * j + par, (sw * na, na), t, range(nt), (), state)

        for t in range(max(XMS)):
            js = [i for i in range(NP) if XMS[i] > t]
            assert js == list(range(js[0], js[-1] + 1))

            @pl.when(jnp.logical_and(j >= js[0], j <= js[-1]))
            def _():
                transpose_v(j, t)

        ie, io = invs
        o = _dot_t(ones32, accp_buf[0]) * jnp.concatenate([ie, jnp.where(lo64, ie, io), io], axis=1)
        op = _pack(o, o)
        for c in range(5):
            xacc_buf[:, 128 * c:128 * (c + 1)] += out_cols(op, 24 * j, 24, c)
        return carry

    def expand(t0, t1):
        return [jnp.where(evn, t0, pltpu.roll(t0, 8, 1)),
                jnp.where(evn, pltpu.roll(t0, 120, 1), t0),
                jnp.where(evn, jnp.where(lo64, t1, pltpu.roll(t1, 56, 1)),
                          jnp.where(lo64, pltpu.roll(t1, 8, 1), pltpu.roll(t1, 64, 1)))]

    def expand_wq(a, carry):
        e = expand(wq_buf[a, 0, 0:8, :], wq_buf[a, 1, 0:8, :])
        wq_buf[a, 0, 0:8, :] = e[0]
        wx_buf[0, a] = e[1]
        wx_buf[1, a] = e[2]
        return carry

    ones_row = jnp.concatenate([ones32] * (D // 128), axis=1)

    def first_cols(i):
        if i in (1, 2):
            return _bf(wx_buf[i - 1].reshape(D // 2, 128))
        return wq_cols(max(i - 2, 0))

    for ref in (so_buf, se_buf, l_buf, qraw_buf, xo_buf):
        ref[...] = jnp.zeros(ref.shape, ref.dtype)
    tm_buf[...] = lane
    zero_ref[0] = 0

    set_row(x0, _mean(x0))
    xacc_buf[...] = x0
    wq_cp.wait()
    lax.fori_loop(0, D // 16, fix_wq, 0)
    wo_cp.wait()
    lax.fori_loop(0, H * DH // 128, fix_wo, 0)
    lax.fori_loop(0, NP, pair1, 0)
    x1 = xacc_buf[...]
    w1_cp.wait()
    lax.fori_loop(0, D // 16, fix_w1, 0, unroll=8)
    m, r = _ln_stats(_pack(x1, x1), _mean(x1))
    lhs = _pack(_unpack(_pack(x1, x1))[0] - m, jnp.ones((8, D), F32))
    b1 = b1_buf[...].astype(F32)
    gs = []
    for k in range(F // 128):
        y = _dot(lhs, w1_cols(k))
        cs1_buf[k:k + 1, :] = y[1:2]
        gs.append(_gelu(jnp.broadcast_to(y[0:1], (8, 128)) * r + b1[k:k + 1, :]))
    x2 = x1 + bias2()
    for cp, r, n in zip(w2_cps, w2_at, W2_ROWS):
        shift = _mean(x2) if cp is w2_cps[-1] else None
        cp.wait()
        for k in range(r // 128, (r + n) // 128):
            x2 = x2 + w2_dot(gs[k], fix5(w2_buf, 8 * k))

    xp, rc, mrc = set_row(x2, shift)
    xacc_buf[...] = x2
    qx = [_dot(xp, first_cols(i)) * rc - csq_buf[i] * mrc for i in range(5)]
    w0 = jnp.concatenate([_pack(jnp.where(evn, q_, zf), jnp.where(evn, zf, q_)) for q_ in qx[0:3]],
                         axis=1)
    store_q([None, qx[3], qx[4]], 0, pars=(1,))
    sg = [None] * ng
    for g in range(ng):
        for c in range(4):
            s = score2(w0, 0, 0, 4 * g + c)
            sg[g] = s if c == 0 else sg[g] + s
    q_pair(1)
    ps0, l0, c0 = softmax_lane(sg)
    for g in range(ng):
        store_p(ps0[g], g, range(8), p_buf0)
    l_buf[0] = l0

    true_mask = [tm_buf[...] >= -i for i in range(3)]
    zq = jnp.clip(zero_ref[0], 0, 1)
    std = [(sw * na, na) for sw in range(NS)]
    steps, info = [], []
    for j in range(NP):
        if j == NP - 1:
            sweeps = [[(tl, range(XE, nt)) for tl in std],
                      [((5, 3), range(XO, nt)), ((2, 3), range(XO, nt)),
                       ((0, 2), range(XO, nt)), ((8, 4), range(XB, nt))]]
        else:
            sweeps = [[(tl, range(XMS[j], nt)) for tl in std]] * 2
        s0 = len(steps)
        steps += [(j, 0, tl, t, ts) for tl, ts in sweeps[0] for t in ts]
        s_odd = len(steps)
        steps += [(j, 1, tl, t, ts) for tl, ts in sweeps[1] for t in ts]
        info.append(dict(s0=s0, s_odd=s_odd, s_end=len(steps),
                         s_tail=len(steps) - len(sweeps[1][-1][1])))
    t_step = [0.0]
    for (_, _, tl, t, _) in steps:
        t_step.append(t_step[-1] + CU * tl[1] * (6 if t < ntb else 4))
    gates, stores, env = {}, {}, {}
    cur = dict(state=None, st=-1, nedge=0, edge=False, p_head=[0, None])

    def get_inv(h):
        return inv_sum(l_buf[zq + (h & 3)])

    def step_at(cyc):
        return next((i for i, tt_ in enumerate(t_step) if tt_ >= cyc), len(t_step))

    def gate(cyc, v):
        st = step_at(cyc)
        while len(gates.get(st, ())) >= 2:
            st += 1
        if cur['st'] < st < len(steps) - NGT:
            gates.setdefault(st, []).append(v)

    def edge(x, n=BE, force=False):
        if cur['st'] < 0 or not (force or cur['edge']):
            return x
        accs = cur['state']['accs']
        cand = [(e_, a) for e_ in range(2) for a in range(accs[0].shape[0])]
        ntile = -(-x.shape[1] // 128)
        parts = [x[:, 128 * i:min(128 * (i + 1), x.shape[1])] for i in range(ntile)]
        for k in range(min(n, 3 * ntile)):
            ce, ca = cand[cur['nedge'] % len(cand)]
            cur['nedge'] += 1
            i = k % ntile
            w_ = parts[i].shape[1]
            parts[i] = jnp.where(true_mask[k // ntile][:, 0:w_], parts[i],
                                 pltpu.bitcast(accs[ce][ca], U32)[:, 0:w_])
        return parts[0] if ntile == 1 else jnp.concatenate(parts, axis=1)

    def sched_stores(ps, lsum, h, t_ready, lo, hi, l_off=10):
        gate(t_ready, ps[-1])
        st_l = min(max(step_at(t_ready + l_off), cur['st'] + 1), len(steps) - 1)
        stores.setdefault(st_l, []).append((lsum, h, None, None))
        t_first = max(t_ready, t_step[lo])
        for i in range(2 * ng):
            g, k = divmod(i, 2)
            st = min(max(step_at(t_first + SDT * i) + 1, cur['st'] + 1), hi)
            assert lo <= st <= hi
            stores.setdefault(st, []).append((ps[g], h, g, range(4 * k, 4 * k + 4)))

    def p_block(h, t):
        assert cur['p_head'][h & 1] == h and not any(
            s_[1] == h and s_[2] is not None for ss in stores.values() for s_ in ss)
        return p_bufs[h & 1][8 * t:8 * t + 8, :]

    def pair_jobs(j):
        inf = info[j]
        first, last = j == 0, j == NP - 1
        h0 = 2 * j
        xm = XMS[j]

        def job_b(h, c, g):
            s_buf = (se_buf, so_buf)[h & 1]

            def fn(td):
                s = score2(edge(qw_buf[h & 3]), h, h & 1, 4 * g + c)
                gate(td + LATP, s)
                pltpu.store(s_buf.at[g], s, mask=sub2 == c)
                if c == 3 and g == ng - 1:
                    sg_ = [s_buf[zq + gg] for gg in range(ng)]
                    if h == 1:
                        ps, lsum, c1 = softmax_lane(sg_)
                        c01_buf[...] = _pack(c0, c1)
                        sched_stores(ps, lsum, h, td + LATP + MOFL, inf['s0'], inf['s_odd'], 130)
                    elif h & 1:
                        ps, lsum = softmax(sg_)
                        sched_stores(ps, lsum, h, td + LATP + MOFF, inf['s0'], inf['s_odd'])
                        if not last:
                            store_q([qraw_buf[zq + i] for i in range(3)], j + 1)
                    else:
                        ps, lsum = softmax(sg_)
                        sched_stores(ps, lsum, h, td + LATP + MOFF2, inf['s_odd'],
                                     inf['s_end'] - 1)
            return fn

        def job_e(td):
            x = _dot_t(edge(c01_buf[...] if j == 1 else ones32), accp_buf[(j - 1) & 1])
            if XMS[j - 1]:
                x = x + xo_buf[zq]

            def row(i, r):
                return jnp.broadcast_to(x[r:r + 1, 128 * i:128 * (i + 1)], (8, 128))

            ie, io = get_inv(h0 - 2), get_inv(h0 - 1)
            o = jnp.concatenate([row(0, 0) * ie, jnp.where(lo64, row(1, 0) * ie, row(1, 1) * io),
                                 row(2, 1) * io], axis=1)
            gate(td + LATP + 10, o[:, 256:384])
            op_buf[...] = _pack(o, o)

        def job_g(c):
            def fn(td):
                xo = out_cols(edge(op_buf[...]), 24 * (j - 1), 24, c)
                xacc_buf[:, 128 * c:128 * (c + 1)] += xo
                gate(td + LATP, xo)
            return fn

        def job_a(c):
            def fn(td):
                qc = q_cols(edge(z_buf[...]), j + 2, c)
                gate(td + LATP, qc)
                qraw_buf[c] = qc
            return fn

        def job_xp(t):
            def fn(td):
                pe, po = p_block(h0, t), p_block(h0 + 1, t)
                if first:
                    ce, co = _unpack(c01_buf[...])
                    pe, po = pe * ce, po * co
                lhs = edge(_pack(pe, po))
                o = jnp.concatenate([_dot(lhs, _bf(v_tiles(h0, 8 * ct, 8, t).reshape(64, 128)))
                                     for ct in range(3)], axis=1)
                env['xp'] = o if t == 0 else env['xp'] + o
                gate(td + LATP, env['xp'][:, 256:384])
                if t == xm - 1:
                    xo_buf[0] = env['xp']
            return fn

        def job_x(par, t, tiles, key):
            def fn(td):
                p = p_block(h0 + par, t)
                rhs = v_tiles(h0 + par, tiles[0], tiles[1], t).reshape(8 * tiles[1], 128)
                o = _dot_t(edge(_pack(p, p)), rhs)
                env[key] = o if key not in env else env[key] + o
                gate(td + LATP, env[key][:, 0:128] if tiles[1] >= 8 else
                     jnp.concatenate([env[key], env[key]], axis=1))
            return fn

        def finish(par, a0, a1, key):
            r0 = par * (DH // 2)
            o = _dot_t(edge(ones32), accp_buf[j & 1, r0 + 8 * a0:r0 + 8 * a1, :]) + env[key]
            inv = get_inv(h0 + par)
            n = 16 * (a1 - a0)
            return o * (inv[:, 0:n] if n <= 128 else
                        jnp.concatenate([inv, inv[:, 0:n - 128]], axis=1))

        env['finish'] = finish

        def job_fin(par, a0, a1, key):
            def fn(td):
                o = finish(par, a0, a1, key)
                gate(td + LATP + 10, o[:, 0:128])
                env['op' + key] = _pack(o, o)
            return fn

        def job_gfin(c):
            def fn(td):
                xo = out_cols(edge(env['opx0']), 12 * h0, 12, c)
                xacc_buf[:, 128 * c:128 * (c + 1)] += xo
                gate(td + LATP, xo)
            return fn

        t_odd = t_step[inf['s_odd'] + 1]
        jobs = [(24, None, job_b(h0 + 1, c, g))
                for g in range(0 if first else ng // 2, ng) for c in range(4)]
        if not first:
            jobs += [(56, t_step[inf['s0']] + EDEL, job_e)]
        out_jobs = [] if first else [(24, None, job_g(c)) for c in range(5)]
        if last:
            t_tail = t_step[inf['s_tail'] + 1]
            jobs += [(24, None, job_x(0, t, (0, 12), 'x0')) for t in range(XE)]
            jobs += out_jobs
            jobs += [(32, t_odd, job_fin(0, 0, 12, 'x0'))]
            jobs += [(16, None, job_x(1, t, (0, 8), 'x1a')) for t in range(XO)]
            jobs += [(12, t_odd + LATP + 60, job_gfin(c)) for c in range(5)]
            jobs += [(8, None, job_x(1, t, (8, 4), 'x1b')) for t in range(XB1)]
            jobs += [(16, t_tail, job_fin(1, 0, 8, 'x1a'))]
            jobs += [(8, None, job_x(1, t, (8, 4), 'x1b')) for t in range(XB1, XB)]
        else:
            jobs += [(24, None, job_b(h0 + 2, c, g)) for g in range(ng) for c in range(4)]
            jobs += [(24, t_odd, job_xp(t)) for t in range(xm)]
            if j + 2 < NP:
                jobs += [(40, None, job_a(c)) for c in range(3)]
            jobs += out_jobs
            jobs += [(24, None, job_b(h0 + 3, c, g)) for g in range(ng // 2) for c in range(4)]
        return jobs

    jobs, times = [], []
    tt = T0
    for j in range(NP):
        if j > 0:
            tt = max(tt, t_step[info[j]['s0']] - LEAD)
        for job in pair_jobs(j):
            tt = tt + job[0] if job[1] is None else max(tt + job[0], job[1])
            jobs.append(job)
            times.append(tt)
    j_first = next(i for i, tt_ in enumerate(times) if tt_ > 0)

    nj = 0
    for st, (j, par, tl, t, ts) in enumerate(steps):
        while nj < len(jobs) and times[nj] <= t_step[st]:
            rel = nj - j_first
            cur['edge'] = (0 <= rel < NE and rel % 2 == 1) or jobs[nj][1] == times[nj]
            jobs[nj][2](times[nj])
            nj += 1
        for val, h, g, rs in stores.pop(st, ()):
            val = pltpu.bitcast(edge(pltpu.bitcast(val, U32), 1, True), F32)
            if g is None:
                l_buf[h & 3] = val
            else:
                store_p(val, g, rs, p_bufs[h & 1])
                cur['p_head'][h & 1] = h
        if st in (info[j]['s0'], info[j]['s_odd']):
            state = dict(par=par, slot=j & 1)
        assert cur['p_head'][par] == 2 * j + par
        pv_step(2 * j + par, tl, t, ts, zip(true_mask, gates.get(st, ())), state)
        cur['state'] = state
        cur['st'] = st
    cur['edge'] = False
    for job, tt in zip(jobs[nj:], times[nj:]):
        job[2](tt)
    assert not stores

    o = env['finish'](1, 8, 12, 'x1b')
    op = _pack(o, o)
    xa = [out_cols(env['opx1a'], 12 * (H - 1), 8, c) for c in range(5)]
    xb = [out_cols(op, 12 * (H - 1) + 8, 4, c) for c in range(5)]
    x3 = (xacc_buf[...] + jnp.concatenate(xa, axis=1)) + jnp.concatenate(xb, axis=1)
    gs = mlp_hidden(x3, shift)
    x4 = x3 + bias2()
    parts = []
    for k in range(NV, F // 128):
        x4 = x4 + w2_dot(gs[k], [w2_buf[8 * k:8 * k + 8, 8 * c:8 * c + 8, :] for c in range(5)])
        parts.append(x4[:, 0:128])
    pins = gs[NV:] + parts
    acc = None
    for k in range(NV):
        col = jnp.broadcast_to(gs[k][0:1, :], (128, 128)).T
        for i in range(8):
            ci = col[16 * i:16 * i + 16, :]
            pin = (8 * k + i - GV0) // GVS
            if (8 * k + i - GV0) % GVS == 0 and 0 <= pin < len(pins):
                ci = jnp.concatenate([jnp.where(true_mask[0], ci[0:8], pins[pin]), ci[8:16]], axis=0)
            y = _bf(w2_buf[8 * k + i]).astype(F32).reshape(5, 16, 128) * ci
            y = y[:, 0:8] + y[:, 8:16]
            acc = y if acc is None else acc + y
    acc = jnp.concatenate([acc[c] for c in range(5)], axis=1)
    x4 = x4 + jnp.sum(acc, axis=0, keepdims=True)
    o_ref[...] = x4[0:1, :].astype(o_ref.dtype)


@jax.jit
def pallas_interleave_layers__sliding_block_cached__dense_activation_gelu__decode_kernel(
    A_x: jax.Array,
    A_k_cache: jax.Array,
    A_v_cache: jax.Array,
    A_wq: jax.Array,
    A_wo: jax.Array,
    B_x: jax.Array,
    B_w1: jax.Array,
    B_b1: jax.Array,
    B_w2: jax.Array,
    B_b2: jax.Array,
):
    sk = A_k_cache.shape[2]
    w = min(4096, max(256, sk // 4))
    ng = w // 1024

    def tile_view(a):
        *lead, r, c = a.shape
        n = len(lead)
        a = a.reshape(*lead, r // 8, 8, c // 128, 128)
        a = a.transpose(*range(n), n, n + 2, n + 1, n + 3)
        return a.reshape(*lead, r // 16, 2, (c // 128) * 8, 128)

    kx = tile_view(jnp.swapaxes(A_k_cache, 2, 3)).reshape(H * DH // 16, 2, sk // 16, 128)
    vx = tile_view(jnp.swapaxes(A_v_cache, 2, 3)).reshape(H * DH // 16, 2, sk // 16, 128)
    wqx = tile_view(A_wq)
    wox = tile_view(A_wo).reshape(H * DH // 16, 80, 128)
    out = pl.pallas_call(
        functools.partial(_kernel, sk=sk, w=w),
        out_shape=jax.ShapeDtypeStruct((1, D), A_x.dtype),
        in_specs=[pl.BlockSpec(memory_space=pl.ANY)] * 9,
        out_specs=pl.BlockSpec(memory_space=pltpu.VMEM),
        scratch_shapes=[
            pltpu.VMEM((H * DH // 16, 2, w // 32, 128), U32),
            pltpu.VMEM((H * DH // 16, 2, w // 32 - 4 * XF, 128), U32),
            pltpu.VMEM((H * DH // 16, 2, 8 * XF, 128), U32),
            pltpu.VMEM((D // 16, 2, H * DH // 32, 128), U32),
            pltpu.VMEM((H * DH // 16, 40, 128), U32),
            pltpu.VMEM((D // 16, 2, F // 32, 128), U32),
            pltpu.VMEM((F // 16, 40, 128), U32),
            pltpu.VMEM((1, D), BF16),
            pltpu.VMEM((F // 128, 128), BF16),
            pltpu.VMEM((D // 128, 128), BF16),
            pltpu.VMEM((w // 16, 128), F32),
            pltpu.VMEM((w // 16, 128), F32),
            pltpu.VMEM((ng + 1, 8, 128), F32),
            pltpu.VMEM((ng + 1, 8, 128), F32),
            pltpu.VMEM((5, 8, 128), F32),
            pltpu.VMEM((4, 8, 128), F32),
            pltpu.VMEM((2, 8, 2 * DH), F32),
            pltpu.VMEM((2, DH, 128), U32),
            pltpu.VMEM((8, D), U32),
            pltpu.VMEM((8, D), F32),
            pltpu.VMEM((4, 8, 2 * DH), U32),
            pltpu.VMEM((5, 8, 128), F32),
            pltpu.VMEM((F // 128, 128), F32),
            pltpu.VMEM((8, 128), F32),
            pltpu.VMEM((8, 2 * DH), U32),
            pltpu.VMEM((2, D // 16, 8, 128), U32),
            pltpu.VMEM((8, 128), U32),
            pltpu.VMEM((8, 128), jnp.int32),
            pltpu.SMEM((1,), jnp.int32),
            pltpu.SemaphoreType.DMA((2,)),
            pltpu.SemaphoreType.DMA((4,)),
            pltpu.SemaphoreType.DMA((6 + len(W2_ROWS),)),
        ],
        compiler_params=pltpu.CompilerParams(vmem_limit_bytes=127 * 1024 * 1024,
                                             disable_semaphore_checks=True),
    )(A_x.reshape(1, D), kx, vx, wqx, wox, tile_view(B_w1), B_b1.reshape(F // 128, 128),
      tile_view(B_w2).reshape(F // 16, 80, 128), B_b2.reshape(D // 128, 128))
    return out.reshape(A_x.shape)
```

```python
import functools
import math

import jax
import jax.numpy as jnp
from jax import lax
import jax.experimental.pallas as pl
import jax.experimental.pallas.tpu as pltpu

F32 = jnp.float32
BF16 = jnp.bfloat16
U32 = jnp.uint32

D = 640
H = 32
DH = 192
F = 1536
EPS = 1e-5
NP = H // 2

CHUNKS = (4, 4, 3, 2, 2, 1)
W2_ROWS = (640, 512, 256, 128)
NS = 4
XF = 6
XMS = (1,) * 14 + (3, 0)
XE, XO, XB, XB1 = 7, 7, 16, 8

CU = 0.2645
T0 = -100.0
LEAD = 100.0
LATP = 160.0
MOFF, MOFF2, MOFL = 160.0, 200.0, 50.0
EDEL = 70.0
SDT = 12.0
NE, BE, NGT = 7, 6, 12
NV, GV0, GVS = 6, 0, 4


def _gelu(x):
    c = math.sqrt(2.0 / math.pi)
    return 0.5 * x * (1.0 + jnp.tanh(c * (x + 0.044715 * (x * x * x))))


def _rows_to_lanes(b, n):
    return jnp.concatenate([b[i:i + 1, :] for i in range(n)], axis=1)


def _bf(x):
    return pltpu.bitcast(x, BF16)


def _halves(x):
    r = lax.bitcast_convert_type(x, U32) + jnp.uint32(0x8000)
    return r >> 16, r & jnp.uint32(0xFFFF0000)


def _store_tile(ref, a, b):
    ref[0:4, :] = pltpu.bitcast(a.astype(BF16), U32)
    ref[4:8, :] = pltpu.bitcast(b.astype(BF16), U32)


def _unpack(x):
    y = _bf(x).astype(F32)
    return y[:, 0:8], y[:, 8:16]


def _dot(lhs, rhs, rows=8):
    return jnp.dot(lhs, rhs, preferred_element_type=F32)[0:rows]


def _dot_t(lhs, rhs):
    return lax.dot_general(lhs, rhs, (((1,), (1,)), ((), ())), preferred_element_type=F32)


def _mean(x):
    return jnp.mean(x, axis=-1, keepdims=True)


def _ln_stats(x, shift):
    x = x - shift
    m = _mean(x)
    v = jnp.maximum(_mean(x * x) - m * m, 0.0)
    return m + shift, lax.rsqrt(v + EPS)


def _kernel(x_hbm, kx_hbm, vx_hbm, wq_hbm, wo_hbm, w1_hbm, b1_hbm, w2_hbm, b2_hbm,
            o_ref,
            kbuf, vbuf, vf_buf, wq_buf, wo_buf, w1_buf, w2_buf, x_buf, b1_buf, b2_buf,
            p_buf0, p_buf1, so_buf, se_buf, l_buf, qraw_buf, xo_buf, accp_buf, z_buf,
            xacc_buf, qw_buf, csq_buf, cs1_buf, st_buf, op_buf, wx_buf, c01_buf,
            tm_buf, zero_ref, sem_k, sem_v, sem_w, *, sk, w):
    c_scale = (DH ** -0.5) * math.log2(math.e)
    nt = w // 128
    ng = nt // 8
    na = 12 // NS
    ntb = nt - XF
    r0w = (sk - w) // 32
    p_bufs = (p_buf0, p_buf1)
    assert ng == 4 and sum(CHUNKS) == NP and all(XMS[:-1])
    starts = [sum(CHUNKS[:c]) for c in range(len(CHUNKS))]
    w2_at = [sum(W2_ROWS[:i]) for i in range(len(W2_ROWS))]

    kx32, vx32 = kx_hbm.bitcast(U32), vx_hbm.bitcast(U32)

    def k_copy(c):
        rows = pl.ds(24 * starts[c], 24 * CHUNKS[c])
        return [pltpu.make_async_copy(kx32.at[rows, :, pl.ds(r0w, 4 * nt), :],
                                      kbuf.at[rows], sem_k.at[c & 1])]

    def v_copy(c):
        rows = pl.ds(24 * starts[c], 24 * CHUNKS[c])
        return [pltpu.make_async_copy(vx32.at[rows, :, pl.ds(r0w, 4 * ntb), :],
                                      vbuf.at[rows], sem_v.at[c & 1]),
                pltpu.make_async_copy(vx32.at[rows, :, pl.ds(r0w + 4 * ntb, 4 * XF), :],
                                      vf_buf.at[rows, :, pl.ds(4 * XF, 4 * XF), :],
                                      sem_v.at[2 + (c & 1)])]

    wq_cp = pltpu.make_async_copy(wq_hbm.bitcast(U32), wq_buf, sem_w.at[0])
    wo_cp = pltpu.make_async_copy(wo_hbm.bitcast(U32), wo_buf, sem_w.at[1])
    w1_cp = pltpu.make_async_copy(w1_hbm.bitcast(U32), w1_buf, sem_w.at[2])
    x_cp = pltpu.make_async_copy(x_hbm, x_buf, sem_w.at[3])
    b1_cp = pltpu.make_async_copy(b1_hbm, b1_buf, sem_w.at[4])
    b2_cp = pltpu.make_async_copy(b2_hbm, b2_buf, sem_w.at[5])
    w2_cps = [pltpu.make_async_copy(w2_hbm.bitcast(U32).at[pl.ds(r // 16, n // 16)],
                                    w2_buf.at[pl.ds(r // 16, n // 16)], sem_w.at[6 + i])
              for i, (r, n) in enumerate(zip(w2_at, W2_ROWS))]

    for cp in [wq_cp, x_cp, b1_cp, b2_cp, wo_cp] + k_copy(0) + v_copy(0):
        cp.start()
    x_cp.wait()
    b1_cp.wait()
    b2_cp.wait()

    x0 = jnp.broadcast_to(x_buf[...].astype(F32), (8, D))

    lane = lax.broadcasted_iota(jnp.int32, (8, 128), 1)
    sub3 = lax.broadcasted_iota(jnp.int32, (8, 2 * DH), 0)
    sub2 = lax.broadcasted_iota(jnp.int32, (8, 128), 0) // 2
    sub_lo = lax.broadcasted_iota(jnp.int32, (1, 8, 128), 1) < 4
    lo64 = lane < 64
    evn = (lane & 8) == 0
    ones = jnp.ones((8, 128), F32)
    k_order = (((0, 8, 0), (0, 8, 1), (8, 4, 0), (8, 4, 1)),
               ((4, 8, 0), (4, 8, 1), (0, 4, 1), (0, 4, 0)))

    def regroup(a, b):
        return jnp.where(sub_lo, a, pltpu.roll(b, 4, 1)), jnp.where(sub_lo, pltpu.roll(a, 4, 1), b)

    def swap_halves(ref2):
        n = ref2.shape[1]
        a, b = regroup(ref2[0].reshape(n // 8, 8, 128), ref2[1].reshape(n // 8, 8, 128))
        ref2[0] = a.reshape(n, 128)
        ref2[1] = b.reshape(n, 128)

    def fix_wq(a, carry):
        swap_halves(wq_buf.at[a])
        return carry

    def fix5(buf, g0):
        v = [buf[pl.ds(g0, 8), 8 * c:8 * c + 8, :] for c in range(5)]
        n = [jnp.where(sub_lo, v[0], v[2]),
             pltpu.roll(jnp.where(sub_lo, v[3], v[0]), 4, 1),
             jnp.where(sub_lo, v[1], v[3]),
             pltpu.roll(jnp.where(sub_lo, v[4], v[1]), 4, 1),
             jnp.where(sub_lo, v[2], v[4])]
        for c in range(5):
            buf[pl.ds(g0, 8), 8 * c:8 * c + 8, :] = n[c]
        return n

    def fix_wo(g8, carry):
        fix5(wo_buf, pl.multiple_of(g8 * 8, 8))
        return carry

    def fix_w1(a, carry):
        swap_halves(w1_buf.at[a])
        return carry

    def fix_v(r2, carry):
        swap_halves(vbuf.at[r2])
        n = 4 * XF
        t0, t1 = regroup(vf_buf[r2, 0, n:2 * n, :].reshape(n // 8, 8, 128),
                         vf_buf[r2, 1, n:2 * n, :].reshape(n // 8, 8, 128))
        t0, t1 = _unpack(t0), _unpack(t1)
        for e in range(2):
            for k in range(XF // 2):
                vf_buf[r2, e, 16 * k:16 * k + 8, :] = pltpu.bitcast(t0[e][k], U32)
                vf_buf[r2, e, 16 * k + 8:16 * k + 16, :] = pltpu.bitcast(t1[e][k], U32)
        return carry

    def v_tiles(h, a0, n, t):
        return vbuf[pl.ds(12 * h + a0, n), t % 2, 8 * (t // 2):8 * (t // 2) + 8, :]

    def transpose_v(j, t):
        y = _bf(v_tiles(2 * j, 0, 24, t).reshape(DH, 128)).astype(F32)
        yt = pltpu.bitcast(y.T.astype(BF16), U32)
        for ct in range(3):
            vbuf[pl.ds(24 * j + 8 * ct, 8), t % 2, 8 * (t // 2):8 * (t // 2) + 8, :] = (
                yt[:, 128 * ct:128 * (ct + 1)].reshape(8, 8, 128))

    def set_row(x, shift):
        xb = x.astype(BF16)
        m, r = _ln_stats(xb.astype(F32), shift)
        xc = xb.astype(F32) - m
        _store_tile(z_buf, xc, xc)
        rc = jnp.broadcast_to(r * c_scale, (8, 128))
        st_buf[...] = rc
        return xb, rc, m * rc

    def wq_cols(ct):
        if isinstance(ct, int):
            r0 = (ct // 2) * 8
        else:
            r0 = pl.multiple_of(lax.shift_right_logical(ct, 1) * 8, 8)
        return _bf(wq_buf[:, ct & 1, pl.ds(r0, 8), :].reshape(D // 2, 128))

    def q_cols(z, j, c):
        return _dot(_bf(z), wq_cols(3 * j + c)) * st_buf[...]

    def store_q(qs, j, pars=(0, 1)):
        q0, q1, q2 = qs
        lo1, hi1 = _halves(q1)
        r56, r64, r8 = pltpu.roll(lo1, 56, 1), pltpu.roll(hi1, 64, 1), pltpu.roll(hi1, 8, 1)

        def put(h, qf, a2, b2):
            lo, hi = _halves(qf)
            qw_buf[h & 3] = jnp.concatenate(
                [jnp.where(evn, lo, pltpu.roll(hi, 8, 1)),
                 jnp.where(evn, pltpu.roll(lo, 120, 1), hi), jnp.where(evn, a2, b2)], axis=1)

        if 0 in pars:
            put(2 * j, q0, jnp.where(lo64, lo1, r56), jnp.where(lo64, r8, r64))
        if 1 in pars:
            put(2 * j + 1, q2, jnp.where(lo64, r56, lo1), jnp.where(lo64, r64, r8))

    def q_pair(j):
        z = z_buf[...]
        store_q([q_cols(z, j, c) for c in range(3)], j)

    def score2(lhs, h, par, k):
        lhs = jnp.where(sub3 == k % 4, lhs, jnp.zeros_like(lhs))
        rhs = jnp.concatenate([kbuf[pl.ds(12 * h + a, n), e, 8 * k:8 * k + 8, :]
                               for a, n, e in k_order[par]], axis=0)
        return _dot(_bf(lhs), _bf(rhs.reshape(DH, 128)))

    def store_p(p, g, rs, p_out):
        for r in rs:
            p_out[pl.ds(64 * g + r, 8, stride=8), :] = p

    def inv_sum(l):
        l = jnp.sum(jnp.sum(l, axis=1, keepdims=True), axis=0, keepdims=True)
        l = jnp.broadcast_to(l, (8, 128))
        r = pl.reciprocal(l, approx=True)
        return r * (2.0 - l * r)

    def softmax(sg):
        mx = sg[0]
        for s in sg[1:]:
            mx = jnp.maximum(mx, s)
        m = jnp.max(jnp.max(mx, axis=1, keepdims=True), axis=0, keepdims=True)
        ps, l = [], None
        for s in sg:
            ps.append(jnp.exp2(s - m))
            l = ps[-1] if l is None else l + ps[-1]
        return ps, l

    def softmax_lane(sg):
        mx = jnp.maximum(jnp.maximum(sg[0], sg[1]), jnp.maximum(sg[2], sg[3]))
        m = jnp.broadcast_to(jnp.max(mx, axis=0, keepdims=True), (8, 128))
        ps = [jnp.exp2(s - m) for s in sg]
        c = jnp.exp2(m - jnp.max(m, axis=1, keepdims=True))
        c = c.astype(BF16).astype(F32)
        return ps, ((ps[0] + ps[1]) + (ps[2] + ps[3])) * c, c

    def pv_step(h, tiles, t, ts, gated, state):
        a0, n = tiles
        p = p_bufs[state['par']][8 * t:8 * t + 8, :]
        for mask, val in gated:
            p = jnp.where(mask, p, val)
        if t < ntb:
            ys = _unpack(v_tiles(h, a0, n, t))
        else:
            r = 8 * (t - ntb)
            ys = [pltpu.bitcast(vf_buf[pl.ds(12 * h + a0, n), e, r:r + 8, :], F32)
                  for e in range(2)]
        if t == ts[0]:
            state['accs'] = [y * p for y in ys]
        else:
            state['accs'] = [acc + y * p for acc, y in zip(state['accs'], ys)]
        if t == ts[-1]:
            for i in range(n):
                _store_tile(accp_buf.at[state['slot'], 12 * state['par'] + a0 + i],
                            state['accs'][0][i], state['accs'][1][i])

    def out_cols(op, g0, ngrp, c):
        rhs = wo_buf[pl.ds(g0, ngrp), 8 * c:8 * c + 8, :].reshape(ngrp * 8, 128)
        return _dot(op, _bf(rhs))

    def w1_cols(k):
        return _bf(w1_buf[:, k % 2, 8 * (k // 2):8 * (k // 2) + 8, :].reshape(D // 2, 128))

    def mlp_hidden(x, shift):
        xb = x.astype(BF16)
        m, r = _ln_stats(xb.astype(F32), shift)
        b1 = b1_buf[...].astype(F32)
        return [_gelu((_dot(xb, w1_cols(k)) - cs1_buf[k:k + 1, :] * m) * r + b1[k:k + 1, :])
                for k in range(F // 128)]

    def bias2():
        return _rows_to_lanes(b2_buf[...].astype(F32), D // 128)

    def w2_dot(g, tiles):
        gb = g.astype(BF16)
        return jnp.concatenate([_dot(gb, _bf(t.reshape(64, 128))) for t in tiles], axis=1)

    def lane_sums(slot, a0, a1):
        return _bf(accp_buf[slot, a0:a1].reshape(8 * (a1 - a0), 128))

    def by_head(e0, mid_e, mid_o, o2):
        return jnp.concatenate([e0, jnp.where(lo64, mid_e, mid_o), o2], axis=1)

    def two_heads(y):
        return by_head(y[0:8, 0:128], y[0:8, 128:256], y[8:16, 128:256], y[8:16, 256:384])

    def next_copies(j, copy_fn, tail_cps):
        for c in range(len(CHUNKS)):
            @pl.when(j == starts[c])
            def _():
                for cp in copy_fn(c):
                    cp.wait()
                for cp in (copy_fn(c + 1) if c + 1 < len(CHUNKS) else tail_cps):
                    cp.start()

    def pair1(j, carry):
        q_pair(j)

        @pl.when(j == 0)
        def _():
            lax.fori_loop(0, D // 16, expand_wq, 0)
            for i in range(5):
                csq_buf[i] = _dot(ones_row.astype(BF16), first_cols(i))

        next_copies(j, k_copy, [w1_cp])
        invs = []
        for par in range(2):
            h = 2 * j + par
            sg = [None] * ng
            lhs = qw_buf[h & 3]
            for c in range(4):
                for g in range(ng):
                    s = score2(lhs, h, par, 4 * g + c)
                    sg[g] = s if c == 0 else sg[g] + s
            ps, l = softmax(sg)
            for g in range(ng):
                store_p(ps[g], g, range(8), p_bufs[par])
            invs.append(inv_sum(l))
        next_copies(j, v_copy, w2_cps)
        lax.fori_loop(0, 24, lambda r, c_: fix_v(24 * j + r, c_), 0)
        for par in range(2):
            state = dict(par=par, slot=0)
            for sw in range(NS):
                for t in range(nt):
                    pv_step(2 * j + par, (sw * na, na), t, range(nt), (), state)

        for t in range(max(XMS)):
            js = [i for i in range(NP) if XMS[i] > t]
            assert js == list(range(js[0], js[-1] + 1))

            @pl.when(jnp.logical_and(j >= js[0], j <= js[-1]))
            def _():
                transpose_v(j, t)

        ie, io = invs
        o = _dot_t(ones.astype(BF16), lane_sums(0, 0, 24)) * by_head(ie, ie, io, io)
        op = o.astype(BF16)
        for c in range(5):
            xacc_buf[:, 128 * c:128 * (c + 1)] += out_cols(op, 24 * j, 24, c)
        return carry

    def expand(t0, t1):
        return [jnp.where(evn, t0, pltpu.roll(t0, 8, 1)),
                jnp.where(evn, pltpu.roll(t0, 120, 1), t0),
                jnp.where(evn, jnp.where(lo64, t1, pltpu.roll(t1, 56, 1)),
                          jnp.where(lo64, pltpu.roll(t1, 8, 1), pltpu.roll(t1, 64, 1)))]

    def expand_wq(a, carry):
        e = expand(wq_buf[a, 0, 0:8, :], wq_buf[a, 1, 0:8, :])
        wq_buf[a, 0, 0:8, :] = e[0]
        wx_buf[0, a] = e[1]
        wx_buf[1, a] = e[2]
        return carry

    ones_row = jnp.ones((8, D), F32)

    def first_cols(i):
        if i in (1, 2):
            return _bf(wx_buf[i - 1].reshape(D // 2, 128))
        return wq_cols(max(i - 2, 0))

    for ref in (so_buf, se_buf, l_buf, qraw_buf, xo_buf):
        ref[...] = jnp.zeros(ref.shape, ref.dtype)
    tm_buf[...] = lane
    zero_ref[0] = 0

    set_row(x0, _mean(x0))
    xacc_buf[...] = x0
    wq_cp.wait()
    lax.fori_loop(0, D // 16, fix_wq, 0)
    wo_cp.wait()
    lax.fori_loop(0, H * DH // 128, fix_wo, 0)
    lax.fori_loop(0, NP, pair1, 0)
    x1 = xacc_buf[...]
    w1_cp.wait()
    lax.fori_loop(0, D // 16, fix_w1, 0, unroll=8)
    x1r = x1.astype(BF16).astype(F32)
    m, r = _ln_stats(x1r, _mean(x1))
    lhs = jnp.concatenate([x1r - m, ones_row], axis=0).astype(BF16)
    b1 = b1_buf[...].astype(F32)
    gs = []
    for k in range(F // 128):
        y = _dot(lhs, w1_cols(k), 16)
        cs1_buf[k:k + 1, :] = y[8:9]
        gs.append(_gelu(y[0:8] * r + b1[k:k + 1, :]))
    x2 = x1 + bias2()
    for cp, r, n in zip(w2_cps, w2_at, W2_ROWS):
        shift = _mean(x2) if cp is w2_cps[-1] else None
        cp.wait()
        for k in range(r // 128, (r + n) // 128):
            x2 = x2 + w2_dot(gs[k], fix5(w2_buf, 8 * k))

    xp, rc, mrc = set_row(x2, shift)
    xacc_buf[...] = x2
    qx = [_dot(xp, first_cols(i)) * rc - csq_buf[i] * mrc for i in range(5)]
    w0 = jnp.concatenate([jnp.where(evn, *_halves(q_)) for q_ in qx[0:3]], axis=1)
    store_q([None, qx[3], qx[4]], 0, pars=(1,))
    sg = [None] * ng
    for g in range(ng):
        for c in range(4):
            s = score2(w0, 0, 0, 4 * g + c)
            sg[g] = s if c == 0 else sg[g] + s
    q_pair(1)
    ps0, l0, c0 = softmax_lane(sg)
    for g in range(ng):
        store_p(ps0[g], g, range(8), p_buf0)
    l_buf[0] = l0

    true_mask = [tm_buf[...] >= -i for i in range(3)]
    zq = jnp.clip(zero_ref[0], 0, 1)
    std = [(sw * na, na) for sw in range(NS)]
    steps, info = [], []
    for j in range(NP):
        if j == NP - 1:
            sweeps = [[(tl, range(XE, nt)) for tl in std],
                      [((5, 3), range(XO, nt)), ((2, 3), range(XO, nt)),
                       ((0, 2), range(XO, nt)), ((8, 4), range(XB, nt))]]
        else:
            sweeps = [[(tl, range(XMS[j], nt)) for tl in std]] * 2
        s0 = len(steps)
        steps += [(j, 0, tl, t, ts) for tl, ts in sweeps[0] for t in ts]
        s_odd = len(steps)
        steps += [(j, 1, tl, t, ts) for tl, ts in sweeps[1] for t in ts]
        info.append(dict(s0=s0, s_odd=s_odd, s_end=len(steps),
                         s_tail=len(steps) - len(sweeps[1][-1][1])))
    t_step = [0.0]
    for (_, _, tl, t, _) in steps:
        t_step.append(t_step[-1] + CU * tl[1] * (6 if t < ntb else 4))
    gates, stores, env = {}, {}, {}
    cur = dict(state=None, st=-1, nedge=0, edge=False, p_head=[0, None])

    def get_inv(h):
        return inv_sum(l_buf[zq + (h & 3)])

    def step_at(cyc):
        return next((i for i, tt_ in enumerate(t_step) if tt_ >= cyc), len(t_step))

    def gate(cyc, v):
        st = step_at(cyc)
        while len(gates.get(st, ())) >= 2:
            st += 1
        if cur['st'] < st < len(steps) - NGT:
            gates.setdefault(st, []).append(v)

    def edge(x, n=BE, force=False):
        if cur['st'] < 0 or not (force or cur['edge']):
            return x
        accs = cur['state']['accs']
        cand = [(e_, a) for e_ in range(2) for a in range(accs[0].shape[0])]
        ntile = -(-x.shape[1] // 128)
        parts = [x[:, 128 * i:min(128 * (i + 1), x.shape[1])] for i in range(ntile)]
        for k in range(min(n, 3 * ntile)):
            ce, ca = cand[cur['nedge'] % len(cand)]
            cur['nedge'] += 1
            i = k % ntile
            w_ = parts[i].shape[1]
            parts[i] = jnp.where(true_mask[k // ntile][:, 0:w_], parts[i],
                                 lax.bitcast_convert_type(accs[ce][ca], x.dtype)[:, 0:w_])
        return parts[0] if ntile == 1 else jnp.concatenate(parts, axis=1)

    def sched_stores(ps, lsum, h, t_ready, lo, hi, l_off=10):
        gate(t_ready, ps[-1])
        st_l = min(max(step_at(t_ready + l_off), cur['st'] + 1), len(steps) - 1)
        stores.setdefault(st_l, []).append((lsum, h, None, None))
        t_first = max(t_ready, t_step[lo])
        for i in range(2 * ng):
            g, k = divmod(i, 2)
            st = min(max(step_at(t_first + SDT * i) + 1, cur['st'] + 1), hi)
            assert lo <= st <= hi
            stores.setdefault(st, []).append((ps[g], h, g, range(4 * k, 4 * k + 4)))

    def p_block(h, t):
        assert cur['p_head'][h & 1] == h and not any(
            s_[1] == h and s_[2] is not None for ss in stores.values() for s_ in ss)
        return p_bufs[h & 1][8 * t:8 * t + 8, :]

    def pair_jobs(j):
        inf = info[j]
        first, last = j == 0, j == NP - 1
        h0 = 2 * j
        xm = XMS[j]

        def job_b(h, c, g):
            s_buf = (se_buf, so_buf)[h & 1]

            def fn(td):
                s = score2(edge(qw_buf[h & 3]), h, h & 1, 4 * g + c)
                gate(td + LATP, s)
                pltpu.store(s_buf.at[g], s, mask=sub2 == c)
                if c == 3 and g == ng - 1:
                    sg_ = [s_buf[zq + gg] for gg in range(ng)]
                    if h == 1:
                        ps, lsum, c1 = softmax_lane(sg_)
                        c01_buf[0] = c0
                        c01_buf[1] = c1
                        sched_stores(ps, lsum, h, td + LATP + MOFL, inf['s0'], inf['s_odd'], 130)
                    elif h & 1:
                        ps, lsum = softmax(sg_)
                        sched_stores(ps, lsum, h, td + LATP + MOFF, inf['s0'], inf['s_odd'])
                        if not last:
                            store_q([qraw_buf[zq + i] for i in range(3)], j + 1)
                    else:
                        ps, lsum = softmax(sg_)
                        sched_stores(ps, lsum, h, td + LATP + MOFF2, inf['s_odd'],
                                     inf['s_end'] - 1)
            return fn

        def job_e(td):
            sums = lane_sums((j - 1) & 1, 0, 24)
            if j == 1:
                lhs = jnp.concatenate([edge(c01_buf[0]), c01_buf[1]], axis=0)
                x = two_heads(_dot_t(lhs.astype(BF16), sums))
            else:
                x = _dot_t(edge(ones).astype(BF16), sums)
            ie, io = get_inv(h0 - 2), get_inv(h0 - 1)
            o = (x + xo_buf[zq]) * by_head(ie, ie, io, io)
            gate(td + LATP + 10, o[:, 256:384])
            _store_tile(op_buf, o, o)

        def job_g(c):
            def fn(td):
                xo = out_cols(_bf(edge(op_buf[...])), 24 * (j - 1), 24, c)
                xacc_buf[:, 128 * c:128 * (c + 1)] += xo
                gate(td + LATP, xo)
            return fn

        def job_a(c):
            def fn(td):
                qc = q_cols(edge(z_buf[...]), j + 2, c)
                gate(td + LATP, qc)
                qraw_buf[c] = qc
            return fn

        def job_xp(t):
            def fn(td):
                pe, po = p_block(h0, t), p_block(h0 + 1, t)
                if first:
                    pe, po = pe * c01_buf[0], po * c01_buf[1]
                lhs = jnp.concatenate([edge(pe), po], axis=0).astype(BF16)
                o = two_heads(jnp.concatenate(
                    [_dot(lhs, _bf(v_tiles(h0, 8 * ct, 8, t).reshape(64, 128)), 16)
                     for ct in range(3)], axis=1))
                env['xp'] = o if t == 0 else env['xp'] + o
                gate(td + LATP, env['xp'][:, 256:384])
                if t == xm - 1:
                    xo_buf[0] = env['xp']
            return fn

        def job_x(par, t, tiles, key):
            def fn(td):
                p = p_block(h0 + par, t)
                rhs = v_tiles(h0 + par, tiles[0], tiles[1], t).reshape(8 * tiles[1], 128)
                o = _dot_t(edge(p).astype(BF16), _bf(rhs))
                env[key] = o if key not in env else env[key] + o
                gate(td + LATP, env[key][:, 0:128] if tiles[1] >= 8 else
                     jnp.concatenate([env[key], env[key]], axis=1))
            return fn

        def finish(par, a0, a1, key):
            o = _dot_t(edge(ones).astype(BF16),
                       lane_sums(j & 1, 12 * par + a0, 12 * par + a1)) + env[key]
            inv = get_inv(h0 + par)
            n = 16 * (a1 - a0)
            return o * (inv[:, 0:n] if n <= 128 else
                        jnp.concatenate([inv, inv[:, 0:n - 128]], axis=1))

        env['finish'] = finish

        def job_fin(par, a0, a1, key):
            def fn(td):
                o = finish(par, a0, a1, key)
                gate(td + LATP + 10, o[:, 0:128])
                env['op' + key] = o
            return fn

        def job_gfin(c):
            def fn(td):
                xo = out_cols(edge(env['opx0']).astype(BF16), 12 * h0, 12, c)
                xacc_buf[:, 128 * c:128 * (c + 1)] += xo
                gate(td + LATP, xo)
            return fn

        t_odd = t_step[inf['s_odd'] + 1]
        jobs = [(24, None, job_b(h0 + 1, c, g))
                for g in range(0 if first else ng // 2, ng) for c in range(4)]
        if not first:
            jobs += [(60, t_step[inf['s0']] + EDEL, job_e)]
        out_jobs = [] if first else [(24, None, job_g(c)) for c in range(5)]
        if last:
            t_tail = t_step[inf['s_tail'] + 1]
            jobs += [(24, None, job_x(0, t, (0, 12), 'x0')) for t in range(XE)]
            jobs += out_jobs
            jobs += [(32, t_odd, job_fin(0, 0, 12, 'x0'))]
            jobs += [(16, None, job_x(1, t, (0, 8), 'x1a')) for t in range(XO)]
            jobs += [(12, t_odd + LATP + 60, job_gfin(c)) for c in range(5)]
            jobs += [(8, None, job_x(1, t, (8, 4), 'x1b')) for t in range(XB1)]
            jobs += [(16, t_tail, job_fin(1, 0, 8, 'x1a'))]
            jobs += [(8, None, job_x(1, t, (8, 4), 'x1b')) for t in range(XB1, XB)]
        else:
            jobs += [(24, None, job_b(h0 + 2, c, g)) for g in range(ng) for c in range(4)]
            jobs += [(24, t_odd, job_xp(t)) for t in range(xm)]
            if j + 2 < NP:
                jobs += [(40, None, job_a(c)) for c in range(3)]
            jobs += out_jobs
            jobs += [(24, None, job_b(h0 + 3, c, g)) for g in range(ng // 2) for c in range(4)]
        return jobs

    jobs, times = [], []
    tt = T0
    for j in range(NP):
        if j > 0:
            tt = max(tt, t_step[info[j]['s0']] - LEAD)
        for job in pair_jobs(j):
            tt = tt + job[0] if job[1] is None else max(tt + job[0], job[1])
            jobs.append(job)
            times.append(tt)
    j_first = next(i for i, tt_ in enumerate(times) if tt_ > 0)

    nj = 0
    for st, (j, par, tl, t, ts) in enumerate(steps):
        while nj < len(jobs) and times[nj] <= t_step[st]:
            rel = nj - j_first
            cur['edge'] = (0 <= rel < NE and rel % 2 == 1) or jobs[nj][1] == times[nj]
            jobs[nj][2](times[nj])
            nj += 1
        for val, h, g, rs in stores.pop(st, ()):
            val = edge(val, 1, True)
            if g is None:
                l_buf[h & 3] = val
            else:
                store_p(val, g, rs, p_bufs[h & 1])
                cur['p_head'][h & 1] = h
        if st in (info[j]['s0'], info[j]['s_odd']):
            state = dict(par=par, slot=j & 1)
        assert cur['p_head'][par] == 2 * j + par
        pv_step(2 * j + par, tl, t, ts, zip(true_mask, gates.get(st, ())), state)
        cur['state'] = state
        cur['st'] = st
    cur['edge'] = False
    for job, tt in zip(jobs[nj:], times[nj:]):
        job[2](tt)
    assert not stores

    op = env['finish'](1, 8, 12, 'x1b').astype(BF16)
    xa = [out_cols(env['opx1a'].astype(BF16), 12 * (H - 1), 8, c) for c in range(5)]
    xb = [out_cols(op, 12 * (H - 1) + 8, 4, c) for c in range(5)]
    x3 = (xacc_buf[...] + jnp.concatenate(xa, axis=1)) + jnp.concatenate(xb, axis=1)
    gs = mlp_hidden(x3, shift)
    x4 = x3 + bias2()
    parts = []
    for k in range(NV, F // 128):
        x4 = x4 + w2_dot(gs[k], [w2_buf[8 * k:8 * k + 8, 8 * c:8 * c + 8, :] for c in range(5)])
        parts.append(x4[:, 0:128])
    pins = gs[NV:] + parts
    acc = None
    for k in range(NV):
        col = jnp.broadcast_to(gs[k][0:1, :], (128, 128)).T
        for i in range(8):
            ci = col[16 * i:16 * i + 16, :]
            pin = (8 * k + i - GV0) // GVS
            if (8 * k + i - GV0) % GVS == 0 and 0 <= pin < len(pins):
                ci = jnp.concatenate([jnp.where(true_mask[0], ci[0:8], pins[pin]), ci[8:16]], axis=0)
            y = _bf(w2_buf[8 * k + i]).astype(F32).reshape(5, 16, 128) * ci
            y = y[:, 0:8] + y[:, 8:16]
            acc = y if acc is None else acc + y
    acc = jnp.concatenate([acc[c] for c in range(5)], axis=1)
    x4 = x4 + jnp.sum(acc, axis=0, keepdims=True)
    o_ref[...] = x4[0:1, :].astype(o_ref.dtype)


@jax.jit
def pallas_interleave_layers__sliding_block_cached__dense_activation_gelu__decode_kernel(
    A_x: jax.Array,
    A_k_cache: jax.Array,
    A_v_cache: jax.Array,
    A_wq: jax.Array,
    A_wo: jax.Array,
    B_x: jax.Array,
    B_w1: jax.Array,
    B_b1: jax.Array,
    B_w2: jax.Array,
    B_b2: jax.Array,
):
    sk = A_k_cache.shape[2]
    w = min(4096, max(256, sk // 4))
    ng = w // 1024

    def tile_view(a):
        *lead, r, c = a.shape
        n = len(lead)
        a = a.reshape(*lead, r // 8, 8, c // 128, 128)
        a = a.transpose(*range(n), n, n + 2, n + 1, n + 3)
        return a.reshape(*lead, r // 16, 2, (c // 128) * 8, 128)

    kx = tile_view(jnp.swapaxes(A_k_cache, 2, 3)).reshape(H * DH // 16, 2, sk // 16, 128)
    vx = tile_view(jnp.swapaxes(A_v_cache, 2, 3)).reshape(H * DH // 16, 2, sk // 16, 128)
    wqx = tile_view(A_wq)
    wox = tile_view(A_wo).reshape(H * DH // 16, 80, 128)
    out = pl.pallas_call(
        functools.partial(_kernel, sk=sk, w=w),
        out_shape=jax.ShapeDtypeStruct((1, D), A_x.dtype),
        in_specs=[pl.BlockSpec(memory_space=pl.ANY)] * 9,
        out_specs=pl.BlockSpec(memory_space=pltpu.VMEM),
        scratch_shapes=[
            pltpu.VMEM((H * DH // 16, 2, w // 32, 128), U32),
            pltpu.VMEM((H * DH // 16, 2, w // 32 - 4 * XF, 128), U32),
            pltpu.VMEM((H * DH // 16, 2, 8 * XF, 128), U32),
            pltpu.VMEM((D // 16, 2, H * DH // 32, 128), U32),
            pltpu.VMEM((H * DH // 16, 40, 128), U32),
            pltpu.VMEM((D // 16, 2, F // 32, 128), U32),
            pltpu.VMEM((F // 16, 40, 128), U32),
            pltpu.VMEM((1, D), BF16),
            pltpu.VMEM((F // 128, 128), BF16),
            pltpu.VMEM((D // 128, 128), BF16),
            pltpu.VMEM((w // 16, 128), F32),
            pltpu.VMEM((w // 16, 128), F32),
            pltpu.VMEM((ng + 1, 8, 128), F32),
            pltpu.VMEM((ng + 1, 8, 128), F32),
            pltpu.VMEM((5, 8, 128), F32),
            pltpu.VMEM((4, 8, 128), F32),
            pltpu.VMEM((2, 8, 2 * DH), F32),
            pltpu.VMEM((2, 24, 8, 128), U32),
            pltpu.VMEM((8, D), U32),
            pltpu.VMEM((8, D), F32),
            pltpu.VMEM((4, 8, 2 * DH), U32),
            pltpu.VMEM((5, 8, 128), F32),
            pltpu.VMEM((F // 128, 128), F32),
            pltpu.VMEM((8, 128), F32),
            pltpu.VMEM((8, 2 * DH), U32),
            pltpu.VMEM((2, D // 16, 8, 128), U32),
            pltpu.VMEM((2, 8, 128), F32),
            pltpu.VMEM((8, 128), jnp.int32),
            pltpu.SMEM((1,), jnp.int32),
            pltpu.SemaphoreType.DMA((2,)),
            pltpu.SemaphoreType.DMA((4,)),
            pltpu.SemaphoreType.DMA((6 + len(W2_ROWS),)),
        ],
        compiler_params=pltpu.CompilerParams(vmem_limit_bytes=127 * 1024 * 1024,
                                             disable_semaphore_checks=True),
    )(A_x.reshape(1, D), kx, vx, wqx, wox, tile_view(B_w1), B_b1.reshape(F // 128, 128),
      tile_view(B_w2).reshape(F // 16, 80, 128), B_b2.reshape(D // 128, 128))
    return out.reshape(A_x.shape)
```
